```python
import jax
import jax.numpy as jnp

def _softmax(x, axis=-1):
    return jax.nn.softmax(x, axis=axis)
def _gelu(x):
    return jax.nn.gelu(x, approximate=True)
def _silu(x):
    return jax.nn.silu(x)
def _sigmoid(x):
    return jax.nn.sigmoid(x)
def _layernorm(x, axis=-1, eps=1e-5):
    m = jnp.mean(x, axis=axis, keepdims=True)
    v = jnp.var(x, axis=axis, keepdims=True)
    return (x - m) / jnp.sqrt(v + eps)
def _scatter_add(tgt, idx, src, axis=0):
    return tgt.at[idx].add(src)
def _segment_sum(src, seg, n):
    return jax.ops.segment_sum(src, seg, n)
class _Rng:
    def __init__(self, key):
        self._k = key
    def _next(self):
        self._k, sub = jax.random.split(self._k)
        return sub
    def normal(self, shape):
        return jax.random.normal(self._next(), shape, dtype=jnp.bfloat16)
    def randint(self, lo, hi, shape):
        return jax.random.randint(self._next(), shape, lo, hi, dtype=jnp.int32)
    def uniform(self, shape, lo=0.0, hi=1.0):
        return jax.random.uniform(self._next(), shape, jnp.bfloat16, lo, hi)
    def permutation(self, n):
        return jax.random.permutation(self._next(), n)


kernel_name = 'interleave_layers__sliding_block__moe_arch_mod__prompt'

def setup_inputs():
    _rng = _Rng(jax.random.key(int.from_bytes(__import__("os").urandom(4), "little")))
    _w = (lambda a: (lambda t: t.astype(jnp.bfloat16) if jnp.issubdtype(t.dtype, jnp.floating) else t)(jnp.asarray(a)))
    def _A_setup():
        B, S, D = 1, 2048, 1024
        return {
            "x": _w((lambda *s: _rng.normal(s) * 0.05)(B, S, D)),
            "wqkv": _w((lambda *s: _rng.normal(s) * 0.05)(D, 3 * D)),
            "wo": _w((lambda *s: _rng.normal(s) * 0.05)(D, D)),
        }
    _A_in = _A_setup()

    def _B_setup():
        B, S, D, F, C = 1, 2048, 1024, 3584, 1
        return {
            "x": _w((lambda *s: _rng.normal(s) * 0.05)(B, S, D)),
            "w_r": _w((lambda *s: _rng.normal(s) * 0.05)(D)),
            "w_gate": _w((lambda *s: _rng.normal(s) * 0.05)(D, F)),
            "w_up": _w((lambda *s: _rng.normal(s) * 0.05)(D, F)),
            "w_down": _w((lambda *s: _rng.normal(s) * 0.05)(F, D)),
        }
    _B_in = _B_setup()

    return {
        "A_x": _A_in["x"],
        "A_wqkv": _A_in["wqkv"],
        "A_wo": _A_in["wo"],
        "B_x": _B_in["x"],
        "B_w_r": _B_in["w_r"],
        "B_w_gate": _B_in["w_gate"],
        "B_w_up": _B_in["w_up"],
        "B_w_down": _B_in["w_down"],
    }

def reference(A_x, A_wqkv, A_wo, B_x, B_w_r, B_w_gate, B_w_up, B_w_down):
    def _A_ref(x, wqkv, wo):
        B, S, D = x.shape
        H = 32; Dh = D // H; W = 256
        qkv = (lambda x, *d: x.transpose(*d))((x @ wqkv).reshape(B, S, 3, H, Dh), 2, 0, 3, 1, 4)
        q, k, v = qkv[0], qkv[1], qkv[2]
        scores = jnp.einsum("bhqd,bhkd->bhqk", q, k) * (Dh ** -0.5)
        idx = jnp.arange(S)
        mask = (idx[:, None] - idx[None, :] >= 0) & (idx[:, None] - idx[None, :] < W)
        scores = jnp.where(mask[None, None], scores, -1e9)
        p = _softmax(scores, axis=-1)
        o = jnp.einsum("bhqk,bhkd->bhqd", p, v)
        return (lambda x, *d: x.transpose(*d))(o, 0, 2, 1, 3).reshape(B, S, D) @ wo

    def _B_ref(x, w_r, w_gate, w_up, w_down):
        B, S, D = x.shape
        C = 1
        r = x @ w_r
        idx = jnp.argsort(-r, axis=-1)[:, :C]
        idx_e = jnp.repeat(idx.reshape(B, C, 1), D, axis=2)
        x_sel = jnp.take_along_axis(x, idx_e, axis=1)
        g = _silu(x_sel @ w_gate)
        u = x_sel @ w_up
        y = (g * u) @ w_down
        r_sel = _sigmoid(jnp.take_along_axis(r, idx, axis=1))
        y = y * r_sel.reshape(B, C, 1)
        b_off = (jnp.arange(B) * S).reshape(B, 1)
        flat_idx = (idx + b_off).reshape(B * C)
        zero = (x * 0.0).reshape(B * S, D)
        upd = _scatter_add(zero, flat_idx, y.reshape(B * C, D), axis=0)
        return x + upd.reshape(B, S, D)

    x = A_x
    x = x + _A_ref(_layernorm(x, axis=-1), A_wqkv, A_wo)
    x = x + _B_ref(_layernorm(x, axis=-1), B_w_r, B_w_gate, B_w_up, B_w_down)
    x = x + _A_ref(_layernorm(x, axis=-1), A_wqkv, A_wo)
    x = x + _B_ref(_layernorm(x, axis=-1), B_w_r, B_w_gate, B_w_up, B_w_down)
    return x
```

```python
import functools
import math

import jax
import jax.numpy as jnp
from jax import lax
import jax.experimental.pallas as pl
import jax.experimental.pallas.tpu as pltpu

S, D, H, DH, WIN, F = 2048, 1024, 32, 32, 256, 3584
NB = S // 128
NG = D // 128
NU = H
TB = 512
NT = S // TB
EPS = 1e-5
NEG = -1e30
QSCALE = (DH ** -0.5) * math.log2(math.e)
LA = 4
NSB = 8
NPB = 8

bf16 = jnp.bfloat16
f32 = jnp.float32
u32 = jnp.uint32
NT_DIMS = (((1,), (1,)), ((), ()))


def _b2u(x):
    return pltpu.bitcast(x, u32)


def _u2b(x):
    return pltpu.bitcast(x, bf16)


def _pack2(a, b):
    w = pltpu.pack_elementwise([a, b], packed_dtype=bf16)
    return w if w.dtype == u32 else pltpu.bitcast(w, u32)


def _kernel(x_hbm, wqkv_hbm, wo_hbm, wr_hbm, wg_hbm, wu_hbm, wd_hbm, out_hbm,
            xin, x_s, xa, xb, k_s, qt_s, vt_s, o_s,
            wk, wq, wv, wqT, wvT, wo, wr, wg, wu, wd,
            r_s, a_s, outb, um_ref, lm_ref, ot_ref, sems, osems, *bufs):
    sb = bufs[0:NSB]
    pb = bufs[NSB:NSB + NPB]
    lb = bufs[NSB + NPB:NSB + 2 * NPB]

    def x_copy(t):
        return pltpu.make_async_copy(x_hbm.at[pl.ds(t * TB, TB), :], xin.at[pl.ds(t * TB, TB), :], sems.at[t])

    wk_copy = pltpu.make_async_copy(wqkv_hbm.at[:, pl.ds(D, D)], wk, sems.at[4])
    wq_copy = pltpu.make_async_copy(wqkv_hbm.at[:, pl.ds(0, D)], wq, sems.at[5])
    wv_copy = pltpu.make_async_copy(wqkv_hbm.at[:, pl.ds(2 * D, D)], wv, sems.at[6])
    wo_copy = pltpu.make_async_copy(wo_hbm, wo, sems.at[7])
    wr_copy = pltpu.make_async_copy(wr_hbm, wr, sems.at[8])
    wg_copy = pltpu.make_async_copy(wg_hbm, wg, sems.at[9])
    wu_copy = pltpu.make_async_copy(wu_hbm, wu, sems.at[10])
    wd_copy = pltpu.make_async_copy(wd_hbm, wd, sems.at[11])

    def out_copy(t):
        return pltpu.make_async_copy(outb.at[pl.ds(t * TB, TB), :], out_hbm.at[pl.ds(t * TB, TB), :], osems.at[t])

    x_copy(0).start()
    wk_copy.start()
    for t in range(1, NT):
        x_copy(t).start()
    wq_copy.start()
    wv_copy.start()

    row2 = lax.broadcasted_iota(jnp.int32, (64, 128), 0)
    col2 = lax.broadcasted_iota(jnp.int32, (64, 128), 1)
    um = (jnp.where(row2 > col2, jnp.uint32(0xFFFF), jnp.uint32(0))
          | jnp.where(row2 + 64 > col2, jnp.uint32(0xFFFF0000), jnp.uint32(0)))
    um_ref[...] = um
    lm_ref[...] = ~um
    for g in range(NG):
        k_s[g, 0:128, :] = jnp.zeros((128, 128), u32)
    vt_s[0] = jnp.zeros((D // 2, 128), u32)
    vt_s[1] = jnp.zeros((D // 2, 128), u32)

    def store_ln(r0, nrows, xc, c):
        xn = xc * c
        xa[pl.ds(r0, nrows), :] = xn.astype(bf16)
        for b in range(nrows // 128):
            h0 = pl.multiple_of((r0 + 128 * b) // 2, 64)
            xb[pl.ds(h0, 64), :] = _pack2(xn[128 * b:128 * b + 64], xn[128 * b + 64:128 * b + 128])

    def plain_ln(r0, nrows, x):
        mu = jnp.mean(x, axis=1, keepdims=True)
        xc = x - mu
        var = jnp.mean(xc * xc, axis=1, keepdims=True)
        store_ln(r0, nrows, xc, lax.rsqrt(var + EPS))

    for t in range(NT):
        x_copy(t).wait()
        for b in range(TB // 128):
            r0 = t * TB + 128 * b
            x = xin[r0:r0 + 128, :].astype(f32)
            x_s[r0:r0 + 128, :] = x
            plain_ln(r0, 128, x)

    wk_copy.wait()
    wo_copy.start()
    wr_copy.start()
    wq_copy.wait()
    for j in range(NG):
        wqT[128 * j:128 * j + 128, :] = wq[:, 128 * j:128 * j + 128].T
    wv_copy.wait()
    for j in range(NG):
        wvT[128 * j:128 * j + 128, :] = wv[:, 128 * j:128 * j + 128].T
    wg_copy.start()
    wu_copy.start()
    wd_copy.start()

    def proj(t, c):
        r0 = pl.multiple_of(t * TB, TB)
        xa_t = xa[pl.ds(r0, TB), :]
        kk = jnp.dot(xa_t, wk[...], preferred_element_type=f32)
        kr = pl.multiple_of(128 + t * (TB // 2), 128)
        for g in range(NG):
            k_s[g, pl.ds(kr, TB // 2), :] = _b2u(kk[:, 128 * g:128 * g + 128].astype(bf16))
        qt = lax.dot_general(wqT[...], xa_t, NT_DIMS, preferred_element_type=f32)
        for b in range(TB // 128):
            qt_s[t * (TB // 128) + b] = _b2u((qt[:, 128 * b:128 * b + 128] * QSCALE).astype(bf16))
        xb_t = _u2b(xb[pl.ds(pl.multiple_of(t * (TB // 2), TB // 2), TB // 2), :])
        vt = lax.dot_general(wvT[...], xb_t, NT_DIMS, preferred_element_type=f32)
        for b in range(TB // 128):
            vt_s[t * (TB // 128) + b + 2] = _b2u(vt[:, 128 * b:128 * b + 128].astype(bf16))
        return c

    CH = 16

    def stage_a(i, u):
        g, h = u // 4, u % 4
        s_ref = sb[u % NSB]
        r0 = pl.multiple_of(i * 64, 64)
        parts = []
        for j in range(128 // CH):
            parts.append(k_s[g, pl.ds(r0 + (CH // 2) * j, CH // 2), :])
            parts.append(k_s[g, pl.ds(r0 + 128 + (CH // 2) * j, CH // 2), :])
        parts.append(k_s[g, pl.ds(r0 + 64, 64), :])
        kt = _u2b(jnp.concatenate(parts, axis=0))
        z = jnp.zeros((16, 128), u32)
        parts = [z] * 4
        parts[h] = qt_s[i, pl.ds(16 * u, 16), :]
        rhs = _u2b(jnp.concatenate(parts, axis=0))
        st = jnp.dot(kt, rhs, preferred_element_type=f32)
        d = lax.broadcasted_iota(jnp.int32, (CH, 128), 1) - lax.broadcasted_iota(jnp.int32, (CH, 128), 0)
        for j in range(128 // CH):
            umask = d < CH * j
            su = st[2 * CH * j:2 * CH * j + CH]
            sl = st[2 * CH * j + CH:2 * CH * j + 2 * CH]
            s_ref[CH * j:CH * j + CH, :] = jnp.where(umask, su, sl)
        s_ref[128:256, :] = st[256:384]

    def stage_b(i, u, masked):
        s_ref = sb[u % NSB]
        p_ref = pb[u % NPB]
        l_ref = lb[u % NPB]
        s = s_ref[...]
        if masked:
            row = lax.broadcasted_iota(jnp.int32, (256, 128), 0)
            col = lax.broadcasted_iota(jnp.int32, (256, 128), 1)
            key = jnp.where(row < 128, jnp.where(row > col, row - 256, row), row - 256) + i * 128
            s = jnp.where(key >= 0, s, NEG)
        m = jnp.max(s, axis=0, keepdims=True)
        p = jnp.exp2(s - m)
        l_ref[...] = jnp.sum(p, axis=0, keepdims=True)
        p_ref[0:64, :] = _pack2(p[0:64], p[64:128])
        p_ref[64:128, :] = _pack2(p[128:192], p[192:256])

    def stage_c(i, u):
        g, h = u // 4, u % 4
        p_ref = pb[u % NPB]
        l_ref = lb[u % NPB]
        r0 = pl.multiple_of(i * 128, 128)
        vt = jnp.concatenate([_u2b(vt_s[i + t, pl.ds(16 * u, 16), :]) for t in range(3)], axis=1)
        pg = p_ref[0:64, :]
        p = jnp.concatenate([pg & um_ref[...], p_ref[64:128, :], pg & lm_ref[...]], axis=0)
        o = jnp.dot(vt, _u2b(p), preferred_element_type=f32)
        ot_ref[32 * h:32 * h + 32, :] = o * (1.0 / l_ref[...])
        if h == 3:
            o_s[pl.ds(r0, 128), 128 * g:128 * g + 128] = ot_ref[...].T.astype(bf16)

    def attn_body(i, c, masked):
        inext = jnp.minimum(i + 1, NB - 1)
        for u in range(NU):
            if u + LA < NU:
                stage_a(i, u + LA)
            else:
                stage_a(inext, u + LA - NU)
            stage_b(i, u, masked)
            if u >= 1:
                stage_c(i, u - 1)
            elif not masked:
                stage_c(i - 1, NU - 1)
            else:
                @pl.when(i > 0)
                def _():
                    stage_c(i - 1, NU - 1)
        return c

    def outproj(t, c, layer):
        r0 = pl.multiple_of(t * TB, TB)
        acc = jnp.dot(o_s[pl.ds(r0, TB), :], wo[...], preferred_element_type=f32)
        x1 = x_s[pl.ds(r0, TB), :] + acc
        mu = jnp.mean(x1, axis=1, keepdims=True)
        xc = x1 - mu
        var = jnp.mean(xc * xc, axis=1, keepdims=True)
        a = lax.rsqrt(var + EPS)
        r = jnp.sum(xc * wr[...].astype(f32), axis=1, keepdims=True) * a
        r_s[pl.ds(r0, TB), :] = r
        a_s[pl.ds(r0, TB), :] = a
        x2 = x1 + xc * a
        x_s[pl.ds(r0, TB), :] = x2

        @pl.when(layer == 0)
        def _():
            a1 = 1.0 + a
            store_ln(r0, TB, xc, a1 * lax.rsqrt(var * a1 * a1 + EPS))

        @pl.when(layer == 1)
        def _():
            outb[pl.ds(r0, TB), :] = x2.astype(bf16)
            out_copy(t).start()
        return c

    def layer_body(layer, c):
        lax.fori_loop(0, NT, proj, 0)
        for u in range(LA):
            stage_a(0, u)
        lax.fori_loop(0, 2, functools.partial(attn_body, masked=True), 0)
        lax.fori_loop(2, NB, functools.partial(attn_body, masked=False), 0)
        stage_c(NB - 1, NU - 1)

        @pl.when(layer == 0)
        def _():
            wo_copy.wait()
            wr_copy.wait()

        lax.fori_loop(0, NT, functools.partial(outproj, layer=layer), 0)

        @pl.when(layer == 0)
        def _():
            wg_copy.wait()
            wu_copy.wait()
            wd_copy.wait()

        r = r_s[...]
        rmax = jnp.max(r)
        rows = lax.broadcasted_iota(jnp.int32, (S, 1), 0)
        idx = jnp.min(jnp.where(r == rmax, rows, S))
        idx = jnp.minimum(idx, S - 1)
        xrow = x_s[pl.ds(idx, 1), :]
        arow = a_s[pl.ds(idx, 1), :]
        xsel = (xrow - jnp.mean(xrow, axis=1, keepdims=True)) * (arow / (1.0 + arow))
        xs = jnp.broadcast_to(xsel, (8, D)).astype(bf16)
        gate = jnp.dot(xs, wg[...], preferred_element_type=f32)
        up = jnp.dot(xs, wu[...], preferred_element_type=f32)
        hid = (gate * jax.nn.sigmoid(gate) * up).astype(bf16)
        y = jnp.dot(hid, wd[...], preferred_element_type=f32)[0:1, :]
        x_s[pl.ds(idx, 1), :] = xrow + y * jax.nn.sigmoid(rmax)

        @pl.when(layer == 0)
        def _():
            b0 = pl.multiple_of((idx // 128) * 128, 128)
            plain_ln(b0, 128, x_s[pl.ds(b0, 128), :])

        @pl.when(layer == 1)
        def _():
            for t in range(NT):
                out_copy(t).wait()
            b0 = pl.multiple_of((idx // 16) * 16, 16)
            outb[pl.ds(b0, 16), :] = x_s[pl.ds(b0, 16), :].astype(bf16)
            fix = pltpu.make_async_copy(outb.at[pl.ds(b0, 16), :], out_hbm.at[pl.ds(b0, 16), :], osems.at[NT])
            fix.start()
            fix.wait()
        return c

    lax.fori_loop(0, 2, layer_body, 0)


@jax.jit
def pallas_interleave_layers__sliding_block__moe_arch_mod__prompt_kernel(
    A_x: jax.Array,
    A_wqkv: jax.Array,
    A_wo: jax.Array,
    B_x: jax.Array,
    B_w_r: jax.Array,
    B_w_gate: jax.Array,
    B_w_up: jax.Array,
    B_w_down: jax.Array,
):
    del B_x
    x = A_x.reshape(S, D)
    wr = B_w_r.reshape(1, D)
    any_spec = pl.BlockSpec(memory_space=pl.ANY)
    scratch = [
        pltpu.VMEM((S, D), bf16),
        pltpu.VMEM((S, D), f32),
        pltpu.VMEM((S, D), bf16),
        pltpu.VMEM((S // 2, D), u32),
        pltpu.VMEM((NG, (S + 256) // 2, 128), u32),
        pltpu.VMEM((NB, D // 2, 128), u32),
        pltpu.VMEM((NB + 2, D // 2, 128), u32),
        pltpu.VMEM((S, D), bf16),
        pltpu.VMEM((D, D), bf16),
        pltpu.VMEM((D, D), bf16),
        pltpu.VMEM((D, D), bf16),
        pltpu.VMEM((D, D), bf16),
        pltpu.VMEM((D, D), bf16),
        pltpu.VMEM((D, D), bf16),
        pltpu.VMEM((1, D), bf16),
        pltpu.VMEM((D, F), bf16),
        pltpu.VMEM((D, F), bf16),
        pltpu.VMEM((F, D), bf16),
        pltpu.VMEM((S, 1), f32),
        pltpu.VMEM((S, 1), f32),
        pltpu.VMEM((S, D), bf16),
        pltpu.VMEM((64, 128), u32),
        pltpu.VMEM((64, 128), u32),
        pltpu.VMEM((128, 128), f32),
        pltpu.SemaphoreType.DMA((12,)),
        pltpu.SemaphoreType.DMA((NT + 1,)),
    ]
    scratch += [pltpu.VMEM((256, 128), f32)] * NSB
    scratch += [pltpu.VMEM((128, 128), u32)] * NPB
    scratch += [pltpu.VMEM((1, 128), f32)] * NPB
    out = pl.pallas_call(
        _kernel,
        out_shape=jax.ShapeDtypeStruct((S, D), bf16),
        in_specs=[any_spec] * 7,
        out_specs=any_spec,
        scratch_shapes=scratch,
        compiler_params=pltpu.CompilerParams(vmem_limit_bytes=110 * 1024 * 1024),
    )(x, A_wqkv, A_wo, wr, B_w_gate, B_w_up, B_w_down)
    return out.reshape(1, S, D)
```

```python
import functools
import math

import jax
import jax.numpy as jnp
from jax import lax
import jax.experimental.pallas as pl
import jax.experimental.pallas.tpu as pltpu

S, D, H, DH, WIN, F = 2048, 1024, 32, 32, 256, 3584
NB = S // 128
NG = D // 128
NU = H
TB = 512
NT = S // TB
EPS = 1e-5
NEG = -1e30
QSCALE = (DH ** -0.5) * math.log2(math.e)
LA = 4
NSB = 2
NPB = 2

bf16 = jnp.bfloat16
f32 = jnp.float32
u32 = jnp.uint32
NT_DIMS = (((1,), (1,)), ((), ()))


def _b2u(x):
    return pltpu.bitcast(x, u32)


def _u2b(x):
    return pltpu.bitcast(x, bf16)


def _pack2(a, b):
    w = pltpu.pack_elementwise([a, b], packed_dtype=bf16)
    return w if w.dtype == u32 else pltpu.bitcast(w, u32)


def _kernel(x_hbm, wqkv_hbm, wo_hbm, wr_hbm, wg_hbm, wu_hbm, wd_hbm, out_hbm,
            xin, x_s, xa, xb, k_s, qt_s, vt_s, o_s,
            wk, wq, wv, wqT, wvT, wo, wou, wr, wg, wu, wd,
            r_s, a_s, outb, um_ref, lm_ref, ot_ref, sems, osems, *bufs):
    sb = bufs[0:NSB]
    pb = bufs[NSB:NSB + NPB]
    lb = bufs[NSB + NPB:NSB + 2 * NPB]

    def x_copy(t):
        return pltpu.make_async_copy(x_hbm.at[pl.ds(t * TB, TB), :], xin.at[pl.ds(t * TB, TB), :], sems.at[t])

    wk_copy = pltpu.make_async_copy(wqkv_hbm.at[:, pl.ds(D, D)], wk, sems.at[4])
    wq_copy = pltpu.make_async_copy(wqkv_hbm.at[:, pl.ds(0, D)], wq, sems.at[5])
    wv_copy = pltpu.make_async_copy(wqkv_hbm.at[:, pl.ds(2 * D, D)], wv, sems.at[6])
    wo_copy = pltpu.make_async_copy(wo_hbm, wo, sems.at[7])
    wr_copy = pltpu.make_async_copy(wr_hbm, wr, sems.at[8])
    wg_copy = pltpu.make_async_copy(wg_hbm, wg, sems.at[9])
    wu_copy = pltpu.make_async_copy(wu_hbm, wu, sems.at[10])
    wd_copy = pltpu.make_async_copy(wd_hbm, wd, sems.at[11])

    def out_copy(i):
        r0 = pl.multiple_of(i * 128, 128)
        return pltpu.make_async_copy(outb.at[pl.ds(r0, 128), :], out_hbm.at[pl.ds(r0, 128), :], osems.at[i])

    x_copy(0).start()
    wk_copy.start()

    row2 = lax.broadcasted_iota(jnp.int32, (64, 128), 0)
    col2 = lax.broadcasted_iota(jnp.int32, (64, 128), 1)
    um = (jnp.where(row2 > col2, jnp.uint32(0xFFFF), jnp.uint32(0))
          | jnp.where(row2 + 64 > col2, jnp.uint32(0xFFFF0000), jnp.uint32(0)))
    um_ref[...] = um
    lm_ref[...] = ~um
    for g in range(NG):
        k_s[g, 0:128, :] = jnp.zeros((128, 128), u32)
    vt_s[0] = jnp.zeros((D // 2, 128), u32)
    vt_s[1] = jnp.zeros((D // 2, 128), u32)

    def store_ln(r0, xn):
        h0 = pl.multiple_of(r0 // 2, 64)
        xa[pl.ds(h0, 64), :] = _b2u(xn.astype(bf16))
        xb[pl.ds(h0, 64), :] = _pack2(xn[0:64], xn[64:128])

    def plain_ln(r0, x):
        mu = jnp.mean(x, axis=1, keepdims=True)
        xc = x - mu
        var = jnp.mean(xc * xc, axis=1, keepdims=True)
        store_ln(r0, xc * lax.rsqrt(var + EPS))

    def kblock(b):
        static = isinstance(b, int)
        r = b * 64 if static else pl.multiple_of(b * 64, 64)
        xa_t = _u2b(xa[pl.ds(r, 64), :])
        kk = jnp.dot(xa_t, wk[...], preferred_element_type=f32)
        kr = 128 + r if static else pl.multiple_of(128 + r, 64)
        for g in range(NG):
            k_s[g, pl.ds(kr, 64), :] = _b2u(kk[:, 128 * g:128 * g + 128].astype(bf16))

    def ln0(b):
        r0 = 128 * b
        x = xin[r0:r0 + 128, :].astype(f32)
        x_s[r0:r0 + 128, :] = x
        plain_ln(r0, x)

    with jax.named_scope("p0_wait_x0"):
        x_copy(0).wait()
        x_copy(1).start()
    with jax.named_scope("p1_ln"):
        for b in range(4):
            ln0(b)
    with jax.named_scope("p2_wait"):
        wk_copy.wait()
        wq_copy.start()
        x_copy(2).start()
        x_copy(1).wait()
    with jax.named_scope("p3_k"):
        for b in range(4):
            kblock(b)
            ln0(4 + b)
    with jax.named_scope("p4_wait"):
        x_copy(3).start()
        wv_copy.start()
        x_copy(2).wait()
        wq_copy.wait()
    with jax.named_scope("p5_k"):
        for b in range(4):
            kblock(4 + b)
            ln0(8 + b)
            for j in range(2 * b, 2 * b + 2):
                wqT[64 * j:64 * j + 64, :] = _b2u(wq[:, 128 * j:128 * j + 128].T)
    with jax.named_scope("p6_wait"):
        wo_copy.start()
        wr_copy.start()
        x_copy(3).wait()
        wv_copy.wait()
    with jax.named_scope("p7_k"):
        for b in range(4):
            kblock(8 + b)
            ln0(12 + b)
            for j in range(2 * b, 2 * b + 2):
                wvT[64 * j:64 * j + 64, :] = _b2u(wv[:, 128 * j:128 * j + 128].T)
    with jax.named_scope("p8_wait"):
        wg_copy.start()
        wu_copy.start()
        wd_copy.start()
        wo_copy.wait()
        wr_copy.wait()
    with jax.named_scope("p9_k"):
        for b in range(4):
            kblock(12 + b)
            for j in range(2 * b, 2 * b + 2):
                wou[64 * j:64 * j + 64, :] = _b2u(wo[128 * j:128 * j + 128, :])

    def q_slice(xa_blk, qt_blk, n):
        lhs = _u2b(wqT[64 * n:64 * n + 64, :])
        rhs = _u2b(xa_blk[...])
        q = lax.dot_general(lhs, rhs, NT_DIMS, preferred_element_type=f32)
        qt_blk[64 * n:64 * n + 64, :] = _b2u((q * QSCALE).astype(bf16))

    def v_slice(xb_blk, vt_blk, n):
        lhs = _u2b(wvT[64 * n:64 * n + 64, :])
        rhs = _u2b(xb_blk[...])
        v = lax.dot_general(lhs, rhs, NT_DIMS, preferred_element_type=f32)
        vt_blk[64 * n:64 * n + 64, :] = _b2u(v.astype(bf16))

    def o_slice(o_blk, x_blk, n):
        lhs = _u2b(o_blk[...])
        rhs = _u2b(wou[:, 128 * n:128 * n + 128])
        acc = jnp.dot(lhs, rhs, preferred_element_type=f32)
        x_blk[:, 128 * n:128 * n + 128] = x_blk[:, 128 * n:128 * n + 128] + acc

    def epilogue(j, x_blk, xa_blk, xb_blk, layer):
        r0 = pl.multiple_of(j * 128, 128)
        x1 = x_blk[...]
        mu = jnp.mean(x1, axis=1, keepdims=True)
        xc = x1 - mu
        var = jnp.mean(xc * xc, axis=1, keepdims=True)
        a = lax.rsqrt(var + EPS)
        r = jnp.sum(xc * wr[...].astype(f32), axis=1, keepdims=True) * a
        r_s[pl.ds(r0, 128), :] = r
        a_s[pl.ds(r0, 128), :] = a
        a1 = 1.0 + a
        x2 = mu + xc * a1
        x_blk[...] = x2
        if layer == 0:
            xn = xc * (a1 * lax.rsqrt(var * a1 * a1 + EPS))
            xa_blk[...] = _b2u(xn.astype(bf16))
            xb_blk[...] = _pack2(xn[0:64], xn[64:128])
        else:
            outb[pl.ds(r0, 128), :] = x2.astype(bf16)

    def views(i, lo):
        r = pl.multiple_of((i + lo) * 64, 64)
        xav = xa.at[pl.ds(r, 192), :]
        xbv = xb.at[pl.ds(r, 192), :]
        ov = o_s.at[pl.ds(r, 128), :]
        return xav, xbv, ov

    CH = 16
    ORDER = "adbc"
    def stage_a(kv, qt_blk, g):
        s_ref = sb[g % NSB]
        parts = []
        for j in range(128 // CH):
            parts.append(kv[g, (CH // 2) * j:(CH // 2) * (j + 1), :])
            parts.append(kv[g, 128 + (CH // 2) * j:128 + (CH // 2) * (j + 1), :])
        parts.append(kv[g, 64:128, :])
        kt = _u2b(jnp.concatenate(parts, axis=0))
        z = jnp.zeros((16, 128), u32)
        cols = []
        for h in range(4):
            parts = [z] * 4
            parts[h] = qt_blk[64 * g + 16 * h:64 * g + 16 * h + 16, :]
            cols.append(_u2b(jnp.concatenate(parts, axis=0)))
        rhs = jnp.concatenate(cols, axis=1)
        st = jnp.dot(kt, rhs, preferred_element_type=f32)
        d = lax.broadcasted_iota(jnp.int32, (CH, 128), 1) - lax.broadcasted_iota(jnp.int32, (CH, 128), 0)
        for j in range(128 // CH):
            umask = d < CH * j
            for h in range(4):
                su = st[2 * CH * j:2 * CH * j + CH, 128 * h:128 * h + 128]
                sl = st[2 * CH * j + CH:2 * CH * j + 2 * CH, 128 * h:128 * h + 128]
                s_ref[h, CH * j:CH * j + CH, :] = jnp.where(umask, su, sl)
        for h in range(4):
            s_ref[h, 128:256, :] = st[256:384, 128 * h:128 * h + 128]

    def stage_b(i, g, masked):
        s_ref = sb[g % NSB]
        p_ref = pb[g % NPB]
        l_ref = lb[g % NPB]
        for h in range(4):
            s = s_ref[h]
            if masked:
                row = lax.broadcasted_iota(jnp.int32, (256, 128), 0)
                col = lax.broadcasted_iota(jnp.int32, (256, 128), 1)
                key = jnp.where(row < 128, jnp.where(row > col, row - 256, row), row - 256) + i * 128
                s = jnp.where(key >= 0, s, NEG)
            m = jnp.max(s, axis=0, keepdims=True)
            p = jnp.exp2(s - m)
            l_ref[h] = jnp.sum(p, axis=0, keepdims=True)
            p_ref[h, 0:64, :] = _pack2(p[0:64], p[64:128])
            p_ref[h, 64:128, :] = _pack2(p[128:192], p[192:256])

    def stage_c(vts, o_blk, g):
        p_ref = pb[g % NPB]
        l_ref = lb[g % NPB]
        outs = []
        for h in range(4):
            vt = jnp.concatenate([_u2b(vts[t][64 * g + 16 * h:64 * g + 16 * h + 16, :]) for t in range(3)], axis=1)
            pg = p_ref[h, 0:64, :]
            p = jnp.concatenate([pg & um_ref[...], p_ref[h, 64:128, :], pg & lm_ref[...]], axis=0)
            o = jnp.dot(vt, _u2b(p), preferred_element_type=f32)
            outs.append(o * (1.0 / l_ref[h]))
        ot = jnp.concatenate(outs, axis=0)
        o_blk[:, 128 * g:128 * g + 128] = _b2u(ot.T.astype(bf16))

    def attn_body(i, c, masked, has_next, prev, layer):
        lo = -1 if prev is True else 0
        r = pl.multiple_of((i + lo) * 64, 64)
        nblk = (2 if has_next else 1) - lo
        xav = xa.at[pl.ds(r, 64 * nblk), :]
        xbv = xb.at[pl.ds(r, 64 * nblk), :]
        ov = o_s.at[pl.ds(r, 64 * (1 - lo)), :]
        xv = x_s.at[pl.ds(pl.multiple_of((i + lo) * 128, 128), 128), :]
        qv = qt_s.at[pl.ds(i, 2)]
        vv = vt_s.at[pl.ds(i + lo, 4 - lo)]
        kv = k_s.at[:, pl.ds(pl.multiple_of(i * 64, 64), 256), :]
        blk = lambda v, b: v.at[pl.ds(64 * (b - lo), 64), :]
        vtile = lambda b: vv.at[b - lo]

        sl = []
        if has_next:
            sl.append(lambda: q_slice(blk(xav, 1), qv.at[1], 0))
        last_o = -1
        if prev is True:
            for n in range(NG):
                sl.append(functools.partial(o_slice, blk(ov, -1), xv, n))
            last_o = len(sl) - 1
        if has_next:
            for n in range(1, NG):
                sl.append(functools.partial(q_slice, blk(xav, 1), qv.at[1], n))
            for n in range(NG):
                sl.append(functools.partial(v_slice, blk(xbv, 1), vtile(3), n))
        per = -(-len(sl) // NG)

        def dense(g):
            for k in range(g * per, min((g + 1) * per, len(sl))):
                sl[k]()
                if k == last_o:
                    epilogue(i - 1, xv, blk(xav, -1), blk(xbv, -1), layer)

        if prev == "cond":
            @pl.when(i > 0)
            def _():
                finish_block(i - 1, layer)
        for g in range(NG):
            def fa():
                if g + 1 < NG:
                    stage_a(kv.at[:, pl.ds(0, 192), :], qv.at[0], g + 1)
                elif has_next:
                    stage_a(kv.at[:, pl.ds(64, 192), :], qv.at[1], 0)
            def fb():
                stage_b(i, g, masked)
            def fc():
                if g >= 1:
                    stage_c([vtile(t) for t in range(3)], blk(ov, 0), g - 1)
                elif prev is True:
                    stage_c([vtile(t - 1) for t in range(3)], blk(ov, -1), NG - 1)
            if g == 0:
                fc()
            for ch in ORDER:
                if ch == "c" and g == 0:
                    continue
                {"a": fa, "b": fb, "c": fc, "d": lambda: dense(g)}[ch]()

        if layer == 1:
            if prev is True:
                out_copy(i - 1).start()
            else:
                @pl.when(i > 0)
                def _():
                    out_copy(i - 1).start()
        return c

    def finish_block(j, layer):
        o_blk = o_s.at[pl.ds(pl.multiple_of(j * 64, 64), 64), :]
        x_blk = x_s.at[pl.ds(pl.multiple_of(j * 128, 128), 128), :]
        stage_c([vt_s.at[j + t] for t in range(3)], o_blk, NG - 1)
        for n in range(NG):
            o_slice(o_blk, x_blk, n)
        epilogue(j, x_blk, xa.at[pl.ds(pl.multiple_of(j * 64, 64), 64), :], xb.at[pl.ds(pl.multiple_of(j * 64, 64), 64), :], layer)

    def layer_body(layer, c):
        with jax.named_scope("qv0"):
            for n in range(NG):
                q_slice(xa.at[pl.ds(0, 64), :], qt_s.at[0], n)
            for n in range(NG):
                v_slice(xb.at[pl.ds(0, 64), :], vt_s.at[2], n)
            stage_a(k_s.at[:, pl.ds(0, 192), :], qt_s.at[0], 0)
        with jax.named_scope("attn"):
            lax.fori_loop(0, 2, functools.partial(attn_body, masked=True, has_next=True, prev="cond", layer=layer), 0)
            lax.fori_loop(2, NB - 1, functools.partial(attn_body, masked=False, has_next=True, prev=True, layer=layer), 0)
            attn_body(NB - 1, 0, masked=False, has_next=False, prev=True, layer=layer)
        with jax.named_scope("tail"):
            finish_block(NB - 1, layer)

        if layer == 0:
            wg_copy.wait()
            wu_copy.wait()
            wd_copy.wait()
            with jax.named_scope("ffn_mid"):
                ffn_mid()
        else:
            out_copy(NB - 1).start()
            with jax.named_scope("ffn_last"):
                ffn_last()
        return c

    FC = 512

    def route():
        r = r_s[...]
        rmax = jnp.max(r)
        rows = lax.broadcasted_iota(jnp.int32, (S, 1), 0)
        idx = jnp.min(jnp.where(r == rmax, rows, S))
        idx = jnp.minimum(idx, S - 1)
        xrow = x_s[pl.ds(idx, 1), :]
        arow = a_s[pl.ds(idx, 1), :]
        xsel = (xrow - jnp.mean(xrow, axis=1, keepdims=True)) * (arow / (1.0 + arow))
        xs = jnp.broadcast_to(xsel, (8, D)).astype(bf16)
        return idx, rmax, xrow, xs

    def ffn_up(xs, c):
        gate = jnp.dot(xs, wg[:, FC * c:FC * (c + 1)], preferred_element_type=f32)
        up = jnp.dot(xs, wu[:, FC * c:FC * (c + 1)], preferred_element_type=f32)
        return (gate * jax.nn.sigmoid(gate) * up).astype(bf16)

    def ffn_down(hid, c):
        return jnp.dot(hid, wd[FC * c:FC * (c + 1), :], preferred_element_type=f32)

    def ffn_mid():
        idx, rmax, xrow, xs = route()
        b0 = idx // 128
        y = None
        nch = F // FC
        hids = []
        for k in range(1, NB):
            kblock((b0 + k) % NB)
            if k - 1 < nch:
                hids.append(ffn_up(xs, k - 1))
            elif k - 1 < 2 * nch:
                part = ffn_down(hids[k - 1 - nch], k - 1 - nch)
                y = part if y is None else y + part
        x_s[pl.ds(idx, 1), :] = xrow + y[0:1, :] * jax.nn.sigmoid(rmax)
        r0 = pl.multiple_of(b0 * 128, 128)
        plain_ln(r0, x_s[pl.ds(r0, 128), :])
        kblock(b0)

    def ffn_last():
        idx, rmax, xrow, xs = route()
        hid = jnp.concatenate([ffn_up(xs, c) for c in range(F // FC)], axis=1)
        y = jnp.dot(hid, wd[...], preferred_element_type=f32)[0:1, :]
        x_s[pl.ds(idx, 1), :] = xrow + y * jax.nn.sigmoid(rmax)
        for i in range(NB):
            out_copy(i).wait()
        b0 = pl.multiple_of((idx // 16) * 16, 16)
        outb[pl.ds(b0, 16), :] = x_s[pl.ds(b0, 16), :].astype(bf16)
        fix = pltpu.make_async_copy(outb.at[pl.ds(b0, 16), :], out_hbm.at[pl.ds(b0, 16), :], osems.at[NB])
        fix.start()
        fix.wait()

    layer_body(0, 0)
    layer_body(1, 0)


@jax.jit
def pallas_interleave_layers__sliding_block__moe_arch_mod__prompt_kernel(
    A_x: jax.Array,
    A_wqkv: jax.Array,
    A_wo: jax.Array,
    B_x: jax.Array,
    B_w_r: jax.Array,
    B_w_gate: jax.Array,
    B_w_up: jax.Array,
    B_w_down: jax.Array,
):
    del B_x
    x = A_x.reshape(S, D)
    wr = B_w_r.reshape(1, D)
    any_spec = pl.BlockSpec(memory_space=pl.ANY)
    scratch = [
        pltpu.VMEM((S, D), bf16),
        pltpu.VMEM((S, D), f32),
        pltpu.VMEM((S // 2, D), u32),
        pltpu.VMEM((S // 2, D), u32),
        pltpu.VMEM((NG, (S + 256) // 2 + 64, 128), u32),
        pltpu.VMEM((NB + 1, D // 2, 128), u32),
        pltpu.VMEM((NB + 3, D // 2, 128), u32),
        pltpu.VMEM((S // 2, D), u32),
        pltpu.VMEM((D, D), bf16),
        pltpu.VMEM((D, D), bf16),
        pltpu.VMEM((D, D), bf16),
        pltpu.VMEM((D // 2, D), u32),
        pltpu.VMEM((D // 2, D), u32),
        pltpu.VMEM((D, D), bf16),
        pltpu.VMEM((D // 2, D), u32),
        pltpu.VMEM((1, D), bf16),
        pltpu.VMEM((D, F), bf16),
        pltpu.VMEM((D, F), bf16),
        pltpu.VMEM((F, D), bf16),
        pltpu.VMEM((S, 1), f32),
        pltpu.VMEM((S, 1), f32),
        pltpu.VMEM((S, D), bf16),
        pltpu.VMEM((64, 128), u32),
        pltpu.VMEM((64, 128), u32),
        pltpu.VMEM((128, 128), f32),
        pltpu.SemaphoreType.DMA((12,)),
        pltpu.SemaphoreType.DMA((NB + 1,)),
    ]
    scratch += [pltpu.VMEM((4, 256, 128), f32)] * NSB
    scratch += [pltpu.VMEM((4, 128, 128), u32)] * NPB
    scratch += [pltpu.VMEM((4, 1, 128), f32)] * NPB
    out = pl.pallas_call(
        _kernel,
        out_shape=jax.ShapeDtypeStruct((S, D), bf16),
        in_specs=[any_spec] * 7,
        out_specs=any_spec,
        scratch_shapes=scratch,
        compiler_params=pltpu.CompilerParams(vmem_limit_bytes=110 * 1024 * 1024),
    )(x, A_wqkv, A_wo, wr, B_w_gate, B_w_up, B_w_down)
    return out.reshape(1, S, D)
```

```python
import functools
import math

import jax
import jax.numpy as jnp
from jax import lax
import jax.experimental.pallas as pl
import jax.experimental.pallas.tpu as pltpu

S, D, H, DH, WIN, F = 2048, 1024, 32, 32, 256, 3584
NB = S // 128
NG = D // 128
NU = H
TB = 512
NT = S // TB
EPS = 1e-5
NEG = -1e30
QSCALE = (DH ** -0.5) * math.log2(math.e)
NEC = 2
LA = 4
NSB = 2
NPB = 2

bf16 = jnp.bfloat16
f32 = jnp.float32
u32 = jnp.uint32
NT_DIMS = (((1,), (1,)), ((), ()))


def _b2u(x):
    return pltpu.bitcast(x, u32)


def _u2b(x):
    return pltpu.bitcast(x, bf16)


def _pack2(a, b):
    w = pltpu.pack_elementwise([a, b], packed_dtype=bf16)
    return w if w.dtype == u32 else pltpu.bitcast(w, u32)


def _pack_adj(x):
    r, c = x.shape
    e = x.reshape(r // 16, 16, c)
    return _pack2(e[:, 0:8, :].reshape(r // 2, c), e[:, 8:16, :].reshape(r // 2, c))


def _kernel(x_hbm, wqkv_hbm, wo_hbm, wr_hbm, wg_hbm, wu_hbm, wd_hbm, out_hbm,
            xin, x_s, xa, xb, k_s, qt_s, vt_s, o_s,
            wk, wq, wv, wqT, wvT, wo, wou, wr, wg, wu, wd,
            r_s, a_s, outb, um_ref, lm_ref, npad, zs, sems, osems, *bufs):
    OPQ = 'p'
    zs[0] = 0
    zs[1] = 0
    sb = bufs[0:NSB]
    pb = bufs[NSB:NSB + NPB]
    lb = bufs[NSB + NPB:NSB + 2 * NPB]

    def x_copy(t):
        return pltpu.make_async_copy(x_hbm.at[pl.ds(t * TB, TB), :], xin.at[pl.ds(t * TB, TB), :], sems.at[t])

    wk_copy = pltpu.make_async_copy(wqkv_hbm.at[:, pl.ds(D, D)], wk, sems.at[4])
    wq_copy = pltpu.make_async_copy(wqkv_hbm.at[:, pl.ds(0, D)], wq, sems.at[5])
    wv_copy = pltpu.make_async_copy(wqkv_hbm.at[:, pl.ds(2 * D, D)], wv, sems.at[6])
    wo_copy = pltpu.make_async_copy(wo_hbm, wo, sems.at[7])
    wr_copy = pltpu.make_async_copy(wr_hbm, wr, sems.at[8])
    wg_copy = pltpu.make_async_copy(wg_hbm, wg, sems.at[9])
    wu_copy = pltpu.make_async_copy(wu_hbm, wu, sems.at[10])
    wd_copy = pltpu.make_async_copy(wd_hbm, wd, sems.at[11])

    def out_copy(i):
        r0 = pl.multiple_of(i * 128, 128)
        return pltpu.make_async_copy(outb.at[pl.ds(r0, 128), :], out_hbm.at[pl.ds(r0, 128), :], osems.at[i])

    x_copy(0).start()
    wk_copy.start()

    row2 = lax.broadcasted_iota(jnp.int32, (64, 128), 0)
    col2 = lax.broadcasted_iota(jnp.int32, (64, 128), 1)
    um = (jnp.where(row2 > col2, jnp.uint32(0xFFFF), jnp.uint32(0))
          | jnp.where(row2 + 64 > col2, jnp.uint32(0xFFFF0000), jnp.uint32(0)))
    um_ref[...] = um
    lm_ref[...] = ~um
    ql1 = lax.broadcasted_iota(jnp.int32, (1, 128), 1) & 31
    for ii in range(3):
        for j in range(4):
            t = 256 - (128 * ii + 32 * j) if ii < 2 else 0
            n = max(0, min(256, t) - 32) + jnp.maximum(0, min(32, t) - 1 - ql1)
            npad[ii, j] = n.astype(f32)
    vt_s[0] = jnp.zeros((D // 2, 128), u32)
    vt_s[1] = jnp.zeros((D // 2, 128), u32)

    def store_ln(r0, xn):
        h0 = pl.multiple_of(r0 // 2, 64)
        xa[pl.ds(h0, 64), :] = _b2u(xn.astype(bf16))
        xb[pl.ds(h0, 64), :] = _pack_adj(xn)

    def plain_ln(r0, x):
        mu = jnp.mean(x, axis=1, keepdims=True)
        xc = x - mu
        var = jnp.mean(xc * xc, axis=1, keepdims=True)
        store_ln(r0, xc * lax.rsqrt(var + EPS))

    def kblock(b):
        static = isinstance(b, int)
        r = b * 64 if static else pl.multiple_of(b * 64, 64)
        xa_t = _u2b(xa[pl.ds(r, 64), :])
        kk = jnp.dot(xa_t, wk[...], preferred_element_type=f32)
        kr = 128 + r if static else pl.multiple_of(128 + r, 64)
        for g in range(NG):
            k_s[g, pl.ds(kr, 64), :] = _b2u(kk[:, 128 * g:128 * g + 128].astype(bf16))

    def fill_kpad():
        for g in range(NG):
            lo = k_s[g, 128:129, :] & jnp.uint32(0xFFFF)
            k_s[g, 0:128, :] = jnp.broadcast_to(lo | (lo << 16), (128, 128))

    def ln0(b):
        r0 = 128 * b
        x = xin[r0:r0 + 128, :].astype(f32)
        x_s[r0:r0 + 128, :] = x
        plain_ln(r0, x)

    with jax.named_scope("p0_wait_x0"):
        x_copy(0).wait()
        x_copy(1).start()
    with jax.named_scope("p1_ln"):
        for b in range(4):
            ln0(b)
    with jax.named_scope("p2_wait"):
        wk_copy.wait()
        wq_copy.start()
        x_copy(2).start()
        x_copy(1).wait()
    with jax.named_scope("p3_k"):
        for b in range(4):
            kblock(b)
            ln0(4 + b)
    with jax.named_scope("p4_wait"):
        x_copy(3).start()
        wv_copy.start()
        x_copy(2).wait()
        wq_copy.wait()
    with jax.named_scope("p5_k"):
        for b in range(4):
            kblock(4 + b)
            ln0(8 + b)
            for j in range(2 * b, 2 * b + 2):
                wqT[64 * j:64 * j + 64, :] = _b2u(wq[128 * j:128 * j + 128, :])
    with jax.named_scope("p6_wait"):
        wo_copy.start()
        wr_copy.start()
        x_copy(3).wait()
        wv_copy.wait()
    with jax.named_scope("p7_k"):
        for b in range(4):
            kblock(8 + b)
            ln0(12 + b)
            for j in range(2 * b, 2 * b + 2):
                wvT[64 * j:64 * j + 64, :] = _b2u(wv[:, 128 * j:128 * j + 128].T)
    with jax.named_scope("p8_wait"):
        wg_copy.start()
        wu_copy.start()
        wd_copy.start()
        wo_copy.wait()
        wr_copy.wait()
    with jax.named_scope("p9_k"):
        for b in range(4):
            kblock(12 + b)
            for j in range(2 * b, 2 * b + 2):
                wou[64 * j:64 * j + 64, :] = _b2u(wo[128 * j:128 * j + 128, :])
        fill_kpad()

    def q_slice(xa_blk, q_blk, n):
        lhs = _u2b(xa_blk[...])
        rhs = _u2b(wqT[:, 128 * n:128 * n + 128])
        q = jnp.dot(lhs, rhs, preferred_element_type=f32)
        q_blk[:, 128 * n:128 * n + 128] = _b2u((q * QSCALE).astype(bf16))

    def v_slice(xb_blk, vt_blk, n):
        lhs = _u2b(wvT[64 * n:64 * n + 64, :])
        rhs = _u2b(xb_blk[...])
        v = lax.dot_general(lhs, rhs, NT_DIMS, preferred_element_type=f32)
        vt_blk[64 * n:64 * n + 64, :] = _b2u(v.astype(bf16))

    def o_slice(o_blk, x_blk, n):
        lhs = _u2b(o_blk[...])
        rhs = _u2b(wou[:, 128 * n:128 * n + 128])
        acc = jnp.dot(lhs, rhs, preferred_element_type=f32)
        x_blk[:, 128 * n:128 * n + 128] = x_blk[:, 128 * n:128 * n + 128] + acc

    def epilogue(j, x_blk, xa_blk, xb_blk, layer, chunks=range(NEC)):
        r0 = pl.multiple_of(j * 128, 128)
        R = 128 // NEC
        for c in chunks:
            lo = R * c
            x1 = x_blk[lo:lo + R, :]
            mu = jnp.mean(x1, axis=1, keepdims=True)
            xc = x1 - mu
            var = jnp.mean(xc * xc, axis=1, keepdims=True)
            a = lax.rsqrt(var + EPS)
            r = jnp.sum(xc * wr[...].astype(f32), axis=1, keepdims=True) * a
            r_s[pl.ds(r0 + lo, R), :] = r
            a_s[pl.ds(r0 + lo, R), :] = a
            a1 = 1.0 + a
            x2 = mu + xc * a1
            x_blk[lo:lo + R, :] = x2
            if layer == 0:
                v = xc * (a1 * lax.rsqrt(var * a1 * a1 + EPS))
                xa_blk[lo // 2:(lo + R) // 2, :] = _b2u(v.astype(bf16))
                xb_blk[lo // 2:(lo + R) // 2, :] = _pack_adj(v)
            else:
                outb[pl.ds(r0 + lo, R), :] = x2.astype(bf16)

    def views(i, lo):
        r = pl.multiple_of((i + lo) * 64, 64)
        xav = xa.at[pl.ds(r, 192), :]
        xbv = xb.at[pl.ds(r, 192), :]
        ov = o_s.at[pl.ds(r, 128), :]
        return xav, xbv, ov

    CH = 16
    ORDER = "a0d1d2d3c"
    EPI_EVERY = 1
    lane8b = lax.broadcasted_iota(jnp.int32, (8, 128), 1) >> 5
    odd = (lane8b & 1) == 1
    high = lane8b >= 2
    lane16b = lax.broadcasted_iota(jnp.int32, (16, 128), 1) >> 5
    d32 = lax.broadcasted_iota(jnp.int32, (32, 128), 0) - (lax.broadcasted_iota(jnp.int32, (32, 128), 1) & 31)
    umask = d32 > 0

    def stage_a(kv, q_blk, g):
        s_ref = sb[g % NSB]
        qg = q_blk[:, 128 * g:128 * g + 128]
        for j in range(4):
            qj = qg[16 * j:16 * j + 16]
            x = jnp.concatenate([jnp.where(lane16b == ((b - j) % 4), qj, jnp.uint32(0)) for b in range(4)], axis=0)
            b0 = 16 * j
            kt = jnp.concatenate([kv[g, b0:b0 + 8, :], kv[g, b0 + 128:b0 + 136, :], kv[g, b0 + 8:b0 + 16, :],
                                  kv[g, b0 + 136:b0 + 144, :], kv[g, b0 + 16:b0 + 128, :]], axis=0)
            st = lax.dot_general(_u2b(kt), _u2b(x), NT_DIMS, preferred_element_type=f32)
            su = jnp.concatenate([st[0:16], st[32:48]], axis=0)
            sl = jnp.concatenate([st[16:32], st[48:64]], axis=0)
            s_ref[j, 0:32, :] = jnp.where(umask, su, sl)
            s_ref[j, 32:256, :] = st[64:288]

    def stage_b(i, g, masked, heads=range(4)):
        if list(heads) != [0]:
            return
        s_ref = sb[g % NSB]
        p_ref = pb[g % NPB].at[zs[0] if 'p' in OPQ else 0]
        l_ref = lb[g % NPB]
        pps = []
        for j in range(4):
            s = s_ref[j]
            m = jnp.max(s, axis=0, keepdims=True)
            p = jnp.exp2(s - m)
            l_ref[j] = jnp.sum(p, axis=0, keepdims=True) - npad[jnp.minimum(i, 2), j] * p[32:33]
            pm = p[0:32]
            e = jnp.concatenate([jnp.where(umask, pm, 0.0), p[32:256], jnp.where(umask, 0.0, pm)], axis=0)
            pps.append(_pack_adj(e))
        for M in range(24):
            y = [pps[j][8 * (M - 2 * j):8 * (M - 2 * j) + 8, :] if 0 <= M - 2 * j < 18 else None for j in range(4)]
            w = bfly(y)
            for h in range(4):
                p_ref[h, 8 * M:8 * M + 8, :] = w[h] if w[h] is not None else jnp.zeros((8, 128), u32)

    def bfly(y):
        def sel(m, a, b):
            if a is None and b is None:
                return None
            z = jnp.zeros((8, 128), (a if a is not None else b).dtype)
            return jnp.where(m, z if a is None else a, z if b is None else b)
        r = [sel(odd, y[(k + 1) % 4], y[k]) for k in range(4)]
        wp = [sel(high, r[(k + 2) % 4], r[k]) for k in range(4)]
        return [wp[(-h) % 4] for h in range(4)]

    def stage_c(vts, o_blk, g):
        p_ref = pb[g % NPB].at[zs[1] if 'p' in OPQ else 0]
        l_ref = lb[g % NPB]
        lh = bfly([jnp.broadcast_to(1.0 / l_ref[j], (8, 128)) for j in range(4)])
        outs = []
        for h in range(4):
            vt = jnp.concatenate([_u2b(vts[t][64 * g + 16 * h:64 * g + 16 * h + 16, :]) for t in range(3)], axis=1)
            o = jnp.dot(vt, _u2b(p_ref[h]), preferred_element_type=f32)
            o = o * lh[h][0:1]
            if h:
                o = pltpu.roll(o, 128 - 32 * h, 1)
            outs.append(o)
        ot = jnp.concatenate(outs, axis=0)
        o_blk[:, 128 * g:128 * g + 128] = _b2u(ot.T.astype(bf16))

    def attn_body(i, c, masked, has_next, prev, layer):
        lo = -1 if prev is True else 0
        r = pl.multiple_of((i + lo) * 64, 64)
        nblk = (2 if has_next else 1) - lo
        xav = xa.at[pl.ds(r, 64 * nblk), :]
        xbv = xb.at[pl.ds(r, 64 * nblk), :]
        ov = o_s.at[pl.ds(r, 64 * (1 - lo)), :]
        xv = x_s.at[pl.ds(pl.multiple_of((i + lo) * 128, 128), 128), :]
        qv = qt_s.at[pl.ds(i, 2)]
        vv = vt_s.at[pl.ds(i + lo, 4 - lo)]
        kv = k_s.at[:, pl.ds(pl.multiple_of(i * 64, 64), 256), :]
        blk = lambda v, b: v.at[pl.ds(64 * (b - lo), 64), :]
        vtile = lambda b: vv.at[b - lo]

        sl = []
        if has_next:
            sl.append(lambda: q_slice(blk(xav, 1), qv.at[1], 0))
        last_o = -1
        if prev is True:
            for n in range(NG):
                sl.append(functools.partial(o_slice, blk(ov, -1), xv, n))
            last_o = len(sl) - 1
        if has_next:
            for n in range(1, NG):
                sl.append(functools.partial(q_slice, blk(xav, 1), qv.at[1], n))
            for n in range(NG):
                sl.append(functools.partial(v_slice, blk(xbv, 1), vtile(3), n))
        per = -(-len(sl) // NG)
        emitted = [0]
        epi_done = [0]

        def dense_one():
            k = emitted[0]
            if k < len(sl):
                sl[k]()
                emitted[0] += 1
                if prev is True and k > last_o and epi_done[0] < NEC and (k - last_o) % EPI_EVERY == 0:
                    epilogue(i - 1, xv, blk(xav, -1), blk(xbv, -1), layer, [epi_done[0]])
                    epi_done[0] += 1

        if prev == "cond":
            @pl.when(i > 0)
            def _():
                finish_block(i - 1, layer)
        for g in range(NG):
            def fa():
                if g + 1 < NG:
                    stage_a(kv.at[:, pl.ds(0, 192), :], qv.at[0], g + 1)
                elif has_next:
                    stage_a(kv.at[:, pl.ds(64, 192), :], qv.at[1], 0)
            def fc():
                if g >= 1:
                    stage_c([vtile(t) for t in range(3)], blk(ov, 0), g - 1)
                elif prev is True:
                    stage_c([vtile(t - 1) for t in range(3)], blk(ov, -1), NG - 1)
            if g == 0:
                fc()
            nd = 0
            for ch in ORDER:
                if ch == "a":
                    fa()
                elif ch == "c":
                    if g > 0:
                        fc()
                elif ch == "d":
                    if nd < per:
                        dense_one()
                        nd += 1
                else:
                    stage_b(i, g, masked, [int(ch)])
        while emitted[0] < len(sl):
            dense_one()
        if prev is True:
            while epi_done[0] < NEC:
                epilogue(i - 1, xv, blk(xav, -1), blk(xbv, -1), layer, [epi_done[0]])
                epi_done[0] += 1

        if layer == 1 and prev is True:
            out_copy(i - 1).start()
        return c

    def finish_block(j, layer):
        o_blk = o_s.at[pl.ds(pl.multiple_of(j * 64, 64), 64), :]
        x_blk = x_s.at[pl.ds(pl.multiple_of(j * 128, 128), 128), :]
        stage_c([vt_s.at[j + t] for t in range(3)], o_blk, NG - 1)
        for n in range(NG):
            o_slice(o_blk, x_blk, n)
        epilogue(j, x_blk, xa.at[pl.ds(pl.multiple_of(j * 64, 64), 64), :], xb.at[pl.ds(pl.multiple_of(j * 64, 64), 64), :], layer)

    def layer_body(layer, c):
        with jax.named_scope("qv0"):
            for n in range(NG):
                q_slice(xa.at[pl.ds(0, 64), :], qt_s.at[0], n)
            for n in range(NG):
                v_slice(xb.at[pl.ds(0, 64), :], vt_s.at[2], n)
            stage_a(k_s.at[:, pl.ds(0, 192), :], qt_s.at[0], 0)
        with jax.named_scope("attn"):
            attn_body(0, 0, masked=False, has_next=True, prev=False, layer=layer)
            lax.fori_loop(1, NB - 1, functools.partial(attn_body, masked=False, has_next=True, prev=True, layer=layer), 0)
            attn_body(NB - 1, 0, masked=False, has_next=False, prev=True, layer=layer)
        with jax.named_scope("tail"):
            finish_block(NB - 1, layer)

        if layer == 0:
            wg_copy.wait()
            wu_copy.wait()
            wd_copy.wait()
            with jax.named_scope("ffn_mid"):
                ffn_mid()
        else:
            out_copy(NB - 1).start()
            with jax.named_scope("ffn_last"):
                ffn_last()
        return c

    FC = 512

    def route():
        r = r_s[...]
        rmax = jnp.max(r)
        rows = lax.broadcasted_iota(jnp.int32, (S, 1), 0)
        idx = jnp.min(jnp.where(r == rmax, rows, S))
        idx = jnp.minimum(idx, S - 1)
        xrow = x_s[pl.ds(idx, 1), :]
        arow = a_s[pl.ds(idx, 1), :]
        xsel = (xrow - jnp.mean(xrow, axis=1, keepdims=True)) * (arow / (1.0 + arow))
        xs = jnp.broadcast_to(xsel, (8, D)).astype(bf16)
        return idx, rmax, xrow, xs

    def ffn_up(xs, c):
        gate = jnp.dot(xs, wg[:, FC * c:FC * (c + 1)], preferred_element_type=f32)
        up = jnp.dot(xs, wu[:, FC * c:FC * (c + 1)], preferred_element_type=f32)
        return (gate * jax.nn.sigmoid(gate) * up).astype(bf16)

    def ffn_down(hid, c):
        return jnp.dot(hid, wd[FC * c:FC * (c + 1), :], preferred_element_type=f32)

    def ffn_mid():
        idx, rmax, xrow, xs = route()
        b0 = idx // 128
        y = None
        nch = F // FC
        hids = []
        for k in range(1, NB):
            kblock((b0 + k) % NB)
            if k - 1 < nch:
                hids.append(ffn_up(xs, k - 1))
            elif k - 1 < 2 * nch:
                part = ffn_down(hids[k - 1 - nch], k - 1 - nch)
                y = part if y is None else y + part
        x_s[pl.ds(idx, 1), :] = xrow + y[0:1, :] * jax.nn.sigmoid(rmax)
        r0 = pl.multiple_of(b0 * 128, 128)
        plain_ln(r0, x_s[pl.ds(r0, 128), :])
        kblock(b0)
        fill_kpad()

    def ffn_last():
        idx, rmax, xrow, xs = route()
        hid = jnp.concatenate([ffn_up(xs, c) for c in range(F // FC)], axis=1)
        y = jnp.dot(hid, wd[...], preferred_element_type=f32)[0:1, :]
        x_s[pl.ds(idx, 1), :] = xrow + y * jax.nn.sigmoid(rmax)
        for i in range(NB):
            out_copy(i).wait()
        b0 = pl.multiple_of((idx // 16) * 16, 16)
        outb[pl.ds(b0, 16), :] = x_s[pl.ds(b0, 16), :].astype(bf16)
        fix = pltpu.make_async_copy(outb.at[pl.ds(b0, 16), :], out_hbm.at[pl.ds(b0, 16), :], osems.at[NB])
        fix.start()
        fix.wait()

    layer_body(0, 0)
    layer_body(1, 0)


@jax.jit
def pallas_interleave_layers__sliding_block__moe_arch_mod__prompt_kernel(
    A_x: jax.Array,
    A_wqkv: jax.Array,
    A_wo: jax.Array,
    B_x: jax.Array,
    B_w_r: jax.Array,
    B_w_gate: jax.Array,
    B_w_up: jax.Array,
    B_w_down: jax.Array,
):
    del B_x
    x = A_x.reshape(S, D)
    wr = B_w_r.reshape(1, D)
    any_spec = pl.BlockSpec(memory_space=pl.ANY)
    scratch = [
        pltpu.VMEM((S, D), bf16),
        pltpu.VMEM((S, D), f32),
        pltpu.VMEM((S // 2, D), u32),
        pltpu.VMEM((S // 2, D), u32),
        pltpu.VMEM((NG, (S + 256) // 2 + 64, 128), u32),
        pltpu.VMEM((NB + 1, 64, D), u32),
        pltpu.VMEM((NB + 3, D // 2, 128), u32),
        pltpu.VMEM((S // 2, D), u32),
        pltpu.VMEM((D, D), bf16),
        pltpu.VMEM((D, D), bf16),
        pltpu.VMEM((D, D), bf16),
        pltpu.VMEM((D // 2, D), u32),
        pltpu.VMEM((D // 2, D), u32),
        pltpu.VMEM((D, D), bf16),
        pltpu.VMEM((D // 2, D), u32),
        pltpu.VMEM((1, D), bf16),
        pltpu.VMEM((D, F), bf16),
        pltpu.VMEM((D, F), bf16),
        pltpu.VMEM((F, D), bf16),
        pltpu.VMEM((S, 1), f32),
        pltpu.VMEM((S, 1), f32),
        pltpu.VMEM((S, D), bf16),
        pltpu.VMEM((64, 128), u32),
        pltpu.VMEM((64, 128), u32),
        pltpu.VMEM((3, 4, 1, 128), f32),
        pltpu.SMEM((2,), jnp.int32),
        pltpu.SemaphoreType.DMA((12,)),
        pltpu.SemaphoreType.DMA((NB + 1,)),
    ]
    scratch += [pltpu.VMEM((4, 256, 128), f32)] * NSB
    scratch += [pltpu.VMEM((1, 4, 192, 128), u32)] * NPB
    scratch += [pltpu.VMEM((4, 1, 128), f32)] * NPB
    out = pl.pallas_call(
        _kernel,
        out_shape=jax.ShapeDtypeStruct((S, D), bf16),
        in_specs=[any_spec] * 7,
        out_specs=any_spec,
        scratch_shapes=scratch,
        compiler_params=pltpu.CompilerParams(vmem_limit_bytes=110 * 1024 * 1024),
    )(x, A_wqkv, A_wo, wr, B_w_gate, B_w_up, B_w_down)
    return out.reshape(1, S, D)
```

```python
import functools
import math

import jax
import jax.numpy as jnp
from jax import lax
import jax.experimental.pallas as pl
import jax.experimental.pallas.tpu as pltpu

S, D, H, DH, WIN, F = 2048, 1024, 32, 32, 256, 3584
NB = S // 128
NG = D // 128
NU = H
TB = 512
NT = S // TB
EPS = 1e-5
NEG = -1e30
QSCALE = (DH ** -0.5) * math.log2(math.e)
NEC = 2
LA = 4
NSB = 2
NPB = 2

bf16 = jnp.bfloat16
f32 = jnp.float32
u32 = jnp.uint32
NT_DIMS = (((1,), (1,)), ((), ()))


def _b2u(x):
    return pltpu.bitcast(x, u32)


def _u2b(x):
    return pltpu.bitcast(x, bf16)


def _pack2(a, b):
    w = pltpu.pack_elementwise([a, b], packed_dtype=bf16)
    return w if w.dtype == u32 else pltpu.bitcast(w, u32)


def _pack_adj(x):
    r, c = x.shape
    e = x.reshape(r // 16, 16, c)
    return _pack2(e[:, 0:8, :].reshape(r // 2, c), e[:, 8:16, :].reshape(r // 2, c))


def _kernel(x_hbm, wqkv_hbm, wo_hbm, wr_hbm, wg_hbm, wu_hbm, wd_hbm, out_hbm,
            xin, x_s, xa, xb, k_s, qt_s, vt_s, o_s,
            wk, wq, wv, wqT, wvT, wo, wou, wr, wg, wu, wd,
            r_s, a_s, outb, um_ref, lm_ref, npad, zs, sems, osems, *bufs):
    OPQ = 'p'
    zs[0] = 0
    zs[1] = 0
    sb = bufs[0:NSB]
    pb = bufs[NSB:NSB + NPB]
    lb = bufs[NSB + NPB:NSB + 2 * NPB]

    XCH = [(0, 128), (128, 384), (512, 512), (1024, 512), (1536, 512)]

    def x_copy(t):
        r0, n = XCH[t]
        return pltpu.make_async_copy(x_hbm.at[pl.ds(r0, n), :], xin.at[pl.ds(r0, n), :], sems.at[t])

    wkl_copy = pltpu.make_async_copy(wqkv_hbm.at[:, pl.ds(D, D // 2)], wk.at[:, pl.ds(0, D // 2)], sems.at[12])
    wkr_copy = pltpu.make_async_copy(wqkv_hbm.at[:, pl.ds(D + D // 2, D // 2)], wk.at[:, pl.ds(D // 2, D // 2)], sems.at[13])
    wq_copy = pltpu.make_async_copy(wqkv_hbm.at[:, pl.ds(0, D)], wq, sems.at[5])
    wv_copy = pltpu.make_async_copy(wqkv_hbm.at[:, pl.ds(2 * D, D)], wv, sems.at[6])
    wo_copy = pltpu.make_async_copy(wo_hbm, wo, sems.at[7])
    wr_copy = pltpu.make_async_copy(wr_hbm, wr, sems.at[8])
    wg_copy = pltpu.make_async_copy(wg_hbm, wg, sems.at[9])
    wu_copy = pltpu.make_async_copy(wu_hbm, wu, sems.at[10])
    wd_copy = pltpu.make_async_copy(wd_hbm, wd, sems.at[11])

    def out_copy(i):
        r0 = pl.multiple_of(i * 128, 128)
        return pltpu.make_async_copy(outb.at[pl.ds(r0, 128), :], out_hbm.at[pl.ds(r0, 128), :], osems.at[i])

    x_copy(0).start()
    wkl_copy.start()

    row2 = lax.broadcasted_iota(jnp.int32, (64, 128), 0)
    col2 = lax.broadcasted_iota(jnp.int32, (64, 128), 1)
    um = (jnp.where(row2 > col2, jnp.uint32(0xFFFF), jnp.uint32(0))
          | jnp.where(row2 + 64 > col2, jnp.uint32(0xFFFF0000), jnp.uint32(0)))
    um_ref[...] = um
    lm_ref[...] = ~um
    ql1 = lax.broadcasted_iota(jnp.int32, (1, 128), 1) & 31
    for ii in range(3):
        for j in range(4):
            t = 256 - (128 * ii + 32 * j) if ii < 2 else 0
            n = max(0, min(256, t) - 32) + jnp.maximum(0, min(32, t) - 1 - ql1)
            npad[ii, j] = n.astype(f32)
    vt_s[0] = jnp.zeros((D // 2, 128), u32)
    vt_s[1] = jnp.zeros((D // 2, 128), u32)

    def store_ln(r0, xn):
        h0 = pl.multiple_of(r0 // 2, 64)
        xa[pl.ds(h0, 64), :] = _b2u(xn.astype(bf16))

    def plain_ln(r0, x):
        mu = jnp.mean(x, axis=1, keepdims=True)
        xc = x - mu
        var = jnp.mean(xc * xc, axis=1, keepdims=True)
        store_ln(r0, xc * lax.rsqrt(var + EPS))

    def kblock(b, g0=0, g1=NG):
        static = isinstance(b, int)
        r = b * 64 if static else pl.multiple_of(b * 64, 64)
        xa_t = _u2b(xa[pl.ds(r, 64), :])
        kk = jnp.dot(xa_t, wk[:, 128 * g0:128 * g1], preferred_element_type=f32)
        kr = 128 + r if static else pl.multiple_of(128 + r, 64)
        for g in range(g0, g1):
            k_s[g, pl.ds(kr, 64), :] = _b2u(kk[:, 128 * (g - g0):128 * (g - g0) + 128].astype(bf16))

    def fill_kpad():
        for g in range(NG):
            lo = k_s[g, 128:129, :] & jnp.uint32(0xFFFF)
            k_s[g, 0:128, :] = jnp.broadcast_to(lo | (lo << 16), (128, 128))

    def ln0(b):
        r0 = 128 * b if isinstance(b, int) else pl.multiple_of(128 * b, 128)
        x = xin[pl.ds(r0, 128), :].astype(f32)
        x_s[pl.ds(r0, 128), :] = x
        plain_ln(r0, x)

    def conv(dst, src):
        for j in range(NG):
            dst[64 * j:64 * j + 64, :] = _b2u(src[128 * j:128 * j + 128, :])

    with jax.named_scope("p0"):
        x_copy(0).wait()
        wkr_copy.start()
        ln0(0)
        wkl_copy.wait()
        x_copy(1).start()
        kblock(0, 0, NG // 2)
    with jax.named_scope("p1a"):
        wkr_copy.wait()
        kblock(0, NG // 2, NG)
    with jax.named_scope("p1"):
        x_copy(1).wait()
        x_copy(2).start()
        x_copy(3).start()
        for b in range(1, 4):
            ln0(b)
        kblock(1)
        kblock(2)
    def pro_body(t, c):
        r0 = pl.multiple_of(512 * (t + 1), 512)
        pltpu.make_async_copy(x_hbm.at[pl.ds(r0, 512), :], xin.at[pl.ds(r0, 512), :], sems.at[t + 2]).wait()

        @pl.when(t == 0)
        def _():
            x_copy(4).start()

        @pl.when(t == 1)
        def _():
            wq_copy.start()
            wv_copy.start()

        @pl.when(t == 2)
        def _():
            wo_copy.start()
            wr_copy.start()

        for b in range(4):
            kblock(4 * t + 3 + b)
            ln0(4 * t + 4 + b)
        return c

    with jax.named_scope("p2"):
        lax.fori_loop(0, 3, pro_body, 0)
    with jax.named_scope("p4"):
        wq_copy.wait()
        kblock(15)
        conv(wqT, wq)
        fill_kpad()
    with jax.named_scope("p5"):
        wv_copy.wait()
        wo_copy.wait()
        wr_copy.wait()
        conv(wvT, wv)
        conv(wou, wo)

    def q_slice(xa_blk, q_blk, n):
        lhs = _u2b(xa_blk[...])
        rhs = _u2b(wqT[:, 128 * n:128 * n + 128])
        q = jnp.dot(lhs, rhs, preferred_element_type=f32)
        qt = _b2u((q * QSCALE).astype(bf16).T)
        parts = [qt[0:16]] + [pltpu.roll(qt[16 * h:16 * h + 16], 32 * h, 1) for h in range(1, 4)]
        q_blk[64 * n:64 * n + 64, :] = jnp.concatenate(parts, axis=0)

    def v_slice(xa_blk, vt_blk, n):
        lhs = _u2b(xa_blk[...])
        rhs = _u2b(wvT[:, 128 * n:128 * n + 128])
        v = jnp.dot(lhs, rhs, preferred_element_type=f32)
        vt_blk[64 * n:64 * n + 64, :] = _b2u(_u2b(_pack_adj(v)).T)

    def o_slice(o_blk, x_blk, n):
        lhs = _u2b(o_blk[...])
        rhs = _u2b(wou[:, 128 * n:128 * n + 128])
        acc = jnp.dot(lhs, rhs, preferred_element_type=f32)
        x_blk[:, 128 * n:128 * n + 128] = x_blk[:, 128 * n:128 * n + 128] + acc

    def epilogue(j, x_blk, xa_blk, xb_blk, layer, chunks=range(NEC)):
        r0 = pl.multiple_of(j * 128, 128)
        R = 128 // NEC
        for c in chunks:
            lo = R * c
            x1 = x_blk[lo:lo + R, :]
            mu = jnp.mean(x1, axis=1, keepdims=True)
            xc = x1 - mu
            var = jnp.mean(xc * xc, axis=1, keepdims=True)
            a = lax.rsqrt(var + EPS)
            r = jnp.sum(xc * wr[...].astype(f32), axis=1, keepdims=True) * a
            r_s[pl.ds(r0 + lo, R), :] = r
            a_s[pl.ds(r0 + lo, R), :] = a
            a1 = 1.0 + a
            x2 = mu + xc * a1
            x_blk[lo:lo + R, :] = x2
            if layer == 0:
                v = xc * (a1 * lax.rsqrt(var * a1 * a1 + EPS))
                xa_blk[lo // 2:(lo + R) // 2, :] = _b2u(v.astype(bf16))
            else:
                outb[pl.ds(r0 + lo, R), :] = x2.astype(bf16)

    def views(i, lo):
        r = pl.multiple_of((i + lo) * 64, 64)
        xav = xa.at[pl.ds(r, 192), :]
        xbv = xb.at[pl.ds(r, 192), :]
        ov = o_s.at[pl.ds(r, 128), :]
        return xav, xbv, ov

    CH = 16
    ORDER = "a0d1d2d3c"
    EPI_EVERY = 1
    lane8b = lax.broadcasted_iota(jnp.int32, (8, 128), 1) >> 5
    odd = (lane8b & 1) == 1
    high = lane8b >= 2
    lane16b = lax.broadcasted_iota(jnp.int32, (16, 128), 1) >> 5
    d32 = lax.broadcasted_iota(jnp.int32, (32, 128), 0) - (lax.broadcasted_iota(jnp.int32, (32, 128), 1) & 31)
    umask = d32 > 0

    def stage_a(kv, q_blk, g):
        s_ref = sb[g % NSB]
        for j in range(4):
            x = jnp.concatenate([jnp.where(lane16b == ((h + j) % 4), q_blk[64 * g + 16 * h:64 * g + 16 * h + 16, :], jnp.uint32(0))
                                 for h in range(4)], axis=0)
            b0 = 16 * j
            kt = jnp.concatenate([kv[g, b0:b0 + 8, :], kv[g, b0 + 128:b0 + 136, :], kv[g, b0 + 8:b0 + 16, :],
                                  kv[g, b0 + 136:b0 + 144, :], kv[g, b0 + 16:b0 + 128, :]], axis=0)
            st = jnp.dot(_u2b(kt), _u2b(x), preferred_element_type=f32)
            su = jnp.concatenate([st[0:16], st[32:48]], axis=0)
            sl = jnp.concatenate([st[16:32], st[48:64]], axis=0)
            s_ref[j, 0:32, :] = jnp.where(umask, su, sl)
            s_ref[j, 32:256, :] = st[64:288]

    def stage_b(i, g, masked, heads=range(4)):
        if list(heads) != [0]:
            return
        s_ref = sb[g % NSB]
        p_ref = pb[g % NPB].at[zs[0] if 'p' in OPQ else 0]
        l_ref = lb[g % NPB]
        pps = []
        for j in range(4):
            s = s_ref[j]
            m = jnp.max(s, axis=0, keepdims=True)
            p = jnp.exp2(s - m)
            l_ref[j] = jnp.sum(p, axis=0, keepdims=True) - npad[jnp.minimum(i, 2), j] * p[32:33]
            pm = p[0:32]
            e = jnp.concatenate([jnp.where(umask, pm, 0.0), p[32:256], jnp.where(umask, 0.0, pm)], axis=0)
            pps.append(_pack_adj(e))
        for M in range(24):
            y = [pps[j][8 * (M - 2 * j):8 * (M - 2 * j) + 8, :] if 0 <= M - 2 * j < 18 else None for j in range(4)]
            w = bfly(y)
            for h in range(4):
                p_ref[h, 8 * M:8 * M + 8, :] = w[h] if w[h] is not None else jnp.zeros((8, 128), u32)

    def bfly(y):
        def sel(m, a, b):
            if a is None and b is None:
                return None
            z = jnp.zeros((8, 128), (a if a is not None else b).dtype)
            return jnp.where(m, z if a is None else a, z if b is None else b)
        r = [sel(odd, y[(k + 1) % 4], y[k]) for k in range(4)]
        wp = [sel(high, r[(k + 2) % 4], r[k]) for k in range(4)]
        return [wp[(-h) % 4] for h in range(4)]

    def stage_c(vts, o_blk, g):
        p_ref = pb[g % NPB].at[zs[1] if 'p' in OPQ else 0]
        l_ref = lb[g % NPB]
        lh = bfly([jnp.broadcast_to(1.0 / l_ref[j], (8, 128)) for j in range(4)])
        outs = []
        for h in range(4):
            vt = jnp.concatenate([_u2b(vts[t][64 * g + 16 * h:64 * g + 16 * h + 16, :]) for t in range(3)], axis=1)
            o = jnp.dot(vt, _u2b(p_ref[h]), preferred_element_type=f32)
            o = o * lh[h][0:1]
            if h:
                o = pltpu.roll(o, 128 - 32 * h, 1)
            outs.append(o)
        ot = jnp.concatenate(outs, axis=0)
        o_blk[:, 128 * g:128 * g + 128] = _b2u(ot.T.astype(bf16))

    def attn_body(i, c, masked, has_next, prev, layer):
        lo = -1 if prev is True else 0
        r = pl.multiple_of((i + lo) * 64, 64)
        nblk = (2 if has_next else 1) - lo
        xav = xa.at[pl.ds(r, 64 * nblk), :]
        xbv = xav
        ov = o_s.at[pl.ds(r, 64 * (1 - lo)), :]
        xv = x_s.at[pl.ds(pl.multiple_of((i + lo) * 128, 128), 128), :]
        qv = qt_s.at[pl.ds(i, 2)]
        vv = vt_s.at[pl.ds(i + lo, 4 - lo)]
        kv = k_s.at[:, pl.ds(pl.multiple_of(i * 64, 64), 256), :]
        blk = lambda v, b: v.at[pl.ds(64 * (b - lo), 64), :]
        vtile = lambda b: vv.at[b - lo]

        sl = []
        if has_next:
            sl.append(lambda: q_slice(blk(xav, 1), qv.at[1], 0))
        last_o = -1
        if prev is True:
            for n in range(NG):
                sl.append(functools.partial(o_slice, blk(ov, -1), xv, n))
            last_o = len(sl) - 1
        if has_next:
            for n in range(1, NG):
                sl.append(functools.partial(q_slice, blk(xav, 1), qv.at[1], n))
            for n in range(NG):
                sl.append(functools.partial(v_slice, blk(xav, 1), vtile(3), n))
        per = -(-len(sl) // NG)
        emitted = [0]
        epi_done = [0]

        def dense_one():
            k = emitted[0]
            if k < len(sl):
                sl[k]()
                emitted[0] += 1
                if prev is True and k > last_o and epi_done[0] < NEC and (k - last_o) % EPI_EVERY == 0:
                    epilogue(i - 1, xv, blk(xav, -1), blk(xbv, -1), layer, [epi_done[0]])
                    epi_done[0] += 1

        if prev == "cond":
            @pl.when(i > 0)
            def _():
                finish_block(i - 1, layer)
        for g in range(NG):
            def fa():
                if g + 1 < NG:
                    stage_a(kv.at[:, pl.ds(0, 192), :], qv.at[0], g + 1)
                elif has_next:
                    stage_a(kv.at[:, pl.ds(64, 192), :], qv.at[1], 0)
            def fc():
                if g >= 1:
                    stage_c([vtile(t) for t in range(3)], blk(ov, 0), g - 1)
                elif prev is True:
                    stage_c([vtile(t - 1) for t in range(3)], blk(ov, -1), NG - 1)
            if g == 0:
                fc()
            nd = 0
            for ch in ORDER:
                if ch == "a":
                    fa()
                elif ch == "c":
                    if g > 0:
                        fc()
                elif ch == "d":
                    if nd < per:
                        dense_one()
                        nd += 1
                else:
                    stage_b(i, g, masked, [int(ch)])
        while emitted[0] < len(sl):
            dense_one()
        if prev is True:
            while epi_done[0] < NEC:
                epilogue(i - 1, xv, blk(xav, -1), blk(xbv, -1), layer, [epi_done[0]])
                epi_done[0] += 1

        if layer == 1 and prev is True:
            out_copy(i - 1).start()
        if layer == 0 and prev is True and has_next:
            @pl.when(i == 1)
            def _():
                wg_copy.start()
                wu_copy.start()
                wd_copy.start()
        return c

    def finish_block(j, layer):
        o_blk = o_s.at[pl.ds(pl.multiple_of(j * 64, 64), 64), :]
        x_blk = x_s.at[pl.ds(pl.multiple_of(j * 128, 128), 128), :]
        stage_c([vt_s.at[j + t] for t in range(3)], o_blk, NG - 1)
        for n in range(NG):
            o_slice(o_blk, x_blk, n)
        epilogue(j, x_blk, xa.at[pl.ds(pl.multiple_of(j * 64, 64), 64), :], None, layer)

    def layer_body(layer, c):
        with jax.named_scope("qv0"):
            for n in range(NG):
                q_slice(xa.at[pl.ds(0, 64), :], qt_s.at[0], n)
            for n in range(NG):
                v_slice(xa.at[pl.ds(0, 64), :], vt_s.at[2], n)
            stage_a(k_s.at[:, pl.ds(0, 192), :], qt_s.at[0], 0)
        with jax.named_scope("attn"):
            with jax.named_scope("first"):
                attn_body(0, 0, masked=False, has_next=True, prev=False, layer=layer)
            with jax.named_scope("main"):
                lax.fori_loop(1, NB - 1, functools.partial(attn_body, masked=False, has_next=True, prev=True, layer=layer), 0)
            with jax.named_scope("last"):
                attn_body(NB - 1, 0, masked=False, has_next=False, prev=True, layer=layer)
        with jax.named_scope("tail"):
            finish_block(NB - 1, layer)

        if layer == 0:
            wg_copy.wait()
            wu_copy.wait()
            wd_copy.wait()
            with jax.named_scope("ffn_mid"):
                ffn_mid()
        else:
            out_copy(NB - 1).start()
            with jax.named_scope("ffn_last"):
                ffn_last()
        return c

    FC = 512

    def route():
        r = r_s[...]
        rmax = jnp.max(r)
        rows = lax.broadcasted_iota(jnp.int32, (S, 1), 0)
        idx = jnp.min(jnp.where(r == rmax, rows, S))
        idx = jnp.minimum(idx, S - 1)
        xrow = x_s[pl.ds(idx, 1), :]
        arow = a_s[pl.ds(idx, 1), :]
        xsel = (xrow - jnp.mean(xrow, axis=1, keepdims=True)) * (arow / (1.0 + arow))
        xs = jnp.broadcast_to(xsel, (8, D)).astype(bf16)
        return idx, rmax, xrow, xs

    def ffn_up(xs, c):
        gate = jnp.dot(xs, wg[:, FC * c:FC * (c + 1)], preferred_element_type=f32)
        up = jnp.dot(xs, wu[:, FC * c:FC * (c + 1)], preferred_element_type=f32)
        return (gate * jax.nn.sigmoid(gate) * up).astype(bf16)

    def ffn_down(hid, c):
        return jnp.dot(hid, wd[FC * c:FC * (c + 1), :], preferred_element_type=f32)

    def kslice(b, g):
        kblock(b, g, g + 1)

    def ffn_mid():
        with jax.named_scope("fm_a"):
            kblock(0)
            idx, rmax, xrow, xs = route()
        with jax.named_scope("fm_b"):
            y = fm_b(xs)
        with jax.named_scope("fm_c"):
            fm_c(idx, rmax, xrow, y)

    def fm_b(xs):
        items = [(b, g) for b in range(1, NB) for g in range(NG)]
        NFS = F // 128
        gates, ups, hid, ys = [], [], [], []
        fi = 0
        def fstep(fi):
            if fi < 2 * NFS:
                c = fi // 2
                w = wg if fi % 2 == 0 else wu
                r = jnp.dot(xs, w[:, 128 * c:128 * (c + 1)], preferred_element_type=f32)
                if fi % 2 == 0:
                    gates.append(r)
                else:
                    g_ = gates[c]
                    hid.append((g_ * jax.nn.sigmoid(g_) * r).astype(bf16))
            elif fi < 2 * NFS + 28:
                c = fi - 2 * NFS
                ys.append(jnp.dot(hid[c], wd[128 * c:128 * (c + 1), :], preferred_element_type=f32))
        for k, (b, g) in enumerate(items):
            kslice(b, g)
            if fi < 2 * NFS + 28:
                fstep(fi)
                fi += 1
        y = ys[0]
        for t in ys[1:]:
            y = y + t
        return y

    def fm_c(idx, rmax, xrow, y):
        x_s[pl.ds(idx, 1), :] = xrow + y[0:1, :] * jax.nn.sigmoid(rmax)
        r0 = pl.multiple_of((idx // 16) * 16, 16)
        h0 = pl.multiple_of((idx // 16) * 8, 8)
        x = x_s[pl.ds(r0, 16), :]
        mu = jnp.mean(x, axis=1, keepdims=True)
        xc = x - mu
        var = jnp.mean(xc * xc, axis=1, keepdims=True)
        xn = (xc * lax.rsqrt(var + EPS)).astype(bf16)
        xa[pl.ds(h0, 8), :] = _b2u(xn)
        kk = jnp.dot(xn, wk[...], preferred_element_type=f32)
        for g in range(NG):
            k_s[g, pl.ds(128 + h0, 8), :] = _b2u(kk[:, 128 * g:128 * g + 128].astype(bf16))
        fill_kpad()

    def ffn_last():
        idx, rmax, xrow, xs = route()
        hid = jnp.concatenate([ffn_up(xs, c) for c in range(F // FC)], axis=1)
        y = jnp.dot(hid, wd[...], preferred_element_type=f32)[0:1, :]
        x_s[pl.ds(idx, 1), :] = xrow + y * jax.nn.sigmoid(rmax)
        for i in range(NB):
            out_copy(i).wait()
        b0 = pl.multiple_of((idx // 16) * 16, 16)
        outb[pl.ds(b0, 16), :] = x_s[pl.ds(b0, 16), :].astype(bf16)
        fix = pltpu.make_async_copy(outb.at[pl.ds(b0, 16), :], out_hbm.at[pl.ds(b0, 16), :], osems.at[NB])
        fix.start()
        fix.wait()

    layer_body(0, 0)
    layer_body(1, 0)


@jax.jit
def pallas_interleave_layers__sliding_block__moe_arch_mod__prompt_kernel(
    A_x: jax.Array,
    A_wqkv: jax.Array,
    A_wo: jax.Array,
    B_x: jax.Array,
    B_w_r: jax.Array,
    B_w_gate: jax.Array,
    B_w_up: jax.Array,
    B_w_down: jax.Array,
):
    del B_x
    x = A_x.reshape(S, D)
    wr = B_w_r.reshape(1, D)
    any_spec = pl.BlockSpec(memory_space=pl.ANY)
    scratch = [
        pltpu.VMEM((S, D), bf16),
        pltpu.VMEM((S, D), f32),
        pltpu.VMEM((S // 2, D), u32),
        pltpu.VMEM((64 * 3, D), u32),
        pltpu.VMEM((NG, (S + 256) // 2 + 64, 128), u32),
        pltpu.VMEM((NB + 1, D // 2, 128), u32),
        pltpu.VMEM((NB + 3, D // 2, 128), u32),
        pltpu.VMEM((S // 2, D), u32),
        pltpu.VMEM((D, D), bf16),
        pltpu.VMEM((D, D), bf16),
        pltpu.VMEM((D, D), bf16),
        pltpu.VMEM((D // 2, D), u32),
        pltpu.VMEM((D // 2, D), u32),
        pltpu.VMEM((D, D), bf16),
        pltpu.VMEM((D // 2, D), u32),
        pltpu.VMEM((1, D), bf16),
        pltpu.VMEM((D, F), bf16),
        pltpu.VMEM((D, F), bf16),
        pltpu.VMEM((F, D), bf16),
        pltpu.VMEM((S, 1), f32),
        pltpu.VMEM((S, 1), f32),
        pltpu.VMEM((S, D), bf16),
        pltpu.VMEM((64, 128), u32),
        pltpu.VMEM((64, 128), u32),
        pltpu.VMEM((3, 4, 1, 128), f32),
        pltpu.SMEM((2,), jnp.int32),
        pltpu.SemaphoreType.DMA((14,)),
        pltpu.SemaphoreType.DMA((NB + 1,)),
    ]
    scratch += [pltpu.VMEM((4, 256, 128), f32)] * NSB
    scratch += [pltpu.VMEM((1, 4, 192, 128), u32)] * NPB
    scratch += [pltpu.VMEM((4, 1, 128), f32)] * NPB
    out = pl.pallas_call(
        _kernel,
        out_shape=jax.ShapeDtypeStruct((S, D), bf16),
        in_specs=[any_spec] * 7,
        out_specs=any_spec,
        scratch_shapes=scratch,
        compiler_params=pltpu.CompilerParams(vmem_limit_bytes=110 * 1024 * 1024),
    )(x, A_wqkv, A_wo, wr, B_w_gate, B_w_up, B_w_down)
    return out.reshape(1, S, D)
```

```python
import functools
import math

import jax
import jax.numpy as jnp
from jax import lax
import jax.experimental.pallas as pl
import jax.experimental.pallas.tpu as pltpu

S, D, H, DH, WIN, F = 2048, 1024, 32, 32, 256, 3584
NB = S // 128
NG = D // 128
NU = H
TB = 512
NT = S // TB
EPS = 1e-5
NEG = -1e30
QSCALE = (DH ** -0.5) * math.log2(math.e)
NEC = 2
LA = 4
NSB = 2
NPB = 2

bf16 = jnp.bfloat16
f32 = jnp.float32
u32 = jnp.uint32
NT_DIMS = (((1,), (1,)), ((), ()))


def _b2u(x):
    return pltpu.bitcast(x, u32)


def _u2b(x):
    return pltpu.bitcast(x, bf16)


def _pack2(a, b):
    w = pltpu.pack_elementwise([a, b], packed_dtype=bf16)
    return w if w.dtype == u32 else pltpu.bitcast(w, u32)


def _pack_adj(x):
    r, c = x.shape
    e = x.reshape(r // 16, 16, c)
    return _pack2(e[:, 0:8, :].reshape(r // 2, c), e[:, 8:16, :].reshape(r // 2, c))


def _kernel(x_hbm, wqkv_hbm, wo_hbm, wr_hbm, wg_hbm, wu_hbm, wd_hbm, out_hbm,
            xin, x_s, xa, xb, k_s, qt_s, vt_s, o_s,
            wk, wq, wv, wqT, wvT, wo, wou, wr, wg, wu, wd,
            r_s, a_s, outb, um_ref, lm_ref, npad, zs, zv, sems, osems, *bufs):
    OPQ = 'p'
    zs[0] = 0
    zs[1] = 0
    zv[...] = jnp.zeros((8, 128), u32)
    sb = bufs[0:NSB]
    pb = bufs[NSB:NSB + NPB]
    lb = bufs[NSB + NPB:NSB + 2 * NPB]

    XCH = [(0, 128), (128, 384), (512, 512), (1024, 512), (1536, 512)]

    def x_copy(t):
        r0, n = XCH[t]
        return pltpu.make_async_copy(x_hbm.at[pl.ds(r0, n), :], xin.at[pl.ds(r0, n), :], sems.at[t])

    wkl_copy = pltpu.make_async_copy(wqkv_hbm.at[:, pl.ds(D, D // 2)], wk.at[:, pl.ds(0, D // 2)], sems.at[12])
    wkr_copy = pltpu.make_async_copy(wqkv_hbm.at[:, pl.ds(D + D // 2, D // 2)], wk.at[:, pl.ds(D // 2, D // 2)], sems.at[13])
    wq_copy = pltpu.make_async_copy(wqkv_hbm.at[:, pl.ds(0, D)], wq, sems.at[5])
    wv_copy = pltpu.make_async_copy(wqkv_hbm.at[:, pl.ds(2 * D, D)], wv, sems.at[6])
    wo_copy = pltpu.make_async_copy(wo_hbm, wo, sems.at[7])
    wr_copy = pltpu.make_async_copy(wr_hbm, wr, sems.at[8])
    wg_copy = pltpu.make_async_copy(wg_hbm, wg, sems.at[9])
    wu_copy = pltpu.make_async_copy(wu_hbm, wu, sems.at[10])
    wd_copy = pltpu.make_async_copy(wd_hbm, wd, sems.at[11])

    def out_copy(i):
        r0 = pl.multiple_of(i * 128, 128)
        return pltpu.make_async_copy(outb.at[pl.ds(r0, 128), :], out_hbm.at[pl.ds(r0, 128), :], osems.at[i])

    x_copy(0).start()
    wkl_copy.start()

    row2 = lax.broadcasted_iota(jnp.int32, (64, 128), 0)
    col2 = lax.broadcasted_iota(jnp.int32, (64, 128), 1)
    um = (jnp.where(row2 > col2, jnp.uint32(0xFFFF), jnp.uint32(0))
          | jnp.where(row2 + 64 > col2, jnp.uint32(0xFFFF0000), jnp.uint32(0)))
    um_ref[...] = um
    lm_ref[...] = ~um
    ql1 = lax.broadcasted_iota(jnp.int32, (1, 128), 1) & 31
    for ii in range(3):
        for j in range(4):
            t = 256 - (128 * ii + 32 * j) if ii < 2 else 0
            n = max(0, min(256, t) - 32) + jnp.maximum(0, min(32, t) - 1 - ql1)
            npad[ii, j] = n.astype(f32)
    vt_s[0] = jnp.zeros((D // 2, 128), u32)
    vt_s[1] = jnp.zeros((D // 2, 128), u32)

    def store_ln(r0, xn):
        h0 = pl.multiple_of(r0 // 2, 64)
        xa[pl.ds(h0, 64), :] = _b2u(xn.astype(bf16))

    def plain_ln(r0, x):
        mu = jnp.mean(x, axis=1, keepdims=True)
        xc = x - mu
        var = jnp.mean(xc * xc, axis=1, keepdims=True)
        store_ln(r0, xc * lax.rsqrt(var + EPS))

    def kblock(b, g0=0, g1=NG):
        static = isinstance(b, int)
        r = b * 64 if static else pl.multiple_of(b * 64, 64)
        xa_t = _u2b(xa[pl.ds(r, 64), :])
        kk = jnp.dot(xa_t, wk[:, 128 * g0:128 * g1], preferred_element_type=f32)
        kr = 128 + r if static else pl.multiple_of(128 + r, 64)
        for g in range(g0, g1):
            k_s[g, pl.ds(kr, 64), :] = _b2u(kk[:, 128 * (g - g0):128 * (g - g0) + 128].astype(bf16))

    def fill_kpad():
        for g in range(NG):
            lo = k_s[g, 128:129, :] & jnp.uint32(0xFFFF)
            k_s[g, 0:128, :] = jnp.broadcast_to(lo | (lo << 16), (128, 128))

    def ln0(b):
        r0 = 128 * b if isinstance(b, int) else pl.multiple_of(128 * b, 128)
        x = xin[pl.ds(r0, 128), :].astype(f32)
        x_s[pl.ds(r0, 128), :] = x
        plain_ln(r0, x)

    def conv(dst, src):
        for j in range(NG):
            dst[64 * j:64 * j + 64, :] = _b2u(src[128 * j:128 * j + 128, :])

    with jax.named_scope("p0"):
        x_copy(0).wait()
        wkr_copy.start()
        ln0(0)
        wkl_copy.wait()
        x_copy(1).start()
        kblock(0, 0, NG // 2)
    with jax.named_scope("p1a"):
        wkr_copy.wait()
        kblock(0, NG // 2, NG)
    with jax.named_scope("p1"):
        x_copy(1).wait()
        x_copy(2).start()
        x_copy(3).start()
        for b in range(1, 4):
            ln0(b)
        kblock(1)
        kblock(2)
    def pro_body(t, c):
        r0 = pl.multiple_of(512 * (t + 1), 512)
        pltpu.make_async_copy(x_hbm.at[pl.ds(r0, 512), :], xin.at[pl.ds(r0, 512), :], sems.at[t + 2]).wait()

        @pl.when(t == 0)
        def _():
            x_copy(4).start()

        @pl.when(t == 1)
        def _():
            wq_copy.start()
            wv_copy.start()

        @pl.when(t == 2)
        def _():
            wo_copy.start()
            wr_copy.start()

        for b in range(4):
            kblock(4 * t + 3 + b)
            ln0(4 * t + 4 + b)
        return c

    with jax.named_scope("p2"):
        lax.fori_loop(0, 3, pro_body, 0)
    with jax.named_scope("p4"):
        wq_copy.wait()
        kblock(15)
        conv(wqT, wq)
        fill_kpad()
    with jax.named_scope("p5"):
        wv_copy.wait()
        wo_copy.wait()
        wr_copy.wait()
        conv(wvT, wv)
        conv(wou, wo)

    def gate(v, tok):
        if tok is None:
            return v
        return v + pltpu.bitcast(tok & zv[...], f32)[0:1, 0:v.shape[1]]

    def q_slice(xa_blk, q_blk, n):
        lhs = _u2b(xa_blk[...])
        rhs = _u2b(wqT[:, 128 * n:128 * n + 128])
        q = jnp.dot(lhs, rhs, preferred_element_type=f32)
        qt = _b2u((q * QSCALE).astype(bf16).T)
        parts = [qt[0:16]] + [pltpu.roll(qt[16 * h:16 * h + 16], 32 * h, 1) for h in range(1, 4)]
        q_blk[64 * n:64 * n + 64, :] = jnp.concatenate(parts, axis=0)
        return parts[0][0:8]

    def v_slice(xa_blk, vt_blk, n):
        lhs = _u2b(xa_blk[...])
        rhs = _u2b(wvT[:, 128 * n:128 * n + 128])
        v = jnp.dot(lhs, rhs, preferred_element_type=f32)
        vt = _b2u(_u2b(_pack_adj(v)).T)
        vt_blk[64 * n:64 * n + 64, :] = vt
        return vt[0:8]

    def o_slice(o_blk, x_blk, n):
        lhs = _u2b(o_blk[...])
        rhs = _u2b(wou[:, 128 * n:128 * n + 128])
        acc = jnp.dot(lhs, rhs, preferred_element_type=f32)
        x_blk[:, 128 * n:128 * n + 128] = x_blk[:, 128 * n:128 * n + 128] + acc
        return pltpu.bitcast(acc[0:8], u32)

    def epilogue(j, x_blk, xa_blk, xb_blk, layer, chunks=range(NEC), tok=None):
        r0 = pl.multiple_of(j * 128, 128)
        R = 128 // NEC
        for c in chunks:
            lo = R * c
            x1 = x_blk[lo:lo + R, :]
            mu = gate(jnp.mean(x1, axis=1, keepdims=True), tok)
            xc = x1 - mu
            var = jnp.mean(xc * xc, axis=1, keepdims=True)
            a = lax.rsqrt(var + EPS)
            r = jnp.sum(xc * wr[...].astype(f32), axis=1, keepdims=True) * a
            r_s[pl.ds(r0 + lo, R), :] = r
            a_s[pl.ds(r0 + lo, R), :] = a
            a1 = 1.0 + a
            x2 = mu + xc * a1
            x_blk[lo:lo + R, :] = x2
            if layer == 0:
                v = xc * (a1 * lax.rsqrt(var * a1 * a1 + EPS))
                xa_blk[lo // 2:(lo + R) // 2, :] = _b2u(v.astype(bf16))
            else:
                outb[pl.ds(r0 + lo, R), :] = x2.astype(bf16)

    def views(i, lo):
        r = pl.multiple_of((i + lo) * 64, 64)
        xav = xa.at[pl.ds(r, 192), :]
        xbv = xb.at[pl.ds(r, 192), :]
        ov = o_s.at[pl.ds(r, 128), :]
        return xav, xbv, ov

    CH = 16
    ORDER = "a0ddcd"
    EPI_EVERY = 1
    lane8b = lax.broadcasted_iota(jnp.int32, (8, 128), 1) >> 5
    odd = (lane8b & 1) == 1
    high = lane8b >= 2
    lane16b = lax.broadcasted_iota(jnp.int32, (16, 128), 1) >> 5
    d32 = lax.broadcasted_iota(jnp.int32, (32, 128), 0) - (lax.broadcasted_iota(jnp.int32, (32, 128), 1) & 31)
    umask = d32 > 0

    def stage_a(kv, q_blk, g):
        s_ref = sb[g % NSB]
        for j in range(4):
            x = jnp.concatenate([jnp.where(lane16b == ((h + j) % 4), q_blk[64 * g + 16 * h:64 * g + 16 * h + 16, :], jnp.uint32(0))
                                 for h in range(4)], axis=0)
            b0 = 16 * j
            kt = jnp.concatenate([kv[g, b0:b0 + 8, :], kv[g, b0 + 128:b0 + 136, :], kv[g, b0 + 8:b0 + 16, :],
                                  kv[g, b0 + 136:b0 + 144, :], kv[g, b0 + 16:b0 + 128, :]], axis=0)
            st = jnp.dot(_u2b(kt), _u2b(x), preferred_element_type=f32)
            su = jnp.concatenate([st[0:16], st[32:48]], axis=0)
            sl = jnp.concatenate([st[16:32], st[48:64]], axis=0)
            s_ref[j, 0:32, :] = jnp.where(umask, su, sl)
            s_ref[j, 32:256, :] = st[64:288]
            if j == 0:
                tok = (pltpu.bitcast(st[64:72], u32), pltpu.bitcast(st[160:168], u32), pltpu.bitcast(st[280:288], u32))
        return tok

    def stage_b(i, g, masked, heads=range(4), toks=(None,) * 4, wtoks=(None,)):
        if list(heads) != [0]:
            return
        s_ref = sb[g % NSB]
        p_ref = pb[g % NPB].at[zs[0] if 'p' in OPQ else 0]
        l_ref = lb[g % NPB]
        pps = []
        for j in range(4):
            s = s_ref[j]
            m = gate(jnp.max(s, axis=0, keepdims=True), toks[j])
            p = jnp.exp2(s - m)
            l_ref[j] = jnp.sum(p, axis=0, keepdims=True) - npad[jnp.minimum(i, 2), j] * p[32:33]
            pm = p[0:32]
            e = jnp.concatenate([jnp.where(umask, pm, 0.0), p[32:256], jnp.where(umask, 0.0, pm)], axis=0)
            pps.append(_pack_adj(e))
        for M in range(24):
            y = [pps[j][8 * (M - 2 * j):8 * (M - 2 * j) + 8, :] if 0 <= M - 2 * j < 18 else None for j in range(4)]
            w = bfly(y, wtoks[M * len(wtoks) // 24])
            for h in range(4):
                p_ref[h, 8 * M:8 * M + 8, :] = w[h] if w[h] is not None else jnp.zeros((8, 128), u32)

    lane8odd = (lane8b & 1).astype(u32)

    def bfly(y, tok=None):
        def sel(m, a, b):
            if a is None and b is None:
                return None
            z = jnp.zeros((8, 128), (a if a is not None else b).dtype)
            return jnp.where(m, z if a is None else a, z if b is None else b)
        od = odd if tok is None else (lane8odd | (tok & zv[...])) == jnp.uint32(1)
        r = [sel(od, y[(k + 1) % 4], y[k]) for k in range(4)]
        wp = [sel(high, r[(k + 2) % 4], r[k]) for k in range(4)]
        return [wp[(-h) % 4] for h in range(4)]

    def stage_c(vts, o_blk, g):
        p_ref = pb[g % NPB].at[zs[1] if 'p' in OPQ else 0]
        l_ref = lb[g % NPB]
        lh = bfly([jnp.broadcast_to(1.0 / l_ref[j], (8, 128)) for j in range(4)])
        outs = []
        for h in range(4):
            vt = jnp.concatenate([_u2b(vts[t][64 * g + 16 * h:64 * g + 16 * h + 16, :]) for t in range(3)], axis=1)
            o = jnp.dot(vt, _u2b(p_ref[h]), preferred_element_type=f32)
            o = o * lh[h][0:1]
            if h:
                o = pltpu.roll(o, 128 - 32 * h, 1)
            outs.append(o)
        ot = jnp.concatenate(outs, axis=0)
        o_blk[:, 128 * g:128 * g + 128] = _b2u(ot.T.astype(bf16))

    def attn_body(i, c, masked, has_next, prev, layer):
        lo = -1 if prev is True else 0
        r = pl.multiple_of((i + lo) * 64, 64)
        nblk = (2 if has_next else 1) - lo
        xav = xa.at[pl.ds(r, 64 * nblk), :]
        xbv = xav
        ov = o_s.at[pl.ds(r, 64 * (1 - lo)), :]
        xv = x_s.at[pl.ds(pl.multiple_of((i + lo) * 128, 128), 128), :]
        qv = qt_s.at[pl.ds(i, 2)]
        vv = vt_s.at[pl.ds(i + lo, 4 - lo)]
        kv = k_s.at[:, pl.ds(pl.multiple_of(i * 64, 64), 256), :]
        blk = lambda v, b: v.at[pl.ds(64 * (b - lo), 64), :]
        vtile = lambda b: vv.at[b - lo]

        qs = [functools.partial(q_slice, blk(xav, 1), qv.at[1], n) for n in range(NG)] if has_next else []
        vs = [functools.partial(v_slice, blk(xav, 1), vtile(3), n) for n in range(NG)] if has_next else []
        os_ = [functools.partial(o_slice, blk(ov, -1), xv, n) for n in range(NG)] if prev is True else []
        SO = "q1,o8,q7,v8".split(",")
        sl = []
        last_o = -1
        pools = {"q": list(qs), "v": list(vs), "o": list(os_)}
        for tok in SO:
            for _ in range(int(tok[1:])):
                if pools[tok[0]]:
                    sl.append(pools[tok[0]].pop(0))
                    if tok[0] == "o":
                        last_o = len(sl) - 1
        assert not any(pools.values())
        per = -(-len(sl) // NG)
        emitted = [0]
        epi_done = [0]

        dtoks = []
        BG = "n,n,m,m".split(",")
        EG = 0
        WG = "n".split(",")

        def dense_one():
            k = emitted[0]
            if k < len(sl):
                t = sl[k]()
                dtoks.append(t)
                emitted[0] += 1
                if prev is True and k > last_o and epi_done[0] < NEC and (k - last_o) % EPI_EVERY == 0:
                    epilogue(i - 1, xv, blk(xav, -1), blk(xbv, -1), layer, [epi_done[0]], tok=t if EG else None)
                    epi_done[0] += 1

        if prev == "cond":
            @pl.when(i > 0)
            def _():
                finish_block(i - 1, layer)
        for g in range(NG):
            def fa():
                if g + 1 < NG:
                    return stage_a(kv.at[:, pl.ds(0, 192), :], qv.at[0], g + 1)
                elif has_next:
                    return stage_a(kv.at[:, pl.ds(64, 192), :], qv.at[1], 0)
            def fc():
                if g >= 1:
                    stage_c([vtile(t) for t in range(3)], blk(ov, 0), g - 1)
                elif prev is True:
                    stage_c([vtile(t - 1) for t in range(3)], blk(ov, -1), NG - 1)
            if g == 0:
                fc()
            nd = 0
            pats = ORDER.split(',')
            pat = pats[g % len(pats)]
            per = pat.count('d')
            k0 = len(dtoks)
            atok = None
            for ch in pat:
                if ch == "a":
                    atok = fa()
                elif ch == "c":
                    if g > 0:
                        fc()
                elif ch == "d":
                    if nd < per:
                        dense_one()
                        nd += 1
                else:
                    def tokof(sp):
                        if sp in ("a", "m", "z"):
                            return None if atok is None else atok["amz".index(sp)]
                        if sp[0] == "p":
                            idx = k0 - int(sp[1:])
                            return dtoks[idx] if 0 <= idx < len(dtoks) else None
                        if sp[0] == "c":
                            idx = k0 + int(sp[1:])
                            return dtoks[idx] if idx < len(dtoks) else None
                        return None
                    stage_b(i, g, masked, [int(ch)], [tokof(sp) for sp in BG], [tokof(sp) for sp in WG])
        while emitted[0] < len(sl):
            dense_one()
        if prev is True:
            while epi_done[0] < NEC:
                epilogue(i - 1, xv, blk(xav, -1), blk(xbv, -1), layer, [epi_done[0]])
                epi_done[0] += 1

        if layer == 1 and prev is True:
            out_copy(i - 1).start()
        if layer == 0 and prev is True and has_next:
            @pl.when(i == 1)
            def _():
                wg_copy.start()
                wu_copy.start()
                wd_copy.start()
        return c

    def finish_block(j, layer):
        o_blk = o_s.at[pl.ds(pl.multiple_of(j * 64, 64), 64), :]
        x_blk = x_s.at[pl.ds(pl.multiple_of(j * 128, 128), 128), :]
        stage_c([vt_s.at[j + t] for t in range(3)], o_blk, NG - 1)
        for n in range(NG):
            o_slice(o_blk, x_blk, n)
        epilogue(j, x_blk, xa.at[pl.ds(pl.multiple_of(j * 64, 64), 64), :], None, layer)

    def layer_body(layer, c):
        with jax.named_scope("qv0"):
            for n in range(NG):
                q_slice(xa.at[pl.ds(0, 64), :], qt_s.at[0], n)
            for n in range(NG):
                v_slice(xa.at[pl.ds(0, 64), :], vt_s.at[2], n)
            stage_a(k_s.at[:, pl.ds(0, 192), :], qt_s.at[0], 0)
        with jax.named_scope("attn"):
            with jax.named_scope("first"):
                attn_body(0, 0, masked=False, has_next=True, prev=False, layer=layer)
            with jax.named_scope("main"):
                lax.fori_loop(1, NB - 1, functools.partial(attn_body, masked=False, has_next=True, prev=True, layer=layer), 0)
            with jax.named_scope("last"):
                attn_body(NB - 1, 0, masked=False, has_next=False, prev=True, layer=layer)
        with jax.named_scope("tail"):
            finish_block(NB - 1, layer)

        if layer == 0:
            wg_copy.wait()
            wu_copy.wait()
            wd_copy.wait()
            with jax.named_scope("ffn_mid"):
                ffn_mid()
        else:
            out_copy(NB - 1).start()
            with jax.named_scope("ffn_last"):
                ffn_last()
        return c

    FC = 512

    def route():
        r = r_s[...]
        rmax = jnp.max(r)
        rows = lax.broadcasted_iota(jnp.int32, (S, 1), 0)
        idx = jnp.min(jnp.where(r == rmax, rows, S))
        idx = jnp.minimum(idx, S - 1)
        xrow = x_s[pl.ds(idx, 1), :]
        arow = a_s[pl.ds(idx, 1), :]
        xsel = (xrow - jnp.mean(xrow, axis=1, keepdims=True)) * (arow / (1.0 + arow))
        xs = jnp.broadcast_to(xsel, (8, D)).astype(bf16)
        return idx, rmax, xrow, xs

    def ffn_up(xs, c):
        gate = jnp.dot(xs, wg[:, FC * c:FC * (c + 1)], preferred_element_type=f32)
        up = jnp.dot(xs, wu[:, FC * c:FC * (c + 1)], preferred_element_type=f32)
        return (gate * jax.nn.sigmoid(gate) * up).astype(bf16)

    def ffn_down(hid, c):
        return jnp.dot(hid, wd[FC * c:FC * (c + 1), :], preferred_element_type=f32)

    def kslice(b, g):
        kblock(b, g, g + 1)

    def ffn_mid():
        with jax.named_scope("fm_a"):
            kblock(0)
            idx, rmax, xrow, xs = route()
        with jax.named_scope("fm_b"):
            y = fm_b(xs)
        with jax.named_scope("fm_c"):
            fm_c(idx, rmax, xrow, y)

    def fm_b(xs):
        items = [(b, g) for b in range(1, NB) for g in range(NG)]
        NFS = F // 128
        gates, ups, hid, ys = [], [], [], []
        fi = 0
        def fstep(fi):
            if fi < 2 * NFS:
                c = fi // 2
                w = wg if fi % 2 == 0 else wu
                r = jnp.dot(xs, w[:, 128 * c:128 * (c + 1)], preferred_element_type=f32)
                if fi % 2 == 0:
                    gates.append(r)
                else:
                    g_ = gates[c]
                    hid.append((g_ * jax.nn.sigmoid(g_) * r).astype(bf16))
            elif fi < 2 * NFS + 28:
                c = fi - 2 * NFS
                ys.append(jnp.dot(hid[c], wd[128 * c:128 * (c + 1), :], preferred_element_type=f32))
        for k, (b, g) in enumerate(items):
            kslice(b, g)
            if fi < 2 * NFS + 28:
                fstep(fi)
                fi += 1
        y = ys[0]
        for t in ys[1:]:
            y = y + t
        return y

    def fm_c(idx, rmax, xrow, y):
        x_s[pl.ds(idx, 1), :] = xrow + y[0:1, :] * jax.nn.sigmoid(rmax)
        r0 = pl.multiple_of((idx // 16) * 16, 16)
        h0 = pl.multiple_of((idx // 16) * 8, 8)
        x = x_s[pl.ds(r0, 16), :]
        mu = jnp.mean(x, axis=1, keepdims=True)
        xc = x - mu
        var = jnp.mean(xc * xc, axis=1, keepdims=True)
        xn = (xc * lax.rsqrt(var + EPS)).astype(bf16)
        xa[pl.ds(h0, 8), :] = _b2u(xn)
        kk = jnp.dot(xn, wk[...], preferred_element_type=f32)
        for g in range(NG):
            k_s[g, pl.ds(128 + h0, 8), :] = _b2u(kk[:, 128 * g:128 * g + 128].astype(bf16))
        fill_kpad()

    def ffn_last():
        idx, rmax, xrow, xs = route()
        hid = jnp.concatenate([ffn_up(xs, c) for c in range(F // FC)], axis=1)
        y = jnp.dot(hid, wd[...], preferred_element_type=f32)[0:1, :]
        x_s[pl.ds(idx, 1), :] = xrow + y * jax.nn.sigmoid(rmax)
        for i in range(NB):
            out_copy(i).wait()
        b0 = pl.multiple_of((idx // 16) * 16, 16)
        outb[pl.ds(b0, 16), :] = x_s[pl.ds(b0, 16), :].astype(bf16)
        fix = pltpu.make_async_copy(outb.at[pl.ds(b0, 16), :], out_hbm.at[pl.ds(b0, 16), :], osems.at[NB])
        fix.start()
        fix.wait()

    layer_body(0, 0)
    layer_body(1, 0)


@jax.jit
def pallas_interleave_layers__sliding_block__moe_arch_mod__prompt_kernel(
    A_x: jax.Array,
    A_wqkv: jax.Array,
    A_wo: jax.Array,
    B_x: jax.Array,
    B_w_r: jax.Array,
    B_w_gate: jax.Array,
    B_w_up: jax.Array,
    B_w_down: jax.Array,
):
    del B_x
    x = A_x.reshape(S, D)
    wr = B_w_r.reshape(1, D)
    any_spec = pl.BlockSpec(memory_space=pl.ANY)
    scratch = [
        pltpu.VMEM((S, D), bf16),
        pltpu.VMEM((S, D), f32),
        pltpu.VMEM((S // 2, D), u32),
        pltpu.VMEM((64 * 3, D), u32),
        pltpu.VMEM((NG, (S + 256) // 2 + 64, 128), u32),
        pltpu.VMEM((NB + 1, D // 2, 128), u32),
        pltpu.VMEM((NB + 3, D // 2, 128), u32),
        pltpu.VMEM((S // 2, D), u32),
        pltpu.VMEM((D, D), bf16),
        pltpu.VMEM((D, D), bf16),
        pltpu.VMEM((D, D), bf16),
        pltpu.VMEM((D // 2, D), u32),
        pltpu.VMEM((D // 2, D), u32),
        pltpu.VMEM((D, D), bf16),
        pltpu.VMEM((D // 2, D), u32),
        pltpu.VMEM((1, D), bf16),
        pltpu.VMEM((D, F), bf16),
        pltpu.VMEM((D, F), bf16),
        pltpu.VMEM((F, D), bf16),
        pltpu.VMEM((S, 1), f32),
        pltpu.VMEM((S, 1), f32),
        pltpu.VMEM((S, D), bf16),
        pltpu.VMEM((64, 128), u32),
        pltpu.VMEM((64, 128), u32),
        pltpu.VMEM((3, 4, 1, 128), f32),
        pltpu.SMEM((2,), jnp.int32),
        pltpu.VMEM((8, 128), u32),
        pltpu.SemaphoreType.DMA((14,)),
        pltpu.SemaphoreType.DMA((NB + 1,)),
    ]
    scratch += [pltpu.VMEM((4, 256, 128), f32)] * NSB
    scratch += [pltpu.VMEM((1, 4, 192, 128), u32)] * NPB
    scratch += [pltpu.VMEM((4, 1, 128), f32)] * NPB
    out = pl.pallas_call(
        _kernel,
        out_shape=jax.ShapeDtypeStruct((S, D), bf16),
        in_specs=[any_spec] * 7,
        out_specs=any_spec,
        scratch_shapes=scratch,
        compiler_params=pltpu.CompilerParams(vmem_limit_bytes=110 * 1024 * 1024),
    )(x, A_wqkv, A_wo, wr, B_w_gate, B_w_up, B_w_down)
    return out.reshape(1, S, D)
```

```python
import functools
import math

import jax
import jax.numpy as jnp
from jax import lax
import jax.experimental.pallas as pl
import jax.experimental.pallas.tpu as pltpu

S, D, H, DH, WIN, F = 2048, 1024, 32, 32, 256, 3584
NB = S // 128
NG = D // 128
NU = H
TB = 512
NT = S // TB
EPS = 1e-5
NEG = -1e30
QSCALE = (DH ** -0.5) * math.log2(math.e)
NEC = 2
LA = 4
NSB = 2
NPB = 2

bf16 = jnp.bfloat16
f32 = jnp.float32
u32 = jnp.uint32
NT_DIMS = (((1,), (1,)), ((), ()))


def _b2u(x):
    return pltpu.bitcast(x, u32)


def _u2b(x):
    return pltpu.bitcast(x, bf16)


def _pack2(a, b):
    w = pltpu.pack_elementwise([a, b], packed_dtype=bf16)
    return w if w.dtype == u32 else pltpu.bitcast(w, u32)


def _pack_adj(x):
    r, c = x.shape
    e = x.reshape(r // 16, 16, c)
    return _pack2(e[:, 0:8, :].reshape(r // 2, c), e[:, 8:16, :].reshape(r // 2, c))


def _kernel(x_hbm, wqkv_hbm, wo_hbm, wr_hbm, wg_hbm, wu_hbm, wd_hbm, out_hbm,
            xin, x_s, xa, xb, k_s, qt_s, vt_s, o_s,
            wk, wq, wv, wqT, wvT, wo, wou, wr, wg, wu, wd,
            r_s, a_s, outb, um_ref, lm_ref, npad, zs, zv, y_s, sems, osems, *bufs):
    OPQ = 'p'
    zs[0] = 0
    zs[1] = 0
    zv[...] = jnp.zeros((8, 128), u32)
    sb = bufs[0:NSB]
    pb = bufs[NSB:NSB + NPB]
    lb = bufs[NSB + NPB:NSB + 2 * NPB]

    XCH = [(0, 128), (128, 384), (512, 512), (1024, 512), (1536, 512)]

    def x_copy(t):
        r0, n = XCH[t]
        return pltpu.make_async_copy(x_hbm.at[pl.ds(r0, n), :], xin.at[pl.ds(r0, n), :], sems.at[t])

    def wk_copy(c):
        return pltpu.make_async_copy(wqkv_hbm.at[:, pl.ds(D + 256 * c, 256)], wk.at[:, pl.ds(256 * c, 256)], sems.at[12 + c])

    wq_copy = pltpu.make_async_copy(wqkv_hbm.at[:, pl.ds(0, D)], wq, sems.at[5])
    wv_copy = pltpu.make_async_copy(wqkv_hbm.at[:, pl.ds(2 * D, D)], wv, sems.at[6])
    wo_copy = pltpu.make_async_copy(wo_hbm, wo, sems.at[7])
    wr_copy = pltpu.make_async_copy(wr_hbm, wr, sems.at[8])
    wg_copy = pltpu.make_async_copy(wg_hbm, wg, sems.at[9])
    wu_copy = pltpu.make_async_copy(wu_hbm, wu, sems.at[10])
    wd_copy = pltpu.make_async_copy(wd_hbm, wd, sems.at[11])

    def out_copy(i):
        r0 = pl.multiple_of(i * 128, 128)
        return pltpu.make_async_copy(outb.at[pl.ds(r0, 128), :], out_hbm.at[pl.ds(r0, 128), :], osems.at[i])

    x_copy(0).start()
    wk_copy(0).start()

    row2 = lax.broadcasted_iota(jnp.int32, (64, 128), 0)
    col2 = lax.broadcasted_iota(jnp.int32, (64, 128), 1)
    um = (jnp.where(row2 > col2, jnp.uint32(0xFFFF), jnp.uint32(0))
          | jnp.where(row2 + 64 > col2, jnp.uint32(0xFFFF0000), jnp.uint32(0)))
    um_ref[...] = um
    lm_ref[...] = ~um
    ql1 = lax.broadcasted_iota(jnp.int32, (1, 128), 1) & 31
    for ii in range(3):
        for j in range(4):
            t = 256 - (128 * ii + 32 * j) if ii < 2 else 0
            n = max(0, min(256, t) - 32) + jnp.maximum(0, min(32, t) - 1 - ql1)
            npad[ii, j] = n.astype(f32)
    vt_s[0] = jnp.zeros((D // 2, 128), u32)
    vt_s[1] = jnp.zeros((D // 2, 128), u32)

    def store_ln(r0, xn):
        h0 = pl.multiple_of(r0 // 2, 64)
        xa[pl.ds(h0, 64), :] = _b2u(xn.astype(bf16))

    def plain_ln(r0, x):
        mu = jnp.mean(x, axis=1, keepdims=True)
        xc = x - mu
        var = jnp.mean(xc * xc, axis=1, keepdims=True)
        store_ln(r0, xc * lax.rsqrt(var + EPS))

    def kblock(b, g0=0, g1=NG):
        static = isinstance(b, int)
        r = b * 64 if static else pl.multiple_of(b * 64, 64)
        xa_t = _u2b(xa[pl.ds(r, 64), :])
        kk = jnp.dot(xa_t, wk[:, 128 * g0:128 * g1], preferred_element_type=f32)
        kr = 128 + r if static else pl.multiple_of(128 + r, 64)
        toks = []
        for g in range(g0, g1):
            v = _b2u(kk[:, 128 * (g - g0):128 * (g - g0) + 128].astype(bf16))
            k_s[g, pl.ds(kr, 64), :] = v
            toks.append(v[0:8])
        return toks

    def fill_kpad():
        for g in range(NG):
            lo = k_s[g, 128:129, :] & jnp.uint32(0xFFFF)
            k_s[g, 0:128, :] = jnp.broadcast_to(lo | (lo << 16), (128, 128))

    def gate(v, tok):
        if tok is None:
            return v
        return v + pltpu.bitcast(tok & zv[...], f32)[0:1, 0:v.shape[1]]

    def ln0(b, toks=None):
        base = 128 * b if isinstance(b, int) else pl.multiple_of(128 * b, 128)
        nch = 1 if toks is None else 2
        n = 128 // nch
        for c in range(nch):
            r0 = base + n * c
            x = xin[pl.ds(r0, n), :].astype(f32)
            x_s[pl.ds(r0, n), :] = x
            mu = jnp.mean(x, axis=1, keepdims=True)
            if toks is not None:
                mu = gate(mu, toks[4 * c])
            xc = x - mu
            var = jnp.mean(xc * xc, axis=1, keepdims=True)
            h0 = r0 // 2 if isinstance(b, int) else pl.multiple_of(r0 // 2, n // 2)
            xa[pl.ds(h0, n // 2), :] = _b2u((xc * lax.rsqrt(var + EPS)).astype(bf16))

    def conv(dst, src):
        for j in range(NG):
            dst[64 * j:64 * j + 64, :] = _b2u(src[128 * j:128 * j + 128, :])

    with jax.named_scope("p0"):
        x_copy(0).wait()
        wk_copy(1).start()
        ln0(0)
        wk_copy(0).wait()
        wk_copy(2).start()
        kblock(0, 0, 2)
        wk_copy(1).wait()
        wk_copy(3).start()
        kblock(0, 2, 4)
        wk_copy(2).wait()
        x_copy(1).start()
        kblock(0, 4, 6)
        wk_copy(3).wait()
        x_copy(2).start()
        kblock(0, 6, 8)
    with jax.named_scope("p1"):
        x_copy(1).wait()
        x_copy(3).start()
        ln0(1)
        kblock(1)
        ln0(2)
        ln0(3)

    def pro_body(t, c):
        r0 = pl.multiple_of(512 * (t + 1), 512)
        pltpu.make_async_copy(x_hbm.at[pl.ds(r0, 512), :], xin.at[pl.ds(r0, 512), :], sems.at[t + 2]).wait()

        @pl.when(t == 0)
        def _():
            x_copy(4).start()

        @pl.when(t == 1)
        def _():
            wq_copy.start()
            wv_copy.start()

        @pl.when(t == 2)
        def _():
            wo_copy.start()
            wr_copy.start()

        for b in range(4):
            toks = kblock(4 * t + 2 + b)
            ln0(4 * t + 4 + b, toks)
        return c

    with jax.named_scope("p2"):
        lax.fori_loop(0, 3, pro_body, 0)
    with jax.named_scope("p4"):
        wq_copy.wait()
        wv_copy.wait()
        kblock(14)
        conv(wqT, wq)
        conv(wvT, wv)
        wo_copy.wait()
        wr_copy.wait()
        kblock(15)
        conv(wou, wo)
        fill_kpad()

    def q_slice(xa_blk, q_blk, n):
        lhs = _u2b(xa_blk[...])
        rhs = _u2b(wqT[:, 128 * n:128 * n + 128])
        q = jnp.dot(lhs, rhs, preferred_element_type=f32)
        qt = _b2u((q * QSCALE).astype(bf16).T)
        parts = [qt[0:16]] + [pltpu.roll(qt[16 * h:16 * h + 16], 32 * h, 1) for h in range(1, 4)]
        q_blk[64 * n:64 * n + 64, :] = jnp.concatenate(parts, axis=0)
        return parts[0][0:8]

    def v_slice(xa_blk, vt_blk, n):
        lhs = _u2b(xa_blk[...])
        rhs = _u2b(wvT[:, 128 * n:128 * n + 128])
        v = jnp.dot(lhs, rhs, preferred_element_type=f32)
        vt = _b2u(_u2b(_pack_adj(v)).T)
        vt_blk[64 * n:64 * n + 64, :] = vt
        return vt[0:8]

    def o_slice(o_blk, x_blk, n):
        lhs = _u2b(o_blk[...])
        rhs = _u2b(wou[:, 128 * n:128 * n + 128])
        acc = jnp.dot(lhs, rhs, preferred_element_type=f32)
        x_blk[:, 128 * n:128 * n + 128] = x_blk[:, 128 * n:128 * n + 128] + acc
        return pltpu.bitcast(acc[0:8], u32)

    def epilogue(j, x_blk, xa_blk, xb_blk, layer, chunks=range(NEC), tok=None):
        r0 = pl.multiple_of(j * 128, 128)
        R = 128 // NEC
        for c in chunks:
            lo = R * c
            x1 = x_blk[lo:lo + R, :]
            mu = gate(jnp.mean(x1, axis=1, keepdims=True), tok)
            xc = x1 - mu
            var = jnp.mean(xc * xc, axis=1, keepdims=True)
            a = lax.rsqrt(var + EPS)
            r = jnp.sum(xc * wr[...].astype(f32), axis=1, keepdims=True) * a
            r_s[pl.ds(r0 + lo, R), :] = r
            a_s[pl.ds(r0 + lo, R), :] = a
            a1 = 1.0 + a
            x2 = mu + xc * a1
            x_blk[lo:lo + R, :] = x2
            if layer == 0:
                v = xc * (a1 * lax.rsqrt(var * a1 * a1 + EPS))
                xa_blk[lo // 2:(lo + R) // 2, :] = _b2u(v.astype(bf16))
            else:
                outb[pl.ds(r0 + lo, R), :] = x2.astype(bf16)

    def views(i, lo):
        r = pl.multiple_of((i + lo) * 64, 64)
        xav = xa.at[pl.ds(r, 192), :]
        xbv = xb.at[pl.ds(r, 192), :]
        ov = o_s.at[pl.ds(r, 128), :]
        return xav, xbv, ov

    CH = 16
    ORDER = "a0ddcd"
    EPI_EVERY = 1
    lane8b = lax.broadcasted_iota(jnp.int32, (8, 128), 1) >> 5
    odd = (lane8b & 1) == 1
    high = lane8b >= 2
    lane16b = lax.broadcasted_iota(jnp.int32, (16, 128), 1) >> 5
    d32 = lax.broadcasted_iota(jnp.int32, (32, 128), 0) - (lax.broadcasted_iota(jnp.int32, (32, 128), 1) & 31)
    umask = d32 > 0

    def stage_a(kv, q_blk, g):
        s_ref = sb[g % NSB]
        for j in range(4):
            x = jnp.concatenate([jnp.where(lane16b == ((h + j) % 4), q_blk[64 * g + 16 * h:64 * g + 16 * h + 16, :], jnp.uint32(0))
                                 for h in range(4)], axis=0)
            b0 = 16 * j
            kt = jnp.concatenate([kv[g, b0:b0 + 8, :], kv[g, b0 + 128:b0 + 136, :], kv[g, b0 + 8:b0 + 16, :],
                                  kv[g, b0 + 136:b0 + 144, :], kv[g, b0 + 16:b0 + 128, :]], axis=0)
            st = jnp.dot(_u2b(kt), _u2b(x), preferred_element_type=f32)
            su = jnp.concatenate([st[0:16], st[32:48]], axis=0)
            sl = jnp.concatenate([st[16:32], st[48:64]], axis=0)
            s_ref[j, 0:32, :] = jnp.where(umask, su, sl)
            s_ref[j, 32:256, :] = st[64:288]
            if j == 0:
                tok = (pltpu.bitcast(st[64:72], u32), pltpu.bitcast(st[160:168], u32), pltpu.bitcast(st[280:288], u32))
        return tok

    def stage_b(i, g, masked, heads=range(4), toks=(None,) * 4, wtoks=(None,)):
        if list(heads) != [0]:
            return
        s_ref = sb[g % NSB]
        p_ref = pb[g % NPB].at[zs[0] if 'p' in OPQ else 0]
        l_ref = lb[g % NPB]
        pps = []
        for j in range(4):
            s = s_ref[j]
            m = gate(jnp.max(s, axis=0, keepdims=True), toks[j])
            p = jnp.exp2(s - m)
            l_ref[j] = jnp.sum(p, axis=0, keepdims=True) - npad[jnp.minimum(i, 2), j] * p[32:33]
            pm = p[0:32]
            e = jnp.concatenate([jnp.where(umask, pm, 0.0), p[32:256], jnp.where(umask, 0.0, pm)], axis=0)
            pps.append(_pack_adj(e))
        for M in range(24):
            y = [pps[j][8 * (M - 2 * j):8 * (M - 2 * j) + 8, :] if 0 <= M - 2 * j < 18 else None for j in range(4)]
            w = bfly(y, wtoks[M * len(wtoks) // 24])
            for h in range(4):
                p_ref[h, 8 * M:8 * M + 8, :] = w[h] if w[h] is not None else jnp.zeros((8, 128), u32)

    lane8odd = (lane8b & 1).astype(u32)

    def bfly(y, tok=None):
        def sel(m, a, b):
            if a is None and b is None:
                return None
            z = jnp.zeros((8, 128), (a if a is not None else b).dtype)
            return jnp.where(m, z if a is None else a, z if b is None else b)
        od = odd if tok is None else (lane8odd | (tok & zv[...])) == jnp.uint32(1)
        r = [sel(od, y[(k + 1) % 4], y[k]) for k in range(4)]
        wp = [sel(high, r[(k + 2) % 4], r[k]) for k in range(4)]
        return [wp[(-h) % 4] for h in range(4)]

    def stage_c(vts, o_blk, g):
        p_ref = pb[g % NPB].at[zs[1] if 'p' in OPQ else 0]
        l_ref = lb[g % NPB]
        lh = bfly([jnp.broadcast_to(1.0 / l_ref[j], (8, 128)) for j in range(4)])
        outs = []
        for h in range(4):
            vt = jnp.concatenate([_u2b(vts[t][64 * g + 16 * h:64 * g + 16 * h + 16, :]) for t in range(3)], axis=1)
            o = jnp.dot(vt, _u2b(p_ref[h]), preferred_element_type=f32)
            o = o * lh[h][0:1]
            if h:
                o = pltpu.roll(o, 128 - 32 * h, 1)
            outs.append(o)
        ot = jnp.concatenate(outs, axis=0)
        o_blk[:, 128 * g:128 * g + 128] = _b2u(ot.T.astype(bf16))

    def attn_body(i, c, masked, has_next, prev, layer, extra=()):
        lo = -1 if prev is True else 0
        r = pl.multiple_of((i + lo) * 64, 64)
        nblk = (2 if has_next else 1) - lo
        xav = xa.at[pl.ds(r, 64 * nblk), :]
        xbv = xav
        ov = o_s.at[pl.ds(r, 64 * (1 - lo)), :]
        xv = x_s.at[pl.ds(pl.multiple_of((i + lo) * 128, 128), 128), :]
        qv = qt_s.at[pl.ds(i, 2)]
        vv = vt_s.at[pl.ds(i + lo, 4 - lo)]
        kv = k_s.at[:, pl.ds(pl.multiple_of(i * 64, 64), 256), :]
        blk = lambda v, b: v.at[pl.ds(64 * (b - lo), 64), :]
        vtile = lambda b: vv.at[b - lo]

        qs = [functools.partial(q_slice, blk(xav, 1), qv.at[1], n) for n in range(NG)] if has_next else []
        vs = [functools.partial(v_slice, blk(xav, 1), vtile(3), n) for n in range(NG)] if has_next else []
        os_ = [functools.partial(o_slice, blk(ov, -1), xv, n) for n in range(NG)] if prev is True else []
        SO = "q1,o8,q7,v8".split(",")
        sl = []
        last_o = -1
        pools = {"q": list(qs), "v": list(vs), "o": list(os_)}
        for tok in SO:
            for _ in range(int(tok[1:])):
                if pools[tok[0]]:
                    sl.append(pools[tok[0]].pop(0))
                    if tok[0] == "o":
                        last_o = len(sl) - 1
        assert not any(pools.values())
        if extra:
            n_it = 2 * NG
            groups = [extra[len(extra) * k // n_it:len(extra) * (k + 1) // n_it] for k in range(n_it)]
            def run(fs):
                t = None
                for f in fs:
                    t = f()
                return t
            comp = [functools.partial(run, fs) for fs in groups]
            sl = comp[0:1] + sl + comp[1:]
            last_o = NG
        per = -(-len(sl) // NG)
        emitted = [0]
        epi_done = [0]

        dtoks = []
        BG = "n,n,m,m".split(",")
        EG = 0
        WG = "n".split(",")

        def dense_one():
            k = emitted[0]
            if k < len(sl):
                t = sl[k]()
                dtoks.append(t)
                emitted[0] += 1
                if prev is True and k > last_o and epi_done[0] < NEC and (k - last_o) % EPI_EVERY == 0:
                    epilogue(i - 1, xv, blk(xav, -1), blk(xbv, -1), layer, [epi_done[0]], tok=t if EG else None)
                    epi_done[0] += 1

        if prev == "cond":
            @pl.when(i > 0)
            def _():
                finish_block(i - 1, layer)
        for g in range(NG):
            def fa():
                if g + 1 < NG:
                    return stage_a(kv.at[:, pl.ds(0, 192), :], qv.at[0], g + 1)
                elif has_next:
                    return stage_a(kv.at[:, pl.ds(64, 192), :], qv.at[1], 0)
            def fc():
                if g >= 1:
                    stage_c([vtile(t) for t in range(3)], blk(ov, 0), g - 1)
                elif prev is True:
                    stage_c([vtile(t - 1) for t in range(3)], blk(ov, -1), NG - 1)
            if g == 0:
                fc()
            nd = 0
            pats = ORDER.split(',')
            pat = pats[g % len(pats)]
            per = pat.count('d')
            k0 = len(dtoks)
            atok = None
            for ch in pat:
                if ch == "a":
                    atok = fa()
                elif ch == "c":
                    if g > 0:
                        fc()
                elif ch == "d":
                    if nd < per:
                        dense_one()
                        nd += 1
                else:
                    def tokof(sp):
                        if sp in ("a", "m", "z"):
                            return None if atok is None else atok["amz".index(sp)]
                        if sp[0] == "p":
                            idx = k0 - int(sp[1:])
                            return dtoks[idx] if 0 <= idx < len(dtoks) else None
                        if sp[0] == "c":
                            idx = k0 + int(sp[1:])
                            return dtoks[idx] if idx < len(dtoks) else None
                        return None
                    stage_b(i, g, masked, [int(ch)], [tokof(sp) for sp in BG], [tokof(sp) for sp in WG])
        while emitted[0] < len(sl):
            dense_one()
        if prev is True:
            while epi_done[0] < NEC:
                epilogue(i - 1, xv, blk(xav, -1), blk(xbv, -1), layer, [epi_done[0]])
                epi_done[0] += 1

        if layer == 1 and prev is True:
            out_copy(i - 1).start()
        if layer == 0 and prev is True and has_next:
            @pl.when(i == 1)
            def _():
                wg_copy.start()
                wu_copy.start()
                wd_copy.start()
        return c

    def finish_block(j, layer):
        o_blk = o_s.at[pl.ds(pl.multiple_of(j * 64, 64), 64), :]
        x_blk = x_s.at[pl.ds(pl.multiple_of(j * 128, 128), 128), :]
        stage_c([vt_s.at[j + t] for t in range(3)], o_blk, NG - 1)
        for n in range(NG):
            o_slice(o_blk, x_blk, n)
        epilogue(j, x_blk, xa.at[pl.ds(pl.multiple_of(j * 64, 64), 64), :], None, layer)

    def layer_body(layer, c):
        with jax.named_scope("qv0"):
            for n in range(NG):
                q_slice(xa.at[pl.ds(0, 64), :], qt_s.at[0], n)
            for n in range(NG):
                v_slice(xa.at[pl.ds(0, 64), :], vt_s.at[2], n)
            stage_a(k_s.at[:, pl.ds(0, 192), :], qt_s.at[0], 0)
        with jax.named_scope("attn"):
            with jax.named_scope("first"):
                attn_body(0, 0, masked=False, has_next=True, prev=False, layer=layer)
            with jax.named_scope("main"):
                lax.fori_loop(1, NB - 1, functools.partial(attn_body, masked=False, has_next=True, prev=True, layer=layer), 0)
            with jax.named_scope("last"):
                if layer == 0:
                    extra = [functools.partial(kslice, b, g) for b in range(K2_EARLY) for g in range(NG)]
                    attn_body(NB - 1, 0, masked=False, has_next=False, prev=True, layer=layer, extra=extra)
                else:
                    attn_body(NB - 1, 0, masked=False, has_next=False, prev=True, layer=layer)
        with jax.named_scope("tail"):
            finish_block(NB - 1, layer)

        if layer == 0:
            wg_copy.wait()
            wu_copy.wait()
            wd_copy.wait()
            with jax.named_scope("ffn_mid"):
                ffn_mid()
        else:
            out_copy(NB - 1).start()
            with jax.named_scope("ffn_last"):
                ffn_last()
        return c

    FC = 512

    def route(nrows=S):
        r = r_s[0:nrows, :]
        rmax = jnp.max(r)
        rows = lax.broadcasted_iota(jnp.int32, (nrows, 1), 0)
        idx = jnp.min(jnp.where(r == rmax, rows, nrows))
        idx = jnp.minimum(idx, nrows - 1)
        xrow = x_s[pl.ds(idx, 1), :]
        arow = a_s[pl.ds(idx, 1), :]
        xsel = (xrow - jnp.mean(xrow, axis=1, keepdims=True)) * (arow / (1.0 + arow))
        xs = jnp.broadcast_to(xsel, (8, D)).astype(bf16)
        return idx, rmax, xrow, xs

    def ffn_up(xs, c):
        gate = jnp.dot(xs, wg[:, FC * c:FC * (c + 1)], preferred_element_type=f32)
        up = jnp.dot(xs, wu[:, FC * c:FC * (c + 1)], preferred_element_type=f32)
        return (gate * jax.nn.sigmoid(gate) * up).astype(bf16)

    def ffn_down(hid, c):
        return jnp.dot(hid, wd[FC * c:FC * (c + 1), :], preferred_element_type=f32)

    K2_EARLY = 2

    def kslice(b, g):
        kblock(b, g, g + 1)
        return None

    def ffn_mid():
        with jax.named_scope("fm_a"):
            kblock(K2_EARLY)
            idx, rmax, xrow, xs = route()
        with jax.named_scope("fm_b"):
            y = fm_b(xs)
        with jax.named_scope("fm_c"):
            fm_c(idx, rmax, xrow, y)

    NFS = F // 128

    def ffn_steps(xs):
        gates, hid, ys = [], [], []

        def up(c, w, first):
            r = jnp.dot(xs, w[:, 128 * c:128 * (c + 1)], preferred_element_type=f32)
            if first:
                gates.append(r)
            else:
                g_ = gates[c]
                hid.append((g_ * jax.nn.sigmoid(g_) * r).astype(bf16))
            return pltpu.bitcast(r, u32)

        def down(c):
            r = jnp.dot(hid[c], wd[128 * c:128 * (c + 1), :], preferred_element_type=f32)
            ys.append(r)
            return pltpu.bitcast(r[:, 0:128], u32)

        steps = []
        for c in range(NFS):
            steps.append(functools.partial(up, c, wg, True))
            steps.append(functools.partial(up, c, wu, False))
            if c >= 1:
                steps.append(functools.partial(down, c - 1))
        steps.append(functools.partial(down, NFS - 1))

        def result():
            y = ys[0]
            for t in ys[1:]:
                y = y + t
            return y
        return steps, result

    def fm_b(xs):
        items = [(b, g) for b in range(K2_EARLY + 1, NB) for g in range(NG)]
        steps, result = ffn_steps(xs)
        fi = 0
        for k, (b, g) in enumerate(items):
            kslice(b, g)
            if fi < len(steps):
                steps[fi]()
                fi += 1
        while fi < len(steps):
            steps[fi]()
            fi += 1
        return result()

    def fm_c(idx, rmax, xrow, y):
        x_s[pl.ds(idx, 1), :] = xrow + y[0:1, :] * jax.nn.sigmoid(rmax)
        r0 = pl.multiple_of((idx // 16) * 16, 16)
        h0 = pl.multiple_of((idx // 16) * 8, 8)
        x = x_s[pl.ds(r0, 16), :]
        mu = jnp.mean(x, axis=1, keepdims=True)
        xc = x - mu
        var = jnp.mean(xc * xc, axis=1, keepdims=True)
        xn = (xc * lax.rsqrt(var + EPS)).astype(bf16)
        xa[pl.ds(h0, 8), :] = _b2u(xn)
        kk = jnp.dot(xn, wk[...], preferred_element_type=f32)
        for g in range(NG):
            k_s[g, pl.ds(128 + h0, 8), :] = _b2u(kk[:, 128 * g:128 * g + 128].astype(bf16))
        fill_kpad()

    def ffn_last():
        idx, rmax, xrow, xs = route()

        steps, result = ffn_steps(xs)
        for f in steps:
            f()
        y = result()
        x_s[pl.ds(idx, 1), :] = xrow + y[0:1, :] * jax.nn.sigmoid(rmax)
        for i in range(NB):
            out_copy(i).wait()
        b0 = pl.multiple_of((idx // 16) * 16, 16)
        outb[pl.ds(b0, 16), :] = x_s[pl.ds(b0, 16), :].astype(bf16)
        fix = pltpu.make_async_copy(outb.at[pl.ds(b0, 16), :], out_hbm.at[pl.ds(b0, 16), :], osems.at[NB])
        fix.start()
        fix.wait()

    layer_body(0, 0)
    layer_body(1, 0)


@jax.jit
def pallas_interleave_layers__sliding_block__moe_arch_mod__prompt_kernel(
    A_x: jax.Array,
    A_wqkv: jax.Array,
    A_wo: jax.Array,
    B_x: jax.Array,
    B_w_r: jax.Array,
    B_w_gate: jax.Array,
    B_w_up: jax.Array,
    B_w_down: jax.Array,
):
    del B_x
    x = A_x.reshape(S, D)
    wr = B_w_r.reshape(1, D)
    any_spec = pl.BlockSpec(memory_space=pl.ANY)
    scratch = [
        pltpu.VMEM((S, D), bf16),
        pltpu.VMEM((S, D), f32),
        pltpu.VMEM((S // 2, D), u32),
        pltpu.VMEM((64 * 3, D), u32),
        pltpu.VMEM((NG, (S + 256) // 2 + 64, 128), u32),
        pltpu.VMEM((NB + 1, D // 2, 128), u32),
        pltpu.VMEM((NB + 3, D // 2, 128), u32),
        pltpu.VMEM((S // 2, D), u32),
        pltpu.VMEM((D, D), bf16),
        pltpu.VMEM((D, D), bf16),
        pltpu.VMEM((D, D), bf16),
        pltpu.VMEM((D // 2, D), u32),
        pltpu.VMEM((D // 2, D), u32),
        pltpu.VMEM((D, D), bf16),
        pltpu.VMEM((D // 2, D), u32),
        pltpu.VMEM((1, D), bf16),
        pltpu.VMEM((D, F), bf16),
        pltpu.VMEM((D, F), bf16),
        pltpu.VMEM((F, D), bf16),
        pltpu.VMEM((S, 1), f32),
        pltpu.VMEM((S, 1), f32),
        pltpu.VMEM((S, D), bf16),
        pltpu.VMEM((64, 128), u32),
        pltpu.VMEM((64, 128), u32),
        pltpu.VMEM((3, 4, 1, 128), f32),
        pltpu.SMEM((3,), jnp.int32),
        pltpu.VMEM((8, 128), u32),
        pltpu.VMEM((8, D), f32),
        pltpu.SemaphoreType.DMA((16,)),
        pltpu.SemaphoreType.DMA((NB + 1,)),
    ]
    scratch += [pltpu.VMEM((4, 256, 128), f32)] * NSB
    scratch += [pltpu.VMEM((1, 4, 192, 128), u32)] * NPB
    scratch += [pltpu.VMEM((4, 1, 128), f32)] * NPB
    out = pl.pallas_call(
        _kernel,
        out_shape=jax.ShapeDtypeStruct((S, D), bf16),
        in_specs=[any_spec] * 7,
        out_specs=any_spec,
        scratch_shapes=scratch,
        compiler_params=pltpu.CompilerParams(vmem_limit_bytes=110 * 1024 * 1024),
    )(x, A_wqkv, A_wo, wr, B_w_gate, B_w_up, B_w_down)
    return out.reshape(1, S, D)
```

```python
import functools
import math

import jax
import jax.numpy as jnp
from jax import lax
import jax.experimental.pallas as pl
import jax.experimental.pallas.tpu as pltpu

S, D, H, DH, WIN, F = 2048, 1024, 32, 32, 256, 3584
NB = S // 128
NG = D // 128
NU = H
TB = 512
NT = S // TB
EPS = 1e-5
NEG = -1e30
QSCALE = (DH ** -0.5) * math.log2(math.e)
NEC = 2
LA = 4
NSB = 2
NPB = 2

bf16 = jnp.bfloat16
f32 = jnp.float32
u32 = jnp.uint32
NT_DIMS = (((1,), (1,)), ((), ()))


def _b2u(x):
    return pltpu.bitcast(x, u32)


def _u2b(x):
    return pltpu.bitcast(x, bf16)


def _pack2(a, b):
    w = pltpu.pack_elementwise([a, b], packed_dtype=bf16)
    return w if w.dtype == u32 else pltpu.bitcast(w, u32)


def _pack_adj(x):
    r, c = x.shape
    e = x.reshape(r // 16, 16, c)
    return _pack2(e[:, 0:8, :].reshape(r // 2, c), e[:, 8:16, :].reshape(r // 2, c))


def _kernel(x_hbm, wqkv_hbm, wo_hbm, wr_hbm, wg_hbm, wu_hbm, wd_hbm, out_hbm,
            xin, x_s, xa, xb, k_s, qt_s, vt_s, o_s,
            wk, wq, wv, wqT, wvT, wo, wou, wr, wg, wu, wd,
            r_s, a_s, outb, um_ref, lm_ref, npad, zs, zv, y_s, sems, osems, *bufs):
    OPQ = 'p'
    zs[0] = 0
    zs[1] = 0
    zv[...] = jnp.zeros((8, 128), u32)
    sb = bufs[0:NSB]
    pb = bufs[NSB:NSB + NPB]
    lb = bufs[NSB + NPB:NSB + 2 * NPB]

    XCH = [(0, 128), (128, 384), (512, 512), (1024, 512), (1536, 512)]

    def x_copy(t):
        r0, n = XCH[t]
        return pltpu.make_async_copy(x_hbm.at[pl.ds(r0, n), :], xin.at[pl.ds(r0, n), :], sems.at[t])

    def wk_copy(c):
        return pltpu.make_async_copy(wqkv_hbm.at[:, pl.ds(D + 256 * c, 256)], wk.at[:, pl.ds(256 * c, 256)], sems.at[12 + c])

    wq_copy = pltpu.make_async_copy(wqkv_hbm.at[:, pl.ds(0, D)], wq, sems.at[5])
    wv_copy = pltpu.make_async_copy(wqkv_hbm.at[:, pl.ds(2 * D, D)], wv, sems.at[6])
    wo_copy = pltpu.make_async_copy(wo_hbm, wo, sems.at[7])
    wr_copy = pltpu.make_async_copy(wr_hbm, wr, sems.at[8])
    wg_copy = pltpu.make_async_copy(wg_hbm, wg, sems.at[9])
    wu_copy = pltpu.make_async_copy(wu_hbm, wu, sems.at[10])
    wd_copy = pltpu.make_async_copy(wd_hbm, wd, sems.at[11])

    def out_copy(i):
        r0 = pl.multiple_of(i * 128, 128)
        return pltpu.make_async_copy(outb.at[pl.ds(r0, 128), :], out_hbm.at[pl.ds(r0, 128), :], osems.at[i])

    x_copy(0).start()
    wk_copy(0).start()

    row2 = lax.broadcasted_iota(jnp.int32, (64, 128), 0)
    col2 = lax.broadcasted_iota(jnp.int32, (64, 128), 1)
    um = (jnp.where(row2 > col2, jnp.uint32(0xFFFF), jnp.uint32(0))
          | jnp.where(row2 + 64 > col2, jnp.uint32(0xFFFF0000), jnp.uint32(0)))
    um_ref[...] = um
    lm_ref[...] = ~um
    ql1 = lax.broadcasted_iota(jnp.int32, (1, 128), 1) & 31
    for ii in range(3):
        for j in range(4):
            t = 256 - (128 * ii + 32 * j) if ii < 2 else 0
            n = max(0, min(256, t) - 32) + jnp.maximum(0, min(32, t) - 1 - ql1)
            npad[ii, j] = n.astype(f32)
    vt_s[0] = jnp.zeros((D // 2, 128), u32)
    vt_s[1] = jnp.zeros((D // 2, 128), u32)

    def store_ln(r0, xn):
        h0 = pl.multiple_of(r0 // 2, 64)
        xa[pl.ds(h0, 64), :] = _b2u(xn.astype(bf16))

    def plain_ln(r0, x):
        mu = jnp.mean(x, axis=1, keepdims=True)
        xc = x - mu
        var = jnp.mean(xc * xc, axis=1, keepdims=True)
        store_ln(r0, xc * lax.rsqrt(var + EPS))

    def kblock(b, g0=0, g1=NG):
        static = isinstance(b, int)
        r = b * 64 if static else pl.multiple_of(b * 64, 64)
        xa_t = _u2b(xa[pl.ds(r, 64), :])
        kk = jnp.dot(xa_t, wk[:, 128 * g0:128 * g1], preferred_element_type=f32)
        kr = 128 + r if static else pl.multiple_of(128 + r, 64)
        toks = []
        for g in range(g0, g1):
            v = _b2u(kk[:, 128 * (g - g0):128 * (g - g0) + 128].astype(bf16))
            k_s[g, pl.ds(kr, 64), :] = v
            toks.append(v[0:8])
        return toks

    def fill_kpad():
        for g in range(NG):
            lo = k_s[g, 128:129, :] & jnp.uint32(0xFFFF)
            k_s[g, 0:128, :] = jnp.broadcast_to(lo | (lo << 16), (128, 128))

    def gate(v, tok):
        if tok is None:
            return v
        return v + pltpu.bitcast(tok & zv[...], f32)[0:1, 0:v.shape[1]]

    def ln0(b, toks=None):
        base = 128 * b if isinstance(b, int) else pl.multiple_of(128 * b, 128)
        nch = 1 if toks is None else 2
        n = 128 // nch
        for c in range(nch):
            r0 = base + n * c
            x = xin[pl.ds(r0, n), :].astype(f32)
            x_s[pl.ds(r0, n), :] = x
            mu = jnp.mean(x, axis=1, keepdims=True)
            if toks is not None:
                mu = gate(mu, toks[4 * c])
            xc = x - mu
            var = jnp.mean(xc * xc, axis=1, keepdims=True)
            h0 = r0 // 2 if isinstance(b, int) else pl.multiple_of(r0 // 2, n // 2)
            xa[pl.ds(h0, n // 2), :] = _b2u((xc * lax.rsqrt(var + EPS)).astype(bf16))

    def conv(dst, src):
        for j in range(NG):
            dst[64 * j:64 * j + 64, :] = _b2u(src[128 * j:128 * j + 128, :])

    with jax.named_scope("p0"):
        x_copy(0).wait()
        wk_copy(1).start()
        ln0(0)
        wk_copy(0).wait()
        wk_copy(2).start()
        kblock(0, 0, 2)
        wk_copy(1).wait()
        wk_copy(3).start()
        kblock(0, 2, 4)
        wk_copy(2).wait()
        x_copy(1).start()
        kblock(0, 4, 6)
        wk_copy(3).wait()
        x_copy(2).start()
        kblock(0, 6, 8)
    with jax.named_scope("p1"):
        x_copy(1).wait()
        x_copy(3).start()
        ln0(1)
        kblock(1)
        ln0(2)
        ln0(3)

    def pro_body(t, c):
        r0 = pl.multiple_of(512 * (t + 1), 512)
        pltpu.make_async_copy(x_hbm.at[pl.ds(r0, 512), :], xin.at[pl.ds(r0, 512), :], sems.at[t + 2]).wait()

        @pl.when(t == 0)
        def _():
            x_copy(4).start()

        @pl.when(t == 1)
        def _():
            wq_copy.start()
            wv_copy.start()

        @pl.when(t == 2)
        def _():
            wo_copy.start()
            wr_copy.start()

        for b in range(4):
            toks = kblock(4 * t + 2 + b)
            ln0(4 * t + 4 + b, toks)
        return c

    with jax.named_scope("p2"):
        lax.fori_loop(0, 3, pro_body, 0)
    with jax.named_scope("p4"):
        wq_copy.wait()
        wv_copy.wait()
        kblock(14)
        conv(wqT, wq)
        conv(wvT, wv)
        wo_copy.wait()
        wr_copy.wait()
        kblock(15)
        conv(wou, wo)
        fill_kpad()

    def q_slice(xa_blk, q_blk, n):
        lhs = _u2b(xa_blk[...])
        rhs = _u2b(wqT[:, 128 * n:128 * n + 128])
        q = jnp.dot(lhs, rhs, preferred_element_type=f32)
        qt = _b2u((q * QSCALE).astype(bf16).T)
        parts = [qt[0:16]] + [pltpu.roll(qt[16 * h:16 * h + 16], 32 * h, 1) for h in range(1, 4)]
        q_blk[64 * n:64 * n + 64, :] = jnp.concatenate(parts, axis=0)
        return parts[0][0:8]

    def v_slice(xa_blk, vt_blk, n):
        lhs = _u2b(xa_blk[...])
        rhs = _u2b(wvT[:, 128 * n:128 * n + 128])
        v = jnp.dot(lhs, rhs, preferred_element_type=f32)
        vt = _b2u(_u2b(_pack_adj(v)).T)
        vt_blk[64 * n:64 * n + 64, :] = vt
        return vt[0:8]

    def o_slice(o_blk, x_blk, n):
        lhs = _u2b(o_blk[...])
        rhs = _u2b(wou[:, 128 * n:128 * n + 128])
        acc = jnp.dot(lhs, rhs, preferred_element_type=f32)
        x_blk[:, 128 * n:128 * n + 128] = x_blk[:, 128 * n:128 * n + 128] + acc
        return pltpu.bitcast(acc[0:8], u32)

    def epilogue(j, x_blk, xa_blk, xb_blk, layer, chunks=range(NEC), tok=None):
        r0 = pl.multiple_of(j * 128, 128)
        R = 128 // NEC
        for c in chunks:
            lo = R * c
            x1 = x_blk[lo:lo + R, :]
            mu = gate(jnp.mean(x1, axis=1, keepdims=True), tok)
            xc = x1 - mu
            var = jnp.mean(xc * xc, axis=1, keepdims=True)
            a = lax.rsqrt(var + EPS)
            r = jnp.sum(xc * wr[...].astype(f32), axis=1, keepdims=True) * a
            r_s[pl.ds(r0 + lo, R), :] = r
            a_s[pl.ds(r0 + lo, R), :] = a
            a1 = 1.0 + a
            x2 = mu + xc * a1
            x_blk[lo:lo + R, :] = x2
            if layer == 0:
                v = xc * (a1 * lax.rsqrt(var * a1 * a1 + EPS))
                xa_blk[lo // 2:(lo + R) // 2, :] = _b2u(v.astype(bf16))
            else:
                outb[pl.ds(r0 + lo, R), :] = x2.astype(bf16)

    def views(i, lo):
        r = pl.multiple_of((i + lo) * 64, 64)
        xav = xa.at[pl.ds(r, 192), :]
        xbv = xb.at[pl.ds(r, 192), :]
        ov = o_s.at[pl.ds(r, 128), :]
        return xav, xbv, ov

    CH = 16
    ORDER = "a0ddcd"
    EPI_EVERY = 1
    lane8b = lax.broadcasted_iota(jnp.int32, (8, 128), 1) >> 5
    odd = (lane8b & 1) == 1
    high = lane8b >= 2
    lane16b = lax.broadcasted_iota(jnp.int32, (16, 128), 1) >> 5
    d32 = lax.broadcasted_iota(jnp.int32, (32, 128), 0) - (lax.broadcasted_iota(jnp.int32, (32, 128), 1) & 31)
    umask = d32 > 0

    def stage_a(kv, q_blk, g):
        s_ref = sb[g % NSB]
        for j in range(4):
            x = jnp.concatenate([jnp.where(lane16b == ((h + j) % 4), q_blk[64 * g + 16 * h:64 * g + 16 * h + 16, :], jnp.uint32(0))
                                 for h in range(4)], axis=0)
            b0 = 16 * j
            kt = jnp.concatenate([kv[g, b0:b0 + 8, :], kv[g, b0 + 128:b0 + 136, :], kv[g, b0 + 8:b0 + 16, :],
                                  kv[g, b0 + 136:b0 + 144, :], kv[g, b0 + 16:b0 + 128, :]], axis=0)
            st = jnp.dot(_u2b(kt), _u2b(x), preferred_element_type=f32)
            su = jnp.concatenate([st[0:16], st[32:48]], axis=0)
            sl = jnp.concatenate([st[16:32], st[48:64]], axis=0)
            s_ref[j, 0:32, :] = jnp.where(umask, su, sl)
            s_ref[j, 32:256, :] = st[64:288]
            if j == 0:
                tok = (pltpu.bitcast(st[64:72], u32), pltpu.bitcast(st[160:168], u32), pltpu.bitcast(st[280:288], u32))
        return tok

    BM = 1

    def stage_b(i, g, masked, heads=range(4), toks=(None,) * 4, wtoks=(None,)):
        if list(heads) != [0]:
            return
        s_ref = sb[g % NSB]
        p_ref = pb[g % NPB].at[zs[0] if 'p' in OPQ else 0]
        l_ref = lb[g % NPB]
        if not BM:
            pps = []
            for j in range(4):
                s = s_ref[j]
                m = gate(jnp.max(s, axis=0, keepdims=True), toks[j])
                p = jnp.exp2(s - m)
                l_ref[j] = jnp.sum(p, axis=0, keepdims=True) - npad[jnp.minimum(i, 2), j] * p[32:33]
                pm = p[0:32]
                e = jnp.concatenate([jnp.where(umask, pm, 0.0), p[32:256], jnp.where(umask, 0.0, pm)], axis=0)
                pps.append(_pack_adj(e))
            for M in range(24):
                y = [pps[j][8 * (M - 2 * j):8 * (M - 2 * j) + 8, :] if 0 <= M - 2 * j < 18 else None for j in range(4)]
                w = bfly(y, wtoks[M * len(wtoks) // 24])
                for h in range(4):
                    p_ref[h, 8 * M:8 * M + 8, :] = w[h] if w[h] is not None else jnp.zeros((8, 128), u32)
            return
        ss = [s_ref[j] for j in range(4)]
        ms = [jnp.max(ss[j], axis=0, keepdims=True) for j in range(4)]
        ls = [None] * 4
        nch = len(toks)
        um16 = [umask[0:16], umask[16:32]]
        for c in range(nch):
            mg = [gate(ms[j], toks[c]) for j in range(4)]
            for M in range(24 * c // nch, 24 * (c + 1) // nch):
                y = []
                for j in range(4):
                    Mp = M - 2 * j
                    if not 0 <= Mp < 18:
                        y.append(None)
                        continue
                    row = 16 * (Mp % 16)
                    p = jnp.exp2(ss[j][row:row + 16] - mg[j])
                    if Mp < 16:
                        ps = p[0:8] + p[8:16]
                        ls[j] = ps if ls[j] is None else ls[j] + ps
                        if Mp == 2:
                            p32 = p[0:1]
                            ls[j] = ls[j] - jnp.where(lax.broadcasted_iota(jnp.int32, (8, 128), 0) == 0,
                                                      npad[jnp.minimum(i, 2), j] * p32, 0.0)
                    if Mp < 2:
                        p = jnp.where(um16[Mp], p, 0.0)
                    elif Mp >= 16:
                        p = jnp.where(um16[Mp - 16], 0.0, p)
                    y.append(_pack2(p[0:8], p[8:16]))
                w = bfly(y)
                for h in range(4):
                    p_ref[h, 8 * M:8 * M + 8, :] = w[h] if w[h] is not None else jnp.zeros((8, 128), u32)
        for j in range(4):
            l_ref[j] = jnp.sum(ls[j], axis=0, keepdims=True)

    lane8odd = (lane8b & 1).astype(u32)

    def bfly(y, tok=None):
        def sel(m, a, b):
            if a is None and b is None:
                return None
            z = jnp.zeros((8, 128), (a if a is not None else b).dtype)
            return jnp.where(m, z if a is None else a, z if b is None else b)
        od = odd if tok is None else (lane8odd | (tok & zv[...])) == jnp.uint32(1)
        r = [sel(od, y[(k + 1) % 4], y[k]) for k in range(4)]
        wp = [sel(high, r[(k + 2) % 4], r[k]) for k in range(4)]
        return [wp[(-h) % 4] for h in range(4)]

    def stage_c(vts, o_blk, g):
        p_ref = pb[g % NPB].at[zs[1] if 'p' in OPQ else 0]
        l_ref = lb[g % NPB]
        lh = bfly([jnp.broadcast_to(1.0 / l_ref[j], (8, 128)) for j in range(4)])
        outs = []
        for h in range(4):
            vt = jnp.concatenate([_u2b(vts[t][64 * g + 16 * h:64 * g + 16 * h + 16, :]) for t in range(3)], axis=1)
            o = jnp.dot(vt, _u2b(p_ref[h]), preferred_element_type=f32)
            o = o * lh[h][0:1]
            if h:
                o = pltpu.roll(o, 128 - 32 * h, 1)
            outs.append(o)
        ot = jnp.concatenate(outs, axis=0)
        o_blk[:, 128 * g:128 * g + 128] = _b2u(ot.T.astype(bf16))

    def attn_body(i, c, masked, has_next, prev, layer, extra=()):
        lo = -1 if prev is True else 0
        r = pl.multiple_of((i + lo) * 64, 64)
        nblk = (2 if has_next else 1) - lo
        xav = xa.at[pl.ds(r, 64 * nblk), :]
        xbv = xav
        ov = o_s.at[pl.ds(r, 64 * (1 - lo)), :]
        xv = x_s.at[pl.ds(pl.multiple_of((i + lo) * 128, 128), 128), :]
        qv = qt_s.at[pl.ds(i, 2)]
        vv = vt_s.at[pl.ds(i + lo, 4 - lo)]
        kv = k_s.at[:, pl.ds(pl.multiple_of(i * 64, 64), 256), :]
        blk = lambda v, b: v.at[pl.ds(64 * (b - lo), 64), :]
        vtile = lambda b: vv.at[b - lo]

        qs = [functools.partial(q_slice, blk(xav, 1), qv.at[1], n) for n in range(NG)] if has_next else []
        vs = [functools.partial(v_slice, blk(xav, 1), vtile(3), n) for n in range(NG)] if has_next else []
        os_ = [functools.partial(o_slice, blk(ov, -1), xv, n) for n in range(NG)] if prev is True else []
        SO = "q1,o8,q7,v8".split(",")
        sl = []
        last_o = -1
        pools = {"q": list(qs), "v": list(vs), "o": list(os_)}
        for tok in SO:
            for _ in range(int(tok[1:])):
                if pools[tok[0]]:
                    sl.append(pools[tok[0]].pop(0))
                    if tok[0] == "o":
                        last_o = len(sl) - 1
        assert not any(pools.values())
        if extra:
            n_it = 2 * NG
            groups = [extra[len(extra) * k // n_it:len(extra) * (k + 1) // n_it] for k in range(n_it)]
            def run(fs):
                t = None
                for f in fs:
                    t = f()
                return t
            comp = [functools.partial(run, fs) for fs in groups]
            sl = comp[0:1] + sl + comp[1:]
            last_o = NG
        per = -(-len(sl) // NG)
        emitted = [0]
        epi_done = [0]

        dtoks = []
        BG = "n,n,a,z".split(",")
        EG = 0
        WG = "n".split(",")

        def dense_one():
            k = emitted[0]
            if k < len(sl):
                t = sl[k]()
                dtoks.append(t)
                emitted[0] += 1
                if prev is True and k > last_o and epi_done[0] < NEC and (k - last_o) % EPI_EVERY == 0:
                    epilogue(i - 1, xv, blk(xav, -1), blk(xbv, -1), layer, [epi_done[0]], tok=t if EG else None)
                    epi_done[0] += 1

        if prev == "cond":
            @pl.when(i > 0)
            def _():
                finish_block(i - 1, layer)
        for g in range(NG):
            def fa():
                if g + 1 < NG:
                    return stage_a(kv.at[:, pl.ds(0, 192), :], qv.at[0], g + 1)
                elif has_next:
                    return stage_a(kv.at[:, pl.ds(64, 192), :], qv.at[1], 0)
            def fc():
                if g >= 1:
                    stage_c([vtile(t) for t in range(3)], blk(ov, 0), g - 1)
                elif prev is True:
                    stage_c([vtile(t - 1) for t in range(3)], blk(ov, -1), NG - 1)
            if g == 0:
                fc()
            nd = 0
            pats = ORDER.split(',')
            pat = pats[g % len(pats)]
            per = pat.count('d')
            k0 = len(dtoks)
            atok = None
            for ch in pat:
                if ch == "a":
                    atok = fa()
                elif ch == "c":
                    if g > 0:
                        fc()
                elif ch == "d":
                    if nd < per:
                        dense_one()
                        nd += 1
                else:
                    def tokof(sp):
                        if sp in ("a", "m", "z"):
                            return None if atok is None else atok["amz".index(sp)]
                        if sp[0] == "p":
                            idx = k0 - int(sp[1:])
                            return dtoks[idx] if 0 <= idx < len(dtoks) else None
                        if sp[0] == "c":
                            idx = k0 + int(sp[1:])
                            return dtoks[idx] if idx < len(dtoks) else None
                        return None
                    stage_b(i, g, masked, [int(ch)], [tokof(sp) for sp in BG], [tokof(sp) for sp in WG])
        while emitted[0] < len(sl):
            dense_one()
        if prev is True:
            while epi_done[0] < NEC:
                epilogue(i - 1, xv, blk(xav, -1), blk(xbv, -1), layer, [epi_done[0]])
                epi_done[0] += 1

        if layer == 1 and prev is True:
            out_copy(i - 1).start()
        if layer == 0 and prev is True and has_next:
            @pl.when(i == 1)
            def _():
                wg_copy.start()
                wu_copy.start()
                wd_copy.start()
        return c

    def finish_block(j, layer):
        o_blk = o_s.at[pl.ds(pl.multiple_of(j * 64, 64), 64), :]
        x_blk = x_s.at[pl.ds(pl.multiple_of(j * 128, 128), 128), :]
        stage_c([vt_s.at[j + t] for t in range(3)], o_blk, NG - 1)
        for n in range(NG):
            o_slice(o_blk, x_blk, n)
        epilogue(j, x_blk, xa.at[pl.ds(pl.multiple_of(j * 64, 64), 64), :], None, layer)

    def layer_body(layer, c):
        with jax.named_scope("qv0"):
            for n in range(NG):
                q_slice(xa.at[pl.ds(0, 64), :], qt_s.at[0], n)
            for n in range(NG):
                v_slice(xa.at[pl.ds(0, 64), :], vt_s.at[2], n)
            stage_a(k_s.at[:, pl.ds(0, 192), :], qt_s.at[0], 0)
        with jax.named_scope("attn"):
            with jax.named_scope("first"):
                attn_body(0, 0, masked=False, has_next=True, prev=False, layer=layer)
            with jax.named_scope("main"):
                lax.fori_loop(1, NB - 1, functools.partial(attn_body, masked=False, has_next=True, prev=True, layer=layer), 0)
            with jax.named_scope("last"):
                if layer == 0:
                    extra = [functools.partial(kslice, b, g) for b in range(K2_EARLY) for g in range(NG)]
                    attn_body(NB - 1, 0, masked=False, has_next=False, prev=True, layer=layer, extra=extra)
                else:
                    attn_body(NB - 1, 0, masked=False, has_next=False, prev=True, layer=layer)
        with jax.named_scope("tail"):
            finish_block(NB - 1, layer)

        if layer == 0:
            wg_copy.wait()
            wu_copy.wait()
            wd_copy.wait()
            with jax.named_scope("ffn_mid"):
                ffn_mid()
        else:
            out_copy(NB - 1).start()
            with jax.named_scope("ffn_last"):
                ffn_last()
        return c

    FC = 512

    def route(nrows=S):
        r = r_s[0:nrows, :]
        rmax = jnp.max(r)
        rows = lax.broadcasted_iota(jnp.int32, (nrows, 1), 0)
        idx = jnp.min(jnp.where(r == rmax, rows, nrows))
        idx = jnp.minimum(idx, nrows - 1)
        xrow = x_s[pl.ds(idx, 1), :]
        arow = a_s[pl.ds(idx, 1), :]
        xsel = (xrow - jnp.mean(xrow, axis=1, keepdims=True)) * (arow / (1.0 + arow))
        xs = jnp.broadcast_to(xsel, (8, D)).astype(bf16)
        return idx, rmax, xrow, xs

    def ffn_up(xs, c):
        gate = jnp.dot(xs, wg[:, FC * c:FC * (c + 1)], preferred_element_type=f32)
        up = jnp.dot(xs, wu[:, FC * c:FC * (c + 1)], preferred_element_type=f32)
        return (gate * jax.nn.sigmoid(gate) * up).astype(bf16)

    def ffn_down(hid, c):
        return jnp.dot(hid, wd[FC * c:FC * (c + 1), :], preferred_element_type=f32)

    K2_EARLY = 2

    def kslice(b, g):
        kblock(b, g, g + 1)
        return None

    def ffn_mid():
        with jax.named_scope("fm_a"):
            kblock(K2_EARLY)
            idx, rmax, xrow, xs = route()
        with jax.named_scope("fm_b"):
            y = fm_b(xs)
        with jax.named_scope("fm_c"):
            fm_c(idx, rmax, xrow, y)

    NFS = F // 128

    def ffn_steps(xs):
        gates, hid, ys = [], [], []

        def up(c, w, first):
            r = jnp.dot(xs, w[:, 128 * c:128 * (c + 1)], preferred_element_type=f32)
            if first:
                gates.append(r)
            else:
                g_ = gates[c]
                hid.append((g_ * jax.nn.sigmoid(g_) * r).astype(bf16))
            return pltpu.bitcast(r, u32)

        def down(c):
            r = jnp.dot(hid[c], wd[128 * c:128 * (c + 1), :], preferred_element_type=f32)
            ys.append(r)
            return pltpu.bitcast(r[:, 0:128], u32)

        steps = []
        for c in range(NFS):
            steps.append(functools.partial(up, c, wg, True))
            steps.append(functools.partial(up, c, wu, False))
            if c >= 1:
                steps.append(functools.partial(down, c - 1))
        steps.append(functools.partial(down, NFS - 1))

        def result():
            y = ys[0]
            for t in ys[1:]:
                y = y + t
            return y
        return steps, result

    def fm_b(xs):
        items = [(b, g) for b in range(K2_EARLY + 1, NB) for g in range(NG)]
        steps, result = ffn_steps(xs)
        fi = 0
        for k, (b, g) in enumerate(items):
            kslice(b, g)
            if fi < len(steps):
                steps[fi]()
                fi += 1
        while fi < len(steps):
            steps[fi]()
            fi += 1
        return result()

    def fm_c(idx, rmax, xrow, y):
        x_s[pl.ds(idx, 1), :] = xrow + y[0:1, :] * jax.nn.sigmoid(rmax)
        r0 = pl.multiple_of((idx // 16) * 16, 16)
        h0 = pl.multiple_of((idx // 16) * 8, 8)
        x = x_s[pl.ds(r0, 16), :]
        mu = jnp.mean(x, axis=1, keepdims=True)
        xc = x - mu
        var = jnp.mean(xc * xc, axis=1, keepdims=True)
        xn = (xc * lax.rsqrt(var + EPS)).astype(bf16)
        xa[pl.ds(h0, 8), :] = _b2u(xn)
        kk = jnp.dot(xn, wk[...], preferred_element_type=f32)
        for g in range(NG):
            k_s[g, pl.ds(128 + h0, 8), :] = _b2u(kk[:, 128 * g:128 * g + 128].astype(bf16))
        fill_kpad()

    def ffn_last():
        idx, rmax, xrow, xs = route()

        steps, result = ffn_steps(xs)
        for f in steps:
            f()
        y = result()
        x_s[pl.ds(idx, 1), :] = xrow + y[0:1, :] * jax.nn.sigmoid(rmax)
        for i in range(NB):
            out_copy(i).wait()
        b0 = pl.multiple_of((idx // 16) * 16, 16)
        outb[pl.ds(b0, 16), :] = x_s[pl.ds(b0, 16), :].astype(bf16)
        fix = pltpu.make_async_copy(outb.at[pl.ds(b0, 16), :], out_hbm.at[pl.ds(b0, 16), :], osems.at[NB])
        fix.start()
        fix.wait()

    layer_body(0, 0)
    layer_body(1, 0)


@jax.jit
def pallas_interleave_layers__sliding_block__moe_arch_mod__prompt_kernel(
    A_x: jax.Array,
    A_wqkv: jax.Array,
    A_wo: jax.Array,
    B_x: jax.Array,
    B_w_r: jax.Array,
    B_w_gate: jax.Array,
    B_w_up: jax.Array,
    B_w_down: jax.Array,
):
    del B_x
    x = A_x.reshape(S, D)
    wr = B_w_r.reshape(1, D)
    any_spec = pl.BlockSpec(memory_space=pl.ANY)
    scratch = [
        pltpu.VMEM((S, D), bf16),
        pltpu.VMEM((S, D), f32),
        pltpu.VMEM((S // 2, D), u32),
        pltpu.VMEM((64 * 3, D), u32),
        pltpu.VMEM((NG, (S + 256) // 2 + 64, 128), u32),
        pltpu.VMEM((NB + 1, D // 2, 128), u32),
        pltpu.VMEM((NB + 3, D // 2, 128), u32),
        pltpu.VMEM((S // 2, D), u32),
        pltpu.VMEM((D, D), bf16),
        pltpu.VMEM((D, D), bf16),
        pltpu.VMEM((D, D), bf16),
        pltpu.VMEM((D // 2, D), u32),
        pltpu.VMEM((D // 2, D), u32),
        pltpu.VMEM((D, D), bf16),
        pltpu.VMEM((D // 2, D), u32),
        pltpu.VMEM((1, D), bf16),
        pltpu.VMEM((D, F), bf16),
        pltpu.VMEM((D, F), bf16),
        pltpu.VMEM((F, D), bf16),
        pltpu.VMEM((S, 1), f32),
        pltpu.VMEM((S, 1), f32),
        pltpu.VMEM((S, D), bf16),
        pltpu.VMEM((64, 128), u32),
        pltpu.VMEM((64, 128), u32),
        pltpu.VMEM((3, 4, 1, 128), f32),
        pltpu.SMEM((3,), jnp.int32),
        pltpu.VMEM((8, 128), u32),
        pltpu.VMEM((8, D), f32),
        pltpu.SemaphoreType.DMA((16,)),
        pltpu.SemaphoreType.DMA((NB + 1,)),
    ]
    scratch += [pltpu.VMEM((4, 256, 128), f32)] * NSB
    scratch += [pltpu.VMEM((1, 4, 192, 128), u32)] * NPB
    scratch += [pltpu.VMEM((4, 1, 128), f32)] * NPB
    out = pl.pallas_call(
        _kernel,
        out_shape=jax.ShapeDtypeStruct((S, D), bf16),
        in_specs=[any_spec] * 7,
        out_specs=any_spec,
        scratch_shapes=scratch,
        compiler_params=pltpu.CompilerParams(vmem_limit_bytes=110 * 1024 * 1024),
    )(x, A_wqkv, A_wo, wr, B_w_gate, B_w_up, B_w_down)
    return out.reshape(1, S, D)
```

```python
import functools
import math

import jax
import jax.numpy as jnp
from jax import lax
import jax.experimental.pallas as pl
import jax.experimental.pallas.tpu as pltpu

S, D, H, DH, WIN, F = 2048, 1024, 32, 32, 256, 3584
NB = S // 128
NG = D // 128
NU = H
TB = 512
NT = S // TB
EPS = 1e-5
NEG = -1e30
QSCALE = (DH ** -0.5) * math.log2(math.e)
NEC = 2
LA = 4
NSB = 2
NPB = 2

bf16 = jnp.bfloat16
f32 = jnp.float32
u32 = jnp.uint32
NT_DIMS = (((1,), (1,)), ((), ()))


def _b2u(x):
    return pltpu.bitcast(x, u32)


def _u2b(x):
    return pltpu.bitcast(x, bf16)


def _pack2(a, b):
    w = pltpu.pack_elementwise([a, b], packed_dtype=bf16)
    return w if w.dtype == u32 else pltpu.bitcast(w, u32)


def _pack_adj(x):
    r, c = x.shape
    e = x.reshape(r // 16, 16, c)
    return _pack2(e[:, 0:8, :].reshape(r // 2, c), e[:, 8:16, :].reshape(r // 2, c))


def _kernel(x_hbm, wqkv_hbm, wo_hbm, wr_hbm, wg_hbm, wu_hbm, wd_hbm, out_hbm,
            xin, x_s, xa, xb, k_s, qt_s, vt_s, o_s,
            wk, wq, wv, wqT, wvT, wo, wou, wr, wg, wu, wd,
            r_s, a_s, outb, um_ref, lm_ref, npad, zs, zv, y_s, sems, osems, *bufs):
    OPQ = 'p'
    zs[0] = 0
    zs[1] = 0
    zv[...] = jnp.zeros((8, 128), u32)
    sb = bufs[0:NSB]
    pb = bufs[NSB:NSB + NPB]
    lb = bufs[NSB + NPB:NSB + 2 * NPB]

    XCH = [(0, 256), (256, 256), (512, 512), (1024, 512), (1536, 512)]

    def x_copy(t):
        r0, n = XCH[t]
        return pltpu.make_async_copy(x_hbm.at[pl.ds(r0, n), :], xin.at[pl.ds(r0, n), :], sems.at[t])

    def wk_copy(c):
        return pltpu.make_async_copy(wqkv_hbm.at[:, pl.ds(D + 256 * c, 256)], wk.at[:, pl.ds(256 * c, 256)], sems.at[12 + c])

    wq_copy = pltpu.make_async_copy(wqkv_hbm.at[:, pl.ds(0, D)], wq, sems.at[5])
    wv_copy = pltpu.make_async_copy(wqkv_hbm.at[:, pl.ds(2 * D, D)], wv, sems.at[6])
    wo_copy = pltpu.make_async_copy(wo_hbm, wo, sems.at[7])
    wr_copy = pltpu.make_async_copy(wr_hbm, wr, sems.at[8])
    wg_copy = pltpu.make_async_copy(wg_hbm, wg, sems.at[9])
    wu_copy = pltpu.make_async_copy(wu_hbm, wu, sems.at[10])
    wd_copy = pltpu.make_async_copy(wd_hbm, wd, sems.at[11])

    def out_copy(i):
        r0 = pl.multiple_of(i * 128, 128)
        return pltpu.make_async_copy(outb.at[pl.ds(r0, 128), :], out_hbm.at[pl.ds(r0, 128), :], osems.at[i])

    x_copy(0).start()
    wk_copy(0).start()

    row2 = lax.broadcasted_iota(jnp.int32, (64, 128), 0)
    col2 = lax.broadcasted_iota(jnp.int32, (64, 128), 1)
    um = (jnp.where(row2 > col2, jnp.uint32(0xFFFF), jnp.uint32(0))
          | jnp.where(row2 + 64 > col2, jnp.uint32(0xFFFF0000), jnp.uint32(0)))
    um_ref[...] = um
    lm_ref[...] = ~um
    ql1 = lax.broadcasted_iota(jnp.int32, (1, 128), 1) & 31
    for ii in range(3):
        for j in range(4):
            t = 256 - (128 * ii + 32 * j) if ii < 2 else 0
            n = max(0, min(256, t) - 32) + jnp.maximum(0, min(32, t) - 1 - ql1)
            npad[ii, j] = n.astype(f32)
    vt_s[0] = jnp.zeros((D // 2, 128), u32)
    vt_s[1] = jnp.zeros((D // 2, 128), u32)

    def store_ln(r0, xn):
        h0 = pl.multiple_of(r0 // 2, 64)
        xa[pl.ds(h0, 64), :] = _b2u(xn.astype(bf16))

    def plain_ln(r0, x):
        mu = jnp.mean(x, axis=1, keepdims=True)
        xc = x - mu
        var = jnp.mean(xc * xc, axis=1, keepdims=True)
        store_ln(r0, xc * lax.rsqrt(var + EPS))

    def kblock(b, g0=0, g1=NG, nb=1):
        static = isinstance(b, int)
        r = b * 64 if static else pl.multiple_of(b * 64, 64)
        xa_t = _u2b(xa[pl.ds(r, 64 * nb), :])
        kk = jnp.dot(xa_t, wk[:, 128 * g0:128 * g1], preferred_element_type=f32)
        kr = 128 + r if static else pl.multiple_of(128 + r, 64)
        toks = []
        for g in range(g0, g1):
            v = _b2u(kk[:, 128 * (g - g0):128 * (g - g0) + 128].astype(bf16))
            k_s[g, pl.ds(kr, 64 * nb), :] = v
            toks.append(v[0:8])
        return toks

    def fill_kpad():
        for g in range(NG):
            lo = k_s[g, 128:129, :] & jnp.uint32(0xFFFF)
            k_s[g, 0:128, :] = jnp.broadcast_to(lo | (lo << 16), (128, 128))

    def gate(v, tok):
        if tok is None:
            return v
        return v + pltpu.bitcast(tok & zv[...], f32)[0:1, 0:v.shape[1]]

    def ln0(b, toks=None):
        base = 128 * b if isinstance(b, int) else pl.multiple_of(128 * b, 128)
        nch = 1 if toks is None else 2
        n = 128 // nch
        for c in range(nch):
            r0 = base + n * c
            x = xin[pl.ds(r0, n), :].astype(f32)
            x_s[pl.ds(r0, n), :] = x
            mu = jnp.mean(x, axis=1, keepdims=True)
            if toks is not None:
                mu = gate(mu, toks[4 * c])
            xc = x - mu
            var = jnp.mean(xc * xc, axis=1, keepdims=True)
            h0 = r0 // 2 if isinstance(b, int) else pl.multiple_of(r0 // 2, n // 2)
            xa[pl.ds(h0, n // 2), :] = _b2u((xc * lax.rsqrt(var + EPS)).astype(bf16))

    def conv(dst, src):
        for j in range(NG):
            dst[64 * j:64 * j + 64, :] = _b2u(src[128 * j:128 * j + 128, :])

    with jax.named_scope("p0"):
        x_copy(0).wait()
        wk_copy(1).start()
        ln0(0)
        ln0(1)
        wk_copy(0).wait()
        x_copy(1).start()
        kblock(0, 0, 2, 2)
        wk_copy(1).wait()
        wk_copy(2).start()
        kblock(0, 2, 4, 2)
        x_copy(1).wait()
        wk_copy(2).wait()
        wk_copy(3).start()
        x_copy(2).start()
        kblock(0, 4, 6, 2)
        ln0(2)
        ln0(3)
        wk_copy(3).wait()
        x_copy(3).start()
        kblock(0, 6, 8, 2)
        kblock(2)

    def pro_body(t, c):
        r0 = pl.multiple_of(512 * (t + 1), 512)
        pltpu.make_async_copy(x_hbm.at[pl.ds(r0, 512), :], xin.at[pl.ds(r0, 512), :], sems.at[t + 2]).wait()

        @pl.when(t == 0)
        def _():
            x_copy(4).start()

        @pl.when(t == 1)
        def _():
            wq_copy.start()
            wv_copy.start()

        @pl.when(t == 2)
        def _():
            wo_copy.start()
            wr_copy.start()

        for b in range(3):
            toks = kblock(4 * t + 3 + b)
            if b == 0:
                ln0(4 * t + 4)
            ln0(4 * t + 5 + b, toks)
        kblock(4 * t + 6)
        return c

    with jax.named_scope("p2"):
        lax.fori_loop(0, 3, pro_body, 0)
    with jax.named_scope("p4"):
        wq_copy.wait()
        wv_copy.wait()
        wo_copy.wait()
        wr_copy.wait()
        kblock(15)
        conv(wqT, wq)
        conv(wvT, wv)
        conv(wou, wo)
        fill_kpad()

    def q_slice(xa_blk, q_blk, n):
        lhs = _u2b(xa_blk[...])
        rhs = _u2b(wqT[:, 128 * n:128 * n + 128])
        q = jnp.dot(lhs, rhs, preferred_element_type=f32)
        qt = _b2u((q * QSCALE).astype(bf16).T)
        parts = [qt[0:16]] + [pltpu.roll(qt[16 * h:16 * h + 16], 32 * h, 1) for h in range(1, 4)]
        q_blk[64 * n:64 * n + 64, :] = jnp.concatenate(parts, axis=0)
        return parts[0][0:8]

    def v_slice(xa_blk, vt_blk, n):
        lhs = _u2b(xa_blk[...])
        rhs = _u2b(wvT[:, 128 * n:128 * n + 128])
        v = jnp.dot(lhs, rhs, preferred_element_type=f32)
        vt = _b2u(_u2b(_pack_adj(v)).T)
        vt_blk[64 * n:64 * n + 64, :] = vt
        return vt[0:8]

    def o_slice(o_blk, x_blk, n):
        lhs = _u2b(o_blk[...])
        rhs = _u2b(wou[:, 128 * n:128 * n + 128])
        acc = jnp.dot(lhs, rhs, preferred_element_type=f32)
        x_blk[:, 128 * n:128 * n + 128] = x_blk[:, 128 * n:128 * n + 128] + acc
        return pltpu.bitcast(acc[0:8], u32)

    def epilogue(j, x_blk, xa_blk, xb_blk, layer, chunks=range(NEC), tok=None):
        r0 = pl.multiple_of(j * 128, 128)
        R = 128 // NEC
        for c in chunks:
            lo = R * c
            x1 = x_blk[lo:lo + R, :]
            mu = gate(jnp.mean(x1, axis=1, keepdims=True), tok)
            xc = x1 - mu
            var = jnp.mean(xc * xc, axis=1, keepdims=True)
            a = lax.rsqrt(var + EPS)
            r = jnp.sum(xc * wr[...].astype(f32), axis=1, keepdims=True) * a
            r_s[pl.ds(r0 + lo, R), :] = r
            a_s[pl.ds(r0 + lo, R), :] = a
            a1 = 1.0 + a
            x2 = mu + xc * a1
            x_blk[lo:lo + R, :] = x2
            if layer == 0:
                v = xc * (a1 * lax.rsqrt(var * a1 * a1 + EPS))
                xa_blk[lo // 2:(lo + R) // 2, :] = _b2u(v.astype(bf16))
            else:
                outb[pl.ds(r0 + lo, R), :] = x2.astype(bf16)

    def views(i, lo):
        r = pl.multiple_of((i + lo) * 64, 64)
        xav = xa.at[pl.ds(r, 192), :]
        xbv = xb.at[pl.ds(r, 192), :]
        ov = o_s.at[pl.ds(r, 128), :]
        return xav, xbv, ov

    CH = 16
    ORDER = "a0ddcd"
    EPI_EVERY = 1
    lane8b = lax.broadcasted_iota(jnp.int32, (8, 128), 1) >> 5
    odd = (lane8b & 1) == 1
    high = lane8b >= 2
    lane16b = lax.broadcasted_iota(jnp.int32, (16, 128), 1) >> 5
    d32 = lax.broadcasted_iota(jnp.int32, (32, 128), 0) - (lax.broadcasted_iota(jnp.int32, (32, 128), 1) & 31)
    umask = d32 > 0

    def stage_a(kv, q_blk, g):
        s_ref = sb[g % NSB]
        for j in range(4):
            x = jnp.concatenate([jnp.where(lane16b == ((h + j) % 4), q_blk[64 * g + 16 * h:64 * g + 16 * h + 16, :], jnp.uint32(0))
                                 for h in range(4)], axis=0)
            b0 = 16 * j
            kt = jnp.concatenate([kv[g, b0:b0 + 8, :], kv[g, b0 + 128:b0 + 136, :], kv[g, b0 + 8:b0 + 16, :],
                                  kv[g, b0 + 136:b0 + 144, :], kv[g, b0 + 16:b0 + 128, :]], axis=0)
            st = jnp.dot(_u2b(kt), _u2b(x), preferred_element_type=f32)
            su = jnp.concatenate([st[0:16], st[32:48]], axis=0)
            sl = jnp.concatenate([st[16:32], st[48:64]], axis=0)
            s_ref[j, 0:32, :] = jnp.where(umask, su, sl)
            s_ref[j, 32:256, :] = st[64:288]
            if j == 0:
                tok = (pltpu.bitcast(st[64:72], u32), pltpu.bitcast(st[160:168], u32), pltpu.bitcast(st[280:288], u32))
        return tok

    BM = 1

    def stage_b(i, g, masked, heads=range(4), toks=(None,) * 4, wtoks=(None,)):
        if list(heads) != [0]:
            return
        s_ref = sb[g % NSB]
        p_ref = pb[g % NPB].at[zs[0] if 'p' in OPQ else 0]
        l_ref = lb[g % NPB]
        if not BM:
            pps = []
            for j in range(4):
                s = s_ref[j]
                m = gate(jnp.max(s, axis=0, keepdims=True), toks[j])
                p = jnp.exp2(s - m)
                l_ref[j] = jnp.sum(p, axis=0, keepdims=True) - npad[jnp.minimum(i, 2), j] * p[32:33]
                pm = p[0:32]
                e = jnp.concatenate([jnp.where(umask, pm, 0.0), p[32:256], jnp.where(umask, 0.0, pm)], axis=0)
                pps.append(_pack_adj(e))
            for M in range(24):
                y = [pps[j][8 * (M - 2 * j):8 * (M - 2 * j) + 8, :] if 0 <= M - 2 * j < 18 else None for j in range(4)]
                w = bfly(y, wtoks[M * len(wtoks) // 24])
                for h in range(4):
                    p_ref[h, 8 * M:8 * M + 8, :] = w[h] if w[h] is not None else jnp.zeros((8, 128), u32)
            return
        ss = [s_ref[j] for j in range(4)]
        ms = [jnp.max(ss[j], axis=0, keepdims=True) for j in range(4)]
        ls = [None] * 4
        nch = len(toks)
        um16 = [umask[0:16], umask[16:32]]
        for c in range(nch):
            mg = [gate(ms[j], toks[c]) for j in range(4)]
            for M in range(24 * c // nch, 24 * (c + 1) // nch):
                y = []
                for j in range(4):
                    Mp = M - 2 * j
                    if not 0 <= Mp < 18:
                        y.append(None)
                        continue
                    row = 16 * (Mp % 16)
                    p = jnp.exp2(ss[j][row:row + 16] - mg[j])
                    if Mp < 16:
                        ps = p[0:8] + p[8:16]
                        ls[j] = ps if ls[j] is None else ls[j] + ps
                        if Mp == 2:
                            p32 = p[0:1]
                            ls[j] = ls[j] - jnp.where(lax.broadcasted_iota(jnp.int32, (8, 128), 0) == 0,
                                                      npad[jnp.minimum(i, 2), j] * p32, 0.0)
                    if Mp < 2:
                        p = jnp.where(um16[Mp], p, 0.0)
                    elif Mp >= 16:
                        p = jnp.where(um16[Mp - 16], 0.0, p)
                    y.append(_pack2(p[0:8], p[8:16]))
                w = bfly(y)
                for h in range(4):
                    p_ref[h, 8 * M:8 * M + 8, :] = w[h] if w[h] is not None else jnp.zeros((8, 128), u32)
        for j in range(4):
            l_ref[j] = jnp.sum(ls[j], axis=0, keepdims=True)

    lane8odd = (lane8b & 1).astype(u32)

    def bfly(y, tok=None):
        def sel(m, a, b):
            if a is None and b is None:
                return None
            z = jnp.zeros((8, 128), (a if a is not None else b).dtype)
            return jnp.where(m, z if a is None else a, z if b is None else b)
        od = odd if tok is None else (lane8odd | (tok & zv[...])) == jnp.uint32(1)
        r = [sel(od, y[(k + 1) % 4], y[k]) for k in range(4)]
        wp = [sel(high, r[(k + 2) % 4], r[k]) for k in range(4)]
        return [wp[(-h) % 4] for h in range(4)]

    def stage_c(vts, o_blk, g):
        p_ref = pb[g % NPB].at[zs[1] if 'p' in OPQ else 0]
        l_ref = lb[g % NPB]
        lh = bfly([jnp.broadcast_to(1.0 / l_ref[j], (8, 128)) for j in range(4)])
        outs = []
        for h in range(4):
            vt = jnp.concatenate([_u2b(vts[t][64 * g + 16 * h:64 * g + 16 * h + 16, :]) for t in range(3)], axis=1)
            o = jnp.dot(vt, _u2b(p_ref[h]), preferred_element_type=f32)
            o = o * lh[h][0:1]
            if h:
                o = pltpu.roll(o, 128 - 32 * h, 1)
            outs.append(o)
        ot = jnp.concatenate(outs, axis=0)
        o_blk[:, 128 * g:128 * g + 128] = _b2u(ot.T.astype(bf16))

    def attn_body(i, c, masked, has_next, prev, layer, extra=()):
        lo = -1 if prev is True else 0
        r = pl.multiple_of((i + lo) * 64, 64)
        nblk = (2 if has_next else 1) - lo
        xav = xa.at[pl.ds(r, 64 * nblk), :]
        xbv = xav
        ov = o_s.at[pl.ds(r, 64 * (1 - lo)), :]
        xv = x_s.at[pl.ds(pl.multiple_of((i + lo) * 128, 128), 128), :]
        qv = qt_s.at[pl.ds(i, 2)]
        vv = vt_s.at[pl.ds(i + lo, 4 - lo)]
        kv = k_s.at[:, pl.ds(pl.multiple_of(i * 64, 64), 256), :]
        blk = lambda v, b: v.at[pl.ds(64 * (b - lo), 64), :]
        vtile = lambda b: vv.at[b - lo]

        qs = [functools.partial(q_slice, blk(xav, 1), qv.at[1], n) for n in range(NG)] if has_next else []
        vs = [functools.partial(v_slice, blk(xav, 1), vtile(3), n) for n in range(NG)] if has_next else []
        os_ = [functools.partial(o_slice, blk(ov, -1), xv, n) for n in range(NG)] if prev is True else []
        SO = "q1,o8,q7,v8".split(",")
        sl = []
        last_o = -1
        pools = {"q": list(qs), "v": list(vs), "o": list(os_)}
        for tok in SO:
            for _ in range(int(tok[1:])):
                if pools[tok[0]]:
                    sl.append(pools[tok[0]].pop(0))
                    if tok[0] == "o":
                        last_o = len(sl) - 1
        assert not any(pools.values())
        if extra:
            n_it = 2 * NG
            groups = [extra[len(extra) * k // n_it:len(extra) * (k + 1) // n_it] for k in range(n_it)]
            def run(fs):
                t = None
                for f in fs:
                    t = f()
                return t
            comp = [functools.partial(run, fs) for fs in groups]
            sl = comp[0:1] + sl + comp[1:]
            last_o = NG
        per = -(-len(sl) // NG)
        emitted = [0]
        epi_done = [0]

        dtoks = []
        BG = "n,n,a,z".split(",")
        EG = 0
        WG = "n".split(",")

        def dense_one():
            k = emitted[0]
            if k < len(sl):
                t = sl[k]()
                dtoks.append(t)
                emitted[0] += 1
                if prev is True and k > last_o and epi_done[0] < NEC and (k - last_o) % EPI_EVERY == 0:
                    epilogue(i - 1, xv, blk(xav, -1), blk(xbv, -1), layer, [epi_done[0]], tok=t if EG else None)
                    epi_done[0] += 1

        if prev == "cond":
            @pl.when(i > 0)
            def _():
                finish_block(i - 1, layer)
        for g in range(NG):
            def fa():
                if g + 1 < NG:
                    return stage_a(kv.at[:, pl.ds(0, 192), :], qv.at[0], g + 1)
                elif has_next:
                    return stage_a(kv.at[:, pl.ds(64, 192), :], qv.at[1], 0)
            def fc():
                if g >= 1:
                    stage_c([vtile(t) for t in range(3)], blk(ov, 0), g - 1)
                elif prev is True:
                    stage_c([vtile(t - 1) for t in range(3)], blk(ov, -1), NG - 1)
            if g == 0:
                fc()
            nd = 0
            pats = ORDER.split(',')
            pat = pats[g % len(pats)]
            per = pat.count('d')
            k0 = len(dtoks)
            atok = None
            for ch in pat:
                if ch == "a":
                    atok = fa()
                elif ch == "c":
                    if g > 0:
                        fc()
                elif ch == "d":
                    if nd < per:
                        dense_one()
                        nd += 1
                else:
                    def tokof(sp):
                        if sp in ("a", "m", "z"):
                            return None if atok is None else atok["amz".index(sp)]
                        if sp[0] == "p":
                            idx = k0 - int(sp[1:])
                            return dtoks[idx] if 0 <= idx < len(dtoks) else None
                        if sp[0] == "c":
                            idx = k0 + int(sp[1:])
                            return dtoks[idx] if idx < len(dtoks) else None
                        return None
                    stage_b(i, g, masked, [int(ch)], [tokof(sp) for sp in BG], [tokof(sp) for sp in WG])
        while emitted[0] < len(sl):
            dense_one()
        if prev is True:
            while epi_done[0] < NEC:
                epilogue(i - 1, xv, blk(xav, -1), blk(xbv, -1), layer, [epi_done[0]])
                epi_done[0] += 1

        if layer == 1 and prev is True:
            out_copy(i - 1).start()
        if layer == 0 and prev is True and has_next:
            @pl.when(i == 1)
            def _():
                wg_copy.start()
                wu_copy.start()
                wd_copy.start()
        return c

    def finish_block(j, layer):
        o_blk = o_s.at[pl.ds(pl.multiple_of(j * 64, 64), 64), :]
        x_blk = x_s.at[pl.ds(pl.multiple_of(j * 128, 128), 128), :]
        stage_c([vt_s.at[j + t] for t in range(3)], o_blk, NG - 1)
        for n in range(NG):
            o_slice(o_blk, x_blk, n)
        epilogue(j, x_blk, xa.at[pl.ds(pl.multiple_of(j * 64, 64), 64), :], None, layer)

    def layer_body(layer, c):
        with jax.named_scope("qv0"):
            for n in range(NG):
                q_slice(xa.at[pl.ds(0, 64), :], qt_s.at[0], n)
            for n in range(NG):
                v_slice(xa.at[pl.ds(0, 64), :], vt_s.at[2], n)
            stage_a(k_s.at[:, pl.ds(0, 192), :], qt_s.at[0], 0)
        with jax.named_scope("attn"):
            with jax.named_scope("first"):
                attn_body(0, 0, masked=False, has_next=True, prev=False, layer=layer)
            with jax.named_scope("main"):
                lax.fori_loop(1, NB - 1, functools.partial(attn_body, masked=False, has_next=True, prev=True, layer=layer), 0)
            with jax.named_scope("last"):
                if layer == 0:
                    extra = [functools.partial(kslice, b, g) for b in range(K2_EARLY) for g in range(NG)]
                    attn_body(NB - 1, 0, masked=False, has_next=False, prev=True, layer=layer, extra=extra)
                else:
                    attn_body(NB - 1, 0, masked=False, has_next=False, prev=True, layer=layer)
        with jax.named_scope("tail"):
            finish_block(NB - 1, layer)

        if layer == 0:
            wg_copy.wait()
            wu_copy.wait()
            wd_copy.wait()
            with jax.named_scope("ffn_mid"):
                ffn_mid()
        else:
            out_copy(NB - 1).start()
            with jax.named_scope("ffn_last"):
                ffn_last()
        return c

    FC = 512

    def route(nrows=S):
        r = r_s[0:nrows, :]
        rmax = jnp.max(r)
        rows = lax.broadcasted_iota(jnp.int32, (nrows, 1), 0)
        idx = jnp.min(jnp.where(r == rmax, rows, nrows))
        idx = jnp.minimum(idx, nrows - 1)
        xrow = x_s[pl.ds(idx, 1), :]
        arow = a_s[pl.ds(idx, 1), :]
        xsel = (xrow - jnp.mean(xrow, axis=1, keepdims=True)) * (arow / (1.0 + arow))
        xs = jnp.broadcast_to(xsel, (8, D)).astype(bf16)
        return idx, rmax, xrow, xs

    def ffn_up(xs, c):
        gate = jnp.dot(xs, wg[:, FC * c:FC * (c + 1)], preferred_element_type=f32)
        up = jnp.dot(xs, wu[:, FC * c:FC * (c + 1)], preferred_element_type=f32)
        return (gate * jax.nn.sigmoid(gate) * up).astype(bf16)

    def ffn_down(hid, c):
        return jnp.dot(hid, wd[FC * c:FC * (c + 1), :], preferred_element_type=f32)

    K2_EARLY = 2

    def kslice(b, g):
        kblock(b, g, g + 1)
        return None

    def ffn_mid():
        with jax.named_scope("fm_a"):
            kblock(K2_EARLY)
            idx, rmax, xrow, xs = route()
        with jax.named_scope("fm_b"):
            y = fm_b(xs)
        with jax.named_scope("fm_c"):
            fm_c(idx, rmax, xrow, y)

    NFS = F // 128

    def ffn_steps(xs):
        gates, hid, ys = [], [], []

        def up(c, w, first):
            r = jnp.dot(xs, w[:, 128 * c:128 * (c + 1)], preferred_element_type=f32)
            if first:
                gates.append(r)
            else:
                g_ = gates[c]
                hid.append((g_ * jax.nn.sigmoid(g_) * r).astype(bf16))
            return pltpu.bitcast(r, u32)

        def down(c):
            r = jnp.dot(hid[c], wd[128 * c:128 * (c + 1), :], preferred_element_type=f32)
            ys.append(r)
            return pltpu.bitcast(r[:, 0:128], u32)

        steps = []
        for c in range(NFS):
            steps.append(functools.partial(up, c, wg, True))
            steps.append(functools.partial(up, c, wu, False))
            if c >= 1:
                steps.append(functools.partial(down, c - 1))
        steps.append(functools.partial(down, NFS - 1))

        def result():
            y = ys[0]
            for t in ys[1:]:
                y = y + t
            return y
        return steps, result

    def fm_b(xs):
        items = [(b, g) for b in range(K2_EARLY + 1, NB) for g in range(NG)]
        steps, result = ffn_steps(xs)
        fi = 0
        for k, (b, g) in enumerate(items):
            kslice(b, g)
            if fi < len(steps):
                steps[fi]()
                fi += 1
        while fi < len(steps):
            steps[fi]()
            fi += 1
        return result()

    def fm_c(idx, rmax, xrow, y):
        x_s[pl.ds(idx, 1), :] = xrow + y[0:1, :] * jax.nn.sigmoid(rmax)
        r0 = pl.multiple_of((idx // 16) * 16, 16)
        h0 = pl.multiple_of((idx // 16) * 8, 8)
        x = x_s[pl.ds(r0, 16), :]
        mu = jnp.mean(x, axis=1, keepdims=True)
        xc = x - mu
        var = jnp.mean(xc * xc, axis=1, keepdims=True)
        xn = (xc * lax.rsqrt(var + EPS)).astype(bf16)
        xa[pl.ds(h0, 8), :] = _b2u(xn)
        kk = jnp.dot(xn, wk[...], preferred_element_type=f32)
        for g in range(NG):
            k_s[g, pl.ds(128 + h0, 8), :] = _b2u(kk[:, 128 * g:128 * g + 128].astype(bf16))
        fill_kpad()

    def ffn_last():
        idx, rmax, xrow, xs = route()

        steps, result = ffn_steps(xs)
        for f in steps:
            f()
        y = result()
        x_s[pl.ds(idx, 1), :] = xrow + y[0:1, :] * jax.nn.sigmoid(rmax)
        for i in range(NB):
            out_copy(i).wait()
        b0 = pl.multiple_of((idx // 16) * 16, 16)
        outb[pl.ds(b0, 16), :] = x_s[pl.ds(b0, 16), :].astype(bf16)
        fix = pltpu.make_async_copy(outb.at[pl.ds(b0, 16), :], out_hbm.at[pl.ds(b0, 16), :], osems.at[NB])
        fix.start()
        fix.wait()

    layer_body(0, 0)
    layer_body(1, 0)


@jax.jit
def pallas_interleave_layers__sliding_block__moe_arch_mod__prompt_kernel(
    A_x: jax.Array,
    A_wqkv: jax.Array,
    A_wo: jax.Array,
    B_x: jax.Array,
    B_w_r: jax.Array,
    B_w_gate: jax.Array,
    B_w_up: jax.Array,
    B_w_down: jax.Array,
):
    del B_x
    x = A_x.reshape(S, D)
    wr = B_w_r.reshape(1, D)
    any_spec = pl.BlockSpec(memory_space=pl.ANY)
    scratch = [
        pltpu.VMEM((S, D), bf16),
        pltpu.VMEM((S, D), f32),
        pltpu.VMEM((S // 2, D), u32),
        pltpu.VMEM((64 * 3, D), u32),
        pltpu.VMEM((NG, (S + 256) // 2 + 64, 128), u32),
        pltpu.VMEM((NB + 1, D // 2, 128), u32),
        pltpu.VMEM((NB + 3, D // 2, 128), u32),
        pltpu.VMEM((S // 2, D), u32),
        pltpu.VMEM((D, D), bf16),
        pltpu.VMEM((D, D), bf16),
        pltpu.VMEM((D, D), bf16),
        pltpu.VMEM((D // 2, D), u32),
        pltpu.VMEM((D // 2, D), u32),
        pltpu.VMEM((D, D), bf16),
        pltpu.VMEM((D // 2, D), u32),
        pltpu.VMEM((1, D), bf16),
        pltpu.VMEM((D, F), bf16),
        pltpu.VMEM((D, F), bf16),
        pltpu.VMEM((F, D), bf16),
        pltpu.VMEM((S, 1), f32),
        pltpu.VMEM((S, 1), f32),
        pltpu.VMEM((S, D), bf16),
        pltpu.VMEM((64, 128), u32),
        pltpu.VMEM((64, 128), u32),
        pltpu.VMEM((3, 4, 1, 128), f32),
        pltpu.SMEM((3,), jnp.int32),
        pltpu.VMEM((8, 128), u32),
        pltpu.VMEM((8, D), f32),
        pltpu.SemaphoreType.DMA((16,)),
        pltpu.SemaphoreType.DMA((NB + 1,)),
    ]
    scratch += [pltpu.VMEM((4, 256, 128), f32)] * NSB
    scratch += [pltpu.VMEM((1, 4, 192, 128), u32)] * NPB
    scratch += [pltpu.VMEM((4, 1, 128), f32)] * NPB
    out = pl.pallas_call(
        _kernel,
        out_shape=jax.ShapeDtypeStruct((S, D), bf16),
        in_specs=[any_spec] * 7,
        out_specs=any_spec,
        scratch_shapes=scratch,
        compiler_params=pltpu.CompilerParams(vmem_limit_bytes=110 * 1024 * 1024),
    )(x, A_wqkv, A_wo, wr, B_w_gate, B_w_up, B_w_down)
    return out.reshape(1, S, D)
```

```python
import functools
import math

import jax
import jax.numpy as jnp
from jax import lax
import jax.experimental.pallas as pl
import jax.experimental.pallas.tpu as pltpu

S, D, H, DH, F = 2048, 1024, 32, 32, 3584
NB = S // 128
NG = D // 128
NFS = F // 128
EPS = 1e-5
QSCALE = (DH ** -0.5) * math.log2(math.e)
NEC = 2
NBUF = 2
K2_EARLY = 2
XCH = [(0, 256), (256, 256), (512, 512), (1024, 512), (1536, 512)]

bf16 = jnp.bfloat16
f32 = jnp.float32
u32 = jnp.uint32


def _b2u(x):
    return pltpu.bitcast(x, u32)


def _u2b(x):
    return pltpu.bitcast(x, bf16)


def _pack2(a, b):
    w = pltpu.pack_elementwise([a, b], packed_dtype=bf16)
    return w if w.dtype == u32 else pltpu.bitcast(w, u32)


def _pack_adj(x):
    r, c = x.shape
    e = x.reshape(r // 16, 16, c)
    return _pack2(e[:, 0:8, :].reshape(r // 2, c), e[:, 8:16, :].reshape(r // 2, c))


def _kernel(x_hbm, wqkv_hbm, wo_hbm, wr_hbm, wg_hbm, wu_hbm, wd_hbm, out_hbm,
            xin, x_s, xa, k_s, qt_s, vt_s, o_s,
            wk, wq, wv, wqu, wvu, wo, wou, wr, wg, wu, wd,
            r_s, a_s, outb, npad, zs, zv, sems, osems, *bufs):
    zs[0] = 0
    zs[1] = 0
    zv[...] = jnp.zeros((8, 128), u32)
    sb = bufs[0:NBUF]
    pb = bufs[NBUF:2 * NBUF]
    lb = bufs[2 * NBUF:3 * NBUF]

    def x_copy(t):
        r0, n = XCH[t]
        return pltpu.make_async_copy(x_hbm.at[pl.ds(r0, n), :], xin.at[pl.ds(r0, n), :], sems.at[t])

    def wk_copy(c):
        return pltpu.make_async_copy(wqkv_hbm.at[:, pl.ds(D + 256 * c, 256)], wk.at[:, pl.ds(256 * c, 256)],
                                     sems.at[12 + c])

    wq_copy = pltpu.make_async_copy(wqkv_hbm.at[:, pl.ds(0, D)], wq, sems.at[5])
    wv_copy = pltpu.make_async_copy(wqkv_hbm.at[:, pl.ds(2 * D, D)], wv, sems.at[6])
    wo_copy = pltpu.make_async_copy(wo_hbm, wo, sems.at[7])
    wr_copy = pltpu.make_async_copy(wr_hbm, wr, sems.at[8])
    wg_copy = pltpu.make_async_copy(wg_hbm, wg, sems.at[9])
    wu_copy = pltpu.make_async_copy(wu_hbm, wu, sems.at[10])
    wd_copy = pltpu.make_async_copy(wd_hbm, wd, sems.at[11])

    def out_copy(i):
        r0 = pl.multiple_of(i * 128, 128)
        return pltpu.make_async_copy(outb.at[pl.ds(r0, 128), :], out_hbm.at[pl.ds(r0, 128), :], osems.at[i])

    x_copy(0).start()
    wk_copy(0).start()

    ql1 = lax.broadcasted_iota(jnp.int32, (1, 128), 1) & 31
    for ii in range(3):
        for j in range(4):
            t = 256 - (128 * ii + 32 * j) if ii < 2 else 0
            n = max(0, min(256, t) - 32) + jnp.maximum(0, min(32, t) - 1 - ql1)
            npad[ii, j] = n.astype(f32)
    vt_s[0] = jnp.zeros((D // 2, 128), u32)
    vt_s[1] = jnp.zeros((D // 2, 128), u32)

    def kblock(b, g0=0, g1=NG, nb=1):
        static = isinstance(b, int)
        r = b * 64 if static else pl.multiple_of(b * 64, 64)
        xa_t = _u2b(xa[pl.ds(r, 64 * nb), :])
        kk = jnp.dot(xa_t, wk[:, 128 * g0:128 * g1], preferred_element_type=f32)
        kr = 128 + r if static else pl.multiple_of(128 + r, 64)
        toks = []
        for g in range(g0, g1):
            v = _b2u(kk[:, 128 * (g - g0):128 * (g - g0) + 128].astype(bf16))
            k_s[g, pl.ds(kr, 64 * nb), :] = v
            toks.append(v[0:8])
        return toks

    def fill_kpad():
        for g in range(NG):
            lo = k_s[g, 128:129, :] & jnp.uint32(0xFFFF)
            k_s[g, 0:128, :] = jnp.broadcast_to(lo | (lo << 16), (128, 128))

    def gate(v, tok):
        if tok is None:
            return v
        return v + pltpu.bitcast(tok & zv[...], f32)[0:1, 0:v.shape[1]]

    def ln0(b, toks=None):
        base = 128 * b if isinstance(b, int) else pl.multiple_of(128 * b, 128)
        nch = 1 if toks is None else 2
        n = 128 // nch
        for c in range(nch):
            r0 = base + n * c
            x = xin[pl.ds(r0, n), :].astype(f32)
            x_s[pl.ds(r0, n), :] = x
            mu = jnp.mean(x, axis=1, keepdims=True)
            if toks is not None:
                mu = gate(mu, toks[4 * c])
            xc = x - mu
            var = jnp.mean(xc * xc, axis=1, keepdims=True)
            h0 = r0 // 2 if isinstance(b, int) else pl.multiple_of(r0 // 2, n // 2)
            xa[pl.ds(h0, n // 2), :] = _b2u((xc * lax.rsqrt(var + EPS)).astype(bf16))

    def conv(dst, src):
        for j in range(NG):
            dst[64 * j:64 * j + 64, :] = _b2u(src[128 * j:128 * j + 128, :])

    x_copy(0).wait()
    wk_copy(1).start()
    ln0(0)
    ln0(1)
    wk_copy(0).wait()
    x_copy(1).start()
    kblock(0, 0, 2, 2)
    wk_copy(1).wait()
    wk_copy(2).start()
    kblock(0, 2, 4, 2)
    x_copy(1).wait()
    wk_copy(2).wait()
    wk_copy(3).start()
    x_copy(2).start()
    kblock(0, 4, 6, 2)
    ln0(2)
    ln0(3)
    wk_copy(3).wait()
    x_copy(3).start()
    kblock(0, 6, 8, 2)
    kblock(2)

    def pro_body(t, c):
        r0 = pl.multiple_of(512 * (t + 1), 512)
        pltpu.make_async_copy(x_hbm.at[pl.ds(r0, 512), :], xin.at[pl.ds(r0, 512), :], sems.at[t + 2]).wait()

        @pl.when(t == 0)
        def _():
            x_copy(4).start()

        @pl.when(t == 1)
        def _():
            wq_copy.start()
            wv_copy.start()

        @pl.when(t == 2)
        def _():
            wo_copy.start()
            wr_copy.start()

        for b in range(3):
            toks = kblock(4 * t + 3 + b)
            if b == 0:
                ln0(4 * t + 4)
            ln0(4 * t + 5 + b, toks)
        kblock(4 * t + 6)
        return c

    lax.fori_loop(0, 3, pro_body, 0)
    wq_copy.wait()
    wv_copy.wait()
    wo_copy.wait()
    wr_copy.wait()
    kblock(15)
    conv(wqu, wq)
    conv(wvu, wv)
    conv(wou, wo)
    fill_kpad()

    def q_slice(xa_blk, q_blk, n):
        lhs = _u2b(xa_blk[...])
        rhs = _u2b(wqu[:, 128 * n:128 * n + 128])
        q = jnp.dot(lhs, rhs, preferred_element_type=f32)
        qt = _b2u((q * QSCALE).astype(bf16).T)
        parts = [qt[0:16]] + [pltpu.roll(qt[16 * h:16 * h + 16], 32 * h, 1) for h in range(1, 4)]
        q_blk[64 * n:64 * n + 64, :] = jnp.concatenate(parts, axis=0)
        return parts[0][0:8]

    def v_slice(xa_blk, vt_blk, n):
        lhs = _u2b(xa_blk[...])
        rhs = _u2b(wvu[:, 128 * n:128 * n + 128])
        v = jnp.dot(lhs, rhs, preferred_element_type=f32)
        vt = _b2u(_u2b(_pack_adj(v)).T)
        vt_blk[64 * n:64 * n + 64, :] = vt
        return vt[0:8]

    def o_slice(o_blk, x_blk, n):
        lhs = _u2b(o_blk[...])
        rhs = _u2b(wou[:, 128 * n:128 * n + 128])
        acc = jnp.dot(lhs, rhs, preferred_element_type=f32)
        x_blk[:, 128 * n:128 * n + 128] = x_blk[:, 128 * n:128 * n + 128] + acc
        return pltpu.bitcast(acc[0:8], u32)

    def epilogue(j, x_blk, xa_blk, layer, chunks=range(NEC)):
        r0 = pl.multiple_of(j * 128, 128)
        R = 128 // NEC
        for c in chunks:
            lo = R * c
            x1 = x_blk[lo:lo + R, :]
            mu = jnp.mean(x1, axis=1, keepdims=True)
            xc = x1 - mu
            var = jnp.mean(xc * xc, axis=1, keepdims=True)
            a = lax.rsqrt(var + EPS)
            r = jnp.sum(xc * wr[...].astype(f32), axis=1, keepdims=True) * a
            r_s[pl.ds(r0 + lo, R), :] = r
            a_s[pl.ds(r0 + lo, R), :] = a
            a1 = 1.0 + a
            x2 = mu + xc * a1
            x_blk[lo:lo + R, :] = x2
            if layer == 0:
                v = xc * (a1 * lax.rsqrt(var * a1 * a1 + EPS))
                xa_blk[lo // 2:(lo + R) // 2, :] = _b2u(v.astype(bf16))
            else:
                outb[pl.ds(r0 + lo, R), :] = x2.astype(bf16)

    lane8b = lax.broadcasted_iota(jnp.int32, (8, 128), 1) >> 5
    odd = (lane8b & 1) == 1
    high = lane8b >= 2
    lane16b = lax.broadcasted_iota(jnp.int32, (16, 128), 1) >> 5
    d32 = lax.broadcasted_iota(jnp.int32, (32, 128), 0) - (lax.broadcasted_iota(jnp.int32, (32, 128), 1) & 31)
    umask = d32 > 0

    def stage_a(kv, q_blk, g):
        s_ref = sb[g % NBUF]
        for j in range(4):
            x = jnp.concatenate([jnp.where(lane16b == ((h + j) % 4), q_blk[64 * g + 16 * h:64 * g + 16 * h + 16, :],
                                           jnp.uint32(0)) for h in range(4)], axis=0)
            b0 = 16 * j
            kt = jnp.concatenate([kv[g, b0:b0 + 8, :], kv[g, b0 + 128:b0 + 136, :], kv[g, b0 + 8:b0 + 16, :],
                                  kv[g, b0 + 136:b0 + 144, :], kv[g, b0 + 16:b0 + 128, :]], axis=0)
            st = jnp.dot(_u2b(kt), _u2b(x), preferred_element_type=f32)
            su = jnp.concatenate([st[0:16], st[32:48]], axis=0)
            sl = jnp.concatenate([st[16:32], st[48:64]], axis=0)
            s_ref[j, 0:32, :] = jnp.where(umask, su, sl)
            s_ref[j, 32:256, :] = st[64:288]
            if j == 0:
                tok = (pltpu.bitcast(st[64:72], u32), pltpu.bitcast(st[160:168], u32),
                       pltpu.bitcast(st[280:288], u32))
        return tok

    def bfly(y):
        def sel(m, a, b):
            if a is None and b is None:
                return None
            z = jnp.zeros((8, 128), (a if a is not None else b).dtype)
            return jnp.where(m, z if a is None else a, z if b is None else b)
        r = [sel(odd, y[(k + 1) % 4], y[k]) for k in range(4)]
        wp = [sel(high, r[(k + 2) % 4], r[k]) for k in range(4)]
        return [wp[(-h) % 4] for h in range(4)]

    def stage_b(i, g, toks):
        s_ref = sb[g % NBUF]
        p_ref = pb[g % NBUF].at[zs[0]]
        l_ref = lb[g % NBUF]
        ss = [s_ref[j] for j in range(4)]
        ms = [jnp.max(ss[j], axis=0, keepdims=True) for j in range(4)]
        ls = [None] * 4
        nch = len(toks)
        um16 = [umask[0:16], umask[16:32]]
        for c in range(nch):
            mg = [gate(ms[j], toks[c]) for j in range(4)]
            for M in range(24 * c // nch, 24 * (c + 1) // nch):
                y = []
                for j in range(4):
                    Mp = M - 2 * j
                    if not 0 <= Mp < 18:
                        y.append(None)
                        continue
                    row = 16 * (Mp % 16)
                    p = jnp.exp2(ss[j][row:row + 16] - mg[j])
                    if Mp < 16:
                        ps = p[0:8] + p[8:16]
                        ls[j] = ps if ls[j] is None else ls[j] + ps
                        if Mp == 2:
                            p32 = p[0:1]
                            ls[j] = ls[j] - jnp.where(lax.broadcasted_iota(jnp.int32, (8, 128), 0) == 0,
                                                      npad[jnp.minimum(i, 2), j] * p32, 0.0)
                    if Mp < 2:
                        p = jnp.where(um16[Mp], p, 0.0)
                    elif Mp >= 16:
                        p = jnp.where(um16[Mp - 16], 0.0, p)
                    y.append(_pack2(p[0:8], p[8:16]))
                w = bfly(y)
                for h in range(4):
                    p_ref[h, 8 * M:8 * M + 8, :] = w[h] if w[h] is not None else jnp.zeros((8, 128), u32)
        for j in range(4):
            l_ref[j] = jnp.sum(ls[j], axis=0, keepdims=True)

    def stage_c(vts, o_blk, g):
        p_ref = pb[g % NBUF].at[zs[1]]
        l_ref = lb[g % NBUF]
        lh = bfly([jnp.broadcast_to(1.0 / l_ref[j], (8, 128)) for j in range(4)])
        outs = []
        for h in range(4):
            vt = jnp.concatenate([_u2b(vts[t][64 * g + 16 * h:64 * g + 16 * h + 16, :]) for t in range(3)], axis=1)
            o = jnp.dot(vt, _u2b(p_ref[h]), preferred_element_type=f32)
            o = o * lh[h][0:1]
            if h:
                o = pltpu.roll(o, 128 - 32 * h, 1)
            outs.append(o)
        ot = jnp.concatenate(outs, axis=0)
        o_blk[:, 128 * g:128 * g + 128] = _b2u(ot.T.astype(bf16))

    def attn_body(i, c, has_next, prev, layer, extra=()):
        lo = -1 if prev else 0
        r = pl.multiple_of((i + lo) * 64, 64)
        nblk = (2 if has_next else 1) - lo
        xav = xa.at[pl.ds(r, 64 * nblk), :]
        ov = o_s.at[pl.ds(r, 64 * (1 - lo)), :]
        xv = x_s.at[pl.ds(pl.multiple_of((i + lo) * 128, 128), 128), :]
        qv = qt_s.at[pl.ds(i, 2)]
        vv = vt_s.at[pl.ds(i + lo, 4 - lo)]
        kv = k_s.at[:, pl.ds(pl.multiple_of(i * 64, 64), 256), :]
        blk = lambda v, b: v.at[pl.ds(64 * (b - lo), 64), :]
        vtile = lambda b: vv.at[b - lo]

        qs = [functools.partial(q_slice, blk(xav, 1), qv.at[1], n) for n in range(NG)] if has_next else []
        vs = [functools.partial(v_slice, blk(xav, 1), vtile(3), n) for n in range(NG)] if has_next else []
        os_ = [functools.partial(o_slice, blk(ov, -1), xv, n) for n in range(NG)] if prev else []
        sl = qs[0:1] + os_ + qs[1:] + vs
        last_o = len(qs[0:1]) + len(os_) - 1 if os_ else -1
        if extra:
            n_it = 2 * NG
            groups = [extra[len(extra) * k // n_it:len(extra) * (k + 1) // n_it] for k in range(n_it)]

            def run(fs):
                for f in fs:
                    f()
            comp = [functools.partial(run, fs) for fs in groups]
            sl = comp[0:1] + sl + comp[1:]
            last_o = NG
        state = {"emitted": 0, "epi": 0}

        def next_epilogue_chunk():
            epilogue(i - 1, xv, blk(xav, -1), layer, [state["epi"]])
            state["epi"] += 1

        def dense_one():
            k = state["emitted"]
            if k < len(sl):
                sl[k]()
                state["emitted"] += 1
                if prev and k > last_o and state["epi"] < NEC:
                    next_epilogue_chunk()

        for g in range(NG):
            def pv():
                if g >= 1:
                    stage_c([vtile(t) for t in range(3)], blk(ov, 0), g - 1)
                elif prev:
                    stage_c([vtile(t - 1) for t in range(3)], blk(ov, -1), NG - 1)
            if g == 0:
                pv()
            tok = (None, None, None)
            if g + 1 < NG:
                tok = stage_a(kv.at[:, pl.ds(0, 192), :], qv.at[0], g + 1)
            elif has_next:
                tok = stage_a(kv.at[:, pl.ds(64, 192), :], qv.at[1], 0)
            stage_b(i, g, [None, None, tok[0], tok[2]])
            dense_one()
            dense_one()
            if g > 0:
                pv()
            dense_one()
        while state["emitted"] < len(sl):
            dense_one()
        if prev:
            while state["epi"] < NEC:
                next_epilogue_chunk()

        if layer == 1 and prev:
            out_copy(i - 1).start()
        if layer == 0 and prev and has_next:
            @pl.when(i == 1)
            def _():
                wg_copy.start()
                wu_copy.start()
                wd_copy.start()
        return c

    def finish_block(j, layer):
        o_blk = o_s.at[pl.ds(pl.multiple_of(j * 64, 64), 64), :]
        x_blk = x_s.at[pl.ds(pl.multiple_of(j * 128, 128), 128), :]
        stage_c([vt_s.at[j + t] for t in range(3)], o_blk, NG - 1)
        for n in range(NG):
            o_slice(o_blk, x_blk, n)
        epilogue(j, x_blk, xa.at[pl.ds(pl.multiple_of(j * 64, 64), 64), :], layer)

    def route():
        r = r_s[0:S, :]
        rmax = jnp.max(r)
        rows = lax.broadcasted_iota(jnp.int32, (S, 1), 0)
        idx = jnp.min(jnp.where(r == rmax, rows, S))
        idx = jnp.minimum(idx, S - 1)
        xrow = x_s[pl.ds(idx, 1), :]
        arow = a_s[pl.ds(idx, 1), :]
        xsel = (xrow - jnp.mean(xrow, axis=1, keepdims=True)) * (arow / (1.0 + arow))
        xs = jnp.broadcast_to(xsel, (8, D)).astype(bf16)
        return idx, rmax, xrow, xs

    def ffn_steps(xs):
        gates, hid, ys = [], [], []

        def up(c, w, first):
            r = jnp.dot(xs, w[:, 128 * c:128 * (c + 1)], preferred_element_type=f32)
            if first:
                gates.append(r)
            else:
                g_ = gates[c]
                hid.append((g_ * jax.nn.sigmoid(g_) * r).astype(bf16))

        def down(c):
            ys.append(jnp.dot(hid[c], wd[128 * c:128 * (c + 1), :], preferred_element_type=f32))

        steps = []
        for c in range(NFS):
            steps.append(functools.partial(up, c, wg, True))
            steps.append(functools.partial(up, c, wu, False))
            if c >= 1:
                steps.append(functools.partial(down, c - 1))
        steps.append(functools.partial(down, NFS - 1))

        def result():
            y = ys[0]
            for t in ys[1:]:
                y = y + t
            return y
        return steps, result

    def kslice(b, g):
        kblock(b, g, g + 1)

    def ffn_mid():
        kblock(K2_EARLY)
        idx, rmax, xrow, xs = route()
        steps, result = ffn_steps(xs)
        fi = 0
        for b in range(K2_EARLY + 1, NB):
            for g in range(NG):
                kslice(b, g)
                if fi < len(steps):
                    steps[fi]()
                    fi += 1
        while fi < len(steps):
            steps[fi]()
            fi += 1
        y = result()
        x_s[pl.ds(idx, 1), :] = xrow + y[0:1, :] * jax.nn.sigmoid(rmax)
        r0 = pl.multiple_of((idx // 16) * 16, 16)
        h0 = pl.multiple_of((idx // 16) * 8, 8)
        x = x_s[pl.ds(r0, 16), :]
        mu = jnp.mean(x, axis=1, keepdims=True)
        xc = x - mu
        var = jnp.mean(xc * xc, axis=1, keepdims=True)
        xn = (xc * lax.rsqrt(var + EPS)).astype(bf16)
        xa[pl.ds(h0, 8), :] = _b2u(xn)
        kk = jnp.dot(xn, wk[...], preferred_element_type=f32)
        for g in range(NG):
            k_s[g, pl.ds(128 + h0, 8), :] = _b2u(kk[:, 128 * g:128 * g + 128].astype(bf16))
        fill_kpad()

    def ffn_last():
        idx, rmax, xrow, xs = route()
        steps, result = ffn_steps(xs)
        for f in steps:
            f()
        y = result()
        x_s[pl.ds(idx, 1), :] = xrow + y[0:1, :] * jax.nn.sigmoid(rmax)
        for i in range(NB):
            out_copy(i).wait()
        b0 = pl.multiple_of((idx // 16) * 16, 16)
        outb[pl.ds(b0, 16), :] = x_s[pl.ds(b0, 16), :].astype(bf16)
        fix = pltpu.make_async_copy(outb.at[pl.ds(b0, 16), :], out_hbm.at[pl.ds(b0, 16), :], osems.at[NB])
        fix.start()
        fix.wait()

    for layer in range(2):
        for n in range(NG):
            q_slice(xa.at[pl.ds(0, 64), :], qt_s.at[0], n)
        for n in range(NG):
            v_slice(xa.at[pl.ds(0, 64), :], vt_s.at[2], n)
        stage_a(k_s.at[:, pl.ds(0, 192), :], qt_s.at[0], 0)
        attn_body(0, 0, has_next=True, prev=False, layer=layer)
        lax.fori_loop(1, NB - 1, functools.partial(attn_body, has_next=True, prev=True, layer=layer), 0)
        extra = [functools.partial(kslice, b, g) for b in range(K2_EARLY) for g in range(NG)] if layer == 0 else ()
        attn_body(NB - 1, 0, has_next=False, prev=True, layer=layer, extra=extra)
        finish_block(NB - 1, layer)
        if layer == 0:
            wg_copy.wait()
            wu_copy.wait()
            wd_copy.wait()
            ffn_mid()
        else:
            out_copy(NB - 1).start()
            ffn_last()


@jax.jit
def pallas_interleave_layers__sliding_block__moe_arch_mod__prompt_kernel(
    A_x: jax.Array,
    A_wqkv: jax.Array,
    A_wo: jax.Array,
    B_x: jax.Array,
    B_w_r: jax.Array,
    B_w_gate: jax.Array,
    B_w_up: jax.Array,
    B_w_down: jax.Array,
):
    del B_x
    x = A_x.reshape(S, D)
    wr = B_w_r.reshape(1, D)
    any_spec = pl.BlockSpec(memory_space=pl.ANY)
    scratch = [
        pltpu.VMEM((S, D), bf16),
        pltpu.VMEM((S, D), f32),
        pltpu.VMEM((S // 2, D), u32),
        pltpu.VMEM((NG, (S + 256) // 2 + 64, 128), u32),
        pltpu.VMEM((NB + 1, D // 2, 128), u32),
        pltpu.VMEM((NB + 3, D // 2, 128), u32),
        pltpu.VMEM((S // 2, D), u32),
        pltpu.VMEM((D, D), bf16),
        pltpu.VMEM((D, D), bf16),
        pltpu.VMEM((D, D), bf16),
        pltpu.VMEM((D // 2, D), u32),
        pltpu.VMEM((D // 2, D), u32),
        pltpu.VMEM((D, D), bf16),
        pltpu.VMEM((D // 2, D), u32),
        pltpu.VMEM((1, D), bf16),
        pltpu.VMEM((D, F), bf16),
        pltpu.VMEM((D, F), bf16),
        pltpu.VMEM((F, D), bf16),
        pltpu.VMEM((S, 1), f32),
        pltpu.VMEM((S, 1), f32),
        pltpu.VMEM((S, D), bf16),
        pltpu.VMEM((3, 4, 1, 128), f32),
        pltpu.SMEM((2,), jnp.int32),
        pltpu.VMEM((8, 128), u32),
        pltpu.SemaphoreType.DMA((16,)),
        pltpu.SemaphoreType.DMA((NB + 1,)),
    ]
    scratch += [pltpu.VMEM((4, 256, 128), f32)] * NBUF
    scratch += [pltpu.VMEM((1, 4, 192, 128), u32)] * NBUF
    scratch += [pltpu.VMEM((4, 1, 128), f32)] * NBUF
    out = pl.pallas_call(
        _kernel,
        out_shape=jax.ShapeDtypeStruct((S, D), bf16),
        in_specs=[any_spec] * 7,
        out_specs=any_spec,
        scratch_shapes=scratch,
        compiler_params=pltpu.CompilerParams(vmem_limit_bytes=110 * 1024 * 1024),
    )(x, A_wqkv, A_wo, wr, B_w_gate, B_w_up, B_w_down)
    return out.reshape(1, S, D)
```

```python
import functools
import math

import jax
import jax.numpy as jnp
from jax import lax
import jax.experimental.pallas as pl
import jax.experimental.pallas.tpu as pltpu

S, D, H, DH, F = 2048, 1024, 32, 32, 3584
NB = S // 128
NG = D // 128
NFS = F // 128
EPS = 1e-5
QSCALE = (DH ** -0.5) * math.log2(math.e)
NEC = 2
NBUF = 2
K2_EARLY = 2
XCH = [(0, 256), (256, 256), (512, 512), (1024, 512), (1536, 512)]

bf16 = jnp.bfloat16
f32 = jnp.float32
u32 = jnp.uint32


def _b2u(x):
    return pltpu.bitcast(x, u32)


def _u2b(x):
    return pltpu.bitcast(x, bf16)


def _pack2(a, b):
    w = pltpu.pack_elementwise([a, b], packed_dtype=bf16)
    return w if w.dtype == u32 else pltpu.bitcast(w, u32)


def _pack_adj(x):
    r, c = x.shape
    e = x.reshape(r // 16, 16, c)
    return _pack2(e[:, 0:8, :].reshape(r // 2, c), e[:, 8:16, :].reshape(r // 2, c))


def _kernel(x_hbm, wqkv_hbm, wo_hbm, wr_hbm, wg_hbm, wu_hbm, wd_hbm, out_hbm,
            xin, x_s, xa, k_s, qt_s, vt_s, o_s,
            wk, wq, wv, wqu, wvu, wo, wou, wr, wg, wu, wd,
            r_s, a_s, outb, npad, zs, zv, sems, osems, *bufs):
    zs[0] = 0
    zs[1] = 0
    zv[...] = jnp.zeros((8, 128), u32)
    sb = bufs[0:NBUF]
    pb = bufs[NBUF:2 * NBUF]
    lb = bufs[2 * NBUF:3 * NBUF]

    def x_copy(t):
        r0, n = XCH[t]
        return pltpu.make_async_copy(x_hbm.at[pl.ds(r0, n), :], xin.at[pl.ds(r0, n), :], sems.at[t])

    def wk_copy(c):
        return pltpu.make_async_copy(wqkv_hbm.at[:, pl.ds(D + 256 * c, 256)], wk.at[:, pl.ds(256 * c, 256)],
                                     sems.at[12 + c])

    wq_copy = pltpu.make_async_copy(wqkv_hbm.at[:, pl.ds(0, D)], wq, sems.at[5])
    wv_copy = pltpu.make_async_copy(wqkv_hbm.at[:, pl.ds(2 * D, D)], wv, sems.at[6])
    wo_copy = pltpu.make_async_copy(wo_hbm, wo, sems.at[7])
    wr_copy = pltpu.make_async_copy(wr_hbm, wr, sems.at[8])
    wg_copy = pltpu.make_async_copy(wg_hbm, wg, sems.at[9])
    wu_copy = pltpu.make_async_copy(wu_hbm, wu, sems.at[10])
    wd_copy = pltpu.make_async_copy(wd_hbm, wd, sems.at[11])

    def out_copy(i):
        r0 = pl.multiple_of(i * 128, 128)
        return pltpu.make_async_copy(outb.at[pl.ds(r0, 128), :], out_hbm.at[pl.ds(r0, 128), :], osems.at[i])

    x_copy(0).start()
    wk_copy(0).start()

    ql1 = lax.broadcasted_iota(jnp.int32, (1, 128), 1) & 31
    for ii in range(3):
        for j in range(4):
            t = 256 - (128 * ii + 32 * j) if ii < 2 else 0
            n = max(0, min(256, t) - 32) + jnp.maximum(0, min(32, t) - 1 - ql1)
            npad[ii, j] = n.astype(f32)
    vt_s[0] = jnp.zeros((D // 2, 128), u32)
    vt_s[1] = jnp.zeros((D // 2, 128), u32)

    def kblock(b, g0=0, g1=NG, nb=1):
        static = isinstance(b, int)
        r = b * 64 if static else pl.multiple_of(b * 64, 64)
        xa_t = _u2b(xa[pl.ds(r, 64 * nb), :])
        kk = jnp.dot(xa_t, wk[:, 128 * g0:128 * g1], preferred_element_type=f32)
        kr = 128 + r if static else pl.multiple_of(128 + r, 64)
        toks = []
        for g in range(g0, g1):
            v = _b2u(kk[:, 128 * (g - g0):128 * (g - g0) + 128].astype(bf16))
            k_s[g, pl.ds(kr, 64 * nb), :] = v
            toks.append(v[0:8])
        return toks

    def fill_kpad():
        for g in range(NG):
            lo = k_s[g, 128:129, :] & jnp.uint32(0xFFFF)
            k_s[g, 0:128, :] = jnp.broadcast_to(lo | (lo << 16), (128, 128))

    def gate(v, tok):
        if tok is None:
            return v
        return v + pltpu.bitcast(tok & zv[...], f32)[0:1, 0:v.shape[1]]

    def ln0(b, toks=None):
        base = 128 * b if isinstance(b, int) else pl.multiple_of(128 * b, 128)
        nch = 1 if toks is None else 2
        n = 128 // nch
        for c in range(nch):
            r0 = base + n * c
            x = xin[pl.ds(r0, n), :].astype(f32)
            x_s[pl.ds(r0, n), :] = x
            mu = jnp.mean(x, axis=1, keepdims=True)
            if toks is not None:
                mu = gate(mu, toks[4 * c])
            xc = x - mu
            var = jnp.mean(xc * xc, axis=1, keepdims=True)
            h0 = r0 // 2 if isinstance(b, int) else pl.multiple_of(r0 // 2, n // 2)
            xa[pl.ds(h0, n // 2), :] = _b2u((xc * lax.rsqrt(var + EPS)).astype(bf16))

    def conv(dst, src):
        for j in range(NG):
            dst[64 * j:64 * j + 64, :] = _b2u(src[128 * j:128 * j + 128, :])

    x_copy(0).wait()
    wk_copy(1).start()
    ln0(0)
    ln0(1)
    wk_copy(0).wait()
    x_copy(1).start()
    kblock(0, 0, 2, 2)
    wk_copy(1).wait()
    wk_copy(2).start()
    kblock(0, 2, 4, 2)
    x_copy(1).wait()
    wk_copy(2).wait()
    wk_copy(3).start()
    x_copy(2).start()
    kblock(0, 4, 6, 2)
    ln0(2)
    ln0(3)
    wk_copy(3).wait()
    x_copy(3).start()
    kblock(0, 6, 8, 2)
    kblock(2)

    def pro_body(t, c):
        r0 = pl.multiple_of(512 * (t + 1), 512)
        pltpu.make_async_copy(x_hbm.at[pl.ds(r0, 512), :], xin.at[pl.ds(r0, 512), :], sems.at[t + 2]).wait()

        @pl.when(t == 0)
        def _():
            x_copy(4).start()

        @pl.when(t == 1)
        def _():
            wq_copy.start()
            wv_copy.start()

        @pl.when(t == 2)
        def _():
            wo_copy.start()
            wr_copy.start()

        for b in range(3):
            toks = kblock(4 * t + 3 + b)
            if b == 0:
                ln0(4 * t + 4)
            ln0(4 * t + 5 + b, toks)
        kblock(4 * t + 6)
        return c

    lax.fori_loop(0, 3, pro_body, 0)
    wq_copy.wait()
    wv_copy.wait()
    wo_copy.wait()
    wr_copy.wait()
    kblock(15)
    conv(wqu, wq)
    conv(wvu, wv)
    conv(wou, wo)
    fill_kpad()

    def q_slice(xa_blk, q_blk, n):
        lhs = _u2b(xa_blk[...])
        rhs = _u2b(wqu[:, 128 * n:128 * n + 128])
        q = jnp.dot(lhs, rhs, preferred_element_type=f32)
        qt = _b2u((q * QSCALE).astype(bf16).T)
        parts = [qt[0:16]] + [pltpu.roll(qt[16 * h:16 * h + 16], 32 * h, 1) for h in range(1, 4)]
        q_blk[64 * n:64 * n + 64, :] = jnp.concatenate(parts, axis=0)
        return parts[0][0:8]

    def v_slice(xa_blk, vt_blk, n):
        lhs = _u2b(xa_blk[...])
        rhs = _u2b(wvu[:, 128 * n:128 * n + 128])
        v = jnp.dot(lhs, rhs, preferred_element_type=f32)
        vt = _b2u(_u2b(_pack_adj(v)).T)
        vt_blk[64 * n:64 * n + 64, :] = vt
        return vt[0:8]

    def o_slice(o_blk, x_blk, n):
        lhs = _u2b(o_blk[...])
        rhs = _u2b(wou[:, 128 * n:128 * n + 128])
        acc = jnp.dot(lhs, rhs, preferred_element_type=f32)
        x_blk[:, 128 * n:128 * n + 128] = x_blk[:, 128 * n:128 * n + 128] + acc
        return pltpu.bitcast(acc[0:8], u32)

    def epilogue(j, x_blk, xa_blk, layer, chunks=range(NEC)):
        r0 = pl.multiple_of(j * 128, 128)
        R = 128 // NEC
        for c in chunks:
            lo = R * c
            x1 = x_blk[lo:lo + R, :]
            mu = jnp.mean(x1, axis=1, keepdims=True)
            xc = x1 - mu
            var = jnp.mean(xc * xc, axis=1, keepdims=True)
            a = lax.rsqrt(var + EPS)
            r = jnp.sum(xc * wr[...].astype(f32), axis=1, keepdims=True) * a
            r_s[pl.ds(r0 + lo, R), :] = r
            a_s[pl.ds(r0 + lo, R), :] = a
            a1 = 1.0 + a
            x2 = mu + xc * a1
            if layer == 0:
                x_blk[lo:lo + R, :] = x2
                v = xc * (a1 * lax.rsqrt(var * a1 * a1 + EPS))
                xa_blk[lo // 2:(lo + R) // 2, :] = _b2u(v.astype(bf16))
            else:
                outb[pl.ds(r0 + lo, R), :] = x2.astype(bf16)

    lane8b = lax.broadcasted_iota(jnp.int32, (8, 128), 1) >> 5
    odd = (lane8b & 1) == 1
    high = lane8b >= 2
    lane16b = lax.broadcasted_iota(jnp.int32, (16, 128), 1) >> 5
    d32 = lax.broadcasted_iota(jnp.int32, (32, 128), 0) - (lax.broadcasted_iota(jnp.int32, (32, 128), 1) & 31)
    umask = d32 > 0

    def stage_a(kv, q_blk, g):
        s_ref = sb[g % NBUF]
        for j in range(4):
            x = jnp.concatenate([jnp.where(lane16b == ((h + j) % 4), q_blk[64 * g + 16 * h:64 * g + 16 * h + 16, :],
                                           jnp.uint32(0)) for h in range(4)], axis=0)
            b0 = 16 * j
            kt = jnp.concatenate([kv[g, b0:b0 + 8, :], kv[g, b0 + 128:b0 + 136, :], kv[g, b0 + 8:b0 + 16, :],
                                  kv[g, b0 + 136:b0 + 144, :], kv[g, b0 + 16:b0 + 128, :]], axis=0)
            st = jnp.dot(_u2b(kt), _u2b(x), preferred_element_type=f32)
            su = jnp.concatenate([st[0:16], st[32:48]], axis=0)
            sl = jnp.concatenate([st[16:32], st[48:64]], axis=0)
            s_ref[j, 0:32, :] = jnp.where(umask, su, sl)
            s_ref[j, 32:256, :] = st[64:288]
            if j == 0:
                tok = (pltpu.bitcast(st[64:72], u32), pltpu.bitcast(st[160:168], u32),
                       pltpu.bitcast(st[280:288], u32))
        return tok

    def bfly(y):
        def sel(m, a, b):
            if a is None and b is None:
                return None
            z = jnp.zeros((8, 128), (a if a is not None else b).dtype)
            return jnp.where(m, z if a is None else a, z if b is None else b)
        r = [sel(odd, y[(k + 1) % 4], y[k]) for k in range(4)]
        wp = [sel(high, r[(k + 2) % 4], r[k]) for k in range(4)]
        return [wp[(-h) % 4] for h in range(4)]

    def stage_b(i, g, toks):
        s_ref = sb[g % NBUF]
        p_ref = pb[g % NBUF].at[zs[0]]
        l_ref = lb[g % NBUF]
        ss = [s_ref[j] for j in range(4)]
        ms = [jnp.max(ss[j], axis=0, keepdims=True) for j in range(4)]
        ls = [None] * 4
        nch = len(toks)
        um16 = [umask[0:16], umask[16:32]]
        for c in range(nch):
            mg = [gate(ms[j], toks[c]) for j in range(4)]
            for M in range(24 * c // nch, 24 * (c + 1) // nch):
                y = []
                for j in range(4):
                    Mp = M - 2 * j
                    if not 0 <= Mp < 18:
                        y.append(None)
                        continue
                    row = 16 * (Mp % 16)
                    p = jnp.exp2(ss[j][row:row + 16] - mg[j])
                    if Mp < 16:
                        ps = p[0:8] + p[8:16]
                        ls[j] = ps if ls[j] is None else ls[j] + ps
                        if Mp == 2:
                            p32 = p[0:1]
                            ls[j] = ls[j] - jnp.where(lax.broadcasted_iota(jnp.int32, (8, 128), 0) == 0,
                                                      npad[jnp.minimum(i, 2), j] * p32, 0.0)
                    if Mp < 2:
                        p = jnp.where(um16[Mp], p, 0.0)
                    elif Mp >= 16:
                        p = jnp.where(um16[Mp - 16], 0.0, p)
                    y.append(_pack2(p[0:8], p[8:16]))
                w = bfly(y)
                for h in range(4):
                    p_ref[h, 8 * M:8 * M + 8, :] = w[h] if w[h] is not None else jnp.zeros((8, 128), u32)
        for j in range(4):
            l_ref[j] = jnp.sum(ls[j], axis=0, keepdims=True)

    def stage_c(vts, o_blk, g):
        p_ref = pb[g % NBUF].at[zs[1]]
        l_ref = lb[g % NBUF]
        lh = bfly([jnp.broadcast_to(1.0 / l_ref[j], (8, 128)) for j in range(4)])
        outs = []
        for h in range(4):
            vt = jnp.concatenate([_u2b(vts[t][64 * g + 16 * h:64 * g + 16 * h + 16, :]) for t in range(3)], axis=1)
            o = jnp.dot(vt, _u2b(p_ref[h]), preferred_element_type=f32)
            o = o * lh[h][0:1]
            if h:
                o = pltpu.roll(o, 128 - 32 * h, 1)
            outs.append(o)
        ot = jnp.concatenate(outs, axis=0)
        o_blk[:, 128 * g:128 * g + 128] = _b2u(ot.T.astype(bf16))

    def attn_body(i, c, has_next, prev, layer, extra=()):
        lo = -1 if prev else 0
        r = pl.multiple_of((i + lo) * 64, 64)
        nblk = (2 if has_next else 1) - lo
        xav = xa.at[pl.ds(r, 64 * nblk), :]
        ov = o_s.at[pl.ds(r, 64 * (1 - lo)), :]
        xv = x_s.at[pl.ds(pl.multiple_of((i + lo) * 128, 128), 128), :]
        qv = qt_s.at[pl.ds(i, 2)]
        vv = vt_s.at[pl.ds(i + lo, 4 - lo)]
        kv = k_s.at[:, pl.ds(pl.multiple_of(i * 64, 64), 256), :]
        blk = lambda v, b: v.at[pl.ds(64 * (b - lo), 64), :]
        vtile = lambda b: vv.at[b - lo]

        qs = [functools.partial(q_slice, blk(xav, 1), qv.at[1], n) for n in range(NG)] if has_next else []
        vs = [functools.partial(v_slice, blk(xav, 1), vtile(3), n) for n in range(NG)] if has_next else []
        os_ = [functools.partial(o_slice, blk(ov, -1), xv, n) for n in range(NG)] if prev else []
        sl = qs[0:1] + os_ + qs[1:] + vs
        last_o = len(qs[0:1]) + len(os_) - 1 if os_ else -1
        if extra:
            n_it = 2 * NG
            groups = [extra[len(extra) * k // n_it:len(extra) * (k + 1) // n_it] for k in range(n_it)]

            def run(fs):
                for f in fs:
                    f()
            comp = [functools.partial(run, fs) for fs in groups]
            sl = comp[0:1] + sl + comp[1:]
            last_o = NG
        state = {"emitted": 0, "epi": 0}

        def next_epilogue_chunk():
            epilogue(i - 1, xv, blk(xav, -1), layer, [state["epi"]])
            state["epi"] += 1

        def dense_one():
            k = state["emitted"]
            if k < len(sl):
                sl[k]()
                state["emitted"] += 1
                if prev and k > last_o and state["epi"] < NEC:
                    next_epilogue_chunk()

        for g in range(NG):
            def pv():
                if g >= 1:
                    stage_c([vtile(t) for t in range(3)], blk(ov, 0), g - 1)
                elif prev:
                    stage_c([vtile(t - 1) for t in range(3)], blk(ov, -1), NG - 1)
            if g == 0:
                pv()
            tok = (None, None, None)
            if g + 1 < NG:
                tok = stage_a(kv.at[:, pl.ds(0, 192), :], qv.at[0], g + 1)
            elif has_next:
                tok = stage_a(kv.at[:, pl.ds(64, 192), :], qv.at[1], 0)
            stage_b(i, g, [None, None, tok[0], tok[2]])
            dense_one()
            dense_one()
            if g > 0:
                pv()
            dense_one()
        while state["emitted"] < len(sl):
            dense_one()
        if prev:
            while state["epi"] < NEC:
                next_epilogue_chunk()

        if layer == 1 and prev:
            out_copy(i - 1).start()
        if layer == 0 and prev and has_next:
            @pl.when(i == 1)
            def _():
                wg_copy.start()
                wu_copy.start()
                wd_copy.start()
        return c

    def finish_block(j, layer):
        o_blk = o_s.at[pl.ds(pl.multiple_of(j * 64, 64), 64), :]
        x_blk = x_s.at[pl.ds(pl.multiple_of(j * 128, 128), 128), :]
        stage_c([vt_s.at[j + t] for t in range(3)], o_blk, NG - 1)
        for n in range(NG):
            o_slice(o_blk, x_blk, n)
        epilogue(j, x_blk, xa.at[pl.ds(pl.multiple_of(j * 64, 64), 64), :], layer)

    def route(raw):
        r = r_s[0:S, :]
        rmax = jnp.max(r)
        rows = lax.broadcasted_iota(jnp.int32, (S, 1), 0)
        idx = jnp.min(jnp.where(r == rmax, rows, S))
        idx = jnp.minimum(idx, S - 1)
        xrow = x_s[pl.ds(idx, 1), :]
        arow = a_s[pl.ds(idx, 1), :]
        mu = jnp.mean(xrow, axis=1, keepdims=True)
        if raw:
            xsel = (xrow - mu) * arow
            xrow = xrow + xsel
        else:
            xsel = (xrow - mu) * (arow / (1.0 + arow))
        xs = jnp.broadcast_to(xsel, (8, D)).astype(bf16)
        return idx, rmax, xrow, xs

    def ffn_steps(xs):
        gates, hid, ys = [], [], []

        def up(c, w, first):
            r = jnp.dot(xs, w[:, 128 * c:128 * (c + 1)], preferred_element_type=f32)
            if first:
                gates.append(r)
            else:
                g_ = gates[c]
                hid.append((g_ * jax.nn.sigmoid(g_) * r).astype(bf16))

        def down(c):
            ys.append(jnp.dot(hid[c], wd[128 * c:128 * (c + 1), :], preferred_element_type=f32))

        steps = []
        for c in range(NFS):
            steps.append(functools.partial(up, c, wg, True))
            steps.append(functools.partial(up, c, wu, False))
            if c >= 1:
                steps.append(functools.partial(down, c - 1))
        steps.append(functools.partial(down, NFS - 1))

        def result():
            y = ys[0]
            for t in ys[1:]:
                y = y + t
            return y
        return steps, result

    def kslice(b, g):
        kblock(b, g, g + 1)

    def ffn_mid():
        kblock(K2_EARLY)
        idx, rmax, xrow, xs = route(raw=False)
        steps, result = ffn_steps(xs)
        fi = 0
        for b in range(K2_EARLY + 1, NB):
            for g in range(NG):
                kslice(b, g)
                if fi < len(steps):
                    steps[fi]()
                    fi += 1
        while fi < len(steps):
            steps[fi]()
            fi += 1
        y = result()
        x_s[pl.ds(idx, 1), :] = xrow + y[0:1, :] * jax.nn.sigmoid(rmax)
        r0 = pl.multiple_of((idx // 16) * 16, 16)
        h0 = pl.multiple_of((idx // 16) * 8, 8)
        x = x_s[pl.ds(r0, 16), :]
        mu = jnp.mean(x, axis=1, keepdims=True)
        xc = x - mu
        var = jnp.mean(xc * xc, axis=1, keepdims=True)
        xn = (xc * lax.rsqrt(var + EPS)).astype(bf16)
        xa[pl.ds(h0, 8), :] = _b2u(xn)
        kk = jnp.dot(xn, wk[...], preferred_element_type=f32)
        for g in range(NG):
            k_s[g, pl.ds(128 + h0, 8), :] = _b2u(kk[:, 128 * g:128 * g + 128].astype(bf16))
        fill_kpad()

    def ffn_last():
        idx, rmax, xrow, xs = route(raw=True)
        steps, result = ffn_steps(xs)
        for f in steps:
            f()
        y = result()
        new = xrow + y[0:1, :] * jax.nn.sigmoid(rmax)
        for i in range(NB):
            out_copy(i).wait()
        b0 = pl.multiple_of((idx // 16) * 16, 16)
        rows = lax.broadcasted_iota(jnp.int32, (16, D), 0) + b0
        outb[pl.ds(b0, 16), :] = jnp.where(rows == idx, new, outb[pl.ds(b0, 16), :].astype(f32)).astype(bf16)
        fix = pltpu.make_async_copy(outb.at[pl.ds(b0, 16), :], out_hbm.at[pl.ds(b0, 16), :], osems.at[NB])
        fix.start()
        fix.wait()

    for layer in range(2):
        for n in range(NG):
            q_slice(xa.at[pl.ds(0, 64), :], qt_s.at[0], n)
        for n in range(NG):
            v_slice(xa.at[pl.ds(0, 64), :], vt_s.at[2], n)
        stage_a(k_s.at[:, pl.ds(0, 192), :], qt_s.at[0], 0)
        attn_body(0, 0, has_next=True, prev=False, layer=layer)
        lax.fori_loop(1, NB - 1, functools.partial(attn_body, has_next=True, prev=True, layer=layer), 0)
        extra = [functools.partial(kslice, b, g) for b in range(K2_EARLY) for g in range(NG)] if layer == 0 else ()
        attn_body(NB - 1, 0, has_next=False, prev=True, layer=layer, extra=extra)
        finish_block(NB - 1, layer)
        if layer == 0:
            wg_copy.wait()
            wu_copy.wait()
            wd_copy.wait()
            ffn_mid()
        else:
            out_copy(NB - 1).start()
            ffn_last()


@jax.jit
def pallas_interleave_layers__sliding_block__moe_arch_mod__prompt_kernel(
    A_x: jax.Array,
    A_wqkv: jax.Array,
    A_wo: jax.Array,
    B_x: jax.Array,
    B_w_r: jax.Array,
    B_w_gate: jax.Array,
    B_w_up: jax.Array,
    B_w_down: jax.Array,
):
    del B_x
    x = A_x.reshape(S, D)
    wr = B_w_r.reshape(1, D)
    any_spec = pl.BlockSpec(memory_space=pl.ANY)
    scratch = [
        pltpu.VMEM((S, D), bf16),
        pltpu.VMEM((S, D), f32),
        pltpu.VMEM((S // 2, D), u32),
        pltpu.VMEM((NG, (S + 256) // 2 + 64, 128), u32),
        pltpu.VMEM((NB + 1, D // 2, 128), u32),
        pltpu.VMEM((NB + 3, D // 2, 128), u32),
        pltpu.VMEM((S // 2, D), u32),
        pltpu.VMEM((D, D), bf16),
        pltpu.VMEM((D, D), bf16),
        pltpu.VMEM((D, D), bf16),
        pltpu.VMEM((D // 2, D), u32),
        pltpu.VMEM((D // 2, D), u32),
        pltpu.VMEM((D, D), bf16),
        pltpu.VMEM((D // 2, D), u32),
        pltpu.VMEM((1, D), bf16),
        pltpu.VMEM((D, F), bf16),
        pltpu.VMEM((D, F), bf16),
        pltpu.VMEM((F, D), bf16),
        pltpu.VMEM((S, 1), f32),
        pltpu.VMEM((S, 1), f32),
        pltpu.VMEM((S, D), bf16),
        pltpu.VMEM((3, 4, 1, 128), f32),
        pltpu.SMEM((2,), jnp.int32),
        pltpu.VMEM((8, 128), u32),
        pltpu.SemaphoreType.DMA((16,)),
        pltpu.SemaphoreType.DMA((NB + 1,)),
    ]
    scratch += [pltpu.VMEM((4, 256, 128), f32)] * NBUF
    scratch += [pltpu.VMEM((1, 4, 192, 128), u32)] * NBUF
    scratch += [pltpu.VMEM((4, 1, 128), f32)] * NBUF
    out = pl.pallas_call(
        _kernel,
        out_shape=jax.ShapeDtypeStruct((S, D), bf16),
        in_specs=[any_spec] * 7,
        out_specs=any_spec,
        scratch_shapes=scratch,
        compiler_params=pltpu.CompilerParams(vmem_limit_bytes=110 * 1024 * 1024),
    )(x, A_wqkv, A_wo, wr, B_w_gate, B_w_up, B_w_down)
    return out.reshape(1, S, D)
```

```python
import functools
import math

import jax
import jax.numpy as jnp
from jax import lax
import jax.experimental.pallas as pl
import jax.experimental.pallas.tpu as pltpu

S, D, H, DH, F = 2048, 1024, 32, 32, 3584
NB = S // 128
NG = D // 128
NFS = F // 128
EPS = 1e-5
QSCALE = (DH ** -0.5) * math.log2(math.e)
NEC = 2
NBUF = 2
K2_EARLY = 2
XCH = [(0, 256), (256, 256), (512, 512), (1024, 512), (1536, 512)]

bf16 = jnp.bfloat16
f32 = jnp.float32
u32 = jnp.uint32


def _b2u(x):
    return pltpu.bitcast(x, u32)


def _u2b(x):
    return pltpu.bitcast(x, bf16)


def _pack2(a, b):
    w = pltpu.pack_elementwise([a, b], packed_dtype=bf16)
    return w if w.dtype == u32 else pltpu.bitcast(w, u32)


def _pack_adj(x):
    r, c = x.shape
    e = x.reshape(r // 16, 16, c)
    return _pack2(e[:, 0:8, :].reshape(r // 2, c), e[:, 8:16, :].reshape(r // 2, c))


def _kernel(x_hbm, wqkv_hbm, wo_hbm, wr_hbm, wg_hbm, wu_hbm, wd_hbm, out_hbm,
            xin, x_s, xa, k_s, qt_s, vt_s, o_s,
            wk, wq, wv, wqu, wvu, wo, wou, wr, wg, wu, wd,
            r_s, a_s, outb, npad, zs, zv, sems, osems, *bufs):
    zs[0] = 0
    zs[1] = 0
    zv[...] = jnp.zeros((8, 128), u32)
    sb = bufs[0:NBUF]
    pb = bufs[NBUF:2 * NBUF]
    lb = bufs[2 * NBUF:3 * NBUF]

    def x_copy(t):
        r0, n = XCH[t]
        return pltpu.make_async_copy(x_hbm.at[pl.ds(r0, n), :], xin.at[pl.ds(r0, n), :], sems.at[t])

    def wk_copy(c):
        return pltpu.make_async_copy(wqkv_hbm.at[:, pl.ds(D + 256 * c, 256)], wk.at[:, pl.ds(256 * c, 256)],
                                     sems.at[12 + c])

    wq_copy = pltpu.make_async_copy(wqkv_hbm.at[:, pl.ds(0, D)], wq, sems.at[5])
    wv_copy = pltpu.make_async_copy(wqkv_hbm.at[:, pl.ds(2 * D, D)], wv, sems.at[6])
    wo_copy = pltpu.make_async_copy(wo_hbm, wo, sems.at[7])
    wr_copy = pltpu.make_async_copy(wr_hbm, wr, sems.at[8])
    wg_copy = pltpu.make_async_copy(wg_hbm, wg, sems.at[9])
    wu_copy = pltpu.make_async_copy(wu_hbm, wu, sems.at[10])
    wd_copy = pltpu.make_async_copy(wd_hbm, wd, sems.at[11])

    def out_copy(i):
        r0 = pl.multiple_of(i * 128, 128)
        return pltpu.make_async_copy(outb.at[pl.ds(r0, 128), :], out_hbm.at[pl.ds(r0, 128), :], osems.at[i])

    x_copy(0).start()
    wk_copy(0).start()

    ql1 = lax.broadcasted_iota(jnp.int32, (1, 128), 1) & 31
    for ii in range(3):
        for j in range(4):
            t = 256 - (128 * ii + 32 * j) if ii < 2 else 0
            n = max(0, min(256, t) - 32) + jnp.maximum(0, min(32, t) - 1 - ql1)
            npad[ii, j] = n.astype(f32)
    vt_s[0] = jnp.zeros((D // 2, 128), u32)
    vt_s[1] = jnp.zeros((D // 2, 128), u32)

    def kblock(b, g0=0, g1=NG, nb=1):
        static = isinstance(b, int)
        r = b * 64 if static else pl.multiple_of(b * 64, 64)
        xa_t = _u2b(xa[pl.ds(r, 64 * nb), :])
        kk = jnp.dot(xa_t, wk[:, 128 * g0:128 * g1], preferred_element_type=f32)
        kr = 128 + r if static else pl.multiple_of(128 + r, 64)
        toks = []
        for g in range(g0, g1):
            v = _b2u(kk[:, 128 * (g - g0):128 * (g - g0) + 128].astype(bf16))
            k_s[g, pl.ds(kr, 64 * nb), :] = v
            toks.append(v[0:8])
        return toks

    def fill_kpad():
        for g in range(NG):
            lo = k_s[g, 128:129, :] & jnp.uint32(0xFFFF)
            k_s[g, 0:128, :] = jnp.broadcast_to(lo | (lo << 16), (128, 128))

    def gate(v, tok):
        if tok is None:
            return v
        return v + pltpu.bitcast(tok & zv[...], f32)[0:1, 0:v.shape[1]]

    def ln0(b, toks=None):
        base = 128 * b if isinstance(b, int) else pl.multiple_of(128 * b, 128)
        nch = 1 if toks is None else 2
        n = 128 // nch
        for c in range(nch):
            r0 = base + n * c
            x = xin[pl.ds(r0, n), :].astype(f32)
            x_s[pl.ds(r0, n), :] = x
            mu = jnp.mean(x, axis=1, keepdims=True)
            if toks is not None:
                mu = gate(mu, toks[4 * c])
            xc = x - mu
            var = jnp.mean(xc * xc, axis=1, keepdims=True)
            h0 = r0 // 2 if isinstance(b, int) else pl.multiple_of(r0 // 2, n // 2)
            xa[pl.ds(h0, n // 2), :] = _b2u((xc * lax.rsqrt(var + EPS)).astype(bf16))

    def conv(dst, src):
        for j in range(NG):
            dst[64 * j:64 * j + 64, :] = _b2u(src[128 * j:128 * j + 128, :])

    x_copy(0).wait()
    wk_copy(1).start()
    ln0(0)
    ln0(1)
    wk_copy(0).wait()
    x_copy(1).start()
    kblock(0, 0, 2, 2)
    wk_copy(1).wait()
    wk_copy(2).start()
    kblock(0, 2, 4, 2)
    x_copy(1).wait()
    wk_copy(2).wait()
    wk_copy(3).start()
    x_copy(2).start()
    kblock(0, 4, 6, 2)
    ln0(2)
    ln0(3)
    wk_copy(3).wait()
    x_copy(3).start()
    kblock(0, 6, 8, 2)
    kblock(2)

    def pro_body(t, c):
        r0 = pl.multiple_of(512 * (t + 1), 512)
        pltpu.make_async_copy(x_hbm.at[pl.ds(r0, 512), :], xin.at[pl.ds(r0, 512), :], sems.at[t + 2]).wait()

        for b in range(3):
            toks = kblock(4 * t + 3 + b)
            if b == 0:
                ln0(4 * t + 4)
            ln0(4 * t + 5 + b, toks)
        kblock(4 * t + 6)
        return c

    x_copy(4).start()
    wq_copy.start()
    wv_copy.start()
    wo_copy.start()
    wr_copy.start()
    lax.fori_loop(0, 3, pro_body, 0)
    wq_copy.wait()
    wv_copy.wait()
    wo_copy.wait()
    wr_copy.wait()
    kblock(15)
    conv(wqu, wq)
    conv(wvu, wv)
    conv(wou, wo)
    fill_kpad()

    def q_slice(xa_blk, q_blk, n):
        lhs = _u2b(xa_blk[...])
        rhs = _u2b(wqu[:, 128 * n:128 * n + 128])
        q = jnp.dot(lhs, rhs, preferred_element_type=f32)
        qt = _b2u((q * QSCALE).astype(bf16).T)
        parts = [qt[0:16]] + [pltpu.roll(qt[16 * h:16 * h + 16], 32 * h, 1) for h in range(1, 4)]
        q_blk[64 * n:64 * n + 64, :] = jnp.concatenate(parts, axis=0)
        return parts[0][0:8]

    def v_slice(xa_blk, vt_blk, n):
        lhs = _u2b(xa_blk[...])
        rhs = _u2b(wvu[:, 128 * n:128 * n + 128])
        v = jnp.dot(lhs, rhs, preferred_element_type=f32)
        vt = _b2u(_u2b(_pack_adj(v)).T)
        vt_blk[64 * n:64 * n + 64, :] = vt
        return vt[0:8]

    def o_slice(o_blk, x_blk, n):
        lhs = _u2b(o_blk[...])
        rhs = _u2b(wou[:, 128 * n:128 * n + 128])
        acc = jnp.dot(lhs, rhs, preferred_element_type=f32)
        x_blk[:, 128 * n:128 * n + 128] = x_blk[:, 128 * n:128 * n + 128] + acc
        return pltpu.bitcast(acc[0:8], u32)

    def epi_stats(j, x_blk, c, tok=None):
        r0 = pl.multiple_of(j * 128, 128)
        R = 128 // NEC
        lo = R * c
        x1 = x_blk[lo:lo + R, :]
        mu = gate(jnp.mean(x1, axis=1, keepdims=True), tok)
        xc = x1 - mu
        var = jnp.mean(xc * xc, axis=1, keepdims=True)
        a = lax.rsqrt(var + EPS)
        r = jnp.sum(xc * wr[...].astype(f32), axis=1, keepdims=True) * a
        r_s[pl.ds(r0 + lo, R), :] = r
        a_s[pl.ds(r0 + lo, R), :] = a
        return mu, xc, var, a

    def epi_norm(j, x_blk, xa_blk, layer, c, st, tok=None):
        r0 = pl.multiple_of(j * 128, 128)
        R = 128 // NEC
        lo = R * c
        mu, xc, var, a = st
        a1 = gate(1.0 + a, tok)
        x2 = mu + xc * a1
        if layer == 0:
            x_blk[lo:lo + R, :] = x2
            v = xc * (a1 * lax.rsqrt(var * a1 * a1 + EPS))
            xa_blk[lo // 2:(lo + R) // 2, :] = _b2u(v.astype(bf16))
        else:
            outb[pl.ds(r0 + lo, R), :] = x2.astype(bf16)

    def epilogue(j, x_blk, xa_blk, layer, chunks=range(NEC)):
        for c in chunks:
            epi_norm(j, x_blk, xa_blk, layer, c, epi_stats(j, x_blk, c))

    lane8b = lax.broadcasted_iota(jnp.int32, (8, 128), 1) >> 5
    odd = (lane8b & 1) == 1
    high = lane8b >= 2
    lane16b = lax.broadcasted_iota(jnp.int32, (16, 128), 1) >> 5
    d32 = lax.broadcasted_iota(jnp.int32, (32, 128), 0) - (lax.broadcasted_iota(jnp.int32, (32, 128), 1) & 31)
    umask = d32 > 0

    def stage_a(kv, q_blk, g):
        s_ref = sb[g % NBUF]
        for j in range(4):
            x = jnp.concatenate([jnp.where(lane16b == ((h + j) % 4), q_blk[64 * g + 16 * h:64 * g + 16 * h + 16, :],
                                           jnp.uint32(0)) for h in range(4)], axis=0)
            b0 = 16 * j
            kt = jnp.concatenate([kv[g, b0:b0 + 8, :], kv[g, b0 + 128:b0 + 136, :], kv[g, b0 + 8:b0 + 16, :],
                                  kv[g, b0 + 136:b0 + 144, :], kv[g, b0 + 16:b0 + 128, :]], axis=0)
            st = jnp.dot(_u2b(kt), _u2b(x), preferred_element_type=f32)
            su = jnp.concatenate([st[0:16], st[32:48]], axis=0)
            sl = jnp.concatenate([st[16:32], st[48:64]], axis=0)
            s_ref[j, 0:32, :] = jnp.where(umask, su, sl)
            s_ref[j, 32:256, :] = st[64:288]
            if j == 0:
                tok = (pltpu.bitcast(st[64:72], u32), pltpu.bitcast(st[160:168], u32),
                       pltpu.bitcast(st[280:288], u32))
        return tok

    def bfly(y):
        def sel(m, a, b):
            if a is None and b is None:
                return None
            z = jnp.zeros((8, 128), (a if a is not None else b).dtype)
            return jnp.where(m, z if a is None else a, z if b is None else b)
        r = [sel(odd, y[(k + 1) % 4], y[k]) for k in range(4)]
        wp = [sel(high, r[(k + 2) % 4], r[k]) for k in range(4)]
        return [wp[(-h) % 4] for h in range(4)]

    def stage_b(i, g, toks):
        s_ref = sb[g % NBUF]
        p_ref = pb[g % NBUF].at[zs[0]]
        l_ref = lb[g % NBUF]
        ss = [s_ref[j] for j in range(4)]
        ms = [jnp.max(ss[j], axis=0, keepdims=True) for j in range(4)]
        ls = [None] * 4
        nch = len(toks)
        um16 = [umask[0:16], umask[16:32]]
        for c in range(nch):
            mg = [gate(ms[j], toks[c]) for j in range(4)]
            for M in range(24 * c // nch, 24 * (c + 1) // nch):
                y = []
                for j in range(4):
                    Mp = M - 2 * j
                    if not 0 <= Mp < 18:
                        y.append(None)
                        continue
                    row = 16 * (Mp % 16)
                    p = jnp.exp2(ss[j][row:row + 16] - mg[j])
                    if Mp < 16:
                        ps = p[0:8] + p[8:16]
                        ls[j] = ps if ls[j] is None else ls[j] + ps
                        if Mp == 2:
                            p32 = p[0:1]
                            ls[j] = ls[j] - jnp.where(lax.broadcasted_iota(jnp.int32, (8, 128), 0) == 0,
                                                      npad[jnp.minimum(i, 2), j] * p32, 0.0)
                    if Mp < 2:
                        p = jnp.where(um16[Mp], p, 0.0)
                    elif Mp >= 16:
                        p = jnp.where(um16[Mp - 16], 0.0, p)
                    y.append(_pack2(p[0:8], p[8:16]))
                w = bfly(y)
                for h in range(4):
                    p_ref[h, 8 * M:8 * M + 8, :] = w[h] if w[h] is not None else jnp.zeros((8, 128), u32)
        for j in range(4):
            l_ref[j] = jnp.sum(ls[j], axis=0, keepdims=True)

    def stage_c(vts, o_blk, g):
        p_ref = pb[g % NBUF].at[zs[1]]
        l_ref = lb[g % NBUF]
        lh = bfly([jnp.broadcast_to(1.0 / l_ref[j], (8, 128)) for j in range(4)])
        outs = []
        for h in range(4):
            vt = jnp.concatenate([_u2b(vts[t][64 * g + 16 * h:64 * g + 16 * h + 16, :]) for t in range(3)], axis=1)
            o = jnp.dot(vt, _u2b(p_ref[h]), preferred_element_type=f32)
            o = o * lh[h][0:1]
            if h:
                o = pltpu.roll(o, 128 - 32 * h, 1)
            outs.append(o)
        ot = jnp.concatenate(outs, axis=0)
        o_blk[:, 128 * g:128 * g + 128] = _b2u(ot.T.astype(bf16))

    def attn_body(i, c, has_next, prev, layer, extra=()):
        lo = -1 if prev else 0
        r = pl.multiple_of((i + lo) * 64, 64)
        nblk = (2 if has_next else 1) - lo
        xav = xa.at[pl.ds(r, 64 * nblk), :]
        ov = o_s.at[pl.ds(r, 64 * (1 - lo)), :]
        xv = x_s.at[pl.ds(pl.multiple_of((i + lo) * 128, 128), 128), :]
        qv = qt_s.at[pl.ds(i, 2)]
        vv = vt_s.at[pl.ds(i + lo, 4 - lo)]
        kv = k_s.at[:, pl.ds(pl.multiple_of(i * 64, 64), 256), :]
        blk = lambda v, b: v.at[pl.ds(64 * (b - lo), 64), :]
        vtile = lambda b: vv.at[b - lo]

        qs = [functools.partial(q_slice, blk(xav, 1), qv.at[1], n) for n in range(NG)] if has_next else []
        vs = [functools.partial(v_slice, blk(xav, 1), vtile(3), n) for n in range(NG)] if has_next else []
        os_ = [functools.partial(o_slice, blk(ov, -1), xv, n) for n in range(NG)] if prev else []
        sl = qs[0:1] + os_ + qs[1:] + vs
        last_o = len(qs[0:1]) + len(os_) - 1 if os_ else -1
        if extra:
            n_it = 2 * NG
            groups = [extra[len(extra) * k // n_it:len(extra) * (k + 1) // n_it] for k in range(n_it)]

            def run(fs):
                for f in fs:
                    f()
            comp = [functools.partial(run, fs) for fs in groups]
            sl = comp[0:1] + sl + comp[1:]
            last_o = NG
        state = {"emitted": 0}
        stats = {}
        if layer == 0:
            esch = [(1, "s", 0, False), (1, "s", 1, False), (4, "n", 0, True), (6, "n", 1, True)]
        else:
            esch = [(1, "s", 0, False), (1, "n", 0, False), (2, "s", 1, False), (2, "n", 1, False)]

        def run_epi(k, tok):
            for (off, kind, ch, paced) in esch:
                if (k is None or off == k) and (kind, ch) not in stats:
                    if kind == "s":
                        stats[kind, ch] = epi_stats(i - 1, xv, ch, tok if paced else None)
                    else:
                        epi_norm(i - 1, xv, blk(xav, -1), layer, ch, stats["s", ch], tok if paced else None)
                        stats[kind, ch] = True

        def dense_one():
            k = state["emitted"]
            if k < len(sl):
                t = sl[k]()
                state["emitted"] += 1
                if prev and k > last_o:
                    run_epi(k - last_o, t)

        for g in range(NG):
            def pv():
                if g >= 1:
                    stage_c([vtile(t) for t in range(3)], blk(ov, 0), g - 1)
                elif prev:
                    stage_c([vtile(t - 1) for t in range(3)], blk(ov, -1), NG - 1)
            if g == 0:
                pv()
            tok = (None, None, None)
            if g + 1 < NG:
                tok = stage_a(kv.at[:, pl.ds(0, 192), :], qv.at[0], g + 1)
            elif has_next:
                tok = stage_a(kv.at[:, pl.ds(64, 192), :], qv.at[1], 0)
            stage_b(i, g, [None, None, tok[0], tok[2]])
            dense_one()
            dense_one()
            if g > 0:
                pv()
            dense_one()
        while state["emitted"] < len(sl):
            dense_one()
        if prev:
            run_epi(None, None)

        if layer == 1 and prev:
            out_copy(i - 1).start()
        if layer == 0 and prev and has_next:
            @pl.when(i == 1)
            def _():
                wg_copy.start()
                wu_copy.start()
                wd_copy.start()
        return c

    def finish_block(j, layer):
        o_blk = o_s.at[pl.ds(pl.multiple_of(j * 64, 64), 64), :]
        x_blk = x_s.at[pl.ds(pl.multiple_of(j * 128, 128), 128), :]
        stage_c([vt_s.at[j + t] for t in range(3)], o_blk, NG - 1)
        for n in range(NG):
            o_slice(o_blk, x_blk, n)
        epilogue(j, x_blk, xa.at[pl.ds(pl.multiple_of(j * 64, 64), 64), :], layer)

    def route(raw):
        r = r_s[0:S, :]
        rmax = jnp.max(r)
        rows = lax.broadcasted_iota(jnp.int32, (S, 1), 0)
        idx = jnp.min(jnp.where(r == rmax, rows, S))
        idx = jnp.minimum(idx, S - 1)
        xrow = x_s[pl.ds(idx, 1), :]
        arow = a_s[pl.ds(idx, 1), :]
        mu = jnp.mean(xrow, axis=1, keepdims=True)
        if raw:
            xsel = (xrow - mu) * arow
            xrow = xrow + xsel
        else:
            xsel = (xrow - mu) * (arow / (1.0 + arow))
        xs = jnp.broadcast_to(xsel, (8, D)).astype(bf16)
        return idx, rmax, xrow, xs

    def ffn_steps(xs):
        gates, hid, ys = [], [], []

        def up(c, w, first):
            r = jnp.dot(xs, w[:, 128 * c:128 * (c + 1)], preferred_element_type=f32)
            if first:
                gates.append(r)
            else:
                g_ = gates[c]
                hid.append((g_ * jax.nn.sigmoid(g_) * r).astype(bf16))

        def down(c):
            ys.append(jnp.dot(hid[c], wd[128 * c:128 * (c + 1), :], preferred_element_type=f32))

        steps = []
        for c in range(NFS):
            steps.append(functools.partial(up, c, wg, True))
            steps.append(functools.partial(up, c, wu, False))
            if c >= 1:
                steps.append(functools.partial(down, c - 1))
        steps.append(functools.partial(down, NFS - 1))

        def result():
            y = ys[0]
            for t in ys[1:]:
                y = y + t
            return y
        return steps, result

    def kslice(b, g):
        kblock(b, g, g + 1)

    def ffn_mid():
        kblock(K2_EARLY)
        idx, rmax, xrow, xs = route(raw=False)
        steps, result = ffn_steps(xs)
        fi = 0
        for b in range(K2_EARLY + 1, NB):
            for g in range(NG):
                kslice(b, g)
                if fi < len(steps):
                    steps[fi]()
                    fi += 1
        while fi < len(steps):
            steps[fi]()
            fi += 1
        y = result()
        x_s[pl.ds(idx, 1), :] = xrow + y[0:1, :] * jax.nn.sigmoid(rmax)
        r0 = pl.multiple_of((idx // 16) * 16, 16)
        h0 = pl.multiple_of((idx // 16) * 8, 8)
        x = x_s[pl.ds(r0, 16), :]
        mu = jnp.mean(x, axis=1, keepdims=True)
        xc = x - mu
        var = jnp.mean(xc * xc, axis=1, keepdims=True)
        xn = (xc * lax.rsqrt(var + EPS)).astype(bf16)
        xa[pl.ds(h0, 8), :] = _b2u(xn)
        kk = jnp.dot(xn, wk[...], preferred_element_type=f32)
        for g in range(NG):
            k_s[g, pl.ds(128 + h0, 8), :] = _b2u(kk[:, 128 * g:128 * g + 128].astype(bf16))
        fill_kpad()

    def ffn_last():
        idx, rmax, xrow, xs = route(raw=True)
        steps, result = ffn_steps(xs)
        for f in steps:
            f()
        y = result()
        new = xrow + y[0:1, :] * jax.nn.sigmoid(rmax)
        for i in range(NB):
            out_copy(i).wait()
        b0 = pl.multiple_of((idx // 16) * 16, 16)
        rows = lax.broadcasted_iota(jnp.int32, (16, D), 0) + b0
        outb[pl.ds(b0, 16), :] = jnp.where(rows == idx, new, outb[pl.ds(b0, 16), :].astype(f32)).astype(bf16)
        fix = pltpu.make_async_copy(outb.at[pl.ds(b0, 16), :], out_hbm.at[pl.ds(b0, 16), :], osems.at[NB])
        fix.start()
        fix.wait()

    for layer in range(2):
        for n in range(NG):
            q_slice(xa.at[pl.ds(0, 64), :], qt_s.at[0], n)
        for n in range(NG):
            v_slice(xa.at[pl.ds(0, 64), :], vt_s.at[2], n)
        stage_a(k_s.at[:, pl.ds(0, 192), :], qt_s.at[0], 0)
        attn_body(0, 0, has_next=True, prev=False, layer=layer)
        lax.fori_loop(1, NB - 1, functools.partial(attn_body, has_next=True, prev=True, layer=layer), 0)
        extra = [functools.partial(kslice, b, g) for b in range(K2_EARLY) for g in range(NG)] if layer == 0 else ()
        attn_body(NB - 1, 0, has_next=False, prev=True, layer=layer, extra=extra)
        finish_block(NB - 1, layer)
        if layer == 0:
            wg_copy.wait()
            wu_copy.wait()
            wd_copy.wait()
            ffn_mid()
        else:
            out_copy(NB - 1).start()
            ffn_last()


@jax.jit
def pallas_interleave_layers__sliding_block__moe_arch_mod__prompt_kernel(
    A_x: jax.Array,
    A_wqkv: jax.Array,
    A_wo: jax.Array,
    B_x: jax.Array,
    B_w_r: jax.Array,
    B_w_gate: jax.Array,
    B_w_up: jax.Array,
    B_w_down: jax.Array,
):
    del B_x
    x = A_x.reshape(S, D)
    wr = B_w_r.reshape(1, D)
    any_spec = pl.BlockSpec(memory_space=pl.ANY)
    scratch = [
        pltpu.VMEM((S, D), bf16),
        pltpu.VMEM((S, D), f32),
        pltpu.VMEM((S // 2, D), u32),
        pltpu.VMEM((NG, (S + 256) // 2 + 64, 128), u32),
        pltpu.VMEM((NB + 1, D // 2, 128), u32),
        pltpu.VMEM((NB + 3, D // 2, 128), u32),
        pltpu.VMEM((S // 2, D), u32),
        pltpu.VMEM((D, D), bf16),
        pltpu.VMEM((D, D), bf16),
        pltpu.VMEM((D, D), bf16),
        pltpu.VMEM((D // 2, D), u32),
        pltpu.VMEM((D // 2, D), u32),
        pltpu.VMEM((D, D), bf16),
        pltpu.VMEM((D // 2, D), u32),
        pltpu.VMEM((1, D), bf16),
        pltpu.VMEM((D, F), bf16),
        pltpu.VMEM((D, F), bf16),
        pltpu.VMEM((F, D), bf16),
        pltpu.VMEM((S, 1), f32),
        pltpu.VMEM((S, 1), f32),
        pltpu.VMEM((S, D), bf16),
        pltpu.VMEM((3, 4, 1, 128), f32),
        pltpu.SMEM((2,), jnp.int32),
        pltpu.VMEM((8, 128), u32),
        pltpu.SemaphoreType.DMA((16,)),
        pltpu.SemaphoreType.DMA((NB + 1,)),
    ]
    scratch += [pltpu.VMEM((4, 256, 128), f32)] * NBUF
    scratch += [pltpu.VMEM((1, 4, 192, 128), u32)] * NBUF
    scratch += [pltpu.VMEM((4, 1, 128), f32)] * NBUF
    out = pl.pallas_call(
        _kernel,
        out_shape=jax.ShapeDtypeStruct((S, D), bf16),
        in_specs=[any_spec] * 7,
        out_specs=any_spec,
        scratch_shapes=scratch,
        compiler_params=pltpu.CompilerParams(vmem_limit_bytes=110 * 1024 * 1024),
    )(x, A_wqkv, A_wo, wr, B_w_gate, B_w_up, B_w_down)
    return out.reshape(1, S, D)
```

```python
import functools
import math

import jax
import jax.numpy as jnp
from jax import lax
import jax.experimental.pallas as pl
import jax.experimental.pallas.tpu as pltpu

S, D, H, DH, F = 2048, 1024, 32, 32, 3584
NB = S // 128
NG = D // 128
NFS = F // 128
EPS = 1e-5
QSCALE = (DH ** -0.5) * math.log2(math.e)
NEC = 2
NBUF = 2
K2_EARLY = 2
XCH = [(0, 256), (256, 256), (512, 512), (1024, 512), (1536, 512)]

bf16 = jnp.bfloat16
f32 = jnp.float32
u32 = jnp.uint32


def _b2u(x):
    return pltpu.bitcast(x, u32)


def _u2b(x):
    return pltpu.bitcast(x, bf16)


def _pack2(a, b):
    w = pltpu.pack_elementwise([a, b], packed_dtype=bf16)
    return w if w.dtype == u32 else pltpu.bitcast(w, u32)


def _pack_adj(x):
    r, c = x.shape
    e = x.reshape(r // 16, 16, c)
    return _pack2(e[:, 0:8, :].reshape(r // 2, c), e[:, 8:16, :].reshape(r // 2, c))


def _kernel(x_hbm, wqkv_hbm, wo_hbm, wr_hbm, wg_hbm, wu_hbm, wd_hbm, out_hbm,
            xin, x_s, xa, k_s, qt_s, vt_s, o_s,
            wk, wq, wv, wqu, wvu, wo, wou, wr, wg, wu, wd,
            r_s, a_s, outb, npad, zs, zv, vraw, sems, osems, *bufs):
    zs[0] = 0
    zs[1] = 0
    zv[...] = jnp.zeros((8, 128), u32)
    sb = bufs[0:NBUF]
    pb = bufs[NBUF:2 * NBUF]
    lb = bufs[2 * NBUF:3 * NBUF]

    def x_copy(t):
        r0, n = XCH[t]
        return pltpu.make_async_copy(x_hbm.at[pl.ds(r0, n), :], xin.at[pl.ds(r0, n), :], sems.at[t])

    def wk_copy(c):
        return pltpu.make_async_copy(wqkv_hbm.at[:, pl.ds(D + 256 * c, 256)], wk.at[:, pl.ds(256 * c, 256)],
                                     sems.at[12 + c])

    wq_copy = pltpu.make_async_copy(wqkv_hbm.at[:, pl.ds(0, D)], wq, sems.at[5])
    wv_copy = pltpu.make_async_copy(wqkv_hbm.at[:, pl.ds(2 * D, D)], wv, sems.at[6])
    wo_copy = pltpu.make_async_copy(wo_hbm, wo, sems.at[7])
    wr_copy = pltpu.make_async_copy(wr_hbm, wr, sems.at[8])
    wg_copy = pltpu.make_async_copy(wg_hbm, wg, sems.at[9])
    wu_copy = pltpu.make_async_copy(wu_hbm, wu, sems.at[10])
    wd_copy = pltpu.make_async_copy(wd_hbm, wd, sems.at[11])

    def out_copy(i):
        r0 = pl.multiple_of(i * 128, 128)
        return pltpu.make_async_copy(outb.at[pl.ds(r0, 128), :], out_hbm.at[pl.ds(r0, 128), :], osems.at[i])

    x_copy(0).start()
    wk_copy(0).start()

    ql1 = lax.broadcasted_iota(jnp.int32, (1, 128), 1) & 31
    for ii in range(3):
        for j in range(4):
            t = 256 - (128 * ii + 32 * j) if ii < 2 else 0
            n = max(0, min(256, t) - 32) + jnp.maximum(0, min(32, t) - 1 - ql1)
            npad[ii, j] = n.astype(f32)
    vt_s[0] = jnp.zeros((D // 2, 128), u32)
    vt_s[1] = jnp.zeros((D // 2, 128), u32)

    def kblock(b, g0=0, g1=NG, nb=1):
        static = isinstance(b, int)
        r = b * 64 if static else pl.multiple_of(b * 64, 64)
        xa_t = _u2b(xa[pl.ds(r, 64 * nb), :])
        kk = jnp.dot(xa_t, wk[:, 128 * g0:128 * g1], preferred_element_type=f32)
        kr = 128 + r if static else pl.multiple_of(128 + r, 64)
        toks = []
        for g in range(g0, g1):
            v = _b2u(kk[:, 128 * (g - g0):128 * (g - g0) + 128].astype(bf16))
            k_s[g, pl.ds(kr, 64 * nb), :] = v
            toks.append(v[0:8])
        return toks

    def fill_kpad():
        for g in range(NG):
            lo = k_s[g, 128:129, :] & jnp.uint32(0xFFFF)
            k_s[g, 0:128, :] = jnp.broadcast_to(lo | (lo << 16), (128, 128))

    def gate(v, tok):
        if tok is None:
            return v
        return v + pltpu.bitcast(tok & zv[...], f32)[0:1, 0:v.shape[1]]

    def ln0(b, toks=None):
        base = 128 * b if isinstance(b, int) else pl.multiple_of(128 * b, 128)
        nch = 1 if toks is None else 2
        n = 128 // nch
        for c in range(nch):
            r0 = base + n * c
            x = xin[pl.ds(r0, n), :].astype(f32)
            x_s[pl.ds(r0, n), :] = x
            mu = jnp.mean(x, axis=1, keepdims=True)
            if toks is not None:
                mu = gate(mu, toks[4 * c])
            xc = x - mu
            var = jnp.mean(xc * xc, axis=1, keepdims=True)
            h0 = r0 // 2 if isinstance(b, int) else pl.multiple_of(r0 // 2, n // 2)
            xa[pl.ds(h0, n // 2), :] = _b2u((xc * lax.rsqrt(var + EPS)).astype(bf16))

    def conv(dst, src):
        for j in range(NG):
            dst[64 * j:64 * j + 64, :] = _b2u(src[128 * j:128 * j + 128, :])

    x_copy(0).wait()
    wk_copy(1).start()
    ln0(0)
    ln0(1)
    wk_copy(0).wait()
    x_copy(1).start()
    kblock(0, 0, 2, 2)
    wk_copy(1).wait()
    wk_copy(2).start()
    kblock(0, 2, 4, 2)
    x_copy(1).wait()
    wk_copy(2).wait()
    wk_copy(3).start()
    x_copy(2).start()
    kblock(0, 4, 6, 2)
    ln0(2)
    ln0(3)
    wk_copy(3).wait()
    x_copy(3).start()
    kblock(0, 6, 8, 2)
    kblock(2)

    def pro_body(t, c):
        r0 = pl.multiple_of(512 * (t + 1), 512)
        pltpu.make_async_copy(x_hbm.at[pl.ds(r0, 512), :], xin.at[pl.ds(r0, 512), :], sems.at[t + 2]).wait()

        for b in range(3):
            toks = kblock(4 * t + 3 + b)
            if b == 0:
                ln0(4 * t + 4)
            ln0(4 * t + 5 + b, toks)
        kblock(4 * t + 6)
        return c

    x_copy(4).start()
    wq_copy.start()
    wv_copy.start()
    wo_copy.start()
    wr_copy.start()
    lax.fori_loop(0, 3, pro_body, 0)
    wq_copy.wait()
    wv_copy.wait()
    wo_copy.wait()
    wr_copy.wait()
    kblock(15)
    conv(wqu, wq)
    conv(wvu, wv)
    conv(wou, wo)
    fill_kpad()

    def q_slice(xa_blk, q_blk, n):
        lhs = _u2b(xa_blk[...])
        rhs = _u2b(wqu[:, 128 * n:128 * n + 128])
        q = jnp.dot(lhs, rhs, preferred_element_type=f32)
        qt = _b2u((q * QSCALE).astype(bf16).T)
        parts = [qt[0:16]] + [pltpu.roll(qt[16 * h:16 * h + 16], 32 * h, 1) for h in range(1, 4)]
        q_blk[64 * n:64 * n + 64, :] = jnp.concatenate(parts, axis=0)
        return parts[0][0:8]

    def v_slice(xa_blk, vt_blk, n):
        lhs = _u2b(xa_blk[...])
        rhs = _u2b(wvu[:, 128 * n:128 * n + 128])
        v = jnp.dot(lhs, rhs, preferred_element_type=f32)
        vt = _b2u(_u2b(_pack_adj(v)).T)
        vt_blk[64 * n:64 * n + 64, :] = vt
        return vt[0:8]

    def v_raw(xa_blk, n):
        vraw[...] = jnp.dot(_u2b(xa_blk[...]), _u2b(wvu[:, 128 * n:128 * n + 128]), preferred_element_type=f32)

    def v_finish(vt_blk, n):
        vt_blk[64 * n:64 * n + 64, :] = _b2u(_u2b(_pack_adj(vraw[...])).T)

    def o_slice(o_blk, x_blk, n):
        lhs = _u2b(o_blk[...])
        rhs = _u2b(wou[:, 128 * n:128 * n + 128])
        acc = jnp.dot(lhs, rhs, preferred_element_type=f32)
        x_blk[:, 128 * n:128 * n + 128] = x_blk[:, 128 * n:128 * n + 128] + acc
        return pltpu.bitcast(acc[0:8], u32)

    def epi_stats(j, x_blk, c, tok=None):
        r0 = pl.multiple_of(j * 128, 128)
        R = 128 // NEC
        lo = R * c
        x1 = x_blk[lo:lo + R, :]
        mu = gate(jnp.mean(x1, axis=1, keepdims=True), tok)
        xc = x1 - mu
        var = jnp.mean(xc * xc, axis=1, keepdims=True)
        a = lax.rsqrt(var + EPS)
        r = jnp.sum(xc * wr[...].astype(f32), axis=1, keepdims=True) * a
        r_s[pl.ds(r0 + lo, R), :] = r
        a_s[pl.ds(r0 + lo, R), :] = a
        return mu, xc, var, a

    def epi_norm(j, x_blk, xa_blk, layer, c, st, tok=None):
        r0 = pl.multiple_of(j * 128, 128)
        R = 128 // NEC
        lo = R * c
        mu, xc, var, a = st
        a1 = gate(1.0 + a, tok)
        x2 = mu + xc * a1
        if layer == 0:
            x_blk[lo:lo + R, :] = x2
            v = xc * (a1 * lax.rsqrt(var * a1 * a1 + EPS))
            xa_blk[lo // 2:(lo + R) // 2, :] = _b2u(v.astype(bf16))
        else:
            outb[pl.ds(r0 + lo, R), :] = x2.astype(bf16)

    def epilogue(j, x_blk, xa_blk, layer, chunks=range(NEC)):
        for c in chunks:
            epi_norm(j, x_blk, xa_blk, layer, c, epi_stats(j, x_blk, c))

    lane8b = lax.broadcasted_iota(jnp.int32, (8, 128), 1) >> 5
    odd = (lane8b & 1) == 1
    high = lane8b >= 2
    lane16b = lax.broadcasted_iota(jnp.int32, (16, 128), 1) >> 5
    d32 = lax.broadcasted_iota(jnp.int32, (32, 128), 0) - (lax.broadcasted_iota(jnp.int32, (32, 128), 1) & 31)
    umask = d32 > 0

    def stage_a(kv, q_blk, g):
        s_ref = sb[g % NBUF]
        for j in range(4):
            x = jnp.concatenate([jnp.where(lane16b == ((h + j) % 4), q_blk[64 * g + 16 * h:64 * g + 16 * h + 16, :],
                                           jnp.uint32(0)) for h in range(4)], axis=0)
            b0 = 16 * j
            kt = jnp.concatenate([kv[g, b0:b0 + 8, :], kv[g, b0 + 128:b0 + 136, :], kv[g, b0 + 8:b0 + 16, :],
                                  kv[g, b0 + 136:b0 + 144, :], kv[g, b0 + 16:b0 + 128, :]], axis=0)
            st = jnp.dot(_u2b(kt), _u2b(x), preferred_element_type=f32)
            su = jnp.concatenate([st[0:16], st[32:48]], axis=0)
            sl = jnp.concatenate([st[16:32], st[48:64]], axis=0)
            s_ref[j, 0:32, :] = jnp.where(umask, su, sl)
            s_ref[j, 32:256, :] = st[64:288]
            if j == 0:
                tok = (pltpu.bitcast(st[64:72], u32), pltpu.bitcast(st[160:168], u32),
                       pltpu.bitcast(st[280:288], u32))
        return tok

    def bfly(y):
        def sel(m, a, b):
            if a is None and b is None:
                return None
            z = jnp.zeros((8, 128), (a if a is not None else b).dtype)
            return jnp.where(m, z if a is None else a, z if b is None else b)
        r = [sel(odd, y[(k + 1) % 4], y[k]) for k in range(4)]
        wp = [sel(high, r[(k + 2) % 4], r[k]) for k in range(4)]
        return [wp[(-h) % 4] for h in range(4)]

    def stage_b(i, g, toks):
        s_ref = sb[g % NBUF]
        p_ref = pb[g % NBUF].at[zs[0]]
        l_ref = lb[g % NBUF]
        ss = [s_ref[j] for j in range(4)]
        ms = [jnp.max(ss[j], axis=0, keepdims=True) for j in range(4)]
        ls = [None] * 4
        nch = len(toks)
        um16 = [umask[0:16], umask[16:32]]
        for c in range(nch):
            mg = [gate(ms[j], toks[c]) for j in range(4)]
            for M in range(24 * c // nch, 24 * (c + 1) // nch):
                y = []
                for j in range(4):
                    Mp = M - 2 * j
                    if not 0 <= Mp < 18:
                        y.append(None)
                        continue
                    row = 16 * (Mp % 16)
                    p = jnp.exp2(ss[j][row:row + 16] - mg[j])
                    if Mp < 16:
                        ps = p[0:8] + p[8:16]
                        ls[j] = ps if ls[j] is None else ls[j] + ps
                        if Mp == 2:
                            p32 = p[0:1]
                            ls[j] = ls[j] - jnp.where(lax.broadcasted_iota(jnp.int32, (8, 128), 0) == 0,
                                                      npad[jnp.minimum(i, 2), j] * p32, 0.0)
                    if Mp < 2:
                        p = jnp.where(um16[Mp], p, 0.0)
                    elif Mp >= 16:
                        p = jnp.where(um16[Mp - 16], 0.0, p)
                    y.append(_pack2(p[0:8], p[8:16]))
                w = bfly(y)
                for h in range(4):
                    p_ref[h, 8 * M:8 * M + 8, :] = w[h] if w[h] is not None else jnp.zeros((8, 128), u32)
        for j in range(4):
            l_ref[j] = jnp.sum(ls[j], axis=0, keepdims=True)

    def stage_c(vts, o_blk, g):
        p_ref = pb[g % NBUF].at[zs[1]]
        l_ref = lb[g % NBUF]
        lh = bfly([jnp.broadcast_to(1.0 / l_ref[j], (8, 128)) for j in range(4)])
        outs = []
        for h in range(4):
            vt = jnp.concatenate([_u2b(vts[t][64 * g + 16 * h:64 * g + 16 * h + 16, :]) for t in range(3)], axis=1)
            o = jnp.dot(vt, _u2b(p_ref[h]), preferred_element_type=f32)
            o = o * lh[h][0:1]
            if h:
                o = pltpu.roll(o, 128 - 32 * h, 1)
            outs.append(o)
        ot = jnp.concatenate(outs, axis=0)
        o_blk[:, 128 * g:128 * g + 128] = _b2u(ot.T.astype(bf16))

    def attn_body(i, c, has_next, prev, layer, extra=()):
        lo = -1 if prev else 0
        r = pl.multiple_of((i + lo) * 64, 64)
        nblk = (2 if has_next else 1) - lo
        xav = xa.at[pl.ds(r, 64 * nblk), :]
        ov = o_s.at[pl.ds(r, 64 * (1 - lo)), :]
        xv = x_s.at[pl.ds(pl.multiple_of((i + lo) * 128, 128), 128), :]
        qv = qt_s.at[pl.ds(i, 2)]
        vv = vt_s.at[pl.ds(i + lo, 4 - lo)]
        kv = k_s.at[:, pl.ds(pl.multiple_of(i * 64, 64), 256), :]
        blk = lambda v, b: v.at[pl.ds(64 * (b - lo), 64), :]
        vtile = lambda b: vv.at[b - lo]

        qs = [functools.partial(q_slice, blk(xav, 1), qv.at[1], n) for n in range(NG)] if has_next else []
        vs = [functools.partial(v_slice, blk(xav, 1), vtile(3), n) for n in range(NG)] if has_next else []
        if has_next:
            vs[NG - 1] = functools.partial(v_raw, blk(xav, 1), NG - 1)
        if prev:
            v_finish(vtile(2), NG - 1)
        os_ = [functools.partial(o_slice, blk(ov, -1), xv, n) for n in range(NG)] if prev else []
        sl = qs[0:1] + os_ + qs[1:] + vs
        last_o = len(qs[0:1]) + len(os_) - 1 if os_ else -1
        if extra:
            n_it = 2 * NG
            groups = [extra[len(extra) * k // n_it:len(extra) * (k + 1) // n_it] for k in range(n_it)]

            def run(fs):
                for f in fs:
                    f()
            comp = [functools.partial(run, fs) for fs in groups]
            sl = comp[0:1] + sl + comp[1:]
            last_o = NG
        state = {"emitted": 0}
        stats = {}
        if layer == 0:
            esch = [(1, "s", 0, False), (1, "s", 1, False), (4, "n", 0, True), (6, "n", 1, True)]
        else:
            esch = [(1, "s", 0, False), (1, "n", 0, False), (2, "s", 1, False), (2, "n", 1, False)]

        def run_epi(k, tok):
            for (off, kind, ch, paced) in esch:
                if (k is None or off == k) and (kind, ch) not in stats:
                    if kind == "s":
                        stats[kind, ch] = epi_stats(i - 1, xv, ch, tok if paced else None)
                    else:
                        epi_norm(i - 1, xv, blk(xav, -1), layer, ch, stats["s", ch], tok if paced else None)
                        stats[kind, ch] = True

        def dense_one():
            k = state["emitted"]
            if k < len(sl):
                t = sl[k]()
                state["emitted"] += 1
                if prev and k > last_o:
                    run_epi(k - last_o, t)

        for g in range(NG):
            def pv():
                if g >= 1:
                    stage_c([vtile(t) for t in range(3)], blk(ov, 0), g - 1)
                elif prev:
                    stage_c([vtile(t - 1) for t in range(3)], blk(ov, -1), NG - 1)
            if g == 0:
                pv()
            tok = (None, None, None)
            if g + 1 < NG:
                tok = stage_a(kv.at[:, pl.ds(0, 192), :], qv.at[0], g + 1)
            elif has_next:
                tok = stage_a(kv.at[:, pl.ds(64, 192), :], qv.at[1], 0)
            stage_b(i, g, [None, None, tok[0], tok[2]])
            dense_one()
            dense_one()
            if g > 0:
                pv()
            dense_one()
        while state["emitted"] < len(sl):
            dense_one()
        if prev:
            run_epi(None, None)

        if layer == 1 and prev:
            out_copy(i - 1).start()
        if layer == 0 and prev and has_next:
            @pl.when(i == 1)
            def _():
                wg_copy.start()
                wu_copy.start()
                wd_copy.start()
        return c

    def finish_block(j, layer):
        o_blk = o_s.at[pl.ds(pl.multiple_of(j * 64, 64), 64), :]
        x_blk = x_s.at[pl.ds(pl.multiple_of(j * 128, 128), 128), :]
        stage_c([vt_s.at[j + t] for t in range(3)], o_blk, NG - 1)
        for n in range(NG):
            o_slice(o_blk, x_blk, n)
        epilogue(j, x_blk, xa.at[pl.ds(pl.multiple_of(j * 64, 64), 64), :], layer)

    def route(raw):
        r = r_s[0:S, :]
        rmax = jnp.max(r)
        rows = lax.broadcasted_iota(jnp.int32, (S, 1), 0)
        idx = jnp.min(jnp.where(r == rmax, rows, S))
        idx = jnp.minimum(idx, S - 1)
        xrow = x_s[pl.ds(idx, 1), :]
        arow = a_s[pl.ds(idx, 1), :]
        mu = jnp.mean(xrow, axis=1, keepdims=True)
        if raw:
            xsel = (xrow - mu) * arow
            xrow = xrow + xsel
        else:
            xsel = (xrow - mu) * (arow / (1.0 + arow))
        xs = jnp.broadcast_to(xsel, (8, D)).astype(bf16)
        return idx, rmax, xrow, xs

    def ffn_steps(xs):
        gates, hid, ys = [], [], []

        def up(c, w, first):
            r = jnp.dot(xs, w[:, 128 * c:128 * (c + 1)], preferred_element_type=f32)
            if first:
                gates.append(r)
            else:
                g_ = gates[c]
                hid.append((g_ * jax.nn.sigmoid(g_) * r).astype(bf16))

        def down(c):
            ys.append(jnp.dot(hid[c], wd[128 * c:128 * (c + 1), :], preferred_element_type=f32))

        steps = []
        for c in range(NFS):
            steps.append(functools.partial(up, c, wg, True))
            steps.append(functools.partial(up, c, wu, False))
            if c >= 1:
                steps.append(functools.partial(down, c - 1))
        steps.append(functools.partial(down, NFS - 1))

        def result():
            y = ys[0]
            for t in ys[1:]:
                y = y + t
            return y
        return steps, result

    def kslice(b, g):
        kblock(b, g, g + 1)

    def ffn_mid():
        kblock(K2_EARLY)
        idx, rmax, xrow, xs = route(raw=False)
        steps, result = ffn_steps(xs)
        fi = 0
        for b in range(K2_EARLY + 1, NB):
            for g in range(NG):
                kslice(b, g)
                if fi < len(steps):
                    steps[fi]()
                    fi += 1
        while fi < len(steps):
            steps[fi]()
            fi += 1
        y = result()
        x_s[pl.ds(idx, 1), :] = xrow + y[0:1, :] * jax.nn.sigmoid(rmax)
        r0 = pl.multiple_of((idx // 16) * 16, 16)
        h0 = pl.multiple_of((idx // 16) * 8, 8)
        x = x_s[pl.ds(r0, 16), :]
        mu = jnp.mean(x, axis=1, keepdims=True)
        xc = x - mu
        var = jnp.mean(xc * xc, axis=1, keepdims=True)
        xn = (xc * lax.rsqrt(var + EPS)).astype(bf16)
        xa[pl.ds(h0, 8), :] = _b2u(xn)
        kk = jnp.dot(xn, wk[...], preferred_element_type=f32)
        for g in range(NG):
            k_s[g, pl.ds(128 + h0, 8), :] = _b2u(kk[:, 128 * g:128 * g + 128].astype(bf16))
        fill_kpad()

    def ffn_last():
        idx, rmax, xrow, xs = route(raw=True)
        steps, result = ffn_steps(xs)
        for f in steps:
            f()
        y = result()
        new = xrow + y[0:1, :] * jax.nn.sigmoid(rmax)
        for i in range(NB):
            out_copy(i).wait()
        b0 = pl.multiple_of((idx // 16) * 16, 16)
        rows = lax.broadcasted_iota(jnp.int32, (16, D), 0) + b0
        outb[pl.ds(b0, 16), :] = jnp.where(rows == idx, new, outb[pl.ds(b0, 16), :].astype(f32)).astype(bf16)
        fix = pltpu.make_async_copy(outb.at[pl.ds(b0, 16), :], out_hbm.at[pl.ds(b0, 16), :], osems.at[NB])
        fix.start()
        fix.wait()

    for layer in range(2):
        for n in range(NG):
            q_slice(xa.at[pl.ds(0, 64), :], qt_s.at[0], n)
        for n in range(NG):
            v_slice(xa.at[pl.ds(0, 64), :], vt_s.at[2], n)
        stage_a(k_s.at[:, pl.ds(0, 192), :], qt_s.at[0], 0)
        attn_body(0, 0, has_next=True, prev=False, layer=layer)
        lax.fori_loop(1, NB - 1, functools.partial(attn_body, has_next=True, prev=True, layer=layer), 0)
        extra = [functools.partial(kslice, b, g) for b in range(K2_EARLY) for g in range(NG)] if layer == 0 else ()
        attn_body(NB - 1, 0, has_next=False, prev=True, layer=layer, extra=extra)
        finish_block(NB - 1, layer)
        if layer == 0:
            wg_copy.wait()
            wu_copy.wait()
            wd_copy.wait()
            ffn_mid()
        else:
            out_copy(NB - 1).start()
            ffn_last()


@jax.jit
def pallas_interleave_layers__sliding_block__moe_arch_mod__prompt_kernel(
    A_x: jax.Array,
    A_wqkv: jax.Array,
    A_wo: jax.Array,
    B_x: jax.Array,
    B_w_r: jax.Array,
    B_w_gate: jax.Array,
    B_w_up: jax.Array,
    B_w_down: jax.Array,
):
    del B_x
    x = A_x.reshape(S, D)
    wr = B_w_r.reshape(1, D)
    any_spec = pl.BlockSpec(memory_space=pl.ANY)
    scratch = [
        pltpu.VMEM((S, D), bf16),
        pltpu.VMEM((S, D), f32),
        pltpu.VMEM((S // 2, D), u32),
        pltpu.VMEM((NG, (S + 256) // 2 + 64, 128), u32),
        pltpu.VMEM((NB + 1, D // 2, 128), u32),
        pltpu.VMEM((NB + 3, D // 2, 128), u32),
        pltpu.VMEM((S // 2, D), u32),
        pltpu.VMEM((D, D), bf16),
        pltpu.VMEM((D, D), bf16),
        pltpu.VMEM((D, D), bf16),
        pltpu.VMEM((D // 2, D), u32),
        pltpu.VMEM((D // 2, D), u32),
        pltpu.VMEM((D, D), bf16),
        pltpu.VMEM((D // 2, D), u32),
        pltpu.VMEM((1, D), bf16),
        pltpu.VMEM((D, F), bf16),
        pltpu.VMEM((D, F), bf16),
        pltpu.VMEM((F, D), bf16),
        pltpu.VMEM((S, 1), f32),
        pltpu.VMEM((S, 1), f32),
        pltpu.VMEM((S, D), bf16),
        pltpu.VMEM((3, 4, 1, 128), f32),
        pltpu.SMEM((2,), jnp.int32),
        pltpu.VMEM((8, 128), u32),
        pltpu.VMEM((128, 128), f32),
        pltpu.SemaphoreType.DMA((16,)),
        pltpu.SemaphoreType.DMA((NB + 1,)),
    ]
    scratch += [pltpu.VMEM((4, 256, 128), f32)] * NBUF
    scratch += [pltpu.VMEM((1, 4, 192, 128), u32)] * NBUF
    scratch += [pltpu.VMEM((4, 1, 128), f32)] * NBUF
    out = pl.pallas_call(
        _kernel,
        out_shape=jax.ShapeDtypeStruct((S, D), bf16),
        in_specs=[any_spec] * 7,
        out_specs=any_spec,
        scratch_shapes=scratch,
        compiler_params=pltpu.CompilerParams(vmem_limit_bytes=110 * 1024 * 1024),
    )(x, A_wqkv, A_wo, wr, B_w_gate, B_w_up, B_w_down)
    return out.reshape(1, S, D)
```

```python
import functools
import math

import jax
import jax.numpy as jnp
from jax import lax
import jax.experimental.pallas as pl
import jax.experimental.pallas.tpu as pltpu

S, D, H, DH, F = 2048, 1024, 32, 32, 3584
NB = S // 128
NG = D // 128
NFS = F // 128
EPS = 1e-5
QSCALE = (DH ** -0.5) * math.log2(math.e)
NEC = 2
NBUF = 2
K2_EARLY = 2
XCH = [(0, 256), (256, 256), (512, 512), (1024, 512), (1536, 512)]

bf16 = jnp.bfloat16
f32 = jnp.float32
u32 = jnp.uint32


def _b2u(x):
    return pltpu.bitcast(x, u32)


def _u2b(x):
    return pltpu.bitcast(x, bf16)


def _pack2(a, b):
    w = pltpu.pack_elementwise([a, b], packed_dtype=bf16)
    return w if w.dtype == u32 else pltpu.bitcast(w, u32)


def _pack_adj(x):
    r, c = x.shape
    e = x.reshape(r // 16, 16, c)
    return _pack2(e[:, 0:8, :].reshape(r // 2, c), e[:, 8:16, :].reshape(r // 2, c))


def _kernel(x_hbm, wqkv_hbm, wo_hbm, wr_hbm, wg_hbm, wu_hbm, wd_hbm, out_hbm,
            xin, x_s, xa, k_s, qt_s, vt_s, o_s,
            wk, wq, wv, wqu, wvu, wo, wou, wr, wg, wu, wd,
            r_s, a_s, outb, npad, zs, zv, vraw, wr1, sems, osems, *bufs):
    zs[0] = 0
    zs[1] = 0
    zv[...] = jnp.zeros((8, 128), u32)
    sb = bufs[0:NBUF]
    pb = bufs[NBUF:2 * NBUF]
    lb = bufs[2 * NBUF:3 * NBUF]

    def x_copy(t):
        r0, n = XCH[t]
        return pltpu.make_async_copy(x_hbm.at[pl.ds(r0, n), :], xin.at[pl.ds(r0, n), :], sems.at[t])

    def wk_copy(c):
        return pltpu.make_async_copy(wqkv_hbm.at[:, pl.ds(D + 256 * c, 256)], wk.at[:, pl.ds(256 * c, 256)],
                                     sems.at[12 + c])

    wq_copy = pltpu.make_async_copy(wqkv_hbm.at[:, pl.ds(0, D)], wq, sems.at[5])
    wv_copy = pltpu.make_async_copy(wqkv_hbm.at[:, pl.ds(2 * D, D)], wv, sems.at[6])
    wo_copy = pltpu.make_async_copy(wo_hbm, wo, sems.at[7])
    wr_copy = pltpu.make_async_copy(wr_hbm, wr1, sems.at[8])
    wg_copy = pltpu.make_async_copy(wg_hbm, wg, sems.at[9])
    wu_copy = pltpu.make_async_copy(wu_hbm, wu, sems.at[10])
    wd_copy = pltpu.make_async_copy(wd_hbm, wd, sems.at[11])

    def out_copy(i):
        r0 = pl.multiple_of(i * 128, 128)
        return pltpu.make_async_copy(outb.at[pl.ds(r0, 128), :], out_hbm.at[pl.ds(r0, 128), :], osems.at[i])

    x_copy(0).start()
    wk_copy(0).start()

    ql1 = lax.broadcasted_iota(jnp.int32, (1, 128), 1) & 31
    for ii in range(3):
        for j in range(4):
            t = 256 - (128 * ii + 32 * j) if ii < 2 else 0
            n = max(0, min(256, t) - 32) + jnp.maximum(0, min(32, t) - 1 - ql1)
            npad[ii, j] = n.astype(f32)
    vt_s[0] = jnp.zeros((D // 2, 128), u32)
    vt_s[1] = jnp.zeros((D // 2, 128), u32)

    def kblock(b, g0=0, g1=NG, nb=1):
        static = isinstance(b, int)
        r = b * 64 if static else pl.multiple_of(b * 64, 64)
        xa_t = _u2b(xa[pl.ds(r, 64 * nb), :])
        kk = jnp.dot(xa_t, wk[:, 128 * g0:128 * g1], preferred_element_type=f32)
        kr = 128 + r if static else pl.multiple_of(128 + r, 64)
        toks = []
        for g in range(g0, g1):
            v = _b2u(kk[:, 128 * (g - g0):128 * (g - g0) + 128].astype(bf16))
            k_s[g, pl.ds(kr, 64 * nb), :] = v
            toks.append(v[0:8])
        return toks

    def fill_kpad():
        for g in range(NG):
            lo = k_s[g, 128:129, :] & jnp.uint32(0xFFFF)
            k_s[g, 0:128, :] = jnp.broadcast_to(lo | (lo << 16), (128, 128))

    def gate(v, tok):
        if tok is None:
            return v
        return v + pltpu.bitcast(tok & zv[...], f32)[0:1, 0:v.shape[1]]

    def ln0(b, toks=None):
        base = 128 * b if isinstance(b, int) else pl.multiple_of(128 * b, 128)
        nch = 1 if toks is None else 2
        n = 128 // nch
        for c in range(nch):
            r0 = base + n * c
            x = xin[pl.ds(r0, n), :].astype(f32)
            x_s[pl.ds(r0, n), :] = x
            mu = jnp.mean(x, axis=1, keepdims=True)
            if toks is not None:
                mu = gate(mu, toks[4 * c])
            xc = x - mu
            var = jnp.mean(xc * xc, axis=1, keepdims=True)
            h0 = r0 // 2 if isinstance(b, int) else pl.multiple_of(r0 // 2, n // 2)
            xa[pl.ds(h0, n // 2), :] = _b2u((xc * lax.rsqrt(var + EPS)).astype(bf16))

    def conv(dst, src):
        for j in range(NG):
            dst[64 * j:64 * j + 64, :] = _b2u(src[128 * j:128 * j + 128, :])

    x_copy(0).wait()
    wk_copy(1).start()
    ln0(0)
    ln0(1)
    wk_copy(0).wait()
    x_copy(1).start()
    kblock(0, 0, 2, 2)
    wk_copy(1).wait()
    wk_copy(2).start()
    kblock(0, 2, 4, 2)
    x_copy(1).wait()
    wk_copy(2).wait()
    wk_copy(3).start()
    x_copy(2).start()
    kblock(0, 4, 6, 2)
    ln0(2)
    ln0(3)
    wk_copy(3).wait()
    x_copy(3).start()
    kblock(0, 6, 8, 2)
    kblock(2)

    def pro_body(t, c):
        r0 = pl.multiple_of(512 * (t + 1), 512)
        pltpu.make_async_copy(x_hbm.at[pl.ds(r0, 512), :], xin.at[pl.ds(r0, 512), :], sems.at[t + 2]).wait()

        for b in range(3):
            toks = kblock(4 * t + 3 + b)
            if b == 0:
                ln0(4 * t + 4)
            ln0(4 * t + 5 + b, toks)
        kblock(4 * t + 6)
        return c

    x_copy(4).start()
    wq_copy.start()
    wv_copy.start()
    wo_copy.start()
    wr_copy.start()
    lax.fori_loop(0, 3, pro_body, 0)
    wq_copy.wait()
    wv_copy.wait()
    wo_copy.wait()
    wr_copy.wait()
    kblock(15)
    conv(wqu, wq)
    conv(wvu, wv)
    conv(wou, wo)
    wr[...] = wr1[...].astype(f32).reshape(1, D).astype(bf16)
    fill_kpad()

    def q_slice(xa_blk, q_blk, n):
        lhs = _u2b(xa_blk[...])
        rhs = _u2b(wqu[:, 128 * n:128 * n + 128])
        q = jnp.dot(lhs, rhs, preferred_element_type=f32)
        qt = _b2u((q * QSCALE).astype(bf16).T)
        parts = [qt[0:16]] + [pltpu.roll(qt[16 * h:16 * h + 16], 32 * h, 1) for h in range(1, 4)]
        q_blk[64 * n:64 * n + 64, :] = jnp.concatenate(parts, axis=0)
        return parts[0][0:8]

    def v_slice(xa_blk, vt_blk, n):
        lhs = _u2b(xa_blk[...])
        rhs = _u2b(wvu[:, 128 * n:128 * n + 128])
        v = jnp.dot(lhs, rhs, preferred_element_type=f32)
        vt = _b2u(_u2b(_pack_adj(v)).T)
        vt_blk[64 * n:64 * n + 64, :] = vt
        return vt[0:8]

    def v_raw(xa_blk, n):
        vraw[...] = jnp.dot(_u2b(xa_blk[...]), _u2b(wvu[:, 128 * n:128 * n + 128]), preferred_element_type=f32)

    def v_finish(vt_blk, n):
        vt_blk[64 * n:64 * n + 64, :] = _b2u(_u2b(_pack_adj(vraw[...])).T)

    def o_slice(o_blk, x_blk, n):
        lhs = _u2b(o_blk[...])
        rhs = _u2b(wou[:, 128 * n:128 * n + 128])
        acc = jnp.dot(lhs, rhs, preferred_element_type=f32)
        x_blk[:, 128 * n:128 * n + 128] = x_blk[:, 128 * n:128 * n + 128] + acc
        return pltpu.bitcast(acc[0:8], u32)

    def epi_stats(j, x_blk, c, tok=None):
        r0 = pl.multiple_of(j * 128, 128)
        R = 128 // NEC
        lo = R * c
        x1 = x_blk[lo:lo + R, :]
        mu = gate(jnp.mean(x1, axis=1, keepdims=True), tok)
        xc = x1 - mu
        var = jnp.mean(xc * xc, axis=1, keepdims=True)
        a = lax.rsqrt(var + EPS)
        r = jnp.sum(xc * wr[...].astype(f32), axis=1, keepdims=True) * a
        r_s[pl.ds(r0 + lo, R), :] = r
        a_s[pl.ds(r0 + lo, R), :] = a
        return mu, xc, var, a

    def epi_norm(j, x_blk, xa_blk, layer, c, st, tok=None):
        r0 = pl.multiple_of(j * 128, 128)
        R = 128 // NEC
        lo = R * c
        mu, xc, var, a = st
        a1 = gate(1.0 + a, tok)
        x2 = mu + xc * a1
        if layer == 0:
            x_blk[lo:lo + R, :] = x2
            v = xc * (a1 * lax.rsqrt(var * a1 * a1 + EPS))
            xa_blk[lo // 2:(lo + R) // 2, :] = _b2u(v.astype(bf16))
        else:
            outb[pl.ds(r0 + lo, R), :] = x2.astype(bf16)

    def epilogue(j, x_blk, xa_blk, layer, chunks=range(NEC)):
        for c in chunks:
            epi_norm(j, x_blk, xa_blk, layer, c, epi_stats(j, x_blk, c))

    lane8b = lax.broadcasted_iota(jnp.int32, (8, 128), 1) >> 5
    odd = (lane8b & 1) == 1
    high = lane8b >= 2
    lane16b = lax.broadcasted_iota(jnp.int32, (16, 128), 1) >> 5
    d32 = lax.broadcasted_iota(jnp.int32, (32, 128), 0) - (lax.broadcasted_iota(jnp.int32, (32, 128), 1) & 31)
    umask = d32 > 0

    def stage_a(kv, q_blk, g):
        s_ref = sb[g % NBUF]
        for j in range(4):
            x = jnp.concatenate([jnp.where(lane16b == ((h + j) % 4), q_blk[64 * g + 16 * h:64 * g + 16 * h + 16, :],
                                           jnp.uint32(0)) for h in range(4)], axis=0)
            b0 = 16 * j
            kt = jnp.concatenate([kv[g, b0:b0 + 8, :], kv[g, b0 + 128:b0 + 136, :], kv[g, b0 + 8:b0 + 16, :],
                                  kv[g, b0 + 136:b0 + 144, :], kv[g, b0 + 16:b0 + 128, :]], axis=0)
            st = jnp.dot(_u2b(kt), _u2b(x), preferred_element_type=f32)
            su = jnp.concatenate([st[0:16], st[32:48]], axis=0)
            sl = jnp.concatenate([st[16:32], st[48:64]], axis=0)
            s_ref[j, 0:32, :] = jnp.where(umask, su, sl)
            s_ref[j, 32:256, :] = st[64:288]
            if j == 0:
                tok = (pltpu.bitcast(st[64:72], u32), pltpu.bitcast(st[160:168], u32),
                       pltpu.bitcast(st[280:288], u32))
        return tok

    def bfly(y):
        def sel(m, a, b):
            if a is None and b is None:
                return None
            z = jnp.zeros((8, 128), (a if a is not None else b).dtype)
            return jnp.where(m, z if a is None else a, z if b is None else b)
        r = [sel(odd, y[(k + 1) % 4], y[k]) for k in range(4)]
        wp = [sel(high, r[(k + 2) % 4], r[k]) for k in range(4)]
        return [wp[(-h) % 4] for h in range(4)]

    def stage_b(i, g, toks):
        s_ref = sb[g % NBUF]
        p_ref = pb[g % NBUF].at[zs[0]]
        l_ref = lb[g % NBUF]
        ss = [s_ref[j] for j in range(4)]
        ms = [jnp.max(ss[j], axis=0, keepdims=True) for j in range(4)]
        ls = [None] * 4
        nch = len(toks)
        um16 = [umask[0:16], umask[16:32]]
        for c in range(nch):
            mg = [gate(ms[j], toks[c]) for j in range(4)]
            for M in range(24 * c // nch, 24 * (c + 1) // nch):
                y = []
                for j in range(4):
                    Mp = M - 2 * j
                    if not 0 <= Mp < 18:
                        y.append(None)
                        continue
                    row = 16 * (Mp % 16)
                    p = jnp.exp2(ss[j][row:row + 16] - mg[j])
                    if Mp < 16:
                        ps = p[0:8] + p[8:16]
                        ls[j] = ps if ls[j] is None else ls[j] + ps
                        if Mp == 2:
                            p32 = p[0:1]
                            ls[j] = ls[j] - jnp.where(lax.broadcasted_iota(jnp.int32, (8, 128), 0) == 0,
                                                      npad[jnp.minimum(i, 2), j] * p32, 0.0)
                    if Mp < 2:
                        p = jnp.where(um16[Mp], p, 0.0)
                    elif Mp >= 16:
                        p = jnp.where(um16[Mp - 16], 0.0, p)
                    y.append(_pack2(p[0:8], p[8:16]))
                w = bfly(y)
                for h in range(4):
                    p_ref[h, 8 * M:8 * M + 8, :] = w[h] if w[h] is not None else jnp.zeros((8, 128), u32)
        for j in range(4):
            l_ref[j] = jnp.sum(ls[j], axis=0, keepdims=True)

    def stage_c(vts, o_blk, g):
        p_ref = pb[g % NBUF].at[zs[1]]
        l_ref = lb[g % NBUF]
        lh = bfly([jnp.broadcast_to(1.0 / l_ref[j], (8, 128)) for j in range(4)])
        outs = []
        for h in range(4):
            vt = jnp.concatenate([_u2b(vts[t][64 * g + 16 * h:64 * g + 16 * h + 16, :]) for t in range(3)], axis=1)
            o = jnp.dot(vt, _u2b(p_ref[h]), preferred_element_type=f32)
            o = o * lh[h][0:1]
            if h:
                o = pltpu.roll(o, 128 - 32 * h, 1)
            outs.append(o)
        ot = jnp.concatenate(outs, axis=0)
        o_blk[:, 128 * g:128 * g + 128] = _b2u(ot.T.astype(bf16))

    def attn_body(i, c, has_next, prev, layer, extra=()):
        lo = -1 if prev else 0
        r = pl.multiple_of((i + lo) * 64, 64)
        nblk = (2 if has_next else 1) - lo
        xav = xa.at[pl.ds(r, 64 * nblk), :]
        ov = o_s.at[pl.ds(r, 64 * (1 - lo)), :]
        xv = x_s.at[pl.ds(pl.multiple_of((i + lo) * 128, 128), 128), :]
        qv = qt_s.at[pl.ds(i, 2)]
        vv = vt_s.at[pl.ds(i + lo, 4 - lo)]
        kv = k_s.at[:, pl.ds(pl.multiple_of(i * 64, 64), 256), :]
        blk = lambda v, b: v.at[pl.ds(64 * (b - lo), 64), :]
        vtile = lambda b: vv.at[b - lo]

        qs = [functools.partial(q_slice, blk(xav, 1), qv.at[1], n) for n in range(NG)] if has_next else []
        vs = [functools.partial(v_slice, blk(xav, 1), vtile(3), n) for n in range(NG)] if has_next else []
        if has_next:
            vs[NG - 1] = functools.partial(v_raw, blk(xav, 1), NG - 1)
        if prev:
            v_finish(vtile(2), NG - 1)
        os_ = [functools.partial(o_slice, blk(ov, -1), xv, n) for n in range(NG)] if prev else []
        sl = qs[0:1] + os_ + qs[1:] + vs
        last_o = len(qs[0:1]) + len(os_) - 1 if os_ else -1
        if extra:
            n_it = 2 * NG
            groups = [extra[len(extra) * k // n_it:len(extra) * (k + 1) // n_it] for k in range(n_it)]

            def run(fs):
                for f in fs:
                    f()
            comp = [functools.partial(run, fs) for fs in groups]
            sl = comp[0:1] + sl + comp[1:]
            last_o = NG
        state = {"emitted": 0}
        stats = {}
        if layer == 0:
            esch = [(1, "s", 0, False), (1, "s", 1, False), (4, "n", 0, True), (6, "n", 1, True)]
        else:
            esch = [(1, "s", 0, False), (1, "n", 0, False), (2, "s", 1, False), (2, "n", 1, False)]

        def run_epi(k, tok):
            for (off, kind, ch, paced) in esch:
                if (k is None or off == k) and (kind, ch) not in stats:
                    if kind == "s":
                        stats[kind, ch] = epi_stats(i - 1, xv, ch, tok if paced else None)
                    else:
                        epi_norm(i - 1, xv, blk(xav, -1), layer, ch, stats["s", ch], tok if paced else None)
                        stats[kind, ch] = True

        def dense_one():
            k = state["emitted"]
            if k < len(sl):
                t = sl[k]()
                state["emitted"] += 1
                if prev and k > last_o:
                    run_epi(k - last_o, t)

        for g in range(NG):
            def pv():
                if g >= 1:
                    stage_c([vtile(t) for t in range(3)], blk(ov, 0), g - 1)
                elif prev:
                    stage_c([vtile(t - 1) for t in range(3)], blk(ov, -1), NG - 1)
            if g == 0:
                pv()
            tok = (None, None, None)
            if g + 1 < NG:
                tok = stage_a(kv.at[:, pl.ds(0, 192), :], qv.at[0], g + 1)
            elif has_next:
                tok = stage_a(kv.at[:, pl.ds(64, 192), :], qv.at[1], 0)
            stage_b(i, g, [None, None, tok[0], tok[2]])
            dense_one()
            dense_one()
            if g > 0:
                pv()
            dense_one()
        while state["emitted"] < len(sl):
            dense_one()
        if prev:
            run_epi(None, None)

        if layer == 1 and prev:
            out_copy(i - 1).start()
        if layer == 0 and prev and has_next:
            @pl.when(i == 1)
            def _():
                wg_copy.start()
                wu_copy.start()
                wd_copy.start()
        return c

    def finish_block(j, layer):
        o_blk = o_s.at[pl.ds(pl.multiple_of(j * 64, 64), 64), :]
        x_blk = x_s.at[pl.ds(pl.multiple_of(j * 128, 128), 128), :]
        stage_c([vt_s.at[j + t] for t in range(3)], o_blk, NG - 1)
        for n in range(NG):
            o_slice(o_blk, x_blk, n)
        epilogue(j, x_blk, xa.at[pl.ds(pl.multiple_of(j * 64, 64), 64), :], layer)

    def route(raw):
        r = r_s[0:S, :]
        rmax = jnp.max(r)
        rows = lax.broadcasted_iota(jnp.int32, (S, 1), 0)
        idx = jnp.min(jnp.where(r == rmax, rows, S))
        idx = jnp.minimum(idx, S - 1)
        xrow = x_s[pl.ds(idx, 1), :]
        arow = a_s[pl.ds(idx, 1), :]
        mu = jnp.mean(xrow, axis=1, keepdims=True)
        if raw:
            xsel = (xrow - mu) * arow
            xrow = xrow + xsel
        else:
            xsel = (xrow - mu) * (arow / (1.0 + arow))
        xs = jnp.broadcast_to(xsel, (8, D)).astype(bf16)
        return idx, rmax, xrow, xs

    def ffn_steps(xs):
        gates, hid, ys = [], [], []

        def up(c, w, first):
            r = jnp.dot(xs, w[:, 128 * c:128 * (c + 1)], preferred_element_type=f32)
            if first:
                gates.append(r)
            else:
                g_ = gates[c]
                hid.append((g_ * jax.nn.sigmoid(g_) * r).astype(bf16))

        def down(c):
            ys.append(jnp.dot(hid[c], wd[128 * c:128 * (c + 1), :], preferred_element_type=f32))

        steps = []
        for c in range(NFS):
            steps.append(functools.partial(up, c, wg, True))
            steps.append(functools.partial(up, c, wu, False))
            if c >= 1:
                steps.append(functools.partial(down, c - 1))
        steps.append(functools.partial(down, NFS - 1))

        def result():
            y = ys[0]
            for t in ys[1:]:
                y = y + t
            return y
        return steps, result

    def kslice(b, g):
        kblock(b, g, g + 1)

    def ffn_mid():
        kblock(K2_EARLY)
        idx, rmax, xrow, xs = route(raw=False)
        steps, result = ffn_steps(xs)
        fi = 0
        for b in range(K2_EARLY + 1, NB):
            for g in range(NG):
                kslice(b, g)
                if fi < len(steps):
                    steps[fi]()
                    fi += 1
        while fi < len(steps):
            steps[fi]()
            fi += 1
        y = result()
        x_s[pl.ds(idx, 1), :] = xrow + y[0:1, :] * jax.nn.sigmoid(rmax)
        r0 = pl.multiple_of((idx // 16) * 16, 16)
        h0 = pl.multiple_of((idx // 16) * 8, 8)
        x = x_s[pl.ds(r0, 16), :]
        mu = jnp.mean(x, axis=1, keepdims=True)
        xc = x - mu
        var = jnp.mean(xc * xc, axis=1, keepdims=True)
        xn = (xc * lax.rsqrt(var + EPS)).astype(bf16)
        xa[pl.ds(h0, 8), :] = _b2u(xn)
        kk = jnp.dot(xn, wk[...], preferred_element_type=f32)
        for g in range(NG):
            k_s[g, pl.ds(128 + h0, 8), :] = _b2u(kk[:, 128 * g:128 * g + 128].astype(bf16))
        fill_kpad()

    def ffn_last():
        idx, rmax, xrow, xs = route(raw=True)
        steps, result = ffn_steps(xs)
        for f in steps:
            f()
        y = result()
        new = xrow + y[0:1, :] * jax.nn.sigmoid(rmax)
        for i in range(NB):
            out_copy(i).wait()
        b0 = pl.multiple_of((idx // 16) * 16, 16)
        rows = lax.broadcasted_iota(jnp.int32, (16, D), 0) + b0
        outb[pl.ds(b0, 16), :] = jnp.where(rows == idx, new, outb[pl.ds(b0, 16), :].astype(f32)).astype(bf16)
        fix = pltpu.make_async_copy(outb.at[pl.ds(b0, 16), :], out_hbm.at[pl.ds(b0, 16), :], osems.at[NB])
        fix.start()
        fix.wait()

    for layer in range(2):
        for n in range(NG):
            q_slice(xa.at[pl.ds(0, 64), :], qt_s.at[0], n)
        for n in range(NG):
            v_slice(xa.at[pl.ds(0, 64), :], vt_s.at[2], n)
        stage_a(k_s.at[:, pl.ds(0, 192), :], qt_s.at[0], 0)
        attn_body(0, 0, has_next=True, prev=False, layer=layer)
        lax.fori_loop(1, NB - 1, functools.partial(attn_body, has_next=True, prev=True, layer=layer), 0)
        extra = [functools.partial(kslice, b, g) for b in range(K2_EARLY) for g in range(NG)] if layer == 0 else ()
        attn_body(NB - 1, 0, has_next=False, prev=True, layer=layer, extra=extra)
        finish_block(NB - 1, layer)
        if layer == 0:
            wg_copy.wait()
            wu_copy.wait()
            wd_copy.wait()
            ffn_mid()
        else:
            out_copy(NB - 1).start()
            ffn_last()


@jax.jit
def pallas_interleave_layers__sliding_block__moe_arch_mod__prompt_kernel(
    A_x: jax.Array,
    A_wqkv: jax.Array,
    A_wo: jax.Array,
    B_x: jax.Array,
    B_w_r: jax.Array,
    B_w_gate: jax.Array,
    B_w_up: jax.Array,
    B_w_down: jax.Array,
):
    del B_x
    x = A_x.reshape(S, D)
    any_spec = pl.BlockSpec(memory_space=pl.ANY)
    scratch = [
        pltpu.VMEM((S, D), bf16),
        pltpu.VMEM((S, D), f32),
        pltpu.VMEM((S // 2, D), u32),
        pltpu.VMEM((NG, (S + 256) // 2 + 64, 128), u32),
        pltpu.VMEM((NB + 1, D // 2, 128), u32),
        pltpu.VMEM((NB + 3, D // 2, 128), u32),
        pltpu.VMEM((S // 2, D), u32),
        pltpu.VMEM((D, D), bf16),
        pltpu.VMEM((D, D), bf16),
        pltpu.VMEM((D, D), bf16),
        pltpu.VMEM((D // 2, D), u32),
        pltpu.VMEM((D // 2, D), u32),
        pltpu.VMEM((D, D), bf16),
        pltpu.VMEM((D // 2, D), u32),
        pltpu.VMEM((1, D), bf16),
        pltpu.VMEM((D, F), bf16),
        pltpu.VMEM((D, F), bf16),
        pltpu.VMEM((F, D), bf16),
        pltpu.VMEM((S, 1), f32),
        pltpu.VMEM((S, 1), f32),
        pltpu.VMEM((S, D), bf16),
        pltpu.VMEM((3, 4, 1, 128), f32),
        pltpu.SMEM((2,), jnp.int32),
        pltpu.VMEM((8, 128), u32),
        pltpu.VMEM((128, 128), f32),
        pltpu.VMEM((D,), bf16),
        pltpu.SemaphoreType.DMA((16,)),
        pltpu.SemaphoreType.DMA((NB + 1,)),
    ]
    scratch += [pltpu.VMEM((4, 256, 128), f32)] * NBUF
    scratch += [pltpu.VMEM((1, 4, 192, 128), u32)] * NBUF
    scratch += [pltpu.VMEM((4, 1, 128), f32)] * NBUF
    out = pl.pallas_call(
        _kernel,
        out_shape=jax.ShapeDtypeStruct((S, D), bf16),
        in_specs=[any_spec] * 7,
        out_specs=any_spec,
        scratch_shapes=scratch,
        compiler_params=pltpu.CompilerParams(vmem_limit_bytes=110 * 1024 * 1024),
    )(x, A_wqkv, A_wo, B_w_r, B_w_gate, B_w_up, B_w_down)
    return out.reshape(1, S, D)
```

```python
import functools
import math

import jax
import jax.numpy as jnp
from jax import lax
import jax.experimental.pallas as pl
import jax.experimental.pallas.tpu as pltpu

S, D, H, DH, F = 2048, 1024, 32, 32, 3584
NB = S // 128
NG = D // 128
NFS = F // 128
EPS = 1e-5
QSCALE = (DH ** -0.5) * math.log2(math.e)
NEC = 2
NBUF = 2
K2_EARLY = 2
XCH = [(0, 256), (256, 256), (512, 512), (1024, 512), (1536, 512)]

bf16 = jnp.bfloat16
f32 = jnp.float32
u32 = jnp.uint32


def _b2u(x):
    return pltpu.bitcast(x, u32)


def _u2b(x):
    return pltpu.bitcast(x, bf16)


def _pack2(a, b):
    w = pltpu.pack_elementwise([a, b], packed_dtype=bf16)
    return w if w.dtype == u32 else pltpu.bitcast(w, u32)


def _pack_adj(x):
    r, c = x.shape
    e = x.reshape(r // 16, 16, c)
    return _pack2(e[:, 0:8, :].reshape(r // 2, c), e[:, 8:16, :].reshape(r // 2, c))


def _kernel(x_hbm, wqkv_hbm, wo_hbm, wr_hbm, wg_hbm, wu_hbm, wd_hbm, out_hbm,
            xin, x_s, xa, k_s, qt_s, vt_s, o_s,
            wk, wq, wv, wqu, wvu, wo, wou, wr, wg, wu, wd,
            r_s, a_s, outb, npad, zs, zv, vraw, wr1, sems, osems, *bufs):
    zs[0] = 0
    zs[1] = 0
    zv[...] = jnp.zeros((8, 128), u32)
    sb = bufs[0:NBUF]
    pb = bufs[NBUF:2 * NBUF]
    lb = bufs[2 * NBUF:3 * NBUF]

    def x_copy(t):
        r0, n = XCH[t]
        return pltpu.make_async_copy(x_hbm.at[pl.ds(r0, n), :], xin.at[pl.ds(r0, n), :], sems.at[t])

    def wk_copy(c):
        return pltpu.make_async_copy(wqkv_hbm.at[:, pl.ds(D + 256 * c, 256)], wk.at[:, pl.ds(256 * c, 256)],
                                     sems.at[12 + c])

    wq_copy = pltpu.make_async_copy(wqkv_hbm.at[:, pl.ds(0, D)], wq, sems.at[5])
    wv_copy = pltpu.make_async_copy(wqkv_hbm.at[:, pl.ds(2 * D, D)], wv, sems.at[6])
    wo_copy = pltpu.make_async_copy(wo_hbm, wo, sems.at[7])
    wr_copy = pltpu.make_async_copy(wr_hbm, wr1, sems.at[8])
    wg_copy = pltpu.make_async_copy(wg_hbm, wg, sems.at[9])
    wu_copy = pltpu.make_async_copy(wu_hbm, wu, sems.at[10])
    wd_copy = pltpu.make_async_copy(wd_hbm, wd, sems.at[11])

    def out_copy(i):
        r0 = pl.multiple_of(i * 128, 128)
        return pltpu.make_async_copy(outb.at[pl.ds(r0, 128), :], out_hbm.at[pl.ds(r0, 128), :], osems.at[i])

    x_copy(0).start()
    wk_copy(0).start()

    ql1 = lax.broadcasted_iota(jnp.int32, (1, 128), 1) & 31
    for ii in range(3):
        for j in range(4):
            t = 256 - (128 * ii + 32 * j) if ii < 2 else 0
            n = max(0, min(256, t) - 32) + jnp.maximum(0, min(32, t) - 1 - ql1)
            npad[ii, j] = n.astype(f32)
    vt_s[0] = jnp.zeros((D // 2, 128), u32)
    vt_s[1] = jnp.zeros((D // 2, 128), u32)

    def kblock(b, g0=0, g1=NG, nb=1):
        static = isinstance(b, int)
        r = b * 64 if static else pl.multiple_of(b * 64, 64)
        xa_t = _u2b(xa[pl.ds(r, 64 * nb), :])
        kk = jnp.dot(xa_t, wk[:, 128 * g0:128 * g1], preferred_element_type=f32)
        kr = 128 + r if static else pl.multiple_of(128 + r, 64)
        toks = []
        for g in range(g0, g1):
            v = _b2u(kk[:, 128 * (g - g0):128 * (g - g0) + 128].astype(bf16))
            k_s[g, pl.ds(kr, 64 * nb), :] = v
            toks.append(v[0:8])
        return toks

    def fill_kpad():
        for g in range(NG):
            lo = k_s[g, 128:129, :] & jnp.uint32(0xFFFF)
            k_s[g, 0:128, :] = jnp.broadcast_to(lo | (lo << 16), (128, 128))

    def gate(v, tok):
        if tok is None:
            return v
        return v + pltpu.bitcast(tok & zv[...], f32)[0:1, 0:v.shape[1]]

    def ln0(b, toks=None):
        base = 128 * b if isinstance(b, int) else pl.multiple_of(128 * b, 128)
        nch = 1 if toks is None else 2
        n = 128 // nch
        for c in range(nch):
            r0 = base + n * c
            x = xin[pl.ds(r0, n), :].astype(f32)
            x_s[pl.ds(r0, n), :] = x
            mu = jnp.mean(x, axis=1, keepdims=True)
            if toks is not None:
                mu = gate(mu, toks[4 * c])
            xc = x - mu
            var = jnp.mean(xc * xc, axis=1, keepdims=True)
            h0 = r0 // 2 if isinstance(b, int) else pl.multiple_of(r0 // 2, n // 2)
            xa[pl.ds(h0, n // 2), :] = _b2u((xc * lax.rsqrt(var + EPS)).astype(bf16))

    def conv(dst, src):
        for j in range(NG):
            dst[64 * j:64 * j + 64, :] = _b2u(src[128 * j:128 * j + 128, :])

    x_copy(0).wait()
    wk_copy(1).start()
    ln0(0)
    ln0(1)
    wk_copy(0).wait()
    x_copy(1).start()
    kblock(0, 0, 2, 2)
    wk_copy(1).wait()
    wk_copy(2).start()
    kblock(0, 2, 4, 2)
    x_copy(1).wait()
    wk_copy(2).wait()
    wk_copy(3).start()
    x_copy(2).start()
    kblock(0, 4, 6, 2)
    ln0(2)
    ln0(3)
    wk_copy(3).wait()
    x_copy(3).start()
    kblock(0, 6, 8, 2)
    kblock(2)

    def pro_body(t, c):
        r0 = pl.multiple_of(512 * (t + 1), 512)
        pltpu.make_async_copy(x_hbm.at[pl.ds(r0, 512), :], xin.at[pl.ds(r0, 512), :], sems.at[t + 2]).wait()

        for b in range(3):
            toks = kblock(4 * t + 3 + b)
            if b == 0:
                ln0(4 * t + 4)
            ln0(4 * t + 5 + b, toks)
        kblock(4 * t + 6)
        return c

    x_copy(4).start()
    wq_copy.start()
    wv_copy.start()
    wo_copy.start()
    wr_copy.start()
    lax.fori_loop(0, 3, pro_body, 0)
    wq_copy.wait()
    wv_copy.wait()
    wo_copy.wait()
    wr_copy.wait()
    kblock(15)
    conv(wqu, wq)
    conv(wvu, wv)
    conv(wou, wo)
    wr[...] = wr1[...].astype(f32).reshape(1, D).astype(bf16)
    fill_kpad()

    def q_slice(xa_blk, q_blk, n):
        lhs = _u2b(xa_blk[...])
        rhs = _u2b(wqu[:, 128 * n:128 * n + 128])
        q = jnp.dot(lhs, rhs, preferred_element_type=f32)
        qt = _b2u((q * QSCALE).astype(bf16).T)
        parts = [qt[0:16]] + [pltpu.roll(qt[16 * h:16 * h + 16], 32 * h, 1) for h in range(1, 4)]
        q_blk[64 * n:64 * n + 64, :] = jnp.concatenate(parts, axis=0)
        return parts[0][0:8]

    def v_slice(xa_blk, vt_blk, n):
        lhs = _u2b(xa_blk[...])
        rhs = _u2b(wvu[:, 128 * n:128 * n + 128])
        v = jnp.dot(lhs, rhs, preferred_element_type=f32)
        vt = _b2u(_u2b(_pack_adj(v)).T)
        vt_blk[64 * n:64 * n + 64, :] = vt
        return vt[0:8]

    def v_raw(xa_blk, n):
        vraw[...] = jnp.dot(_u2b(xa_blk[...]), _u2b(wvu[:, 128 * n:128 * n + 128]), preferred_element_type=f32)

    def v_finish(vt_blk, n):
        vt_blk[64 * n:64 * n + 64, :] = _b2u(_u2b(_pack_adj(vraw[...])).T)

    def o_slice(o_blk, x_blk, n):
        lhs = _u2b(o_blk[...])
        rhs = _u2b(wou[:, 128 * n:128 * n + 128])
        acc = jnp.dot(lhs, rhs, preferred_element_type=f32)
        x_blk[:, 128 * n:128 * n + 128] = x_blk[:, 128 * n:128 * n + 128] + acc
        return pltpu.bitcast(acc[0:8], u32)

    def epi_stats(j, x_blk, c, tok=None):
        r0 = pl.multiple_of(j * 128, 128)
        R = 128 // NEC
        lo = R * c
        x1 = x_blk[lo:lo + R, :]
        mu = gate(jnp.mean(x1, axis=1, keepdims=True), tok)
        xc = x1 - mu
        var = jnp.mean(xc * xc, axis=1, keepdims=True)
        a = lax.rsqrt(var + EPS)
        r = jnp.sum(xc * wr[...].astype(f32), axis=1, keepdims=True) * a
        r_s[pl.ds(r0 + lo, R), :] = r
        a_s[pl.ds(r0 + lo, R), :] = a
        return mu, xc, var, a

    def epi_norm(j, x_blk, xa_blk, layer, c, st, tok=None):
        r0 = pl.multiple_of(j * 128, 128)
        R = 128 // NEC
        lo = R * c
        mu, xc, var, a = st
        a1 = gate(1.0 + a, tok)
        x2 = mu + xc * a1
        if layer == 0:
            x_blk[lo:lo + R, :] = x2
            v = xc * (a1 * lax.rsqrt(var * a1 * a1 + EPS))
            xa_blk[lo // 2:(lo + R) // 2, :] = _b2u(v.astype(bf16))
        else:
            outb[pl.ds(r0 + lo, R), :] = x2.astype(bf16)

    def epilogue(j, x_blk, xa_blk, layer, chunks=range(NEC)):
        for c in chunks:
            epi_norm(j, x_blk, xa_blk, layer, c, epi_stats(j, x_blk, c))

    lane8b = lax.broadcasted_iota(jnp.int32, (8, 128), 1) >> 5
    odd = (lane8b & 1) == 1
    high = lane8b >= 2
    lane16b = lax.broadcasted_iota(jnp.int32, (16, 128), 1) >> 5
    d32 = lax.broadcasted_iota(jnp.int32, (32, 128), 0) - (lax.broadcasted_iota(jnp.int32, (32, 128), 1) & 31)
    umask = d32 > 0

    def stage_a(kv, q_blk, g):
        s_ref = sb[g % NBUF]
        for j in range(4):
            x = jnp.concatenate([jnp.where(lane16b == ((h + j) % 4), q_blk[64 * g + 16 * h:64 * g + 16 * h + 16, :],
                                           jnp.uint32(0)) for h in range(4)], axis=0)
            b0 = 16 * j
            kt = jnp.concatenate([kv[g, b0:b0 + 8, :], kv[g, b0 + 128:b0 + 136, :], kv[g, b0 + 8:b0 + 16, :],
                                  kv[g, b0 + 136:b0 + 144, :], kv[g, b0 + 16:b0 + 128, :]], axis=0)
            st = jnp.dot(_u2b(kt), _u2b(x), preferred_element_type=f32)
            su = jnp.concatenate([st[0:16], st[32:48]], axis=0)
            sl = jnp.concatenate([st[16:32], st[48:64]], axis=0)
            s_ref[j, 0:32, :] = jnp.where(umask, su, sl)
            s_ref[j, 32:256, :] = st[64:288]
            if j == 0:
                tok = (pltpu.bitcast(st[64:72], u32), pltpu.bitcast(st[160:168], u32),
                       pltpu.bitcast(st[280:288], u32))
        return tok

    def bfly(y):
        def sel(m, a, b):
            if a is None and b is None:
                return None
            z = jnp.zeros((8, 128), (a if a is not None else b).dtype)
            return jnp.where(m, z if a is None else a, z if b is None else b)
        r = [sel(odd, y[(k + 1) % 4], y[k]) for k in range(4)]
        wp = [sel(high, r[(k + 2) % 4], r[k]) for k in range(4)]
        return [wp[(-h) % 4] for h in range(4)]

    def stage_b(i, g, toks):
        s_ref = sb[g % NBUF]
        p_ref = pb[g % NBUF].at[zs[0]]
        l_ref = lb[g % NBUF]
        ss = [s_ref[j] for j in range(4)]
        ms = [jnp.max(ss[j], axis=0, keepdims=True) for j in range(4)]
        ls = [None] * 4
        nch = len(toks)
        um16 = [umask[0:16], umask[16:32]]
        for c in range(nch):
            mg = [gate(ms[j], toks[c]) for j in range(4)]
            for M in range(24 * c // nch, 24 * (c + 1) // nch):
                y = []
                for j in range(4):
                    Mp = M - 2 * j
                    if not 0 <= Mp < 18:
                        y.append(None)
                        continue
                    row = 16 * (Mp % 16)
                    p = jnp.exp2(ss[j][row:row + 16] - mg[j])
                    if Mp < 16:
                        ps = p[0:8] + p[8:16]
                        ls[j] = ps if ls[j] is None else ls[j] + ps
                        if Mp == 2:
                            p32 = p[0:1]
                            ls[j] = ls[j] - jnp.where(lax.broadcasted_iota(jnp.int32, (8, 128), 0) == 0,
                                                      npad[jnp.minimum(i, 2), j] * p32, 0.0)
                    if Mp < 2:
                        p = jnp.where(um16[Mp], p, 0.0)
                    elif Mp >= 16:
                        p = jnp.where(um16[Mp - 16], 0.0, p)
                    y.append(_pack2(p[0:8], p[8:16]))
                w = bfly(y)
                for h in range(4):
                    p_ref[h, 8 * M:8 * M + 8, :] = w[h] if w[h] is not None else jnp.zeros((8, 128), u32)
        for j in range(4):
            l_ref[j] = jnp.sum(ls[j], axis=0, keepdims=True)

    def stage_c(vts, o_blk, g):
        p_ref = pb[g % NBUF].at[zs[1]]
        l_ref = lb[g % NBUF]
        lh = bfly([jnp.broadcast_to(1.0 / l_ref[j], (8, 128)) for j in range(4)])
        outs = []
        for h in range(4):
            vt = jnp.concatenate([_u2b(vts[t][64 * g + 16 * h:64 * g + 16 * h + 16, :]) for t in range(3)], axis=1)
            o = jnp.dot(vt, _u2b(p_ref[h]), preferred_element_type=f32)
            o = o * lh[h][0:1]
            if h:
                o = pltpu.roll(o, 128 - 32 * h, 1)
            outs.append(o)
        ot = jnp.concatenate(outs, axis=0)
        o_blk[:, 128 * g:128 * g + 128] = _b2u(ot.T.astype(bf16))

    def attn_body(i, c, has_next, prev, layer, extra=()):
        lo = -1 if prev else 0
        r = pl.multiple_of((i + lo) * 64, 64)
        nblk = (2 if has_next else 1) - lo
        xav = xa.at[pl.ds(r, 64 * nblk), :]
        ov = o_s.at[pl.ds(r, 64 * (1 - lo)), :]
        xv = x_s.at[pl.ds(pl.multiple_of((i + lo) * 128, 128), 128), :]
        qv = qt_s.at[pl.ds(i, 2)]
        vv = vt_s.at[pl.ds(i + lo, 4 - lo)]
        kv = k_s.at[:, pl.ds(pl.multiple_of(i * 64, 64), 256), :]
        blk = lambda v, b: v.at[pl.ds(64 * (b - lo), 64), :]
        vtile = lambda b: vv.at[b - lo]

        qs = [functools.partial(q_slice, blk(xav, 1), qv.at[1], n) for n in range(NG)] if has_next else []
        vs = [functools.partial(v_slice, blk(xav, 1), vtile(3), n) for n in range(NG)] if has_next else []
        if has_next:
            vs[NG - 1] = functools.partial(v_raw, blk(xav, 1), NG - 1)
        if prev:
            v_finish(vtile(2), NG - 1)
        os_ = [functools.partial(o_slice, blk(ov, -1), xv, n) for n in range(NG)] if prev else []
        sl = qs[0:1] + os_ + qs[1:] + vs
        last_o = len(qs[0:1]) + len(os_) - 1 if os_ else -1
        if extra:
            n_it = 2 * NG
            groups = [extra[len(extra) * k // n_it:len(extra) * (k + 1) // n_it] for k in range(n_it)]

            def run(fs):
                for f in fs:
                    f()
            comp = [functools.partial(run, fs) for fs in groups]
            sl = comp[0:1] + sl + comp[1:]
            last_o = NG
        state = {"emitted": 0}
        stats = {}
        if layer == 0:
            esch = [(1, "s", 0, False), (2, "s", 1, True), (4, "n", 0, True), (6, "n", 1, True)]
        else:
            esch = [(1, "s", 0, False), (2, "s", 1, True), (3, "n", 0, True), (5, "n", 1, True)]

        def run_epi(k, tok):
            for (off, kind, ch, paced) in esch:
                if (k is None or off == k) and (kind, ch) not in stats:
                    if kind == "s":
                        stats[kind, ch] = epi_stats(i - 1, xv, ch, tok if paced else None)
                    else:
                        epi_norm(i - 1, xv, blk(xav, -1), layer, ch, stats["s", ch], tok if paced else None)
                        stats[kind, ch] = True

        def dense_one():
            k = state["emitted"]
            if k < len(sl):
                t = sl[k]()
                state["emitted"] += 1
                if prev and k > last_o:
                    run_epi(k - last_o, t)

        for g in range(NG):
            def pv():
                if g >= 1:
                    stage_c([vtile(t) for t in range(3)], blk(ov, 0), g - 1)
                elif prev:
                    stage_c([vtile(t - 1) for t in range(3)], blk(ov, -1), NG - 1)
            if g == 0:
                pv()
            tok = (None, None, None)
            if g + 1 < NG:
                tok = stage_a(kv.at[:, pl.ds(0, 192), :], qv.at[0], g + 1)
            elif has_next:
                tok = stage_a(kv.at[:, pl.ds(64, 192), :], qv.at[1], 0)
            stage_b(i, g, [None, None, tok[0], tok[1]])
            dense_one()
            dense_one()
            if g > 0:
                pv()
            dense_one()
        while state["emitted"] < len(sl):
            dense_one()
        if prev:
            run_epi(None, None)

        if layer == 1 and prev:
            out_copy(i - 1).start()
        if layer == 0 and prev and has_next:
            @pl.when(i == 1)
            def _():
                wg_copy.start()
                wu_copy.start()
                wd_copy.start()
        return c

    def finish_block(j, layer):
        o_blk = o_s.at[pl.ds(pl.multiple_of(j * 64, 64), 64), :]
        x_blk = x_s.at[pl.ds(pl.multiple_of(j * 128, 128), 128), :]
        stage_c([vt_s.at[j + t] for t in range(3)], o_blk, NG - 1)
        for n in range(NG):
            o_slice(o_blk, x_blk, n)
        epilogue(j, x_blk, xa.at[pl.ds(pl.multiple_of(j * 64, 64), 64), :], layer)

    def route(raw):
        def best(r0, n):
            r = r_s[r0:r0 + n, :]
            m = jnp.max(r)
            rows = lax.broadcasted_iota(jnp.int32, (n, 1), 0) + r0
            return m, jnp.min(jnp.where(r == m, rows, S))
        ma, ia = best(0, S - 128)
        mb, ib = best(S - 128, 128)
        rmax = jnp.maximum(ma, mb)
        idx = jnp.where(mb > ma, ib, ia)
        idx = jnp.minimum(idx, S - 1)
        xrow = x_s[pl.ds(idx, 1), :]
        arow = a_s[pl.ds(idx, 1), :]
        mu = jnp.mean(xrow, axis=1, keepdims=True)
        if raw:
            xsel = (xrow - mu) * arow
            xrow = xrow + xsel
        else:
            xsel = (xrow - mu) * (arow / (1.0 + arow))
        xs = jnp.broadcast_to(xsel, (8, D)).astype(bf16)
        return idx, rmax, xrow, xs

    def ffn_steps(xs):
        gates, hid, ys = [], [], []

        def up(c, w, first):
            r = jnp.dot(xs, w[:, 128 * c:128 * (c + 1)], preferred_element_type=f32)
            if first:
                gates.append(r)
            else:
                g_ = gates[c]
                hid.append((g_ * jax.nn.sigmoid(g_) * r).astype(bf16))

        def down(c):
            ys.append(jnp.dot(hid[c], wd[128 * c:128 * (c + 1), :], preferred_element_type=f32))

        steps = []
        for c in range(NFS):
            steps.append(functools.partial(up, c, wg, True))
            steps.append(functools.partial(up, c, wu, False))
            if c >= 1:
                steps.append(functools.partial(down, c - 1))
        steps.append(functools.partial(down, NFS - 1))

        def result():
            y = ys[0]
            for t in ys[1:]:
                y = y + t
            return y
        return steps, result

    def kslice(b, g):
        kblock(b, g, g + 1)

    def ffn_mid():
        kblock(K2_EARLY)
        idx, rmax, xrow, xs = route(raw=False)
        steps, result = ffn_steps(xs)
        fi = 0
        for b in range(K2_EARLY + 1, NB):
            for g in range(NG):
                kslice(b, g)
                if fi < len(steps):
                    steps[fi]()
                    fi += 1
        while fi < len(steps):
            steps[fi]()
            fi += 1
        y = result()
        x_s[pl.ds(idx, 1), :] = xrow + y[0:1, :] * jax.nn.sigmoid(rmax)
        r0 = pl.multiple_of((idx // 16) * 16, 16)
        h0 = pl.multiple_of((idx // 16) * 8, 8)
        x = x_s[pl.ds(r0, 16), :]
        mu = jnp.mean(x, axis=1, keepdims=True)
        xc = x - mu
        var = jnp.mean(xc * xc, axis=1, keepdims=True)
        xn = (xc * lax.rsqrt(var + EPS)).astype(bf16)
        xa[pl.ds(h0, 8), :] = _b2u(xn)
        kk = jnp.dot(xn, wk[...], preferred_element_type=f32)
        for g in range(NG):
            k_s[g, pl.ds(128 + h0, 8), :] = _b2u(kk[:, 128 * g:128 * g + 128].astype(bf16))
        fill_kpad()

    def ffn_last():
        idx, rmax, xrow, xs = route(raw=True)
        steps, result = ffn_steps(xs)
        for f in steps:
            f()
        y = result()
        new = xrow + y[0:1, :] * jax.nn.sigmoid(rmax)
        for i in range(NB):
            out_copy(i).wait()
        b0 = pl.multiple_of((idx // 16) * 16, 16)
        rows = lax.broadcasted_iota(jnp.int32, (16, D), 0) + b0
        outb[pl.ds(b0, 16), :] = jnp.where(rows == idx, new, outb[pl.ds(b0, 16), :].astype(f32)).astype(bf16)
        fix = pltpu.make_async_copy(outb.at[pl.ds(b0, 16), :], out_hbm.at[pl.ds(b0, 16), :], osems.at[NB])
        fix.start()
        fix.wait()

    for layer in range(2):
        for n in range(NG):
            q_slice(xa.at[pl.ds(0, 64), :], qt_s.at[0], n)
        for n in range(NG):
            v_slice(xa.at[pl.ds(0, 64), :], vt_s.at[2], n)
        stage_a(k_s.at[:, pl.ds(0, 192), :], qt_s.at[0], 0)
        attn_body(0, 0, has_next=True, prev=False, layer=layer)
        lax.fori_loop(1, NB - 1, functools.partial(attn_body, has_next=True, prev=True, layer=layer), 0)
        extra = [functools.partial(kslice, b, g) for b in range(K2_EARLY) for g in range(NG)] if layer == 0 else ()
        attn_body(NB - 1, 0, has_next=False, prev=True, layer=layer, extra=extra)
        finish_block(NB - 1, layer)
        if layer == 0:
            wg_copy.wait()
            wu_copy.wait()
            wd_copy.wait()
            ffn_mid()
        else:
            out_copy(NB - 1).start()
            ffn_last()


@jax.jit
def pallas_interleave_layers__sliding_block__moe_arch_mod__prompt_kernel(
    A_x: jax.Array,
    A_wqkv: jax.Array,
    A_wo: jax.Array,
    B_x: jax.Array,
    B_w_r: jax.Array,
    B_w_gate: jax.Array,
    B_w_up: jax.Array,
    B_w_down: jax.Array,
):
    del B_x
    x = A_x.reshape(S, D)
    any_spec = pl.BlockSpec(memory_space=pl.ANY)
    scratch = [
        pltpu.VMEM((S, D), bf16),
        pltpu.VMEM((S, D), f32),
        pltpu.VMEM((S // 2, D), u32),
        pltpu.VMEM((NG, (S + 256) // 2 + 64, 128), u32),
        pltpu.VMEM((NB + 1, D // 2, 128), u32),
        pltpu.VMEM((NB + 3, D // 2, 128), u32),
        pltpu.VMEM((S // 2, D), u32),
        pltpu.VMEM((D, D), bf16),
        pltpu.VMEM((D, D), bf16),
        pltpu.VMEM((D, D), bf16),
        pltpu.VMEM((D // 2, D), u32),
        pltpu.VMEM((D // 2, D), u32),
        pltpu.VMEM((D, D), bf16),
        pltpu.VMEM((D // 2, D), u32),
        pltpu.VMEM((1, D), bf16),
        pltpu.VMEM((D, F), bf16),
        pltpu.VMEM((D, F), bf16),
        pltpu.VMEM((F, D), bf16),
        pltpu.VMEM((S, 1), f32),
        pltpu.VMEM((S, 1), f32),
        pltpu.VMEM((S, D), bf16),
        pltpu.VMEM((3, 4, 1, 128), f32),
        pltpu.SMEM((2,), jnp.int32),
        pltpu.VMEM((8, 128), u32),
        pltpu.VMEM((128, 128), f32),
        pltpu.VMEM((D,), bf16),
        pltpu.SemaphoreType.DMA((16,)),
        pltpu.SemaphoreType.DMA((NB + 1,)),
    ]
    scratch += [pltpu.VMEM((4, 256, 128), f32)] * NBUF
    scratch += [pltpu.VMEM((1, 4, 192, 128), u32)] * NBUF
    scratch += [pltpu.VMEM((4, 1, 128), f32)] * NBUF
    out = pl.pallas_call(
        _kernel,
        out_shape=jax.ShapeDtypeStruct((S, D), bf16),
        in_specs=[any_spec] * 7,
        out_specs=any_spec,
        scratch_shapes=scratch,
        compiler_params=pltpu.CompilerParams(vmem_limit_bytes=110 * 1024 * 1024),
    )(x, A_wqkv, A_wo, B_w_r, B_w_gate, B_w_up, B_w_down)
    return out.reshape(1, S, D)
```

```python
import functools
import math

import jax
import jax.numpy as jnp
from jax import lax
import jax.experimental.pallas as pl
import jax.experimental.pallas.tpu as pltpu

S, D, H, DH, F = 2048, 1024, 32, 32, 3584
NB = S // 128
NG = D // 128
NFS = F // 128
EPS = 1e-5
QSCALE = (DH ** -0.5) * math.log2(math.e)
NEC = 2
NBUF = 2
K2_EARLY = 2
XCH = [(0, 256), (256, 256), (512, 128), (640, 512), (1152, 512), (1664, 384)]

bf16 = jnp.bfloat16
f32 = jnp.float32
u32 = jnp.uint32


def _b2u(x):
    return pltpu.bitcast(x, u32)


def _u2b(x):
    return pltpu.bitcast(x, bf16)


def _pack2(a, b):
    w = pltpu.pack_elementwise([a, b], packed_dtype=bf16)
    return w if w.dtype == u32 else pltpu.bitcast(w, u32)


def _pack_adj(x):
    r, c = x.shape
    e = x.reshape(r // 16, 16, c)
    return _pack2(e[:, 0:8, :].reshape(r // 2, c), e[:, 8:16, :].reshape(r // 2, c))


def _kernel(x_hbm, wqkv_hbm, wo_hbm, wr_hbm, wg_hbm, wu_hbm, wd_hbm, out_hbm,
            xin, x_s, xa, k_s, qt_s, vt_s, o_s,
            wk, wq, wv, wqu, wvu, wo, wou, wr, wg, wu, wd,
            r_s, a_s, outb, npad, zs, zv, vraw, wr1, sems, osems, *bufs):
    zs[0] = 0
    zs[1] = 0
    zv[...] = jnp.zeros((8, 128), u32)
    sb = bufs[0:NBUF]
    pb = bufs[NBUF:2 * NBUF]
    lb = bufs[2 * NBUF:3 * NBUF]

    def x_copy(t):
        r0, n = XCH[t]
        return pltpu.make_async_copy(x_hbm.at[pl.ds(r0, n), :], xin.at[pl.ds(r0, n), :], sems.at[16 + t])

    def wk_copy(c):
        return pltpu.make_async_copy(wqkv_hbm.at[:, pl.ds(D + 256 * c, 256)], wk.at[:, pl.ds(256 * c, 256)],
                                     sems.at[12 + c])

    wq_copy = pltpu.make_async_copy(wqkv_hbm.at[:, pl.ds(0, D)], wq, sems.at[5])
    wv_copy = pltpu.make_async_copy(wqkv_hbm.at[:, pl.ds(2 * D, D)], wv, sems.at[6])
    wo_copy = pltpu.make_async_copy(wo_hbm, wo, sems.at[7])
    wr_copy = pltpu.make_async_copy(wr_hbm, wr1, sems.at[8])
    wg_copy = pltpu.make_async_copy(wg_hbm, wg, sems.at[9])
    wu_copy = pltpu.make_async_copy(wu_hbm, wu, sems.at[10])
    wd_copy = pltpu.make_async_copy(wd_hbm, wd, sems.at[11])

    def out_copy(i):
        r0 = pl.multiple_of(i * 128, 128)
        return pltpu.make_async_copy(outb.at[pl.ds(r0, 128), :], out_hbm.at[pl.ds(r0, 128), :], osems.at[i])

    x_copy(0).start()
    wk_copy(0).start()

    ql1 = lax.broadcasted_iota(jnp.int32, (1, 128), 1) & 31
    for ii in range(3):
        for j in range(4):
            t = 256 - (128 * ii + 32 * j) if ii < 2 else 0
            n = max(0, min(256, t) - 32) + jnp.maximum(0, min(32, t) - 1 - ql1)
            npad[ii, j] = n.astype(f32)
    vt_s[0] = jnp.zeros((D // 2, 128), u32)
    vt_s[1] = jnp.zeros((D // 2, 128), u32)

    def kblock(b, g0=0, g1=NG, nb=1):
        static = isinstance(b, int)
        r = b * 64 if static else pl.multiple_of(b * 64, 64)
        xa_t = _u2b(xa[pl.ds(r, 64 * nb), :])
        kk = jnp.dot(xa_t, wk[:, 128 * g0:128 * g1], preferred_element_type=f32)
        kr = 128 + r if static else pl.multiple_of(128 + r, 64)
        toks = []
        for g in range(g0, g1):
            v = _b2u(kk[:, 128 * (g - g0):128 * (g - g0) + 128].astype(bf16))
            k_s[g, pl.ds(kr, 64 * nb), :] = v
            toks.append(v[0:8])
        return toks

    def fill_kpad():
        for g in range(NG):
            lo = k_s[g, 128:129, :] & jnp.uint32(0xFFFF)
            k_s[g, 0:128, :] = jnp.broadcast_to(lo | (lo << 16), (128, 128))

    def gate(v, tok):
        if tok is None:
            return v
        return v + pltpu.bitcast(tok & zv[...], f32)[0:1, 0:v.shape[1]]

    def ln0(b, toks=None):
        base = 128 * b if isinstance(b, int) else pl.multiple_of(128 * b, 128)
        nch = 1 if toks is None else 2
        n = 128 // nch
        for c in range(nch):
            r0 = base + n * c
            x = xin[pl.ds(r0, n), :].astype(f32)
            x_s[pl.ds(r0, n), :] = x
            mu = jnp.mean(x, axis=1, keepdims=True)
            if toks is not None:
                mu = gate(mu, toks[4 * c])
            xc = x - mu
            var = jnp.mean(xc * xc, axis=1, keepdims=True)
            h0 = r0 // 2 if isinstance(b, int) else pl.multiple_of(r0 // 2, n // 2)
            xa[pl.ds(h0, n // 2), :] = _b2u((xc * lax.rsqrt(var + EPS)).astype(bf16))

    def conv(dst, src):
        for j in range(NG):
            dst[64 * j:64 * j + 64, :] = _b2u(src[128 * j:128 * j + 128, :])

    x_copy(0).wait()
    x_copy(1).start()
    ln0(0)
    ln0(1)
    wk_copy(0).wait()
    wk_copy(1).start()
    kblock(0, 0, 2, 2)
    x_copy(1).wait()
    wk_copy(2).start()
    ln0(2)
    kblock(2, 0, 2)
    ln0(3)
    wk_copy(1).wait()
    wk_copy(3).start()
    kblock(0, 2, 4, 3)
    wk_copy(2).wait()
    x_copy(2).start()
    x_copy(3).start()
    kblock(0, 4, 6, 3)
    wk_copy(3).wait()
    x_copy(2).wait()
    x_copy(4).start()
    kblock(0, 6, 8, 3)
    ln0(4)

    def pro_body(t, c):
        @pl.when(t == 0)
        def _():
            x_copy(3).wait()

        @pl.when(t == 1)
        def _():
            x_copy(4).wait()

        @pl.when(t == 2)
        def _():
            x_copy(5).wait()

        for b in range(4):
            toks = kblock(4 * t + 3 + b)
            ln0(jnp.minimum(4 * t + 5 + b, NB - 1), toks)
        return c

    x_copy(5).start()
    wq_copy.start()
    wv_copy.start()
    wo_copy.start()
    wr_copy.start()
    lax.fori_loop(0, 3, pro_body, 0)
    wq_copy.wait()
    wv_copy.wait()
    wo_copy.wait()
    wr_copy.wait()
    kblock(15)
    conv(wqu, wq)
    conv(wvu, wv)
    conv(wou, wo)
    wr[...] = wr1[...].astype(f32).reshape(1, D).astype(bf16)
    fill_kpad()

    def q_slice(xa_blk, q_blk, n):
        lhs = _u2b(xa_blk[...])
        rhs = _u2b(wqu[:, 128 * n:128 * n + 128])
        q = jnp.dot(lhs, rhs, preferred_element_type=f32)
        qt = _b2u((q * QSCALE).astype(bf16).T)
        parts = [qt[0:16]] + [pltpu.roll(qt[16 * h:16 * h + 16], 32 * h, 1) for h in range(1, 4)]
        q_blk[64 * n:64 * n + 64, :] = jnp.concatenate(parts, axis=0)
        return parts[0][0:8]

    def v_slice(xa_blk, vt_blk, n):
        lhs = _u2b(xa_blk[...])
        rhs = _u2b(wvu[:, 128 * n:128 * n + 128])
        v = jnp.dot(lhs, rhs, preferred_element_type=f32)
        vt = _b2u(_u2b(_pack_adj(v)).T)
        vt_blk[64 * n:64 * n + 64, :] = vt
        return vt[0:8]

    def v_raw(xa_blk, n):
        vraw[...] = jnp.dot(_u2b(xa_blk[...]), _u2b(wvu[:, 128 * n:128 * n + 128]), preferred_element_type=f32)

    def v_finish(vt_blk, n):
        vt_blk[64 * n:64 * n + 64, :] = _b2u(_u2b(_pack_adj(vraw[...])).T)

    def o_slice(o_blk, x_blk, n):
        lhs = _u2b(o_blk[...])
        rhs = _u2b(wou[:, 128 * n:128 * n + 128])
        acc = jnp.dot(lhs, rhs, preferred_element_type=f32)
        x_blk[:, 128 * n:128 * n + 128] = x_blk[:, 128 * n:128 * n + 128] + acc
        return pltpu.bitcast(acc[0:8], u32)

    def epi_stats(j, x_blk, c, tok=None):
        r0 = pl.multiple_of(j * 128, 128)
        R = 128 // NEC
        lo = R * c
        x1 = x_blk[lo:lo + R, :]
        mu = gate(jnp.mean(x1, axis=1, keepdims=True), tok)
        xc = x1 - mu
        var = jnp.mean(xc * xc, axis=1, keepdims=True)
        a = lax.rsqrt(var + EPS)
        r = jnp.sum(xc * wr[...].astype(f32), axis=1, keepdims=True) * a
        r_s[pl.ds(r0 + lo, R), :] = r
        a_s[pl.ds(r0 + lo, R), :] = a
        return mu, xc, var, a

    def epi_norm(j, x_blk, xa_blk, layer, c, st, tok=None):
        r0 = pl.multiple_of(j * 128, 128)
        R = 128 // NEC
        lo = R * c
        mu, xc, var, a = st
        a1 = gate(1.0 + a, tok)
        x2 = mu + xc * a1
        if layer == 0:
            x_blk[lo:lo + R, :] = x2
            v = xc * (a1 * lax.rsqrt(var * a1 * a1 + EPS))
            xa_blk[lo // 2:(lo + R) // 2, :] = _b2u(v.astype(bf16))
        else:
            outb[pl.ds(r0 + lo, R), :] = x2.astype(bf16)

    def epilogue(j, x_blk, xa_blk, layer, chunks=range(NEC)):
        for c in chunks:
            epi_norm(j, x_blk, xa_blk, layer, c, epi_stats(j, x_blk, c))

    lane8b = lax.broadcasted_iota(jnp.int32, (8, 128), 1) >> 5
    odd = (lane8b & 1) == 1
    high = lane8b >= 2
    lane16b = lax.broadcasted_iota(jnp.int32, (16, 128), 1) >> 5
    d32 = lax.broadcasted_iota(jnp.int32, (32, 128), 0) - (lax.broadcasted_iota(jnp.int32, (32, 128), 1) & 31)
    umask = d32 > 0

    def stage_a(kv, q_blk, g):
        s_ref = sb[g % NBUF]
        for j in range(4):
            x = jnp.concatenate([jnp.where(lane16b == ((h + j) % 4), q_blk[64 * g + 16 * h:64 * g + 16 * h + 16, :],
                                           jnp.uint32(0)) for h in range(4)], axis=0)
            b0 = 16 * j
            kt = jnp.concatenate([kv[g, b0:b0 + 8, :], kv[g, b0 + 128:b0 + 136, :], kv[g, b0 + 8:b0 + 16, :],
                                  kv[g, b0 + 136:b0 + 144, :], kv[g, b0 + 16:b0 + 128, :]], axis=0)
            st = jnp.dot(_u2b(kt), _u2b(x), preferred_element_type=f32)
            su = jnp.concatenate([st[0:16], st[32:48]], axis=0)
            sl = jnp.concatenate([st[16:32], st[48:64]], axis=0)
            s_ref[j, 0:32, :] = jnp.where(umask, su, sl)
            s_ref[j, 32:256, :] = st[64:288]
            if j == 0:
                tok = (pltpu.bitcast(st[64:72], u32), pltpu.bitcast(st[160:168], u32),
                       pltpu.bitcast(st[280:288], u32))
        return tok

    def bfly(y):
        def sel(m, a, b):
            if a is None and b is None:
                return None
            z = jnp.zeros((8, 128), (a if a is not None else b).dtype)
            return jnp.where(m, z if a is None else a, z if b is None else b)
        r = [sel(odd, y[(k + 1) % 4], y[k]) for k in range(4)]
        wp = [sel(high, r[(k + 2) % 4], r[k]) for k in range(4)]
        return [wp[(-h) % 4] for h in range(4)]

    def stage_b(i, g, toks):
        s_ref = sb[g % NBUF]
        p_ref = pb[g % NBUF].at[zs[0]]
        l_ref = lb[g % NBUF]
        ss = [s_ref[j] for j in range(4)]
        ms = [jnp.max(ss[j], axis=0, keepdims=True) for j in range(4)]
        ls = [None] * 4
        nch = len(toks)
        um16 = [umask[0:16], umask[16:32]]
        for c in range(nch):
            mg = [gate(ms[j], toks[c]) for j in range(4)]
            for M in range(24 * c // nch, 24 * (c + 1) // nch):
                y = []
                for j in range(4):
                    Mp = M - 2 * j
                    if not 0 <= Mp < 18:
                        y.append(None)
                        continue
                    row = 16 * (Mp % 16)
                    p = jnp.exp2(ss[j][row:row + 16] - mg[j])
                    if Mp < 16:
                        ps = p[0:8] + p[8:16]
                        ls[j] = ps if ls[j] is None else ls[j] + ps
                        if Mp == 2:
                            p32 = p[0:1]
                            ls[j] = ls[j] - jnp.where(lax.broadcasted_iota(jnp.int32, (8, 128), 0) == 0,
                                                      npad[jnp.minimum(i, 2), j] * p32, 0.0)
                    if Mp < 2:
                        p = jnp.where(um16[Mp], p, 0.0)
                    elif Mp >= 16:
                        p = jnp.where(um16[Mp - 16], 0.0, p)
                    y.append(_pack2(p[0:8], p[8:16]))
                w = bfly(y)
                for h in range(4):
                    p_ref[h, 8 * M:8 * M + 8, :] = w[h] if w[h] is not None else jnp.zeros((8, 128), u32)
        for j in range(4):
            l_ref[j] = jnp.sum(ls[j], axis=0, keepdims=True)

    def stage_c(vts, o_blk, g):
        p_ref = pb[g % NBUF].at[zs[1]]
        l_ref = lb[g % NBUF]
        lh = bfly([jnp.broadcast_to(1.0 / l_ref[j], (8, 128)) for j in range(4)])
        outs = []
        for h in range(4):
            vt = jnp.concatenate([_u2b(vts[t][64 * g + 16 * h:64 * g + 16 * h + 16, :]) for t in range(3)], axis=1)
            o = jnp.dot(vt, _u2b(p_ref[h]), preferred_element_type=f32)
            o = o * lh[h][0:1]
            if h:
                o = pltpu.roll(o, 128 - 32 * h, 1)
            outs.append(o)
        ot = jnp.concatenate(outs, axis=0)
        o_blk[:, 128 * g:128 * g + 128] = _b2u(ot.T.astype(bf16))

    def attn_body(i, c, has_next, prev, layer, extra=()):
        lo = -1 if prev else 0
        r = pl.multiple_of((i + lo) * 64, 64)
        nblk = (2 if has_next else 1) - lo
        xav = xa.at[pl.ds(r, 64 * nblk), :]
        ov = o_s.at[pl.ds(r, 64 * (1 - lo)), :]
        xv = x_s.at[pl.ds(pl.multiple_of((i + lo) * 128, 128), 128), :]
        qv = qt_s.at[pl.ds(i, 2)]
        vv = vt_s.at[pl.ds(i + lo, 4 - lo)]
        kv = k_s.at[:, pl.ds(pl.multiple_of(i * 64, 64), 256), :]
        blk = lambda v, b: v.at[pl.ds(64 * (b - lo), 64), :]
        vtile = lambda b: vv.at[b - lo]

        qs = [functools.partial(q_slice, blk(xav, 1), qv.at[1], n) for n in range(NG)] if has_next else []
        vs = [functools.partial(v_slice, blk(xav, 1), vtile(3), n) for n in range(NG)] if has_next else []
        if has_next:
            vs[NG - 1] = functools.partial(v_raw, blk(xav, 1), NG - 1)
        if prev:
            v_finish(vtile(2), NG - 1)
        os_ = [functools.partial(o_slice, blk(ov, -1), xv, n) for n in range(NG)] if prev else []
        sl = qs[0:1] + os_ + qs[1:] + vs
        last_o = len(qs[0:1]) + len(os_) - 1 if os_ else -1
        if extra:
            n_it = 2 * NG
            groups = [extra[len(extra) * k // n_it:len(extra) * (k + 1) // n_it] for k in range(n_it)]

            def run(fs):
                for f in fs:
                    f()
            comp = [functools.partial(run, fs) for fs in groups]
            sl = comp[0:1] + sl + comp[1:]
            last_o = NG
        state = {"emitted": 0}
        stats = {}
        if layer == 0:
            esch = [(1, "s", 0, False), (2, "s", 1, True), (4, "n", 0, True), (6, "n", 1, True)]
        else:
            esch = [(1, "s", 0, False), (2, "s", 1, True), (3, "n", 0, True), (5, "n", 1, True)]

        def run_epi(k, tok):
            for (off, kind, ch, paced) in esch:
                if (k is None or off == k) and (kind, ch) not in stats:
                    if kind == "s":
                        stats[kind, ch] = epi_stats(i - 1, xv, ch, tok if paced else None)
                    else:
                        epi_norm(i - 1, xv, blk(xav, -1), layer, ch, stats["s", ch], tok if paced else None)
                        stats[kind, ch] = True

        def dense_one():
            k = state["emitted"]
            if k < len(sl):
                t = sl[k]()
                state["emitted"] += 1
                if prev and k > last_o:
                    run_epi(k - last_o, t)

        for g in range(NG):
            def pv():
                if g >= 1:
                    stage_c([vtile(t) for t in range(3)], blk(ov, 0), g - 1)
                elif prev:
                    stage_c([vtile(t - 1) for t in range(3)], blk(ov, -1), NG - 1)
            if g == 0:
                pv()
            tok = (None, None, None)
            if g + 1 < NG:
                tok = stage_a(kv.at[:, pl.ds(0, 192), :], qv.at[0], g + 1)
            elif has_next:
                tok = stage_a(kv.at[:, pl.ds(64, 192), :], qv.at[1], 0)
            stage_b(i, g, [None, None, tok[0], tok[1]])
            dense_one()
            dense_one()
            if g > 0:
                pv()
            dense_one()
        while state["emitted"] < len(sl):
            dense_one()
        if prev:
            run_epi(None, None)

        if layer == 1 and prev:
            out_copy(i - 1).start()
        if layer == 0 and prev and has_next:
            @pl.when(i == 1)
            def _():
                wg_copy.start()
                wu_copy.start()
                wd_copy.start()
        return c

    def finish_block(j, layer):
        o_blk = o_s.at[pl.ds(pl.multiple_of(j * 64, 64), 64), :]
        x_blk = x_s.at[pl.ds(pl.multiple_of(j * 128, 128), 128), :]
        stage_c([vt_s.at[j + t] for t in range(3)], o_blk, NG - 1)
        for n in range(NG):
            o_slice(o_blk, x_blk, n)
        epilogue(j, x_blk, xa.at[pl.ds(pl.multiple_of(j * 64, 64), 64), :], layer)

    def route(raw):
        def best(r0, n):
            r = r_s[r0:r0 + n, :]
            m = jnp.max(r)
            rows = lax.broadcasted_iota(jnp.int32, (n, 1), 0) + r0
            return m, jnp.min(jnp.where(r == m, rows, S))
        ma, ia = best(0, S - 128)
        mb, ib = best(S - 128, 128)
        rmax = jnp.maximum(ma, mb)
        idx = jnp.where(mb > ma, ib, ia)
        idx = jnp.minimum(idx, S - 1)
        xrow = x_s[pl.ds(idx, 1), :]
        arow = a_s[pl.ds(idx, 1), :]
        mu = jnp.mean(xrow, axis=1, keepdims=True)
        if raw:
            xsel = (xrow - mu) * arow
            xrow = xrow + xsel
        else:
            xsel = (xrow - mu) * (arow / (1.0 + arow))
        xs = jnp.broadcast_to(xsel, (8, D)).astype(bf16)
        return idx, rmax, xrow, xs

    def ffn_steps(xs):
        gates, hid, ys = [], [], []

        def up(c, w, first):
            r = jnp.dot(xs, w[:, 128 * c:128 * (c + 1)], preferred_element_type=f32)
            if first:
                gates.append(r)
            else:
                g_ = gates[c]
                hid.append((g_ * jax.nn.sigmoid(g_) * r).astype(bf16))

        def down(c):
            ys.append(jnp.dot(hid[c], wd[128 * c:128 * (c + 1), :], preferred_element_type=f32))

        steps = []
        for c in range(NFS):
            steps.append(functools.partial(up, c, wg, True))
            steps.append(functools.partial(up, c, wu, False))
            if c >= 1:
                steps.append(functools.partial(down, c - 1))
        steps.append(functools.partial(down, NFS - 1))

        def result():
            y = ys[0]
            for t in ys[1:]:
                y = y + t
            return y
        return steps, result

    def kslice(b, g):
        kblock(b, g, g + 1)

    def ffn_mid():
        kblock(K2_EARLY)
        idx, rmax, xrow, xs = route(raw=False)
        steps, result = ffn_steps(xs)
        fi = 0
        for b in range(K2_EARLY + 1, NB):
            for g in range(NG):
                kslice(b, g)
                if fi < len(steps):
                    steps[fi]()
                    fi += 1
        while fi < len(steps):
            steps[fi]()
            fi += 1
        y = result()
        x_s[pl.ds(idx, 1), :] = xrow + y[0:1, :] * jax.nn.sigmoid(rmax)
        r0 = pl.multiple_of((idx // 16) * 16, 16)
        h0 = pl.multiple_of((idx // 16) * 8, 8)
        x = x_s[pl.ds(r0, 16), :]
        mu = jnp.mean(x, axis=1, keepdims=True)
        xc = x - mu
        var = jnp.mean(xc * xc, axis=1, keepdims=True)
        xn = (xc * lax.rsqrt(var + EPS)).astype(bf16)
        xa[pl.ds(h0, 8), :] = _b2u(xn)
        kk = jnp.dot(xn, wk[...], preferred_element_type=f32)
        for g in range(NG):
            k_s[g, pl.ds(128 + h0, 8), :] = _b2u(kk[:, 128 * g:128 * g + 128].astype(bf16))
        fill_kpad()

    def ffn_last():
        idx, rmax, xrow, xs = route(raw=True)
        steps, result = ffn_steps(xs)
        for f in steps:
            f()
        y = result()
        new = xrow + y[0:1, :] * jax.nn.sigmoid(rmax)
        for i in range(NB):
            out_copy(i).wait()
        b0 = pl.multiple_of((idx // 16) * 16, 16)
        rows = lax.broadcasted_iota(jnp.int32, (16, D), 0) + b0
        outb[pl.ds(b0, 16), :] = jnp.where(rows == idx, new, outb[pl.ds(b0, 16), :].astype(f32)).astype(bf16)
        fix = pltpu.make_async_copy(outb.at[pl.ds(b0, 16), :], out_hbm.at[pl.ds(b0, 16), :], osems.at[NB])
        fix.start()
        fix.wait()

    for layer in range(2):
        for n in range(NG):
            q_slice(xa.at[pl.ds(0, 64), :], qt_s.at[0], n)
        for n in range(NG):
            v_slice(xa.at[pl.ds(0, 64), :], vt_s.at[2], n)
        stage_a(k_s.at[:, pl.ds(0, 192), :], qt_s.at[0], 0)
        attn_body(0, 0, has_next=True, prev=False, layer=layer)
        lax.fori_loop(1, NB - 1, functools.partial(attn_body, has_next=True, prev=True, layer=layer), 0)
        extra = [functools.partial(kslice, b, g) for b in range(K2_EARLY) for g in range(NG)] if layer == 0 else ()
        attn_body(NB - 1, 0, has_next=False, prev=True, layer=layer, extra=extra)
        finish_block(NB - 1, layer)
        if layer == 0:
            wg_copy.wait()
            wu_copy.wait()
            wd_copy.wait()
            ffn_mid()
        else:
            out_copy(NB - 1).start()
            ffn_last()


@jax.jit
def pallas_interleave_layers__sliding_block__moe_arch_mod__prompt_kernel(
    A_x: jax.Array,
    A_wqkv: jax.Array,
    A_wo: jax.Array,
    B_x: jax.Array,
    B_w_r: jax.Array,
    B_w_gate: jax.Array,
    B_w_up: jax.Array,
    B_w_down: jax.Array,
):
    del B_x
    x = A_x.reshape(S, D)
    any_spec = pl.BlockSpec(memory_space=pl.ANY)
    scratch = [
        pltpu.VMEM((S, D), bf16),
        pltpu.VMEM((S, D), f32),
        pltpu.VMEM((S // 2, D), u32),
        pltpu.VMEM((NG, (S + 256) // 2 + 64, 128), u32),
        pltpu.VMEM((NB + 1, D // 2, 128), u32),
        pltpu.VMEM((NB + 3, D // 2, 128), u32),
        pltpu.VMEM((S // 2, D), u32),
        pltpu.VMEM((D, D), bf16),
        pltpu.VMEM((D, D), bf16),
        pltpu.VMEM((D, D), bf16),
        pltpu.VMEM((D // 2, D), u32),
        pltpu.VMEM((D // 2, D), u32),
        pltpu.VMEM((D, D), bf16),
        pltpu.VMEM((D // 2, D), u32),
        pltpu.VMEM((1, D), bf16),
        pltpu.VMEM((D, F), bf16),
        pltpu.VMEM((D, F), bf16),
        pltpu.VMEM((F, D), bf16),
        pltpu.VMEM((S, 1), f32),
        pltpu.VMEM((S, 1), f32),
        pltpu.VMEM((S, D), bf16),
        pltpu.VMEM((3, 4, 1, 128), f32),
        pltpu.SMEM((2,), jnp.int32),
        pltpu.VMEM((8, 128), u32),
        pltpu.VMEM((128, 128), f32),
        pltpu.VMEM((D,), bf16),
        pltpu.SemaphoreType.DMA((22,)),
        pltpu.SemaphoreType.DMA((NB + 1,)),
    ]
    scratch += [pltpu.VMEM((4, 256, 128), f32)] * NBUF
    scratch += [pltpu.VMEM((1, 4, 192, 128), u32)] * NBUF
    scratch += [pltpu.VMEM((4, 1, 128), f32)] * NBUF
    out = pl.pallas_call(
        _kernel,
        out_shape=jax.ShapeDtypeStruct((S, D), bf16),
        in_specs=[any_spec] * 7,
        out_specs=any_spec,
        scratch_shapes=scratch,
        compiler_params=pltpu.CompilerParams(vmem_limit_bytes=110 * 1024 * 1024),
    )(x, A_wqkv, A_wo, B_w_r, B_w_gate, B_w_up, B_w_down)
    return out.reshape(1, S, D)
```

```python
import functools
import math

import jax
import jax.numpy as jnp
from jax import lax
import jax.experimental.pallas as pl
import jax.experimental.pallas.tpu as pltpu

S, D, H, DH, F = 2048, 1024, 32, 32, 3584
NB = S // 128
NG = D // 128
NFS = F // 128
EPS = 1e-5
QSCALE = (DH ** -0.5) * math.log2(math.e)
NEC = 2
NBUF = 2
K2_EARLY = 2
XCH = [(0, 256), (256, 256), (512, 128), (640, 512), (1152, 512), (1664, 384)]

bf16 = jnp.bfloat16
f32 = jnp.float32
u32 = jnp.uint32


def _b2u(x):
    return pltpu.bitcast(x, u32)


def _u2b(x):
    return pltpu.bitcast(x, bf16)


def _pack2(a, b):
    w = pltpu.pack_elementwise([a, b], packed_dtype=bf16)
    return w if w.dtype == u32 else pltpu.bitcast(w, u32)


def _pack_adj(x):
    r, c = x.shape
    e = x.reshape(r // 16, 16, c)
    return _pack2(e[:, 0:8, :].reshape(r // 2, c), e[:, 8:16, :].reshape(r // 2, c))


def _kernel(x_hbm, wqkv_hbm, wo_hbm, wr_hbm, wg_hbm, wu_hbm, wd_hbm, out_hbm,
            xin, x_s, xa, k_s, qt_s, vt_s, o_s,
            wk, wq, wv, wqu, wvu, wo, wou, wr, wg, wu, wd,
            r_s, a_s, outb, npad, zs, zv, vraw, wr1, sems, osems, *bufs):
    zs[0] = 0
    zs[1] = 0
    zv[...] = jnp.zeros((8, 128), u32)
    sb = bufs[0:NBUF]
    pb = bufs[NBUF:2 * NBUF]
    lb = bufs[2 * NBUF:3 * NBUF]

    def x_copy(t):
        r0, n = XCH[t]
        return pltpu.make_async_copy(x_hbm.at[pl.ds(r0, n), :], xin.at[pl.ds(r0, n), :], sems.at[16 + t])

    def wk_copy(c):
        return pltpu.make_async_copy(wqkv_hbm.at[:, pl.ds(D + 256 * c, 256)], wk.at[:, pl.ds(256 * c, 256)],
                                     sems.at[12 + c])

    wq_copy = pltpu.make_async_copy(wqkv_hbm.at[:, pl.ds(0, D)], wq, sems.at[5])
    wv_copy = pltpu.make_async_copy(wqkv_hbm.at[:, pl.ds(2 * D, D)], wv, sems.at[6])
    wo_copy = pltpu.make_async_copy(wo_hbm, wo, sems.at[7])
    wr_copy = pltpu.make_async_copy(wr_hbm, wr1, sems.at[8])
    wg_copy = pltpu.make_async_copy(wg_hbm, wg, sems.at[9])
    wu_copy = pltpu.make_async_copy(wu_hbm, wu, sems.at[10])
    wd_copy = pltpu.make_async_copy(wd_hbm, wd, sems.at[11])

    def out_copy(i):
        r0 = pl.multiple_of(i * 128, 128)
        return pltpu.make_async_copy(outb.at[pl.ds(r0, 128), :], out_hbm.at[pl.ds(r0, 128), :], osems.at[i])

    x_copy(0).start()
    wk_copy(0).start()

    ql1 = lax.broadcasted_iota(jnp.int32, (1, 128), 1) & 31
    for ii in range(3):
        for j in range(4):
            t = 256 - (128 * ii + 32 * j) if ii < 2 else 0
            n = max(0, min(256, t) - 32) + jnp.maximum(0, min(32, t) - 1 - ql1)
            npad[ii, j] = n.astype(f32)
    vt_s[0] = jnp.zeros((D // 2, 128), u32)
    vt_s[1] = jnp.zeros((D // 2, 128), u32)

    def kblock(b, g0=0, g1=NG, nb=1):
        static = isinstance(b, int)
        r = b * 64 if static else pl.multiple_of(b * 64, 64)
        xa_t = _u2b(xa[pl.ds(r, 64 * nb), :])
        kk = jnp.dot(xa_t, wk[:, 128 * g0:128 * g1], preferred_element_type=f32)
        kr = 128 + r if static else pl.multiple_of(128 + r, 64)
        toks = []
        for g in range(g0, g1):
            v = _b2u(kk[:, 128 * (g - g0):128 * (g - g0) + 128].astype(bf16))
            k_s[g, pl.ds(kr, 64 * nb), :] = v
            toks.append(v[0:8])
        return toks

    def fill_kpad():
        for g in range(NG):
            lo = k_s[g, 128:129, :] & jnp.uint32(0xFFFF)
            k_s[g, 0:128, :] = jnp.broadcast_to(lo | (lo << 16), (128, 128))

    def gate(v, tok):
        if tok is None:
            return v
        return v + pltpu.bitcast(tok & zv[...], f32)[0:1, 0:v.shape[1]]

    def ln0(b, toks=None):
        base = 128 * b if isinstance(b, int) else pl.multiple_of(128 * b, 128)
        nch = 1 if toks is None else 2
        n = 128 // nch
        for c in range(nch):
            r0 = base + n * c
            x = xin[pl.ds(r0, n), :].astype(f32)
            x_s[pl.ds(r0, n), :] = x
            mu = jnp.mean(x, axis=1, keepdims=True)
            if toks is not None:
                mu = gate(mu, toks[4 * c])
            xc = x - mu
            var = jnp.mean(xc * xc, axis=1, keepdims=True)
            h0 = r0 // 2 if isinstance(b, int) else pl.multiple_of(r0 // 2, n // 2)
            xa[pl.ds(h0, n // 2), :] = _b2u((xc * lax.rsqrt(var + EPS)).astype(bf16))

    def conv(dst, src):
        for j in range(NG):
            dst[64 * j:64 * j + 64, :] = _b2u(src[128 * j:128 * j + 128, :])

    x_copy(0).wait()
    x_copy(1).start()
    ln0(0)
    ln0(1)
    wk_copy(0).wait()
    wk_copy(1).start()
    kblock(0, 0, 2, 2)
    x_copy(1).wait()
    wk_copy(2).start()
    ln0(2)
    kblock(2, 0, 2)
    ln0(3)
    wk_copy(1).wait()
    wk_copy(3).start()
    kblock(0, 2, 4, 3)
    wk_copy(2).wait()
    x_copy(2).start()
    x_copy(3).start()
    kblock(0, 4, 6, 3)
    wk_copy(3).wait()
    x_copy(2).wait()
    x_copy(4).start()
    kblock(0, 6, 8, 3)
    ln0(4)

    def pro_body(t, c):
        @pl.when(t == 0)
        def _():
            x_copy(3).wait()

        @pl.when(t == 1)
        def _():
            x_copy(4).wait()

        @pl.when(t == 2)
        def _():
            x_copy(5).wait()

        for b in range(4):
            toks = kblock(4 * t + 3 + b)
            ln0(jnp.minimum(4 * t + 5 + b, NB - 1), toks)
        return c

    x_copy(5).start()
    wq_copy.start()
    wv_copy.start()
    wo_copy.start()
    wr_copy.start()
    lax.fori_loop(0, 3, pro_body, 0)
    wq_copy.wait()
    wv_copy.wait()
    wo_copy.wait()
    wr_copy.wait()
    kblock(15)
    conv(wqu, wq)
    conv(wvu, wv)
    conv(wou, wo)
    wr[...] = wr1[...].astype(f32).reshape(1, D).astype(bf16)
    fill_kpad()

    def q_slice(xa_blk, q_blk, n):
        lhs = _u2b(xa_blk[...])
        rhs = _u2b(wqu[:, 128 * n:128 * n + 128])
        q = jnp.dot(lhs, rhs, preferred_element_type=f32)
        qt = _b2u((q * QSCALE).astype(bf16).T)
        parts = [qt[0:16]] + [pltpu.roll(qt[16 * h:16 * h + 16], 32 * h, 1) for h in range(1, 4)]
        q_blk[64 * n:64 * n + 64, :] = jnp.concatenate(parts, axis=0)
        return parts[0][0:8]

    def v_slice(xa_blk, vt_blk, n):
        lhs = _u2b(xa_blk[...])
        rhs = _u2b(wvu[:, 128 * n:128 * n + 128])
        v = jnp.dot(lhs, rhs, preferred_element_type=f32)
        vt = _b2u(_u2b(_pack_adj(v)).T)
        vt_blk[64 * n:64 * n + 64, :] = vt
        return vt[0:8]

    def v_raw(xa_blk, n):
        vraw[...] = jnp.dot(_u2b(xa_blk[...]), _u2b(wvu[:, 128 * n:128 * n + 128]), preferred_element_type=f32)

    def v_finish(vt_blk, n):
        vt_blk[64 * n:64 * n + 64, :] = _b2u(_u2b(_pack_adj(vraw[...])).T)

    def o_slice(o_blk, x_blk, n):
        lhs = _u2b(o_blk[...])
        rhs = _u2b(wou[:, 128 * n:128 * n + 128])
        acc = jnp.dot(lhs, rhs, preferred_element_type=f32)
        x_blk[:, 128 * n:128 * n + 128] = x_blk[:, 128 * n:128 * n + 128] + acc
        return pltpu.bitcast(acc[0:8], u32)

    def epi_stats(j, x_blk, c, tok=None):
        r0 = pl.multiple_of(j * 128, 128)
        R = 128 // NEC
        lo = R * c
        x1 = x_blk[lo:lo + R, :]
        mu = gate(jnp.mean(x1, axis=1, keepdims=True), tok)
        xc = x1 - mu
        var = jnp.mean(xc * xc, axis=1, keepdims=True)
        a = lax.rsqrt(var + EPS)
        r = jnp.sum(xc * wr[...].astype(f32), axis=1, keepdims=True) * a
        r_s[pl.ds(r0 + lo, R), :] = r
        a_s[pl.ds(r0 + lo, R), :] = a
        return mu, xc, var, a

    def epi_norm(j, x_blk, xa_blk, layer, c, st, tok=None):
        r0 = pl.multiple_of(j * 128, 128)
        R = 128 // NEC
        lo = R * c
        mu, xc, var, a = st
        a1 = gate(1.0 + a, tok)
        x2 = mu + xc * a1
        if layer == 0:
            x_blk[lo:lo + R, :] = x2
            v = xc * (a1 * lax.rsqrt(var * a1 * a1 + EPS))
            xa_blk[lo // 2:(lo + R) // 2, :] = _b2u(v.astype(bf16))
        else:
            outb[pl.ds(r0 + lo, R), :] = x2.astype(bf16)

    def epilogue(j, x_blk, xa_blk, layer, chunks=range(NEC)):
        for c in chunks:
            epi_norm(j, x_blk, xa_blk, layer, c, epi_stats(j, x_blk, c))

    lane8b = lax.broadcasted_iota(jnp.int32, (8, 128), 1) >> 5
    odd = (lane8b & 1) == 1
    high = lane8b >= 2
    lane16b = lax.broadcasted_iota(jnp.int32, (16, 128), 1) >> 5
    d32 = lax.broadcasted_iota(jnp.int32, (32, 128), 0) - (lax.broadcasted_iota(jnp.int32, (32, 128), 1) & 31)
    umask = d32 > 0

    def stage_a(kv, q_blk, g):
        s_ref = sb[g % NBUF]
        for j in range(4):
            x = jnp.concatenate([jnp.where(lane16b == ((h + j) % 4), q_blk[64 * g + 16 * h:64 * g + 16 * h + 16, :],
                                           jnp.uint32(0)) for h in range(4)], axis=0)
            b0 = 16 * j
            kt = jnp.concatenate([kv[g, b0:b0 + 8, :], kv[g, b0 + 128:b0 + 136, :], kv[g, b0 + 8:b0 + 16, :],
                                  kv[g, b0 + 136:b0 + 144, :], kv[g, b0 + 16:b0 + 128, :]], axis=0)
            st = jnp.dot(_u2b(kt), _u2b(x), preferred_element_type=f32)
            su = jnp.concatenate([st[0:16], st[32:48]], axis=0)
            sl = jnp.concatenate([st[16:32], st[48:64]], axis=0)
            s_ref[j, 0:32, :] = jnp.where(umask, su, sl)
            s_ref[j, 32:256, :] = st[64:288]
            if j == 0:
                tok = (pltpu.bitcast(st[64:72], u32), pltpu.bitcast(st[160:168], u32),
                       pltpu.bitcast(st[280:288], u32))
        return tok

    def bfly(y):
        def sel(m, a, b):
            if a is None and b is None:
                return None
            z = jnp.zeros((8, 128), (a if a is not None else b).dtype)
            return jnp.where(m, z if a is None else a, z if b is None else b)
        r = [sel(odd, y[(k + 1) % 4], y[k]) for k in range(4)]
        wp = [sel(high, r[(k + 2) % 4], r[k]) for k in range(4)]
        return [wp[(-h) % 4] for h in range(4)]

    def stage_b(i, g, toks):
        s_ref = sb[g % NBUF]
        p_ref = pb[g % NBUF].at[zs[0]]
        l_ref = lb[g % NBUF]
        ss = [s_ref[j] for j in range(4)]
        ms = [jnp.max(ss[j], axis=0, keepdims=True) for j in range(4)]
        ls = [None] * 4
        nch = len(toks)
        um16 = [umask[0:16], umask[16:32]]
        for c in range(nch):
            mg = [gate(ms[j], toks[c]) for j in range(4)]
            for M in range(24 * c // nch, 24 * (c + 1) // nch):
                y = []
                for j in range(4):
                    Mp = M - 2 * j
                    if not 0 <= Mp < 18:
                        y.append(None)
                        continue
                    row = 16 * (Mp % 16)
                    p = jnp.exp2(ss[j][row:row + 16] - mg[j])
                    if Mp < 16:
                        ps = p[0:8] + p[8:16]
                        ls[j] = ps if ls[j] is None else ls[j] + ps
                        if Mp == 2:
                            p32 = p[0:1]
                            ls[j] = ls[j] - jnp.where(lax.broadcasted_iota(jnp.int32, (8, 128), 0) == 0,
                                                      npad[jnp.minimum(i, 2), j] * p32, 0.0)
                    if Mp < 2:
                        p = jnp.where(um16[Mp], p, 0.0)
                    elif Mp >= 16:
                        p = jnp.where(um16[Mp - 16], 0.0, p)
                    y.append(_pack2(p[0:8], p[8:16]))
                w = bfly(y)
                for h in range(4):
                    p_ref[h, 8 * M:8 * M + 8, :] = w[h] if w[h] is not None else jnp.zeros((8, 128), u32)
        for j in range(4):
            l_ref[j] = jnp.sum(ls[j], axis=0, keepdims=True)

    def stage_c(vts, o_blk, g):
        p_ref = pb[g % NBUF].at[zs[1]]
        l_ref = lb[g % NBUF]
        lh = bfly([jnp.broadcast_to(1.0 / l_ref[j], (8, 128)) for j in range(4)])
        outs = []
        for h in range(4):
            vt = jnp.concatenate([_u2b(vts[t][64 * g + 16 * h:64 * g + 16 * h + 16, :]) for t in range(3)], axis=1)
            o = jnp.dot(vt, _u2b(p_ref[h]), preferred_element_type=f32)
            o = o * lh[h][0:1]
            if h:
                o = pltpu.roll(o, 128 - 32 * h, 1)
            outs.append(o)
        ot = jnp.concatenate(outs, axis=0)
        o_blk[:, 128 * g:128 * g + 128] = _b2u(ot.T.astype(bf16))

    def attn_body(i, c, has_next, prev, layer, extra=()):
        lo = -1 if prev else 0
        r = pl.multiple_of((i + lo) * 64, 64)
        nblk = (2 if has_next else 1) - lo
        xav = xa.at[pl.ds(r, 64 * nblk), :]
        ov = o_s.at[pl.ds(r, 64 * (1 - lo)), :]
        xv = x_s.at[pl.ds(pl.multiple_of((i + lo) * 128, 128), 128), :]
        qv = qt_s.at[pl.ds(i, 2)]
        vv = vt_s.at[pl.ds(i + lo, 4 - lo)]
        kv = k_s.at[:, pl.ds(pl.multiple_of(i * 64, 64), 256), :]
        blk = lambda v, b: v.at[pl.ds(64 * (b - lo), 64), :]
        vtile = lambda b: vv.at[b - lo]

        qs = [functools.partial(q_slice, blk(xav, 1), qv.at[1], n) for n in range(NG)] if has_next else []
        vs = [functools.partial(v_slice, blk(xav, 1), vtile(3), n) for n in range(NG)] if has_next else []
        if has_next:
            vs[NG - 1] = functools.partial(v_raw, blk(xav, 1), NG - 1)
        if prev:
            v_finish(vtile(2), NG - 1)
        os_ = [functools.partial(o_slice, blk(ov, -1), xv, n) for n in range(NG)] if prev else []
        sl = qs[0:1] + os_ + qs[1:] + vs
        last_o = len(qs[0:1]) + len(os_) - 1 if os_ else -1
        if extra:
            n_it = 2 * NG
            groups = [extra[len(extra) * k // n_it:len(extra) * (k + 1) // n_it] for k in range(n_it)]

            def run(fs):
                for f in fs:
                    f()
            comp = [functools.partial(run, fs) for fs in groups]
            sl = comp[0:1] + sl + comp[1:]
            last_o = NG
        state = {"emitted": 0}
        stats = {}
        if layer == 0:
            esch = [(1, "s", 0, False), (2, "s", 1, True), (4, "n", 0, True), (6, "n", 1, True)]
        else:
            esch = [(1, "s", 0, False), (2, "s", 1, True), (3, "n", 0, True), (5, "n", 1, True)]

        def run_epi(k, tok):
            for (off, kind, ch, paced) in esch:
                if (k is None or off == k) and (kind, ch) not in stats:
                    if kind == "s":
                        stats[kind, ch] = epi_stats(i - 1, xv, ch, tok if paced else None)
                    else:
                        epi_norm(i - 1, xv, blk(xav, -1), layer, ch, stats["s", ch], tok if paced else None)
                        stats[kind, ch] = True

        def dense_one():
            k = state["emitted"]
            if k < len(sl):
                t = sl[k]()
                state["emitted"] += 1
                if prev and k > last_o:
                    run_epi(k - last_o, t)

        for g in range(NG):
            def pv():
                if g >= 1:
                    stage_c([vtile(t) for t in range(3)], blk(ov, 0), g - 1)
                elif prev:
                    stage_c([vtile(t - 1) for t in range(3)], blk(ov, -1), NG - 1)
            if g == 0:
                pv()
            tok = (None, None, None)
            if g + 1 < NG:
                tok = stage_a(kv.at[:, pl.ds(0, 192), :], qv.at[0], g + 1)
            elif has_next:
                tok = stage_a(kv.at[:, pl.ds(64, 192), :], qv.at[1], 0)
            stage_b(i, g, [None, None, tok[0], tok[1]])
            nd = len(sl) * (g + 1) // NG - len(sl) * g // NG
            for _ in range(min(nd, 2) if nd > 1 else 0):
                dense_one()
            if g > 0:
                pv()
            for _ in range(nd - (min(nd, 2) if nd > 1 else 0)):
                dense_one()
        while state["emitted"] < len(sl):
            dense_one()
        if prev:
            run_epi(None, None)

        if layer == 1 and prev:
            out_copy(i - 1).start()
        if layer == 0 and prev and has_next:
            @pl.when(i == 1)
            def _():
                wg_copy.start()
                wu_copy.start()
                wd_copy.start()
        return c

    def finish_block(j, layer):
        o_blk = o_s.at[pl.ds(pl.multiple_of(j * 64, 64), 64), :]
        x_blk = x_s.at[pl.ds(pl.multiple_of(j * 128, 128), 128), :]
        stage_c([vt_s.at[j + t] for t in range(3)], o_blk, NG - 1)
        for n in range(NG):
            o_slice(o_blk, x_blk, n)
        epilogue(j, x_blk, xa.at[pl.ds(pl.multiple_of(j * 64, 64), 64), :], layer)

    def route(raw):
        def best(r0, n):
            r = r_s[r0:r0 + n, :]
            m = jnp.max(r)
            rows = lax.broadcasted_iota(jnp.int32, (n, 1), 0) + r0
            return m, jnp.min(jnp.where(r == m, rows, S))
        ma, ia = best(0, S - 128)
        mb, ib = best(S - 128, 128)
        rmax = jnp.maximum(ma, mb)
        idx = jnp.where(mb > ma, ib, ia)
        idx = jnp.minimum(idx, S - 1)
        xrow = x_s[pl.ds(idx, 1), :]
        arow = a_s[pl.ds(idx, 1), :]
        mu = jnp.mean(xrow, axis=1, keepdims=True)
        if raw:
            xsel = (xrow - mu) * arow
            xrow = xrow + xsel
        else:
            xsel = (xrow - mu) * (arow / (1.0 + arow))
        xs = jnp.broadcast_to(xsel, (8, D)).astype(bf16)
        return idx, rmax, xrow, xs

    def ffn_steps(xs):
        gates, hid, ys = [], [], []

        def up(c, w, first):
            r = jnp.dot(xs, w[:, 128 * c:128 * (c + 1)], preferred_element_type=f32)
            if first:
                gates.append(r)
            else:
                g_ = gates[c]
                hid.append((g_ * jax.nn.sigmoid(g_) * r).astype(bf16))

        def down(c):
            ys.append(jnp.dot(hid[c], wd[128 * c:128 * (c + 1), :], preferred_element_type=f32))

        steps = []
        for c in range(NFS):
            steps.append(functools.partial(up, c, wg, True))
            steps.append(functools.partial(up, c, wu, False))
            if c >= 1:
                steps.append(functools.partial(down, c - 1))
        steps.append(functools.partial(down, NFS - 1))

        def result():
            y = ys[0]
            for t in ys[1:]:
                y = y + t
            return y
        return steps, result

    def kslice(b, g):
        kblock(b, g, g + 1)

    def ffn_mid():
        kblock(K2_EARLY)
        idx, rmax, xrow, xs = route(raw=False)
        steps, result = ffn_steps(xs)
        fi = 0
        for b in range(K2_EARLY + 1, NB):
            for g in range(NG):
                kslice(b, g)
                if fi < len(steps):
                    steps[fi]()
                    fi += 1
        while fi < len(steps):
            steps[fi]()
            fi += 1
        y = result()
        x_s[pl.ds(idx, 1), :] = xrow + y[0:1, :] * jax.nn.sigmoid(rmax)
        r0 = pl.multiple_of((idx // 16) * 16, 16)
        h0 = pl.multiple_of((idx // 16) * 8, 8)
        x = x_s[pl.ds(r0, 16), :]
        mu = jnp.mean(x, axis=1, keepdims=True)
        xc = x - mu
        var = jnp.mean(xc * xc, axis=1, keepdims=True)
        xn = (xc * lax.rsqrt(var + EPS)).astype(bf16)
        xa[pl.ds(h0, 8), :] = _b2u(xn)
        kk = jnp.dot(xn, wk[...], preferred_element_type=f32)
        for g in range(NG):
            k_s[g, pl.ds(128 + h0, 8), :] = _b2u(kk[:, 128 * g:128 * g + 128].astype(bf16))
        fill_kpad()

    def ffn_last():
        idx, rmax, xrow, xs = route(raw=True)
        steps, result = ffn_steps(xs)
        for f in steps:
            f()
        y = result()
        new = xrow + y[0:1, :] * jax.nn.sigmoid(rmax)
        for i in range(NB):
            out_copy(i).wait()
        b0 = pl.multiple_of((idx // 16) * 16, 16)
        rows = lax.broadcasted_iota(jnp.int32, (16, D), 0) + b0
        outb[pl.ds(b0, 16), :] = jnp.where(rows == idx, new, outb[pl.ds(b0, 16), :].astype(f32)).astype(bf16)
        fix = pltpu.make_async_copy(outb.at[pl.ds(b0, 16), :], out_hbm.at[pl.ds(b0, 16), :], osems.at[NB])
        fix.start()
        fix.wait()

    for layer in range(2):
        for n in range(NG):
            q_slice(xa.at[pl.ds(0, 64), :], qt_s.at[0], n)
        for n in range(NG):
            v_slice(xa.at[pl.ds(0, 64), :], vt_s.at[2], n)
        stage_a(k_s.at[:, pl.ds(0, 192), :], qt_s.at[0], 0)
        attn_body(0, 0, has_next=True, prev=False, layer=layer)
        lax.fori_loop(1, NB - 1, functools.partial(attn_body, has_next=True, prev=True, layer=layer), 0)
        extra = [functools.partial(kslice, b, g) for b in range(K2_EARLY) for g in range(NG)] if layer == 0 else ()
        attn_body(NB - 1, 0, has_next=False, prev=True, layer=layer, extra=extra)
        finish_block(NB - 1, layer)
        if layer == 0:
            wg_copy.wait()
            wu_copy.wait()
            wd_copy.wait()
            ffn_mid()
        else:
            out_copy(NB - 1).start()
            ffn_last()


@jax.jit
def pallas_interleave_layers__sliding_block__moe_arch_mod__prompt_kernel(
    A_x: jax.Array,
    A_wqkv: jax.Array,
    A_wo: jax.Array,
    B_x: jax.Array,
    B_w_r: jax.Array,
    B_w_gate: jax.Array,
    B_w_up: jax.Array,
    B_w_down: jax.Array,
):
    del B_x
    x = A_x.reshape(S, D)
    any_spec = pl.BlockSpec(memory_space=pl.ANY)
    scratch = [
        pltpu.VMEM((S, D), bf16),
        pltpu.VMEM((S, D), f32),
        pltpu.VMEM((S // 2, D), u32),
        pltpu.VMEM((NG, (S + 256) // 2 + 64, 128), u32),
        pltpu.VMEM((NB + 1, D // 2, 128), u32),
        pltpu.VMEM((NB + 3, D // 2, 128), u32),
        pltpu.VMEM((S // 2, D), u32),
        pltpu.VMEM((D, D), bf16),
        pltpu.VMEM((D, D), bf16),
        pltpu.VMEM((D, D), bf16),
        pltpu.VMEM((D // 2, D), u32),
        pltpu.VMEM((D // 2, D), u32),
        pltpu.VMEM((D, D), bf16),
        pltpu.VMEM((D // 2, D), u32),
        pltpu.VMEM((1, D), bf16),
        pltpu.VMEM((D, F), bf16),
        pltpu.VMEM((D, F), bf16),
        pltpu.VMEM((F, D), bf16),
        pltpu.VMEM((S, 1), f32),
        pltpu.VMEM((S, 1), f32),
        pltpu.VMEM((S, D), bf16),
        pltpu.VMEM((3, 4, 1, 128), f32),
        pltpu.SMEM((2,), jnp.int32),
        pltpu.VMEM((8, 128), u32),
        pltpu.VMEM((128, 128), f32),
        pltpu.VMEM((D,), bf16),
        pltpu.SemaphoreType.DMA((22,)),
        pltpu.SemaphoreType.DMA((NB + 1,)),
    ]
    scratch += [pltpu.VMEM((4, 256, 128), f32)] * NBUF
    scratch += [pltpu.VMEM((1, 4, 192, 128), u32)] * NBUF
    scratch += [pltpu.VMEM((4, 1, 128), f32)] * NBUF
    out = pl.pallas_call(
        _kernel,
        out_shape=jax.ShapeDtypeStruct((S, D), bf16),
        in_specs=[any_spec] * 7,
        out_specs=any_spec,
        scratch_shapes=scratch,
        compiler_params=pltpu.CompilerParams(vmem_limit_bytes=110 * 1024 * 1024),
    )(x, A_wqkv, A_wo, B_w_r, B_w_gate, B_w_up, B_w_down)
    return out.reshape(1, S, D)
```
